```python
import jax
import jax.numpy as jnp

def _softmax(x, axis=-1):
    return jax.nn.softmax(x, axis=axis)
def _gelu(x):
    return jax.nn.gelu(x, approximate=True)
def _silu(x):
    return jax.nn.silu(x)
def _sigmoid(x):
    return jax.nn.sigmoid(x)
def _layernorm(x, axis=-1, eps=1e-5):
    m = jnp.mean(x, axis=axis, keepdims=True)
    v = jnp.var(x, axis=axis, keepdims=True)
    return (x - m) / jnp.sqrt(v + eps)
def _scatter_add(tgt, idx, src, axis=0):
    return tgt.at[idx].add(src)
def _segment_sum(src, seg, n):
    return jax.ops.segment_sum(src, seg, n)
class _Rng:
    def __init__(self, key):
        self._k = key
    def _next(self):
        self._k, sub = jax.random.split(self._k)
        return sub
    def normal(self, shape):
        return jax.random.normal(self._next(), shape, dtype=jnp.bfloat16)
    def randint(self, lo, hi, shape):
        return jax.random.randint(self._next(), shape, lo, hi, dtype=jnp.int32)
    def uniform(self, shape, lo=0.0, hi=1.0):
        return jax.random.uniform(self._next(), shape, jnp.bfloat16, lo, hi)
    def permutation(self, n):
        return jax.random.permutation(self._next(), n)


kernel_name = 'interleave_layers__sliding_block__moe_arch_mod__prompt'

def setup_inputs():
    _rng = _Rng(jax.random.key(int.from_bytes(__import__("os").urandom(4), "little")))
    _w = (lambda a: (lambda t: t.astype(jnp.bfloat16) if jnp.issubdtype(t.dtype, jnp.floating) else t)(jnp.asarray(a)))
    def _A_setup():
        B, S, D = 1, 2048, 1024
        return {
            "x": _w((lambda *s: _rng.normal(s) * 0.05)(B, S, D)),
            "wqkv": _w((lambda *s: _rng.normal(s) * 0.05)(D, 3 * D)),
            "wo": _w((lambda *s: _rng.normal(s) * 0.05)(D, D)),
        }
    _A_in = _A_setup()

    def _B_setup():
        B, S, D, F, C = 1, 2048, 1024, 3584, 1
        return {
            "x": _w((lambda *s: _rng.normal(s) * 0.05)(B, S, D)),
            "w_r": _w((lambda *s: _rng.normal(s) * 0.05)(D)),
            "w_gate": _w((lambda *s: _rng.normal(s) * 0.05)(D, F)),
            "w_up": _w((lambda *s: _rng.normal(s) * 0.05)(D, F)),
            "w_down": _w((lambda *s: _rng.normal(s) * 0.05)(F, D)),
        }
    _B_in = _B_setup()

    return {
        "A_x": _A_in["x"],
        "A_wqkv": _A_in["wqkv"],
        "A_wo": _A_in["wo"],
        "B_x": _B_in["x"],
        "B_w_r": _B_in["w_r"],
        "B_w_gate": _B_in["w_gate"],
        "B_w_up": _B_in["w_up"],
        "B_w_down": _B_in["w_down"],
    }

def reference(A_x, A_wqkv, A_wo, B_x, B_w_r, B_w_gate, B_w_up, B_w_down):
    def _A_ref(x, wqkv, wo):
        B, S, D = x.shape
        H = 32; Dh = D // H; W = 256
        qkv = (lambda x, *d: x.transpose(*d))((x @ wqkv).reshape(B, S, 3, H, Dh), 2, 0, 3, 1, 4)
        q, k, v = qkv[0], qkv[1], qkv[2]
        scores = jnp.einsum("bhqd,bhkd->bhqk", q, k) * (Dh ** -0.5)
        idx = jnp.arange(S)
        mask = (idx[:, None] - idx[None, :] >= 0) & (idx[:, None] - idx[None, :] < W)
        scores = jnp.where(mask[None, None], scores, -1e9)
        p = _softmax(scores, axis=-1)
        o = jnp.einsum("bhqk,bhkd->bhqd", p, v)
        return (lambda x, *d: x.transpose(*d))(o, 0, 2, 1, 3).reshape(B, S, D) @ wo

    def _B_ref(x, w_r, w_gate, w_up, w_down):
        B, S, D = x.shape
        C = 1
        r = x @ w_r
        idx = jnp.argsort(-r, axis=-1)[:, :C]
        idx_e = jnp.repeat(idx.reshape(B, C, 1), D, axis=2)
        x_sel = jnp.take_along_axis(x, idx_e, axis=1)
        g = _silu(x_sel @ w_gate)
        u = x_sel @ w_up
        y = (g * u) @ w_down
        r_sel = _sigmoid(jnp.take_along_axis(r, idx, axis=1))
        y = y * r_sel.reshape(B, C, 1)
        b_off = (jnp.arange(B) * S).reshape(B, 1)
        flat_idx = (idx + b_off).reshape(B * C)
        zero = (x * 0.0).reshape(B * S, D)
        upd = _scatter_add(zero, flat_idx, y.reshape(B * C, D), axis=0)
        return x + upd.reshape(B, S, D)

    x = A_x
    x = x + _A_ref(_layernorm(x, axis=-1), A_wqkv, A_wo)
    x = x + _B_ref(_layernorm(x, axis=-1), B_w_r, B_w_gate, B_w_up, B_w_down)
    x = x + _A_ref(_layernorm(x, axis=-1), A_wqkv, A_wo)
    x = x + _B_ref(_layernorm(x, axis=-1), B_w_r, B_w_gate, B_w_up, B_w_down)
    return x
```

```python
import jax
import jax.numpy as jnp
from jax import lax
import jax.experimental.pallas as pl
import jax.experimental.pallas.tpu as pltpu

bf16 = jnp.bfloat16
f32 = jnp.float32
u32 = jnp.uint32
i32 = jnp.int32

S = 2048
D = 1024
H = 32
DH = 32
W = 256
F = 3584
G = 8
PAD = 256
TQ = 256
NB = S // TQ
NSB = S // 128
EPS = 1e-5
NEG = -1e30
QSCALE = (DH ** -0.5) * 1.4426950408889634
NT = (((1,), (1,)), ((), ()))


def _ln(x):
    m = jnp.mean(x, axis=-1, keepdims=True)
    xc = x - m
    v = jnp.mean(xc * xc, axis=-1, keepdims=True)
    return xc * lax.rsqrt(v + EPS)


def _pack_rows(x):
    return pltpu.bitcast(x.astype(bf16), u32)


def _pack_rows_interleaved(x):
    n = x.shape[0] // 16
    x3 = x.reshape(n, 16, x.shape[1])
    a = x3[:, 0:8, :].reshape(n * 8, x.shape[1])
    b = x3[:, 8:16, :].reshape(n * 8, x.shape[1])
    return pltpu.pack_elementwise([a, b], packed_dtype=bf16)


def _kernel(x_hbm, wqkv_hbm, wo_hbm, wr_hbm, wg_hbm, wu_hbm, wd_hbm,
            out_hbm,
            xio, wqk_v, wv_v, wvt_v, wo_v, wr_v, wg_v, wu_v, wd_v,
            xres, xn1_s, r_s,
            xca, xia, xcb, xib,
            q_s, k_s, vt_s, o_s, s_s, m_s,
            ata, atb,
            sem_x, sem_w, sem_o):
    def x_copy(i):
        r0 = pl.multiple_of(i * TQ, TQ)
        return pltpu.make_async_copy(x_hbm.at[pl.ds(r0, TQ), :], xio.at[pl.ds(r0, TQ), :], sem_x.at[i])

    def out_copy(i):
        r0 = pl.multiple_of(i * TQ, TQ)
        return pltpu.make_async_copy(xio.at[pl.ds(r0, TQ), :], out_hbm.at[pl.ds(r0, TQ), :], sem_o.at[i])

    cp_wv = pltpu.make_async_copy(wqkv_hbm.at[:, pl.ds(2 * D, D)], wv_v, sem_w.at[0])
    cp_wqk = pltpu.make_async_copy(wqkv_hbm.at[:, pl.ds(0, 2 * D)], wqk_v, sem_w.at[1])
    cp_wo = pltpu.make_async_copy(wo_hbm, wo_v, sem_w.at[2])
    cp_wr = pltpu.make_async_copy(wr_hbm, wr_v, sem_w.at[3])
    cp_wg = pltpu.make_async_copy(wg_hbm, wg_v, sem_w.at[4])
    cp_wu = pltpu.make_async_copy(wu_hbm, wu_v, sem_w.at[5])
    cp_wd = pltpu.make_async_copy(wd_hbm, wd_v, sem_w.at[6])

    x_copy(0).start()
    cp_wv.start()
    cp_wqk.start()
    for i in range(1, NB):
        x_copy(i).start()
    cp_wo.start()
    cp_wr.start()
    cp_wg.start()
    cp_wu.start()
    cp_wd.start()

    k_s[:, 0:PAD // 2, :] = jnp.zeros((G, PAD // 2, 128), u32)
    vt_s[:, 0:PAD] = jnp.zeros((D // 2, PAD), u32)

    cp_wv.wait()
    wvt_v[...] = pltpu.bitcast(wv_v[...].T, u32)

    def ln_block(layer, i, xc_ref, xi_ref):
        r0 = pl.multiple_of(i * TQ, TQ)
        x_in = xio[pl.ds(r0, TQ), :].astype(f32)
        x_rs = xres[pl.ds(r0, TQ), :]
        x = jnp.where(layer == 0, x_in, x_rs)
        xn = _ln(x)
        xc_ref[...] = _pack_rows(xn)
        xi_ref[...] = _pack_rows_interleaved(xn)

    def proj_block(i, xc_ref, xi_ref):
        h0 = pl.multiple_of(i * (TQ // 2), TQ // 2)
        y = jnp.dot(pltpu.bitcast(xc_ref[...], bf16), wqk_v[...], preferred_element_type=f32)
        for g in range(G):
            q_s[g, pl.ds(h0, TQ // 2), :] = _pack_rows(y[:, g * 128:(g + 1) * 128] * QSCALE)
            k_s[g, pl.ds(PAD // 2 + h0, TQ // 2), :] = _pack_rows(y[:, D + g * 128:D + (g + 1) * 128])
        vt = lax.dot_general(pltpu.bitcast(wvt_v[...], bf16), pltpu.bitcast(xi_ref[...], bf16), NT,
                             preferred_element_type=f32)
        c0 = pl.multiple_of(PAD + i * TQ, TQ)
        vt_s[:, pl.ds(c0, TQ)] = _pack_rows(vt)

    def phase_a(layer):
        @pl.when(layer == 0)
        def _():
            x_copy(0).wait()
            cp_wqk.wait()

        ln_block(layer, 0, xca, xia)

        def body(j, c):
            i0 = 2 * j
            i2 = jnp.minimum(i0 + 2, NB - 1)

            @pl.when(layer == 0)
            def _():
                x_copy(i0 + 1).wait()

                @pl.when(i0 + 2 < NB)
                def _():
                    x_copy(i2).wait()

            proj_block(i0, xca, xia)
            ln_block(layer, i0 + 1, xcb, xib)
            proj_block(i0 + 1, xcb, xib)
            ln_block(layer, i2, xca, xia)
            return c

        lax.fori_loop(0, NB // 2, body, 0)

    def qk_stage(g, q0, slot, masked):
        lane16 = lax.broadcasted_iota(i32, (16, 128), 1)
        r16 = lax.broadcasted_iota(i32, (16, 128), 0)
        hb16 = lane16 // 32
        dd = r16 - lane16 % 32
        h0 = q0 // 2
        for b in range(4):
            base = pl.multiple_of(h0 + 16 * b, 16)
            parts = [k_s[g, pl.ds(base, 8), :], k_s[g, pl.ds(base + 128, 8), :],
                     k_s[g, pl.ds(base + 8, 8), :], k_s[g, pl.ds(base + 136, 8), :],
                     k_s[g, pl.ds(base + 16, 112), :]]
            kw = pltpu.bitcast(jnp.concatenate(parts, axis=0), bf16)
            qu = q_s[g, pl.ds(base, 16), :]
            qall = pltpu.bitcast(
                jnp.concatenate([jnp.where(hb16 == (p - b) % 4, qu, jnp.uint32(0)) for p in range(4)], axis=0),
                bf16)
            st = lax.dot_general(kw, qall, NT, preferred_element_type=f32)
            lo0, hi0, lo1, hi1, mid = st[0:16], st[16:32], st[32:48], st[48:64], st[64:288]
            if masked:
                first = PAD - (q0 + 32 * b)
                lo0 = jnp.where(r16 >= first, lo0, NEG)
                lo1 = jnp.where(r16 + 16 >= first, lo1, NEG)
                rm = lax.broadcasted_iota(i32, (224, 128), 0)
                mid = jnp.where(rm + 32 >= first, mid, NEG)
            c0 = jnp.where(dd > 0, lo0, hi0)
            c1 = jnp.where(dd > -16, lo1, hi1)
            x = jnp.concatenate([c0, c1, mid], axis=0)
            s_s[slot, b] = x
            mm = jnp.max(x.reshape(32, 8, 128), axis=0)
            m_s[slot, b] = jnp.broadcast_to(jnp.max(mm, axis=0, keepdims=True), (8, 128))

    def pv_stage(g, q0, slot):
        r8 = lax.broadcasted_iota(i32, (8, 128), 0)
        c8 = lax.broadcasted_iota(i32, (8, 128), 1)
        blk = c8 // 32
        j = c8 % 32

        def tri(u):
            return (jnp.where(16 * u + r8 > j, jnp.uint32(0xFFFF), jnp.uint32(0)) |
                    jnp.where(16 * u + 8 + r8 > j, jnp.uint32(0xFFFF0000), jnp.uint32(0)))

        tris = [tri(0), tri(1)]
        ms = [m_s[slot, b] for b in range(4)]
        L = [None] * 4
        cache = {}

        def pexp(b, u):
            x = s_s[slot, b, 16 * u:16 * u + 16, :]
            p0 = jnp.exp2(x[0:8] - ms[b])
            p1 = jnp.exp2(x[8:16] - ms[b])
            sm = p0 + p1
            L[b] = sm if L[b] is None else L[b] + sm
            return pltpu.pack_elementwise([p0, p1], packed_dtype=bf16)

        def get_p(b, u):
            if u < 2:
                pk = pexp(b, u)
                lo = pk & tris[u]
                cache[(b, u + 16)] = pk ^ lo
                return lo
            if u >= 16:
                return cache.pop((b, u))
            return pexp(b, u)

        zero = jnp.zeros((8, 128), u32)
        accs = [None] * 4
        for k in range(3):
            wts = [[] for _ in range(4)]
            for t in range(8 * k, 8 * k + 8):
                srcs = [(b, get_p(b, t - 2 * b)) for b in range(4) if 0 <= t - 2 * b < 18]
                for h in range(4):
                    acc = zero if len(srcs) < 4 else None
                    for (b, v) in srcs:
                        acc = v if acc is None else jnp.where(blk == (h + b) % 4, v, acc)
                    wts[h].append(acc)
            c0 = pl.multiple_of(q0 + 128 * k, 128)
            for h in range(4):
                pt = pltpu.bitcast(jnp.concatenate(wts[h], axis=0), bf16)
                vth = pltpu.bitcast(vt_s[pl.ds((g * 4 + h) * 16, 16), pl.ds(c0, 128)], bf16)
                d = jnp.dot(vth, pt, preferred_element_type=f32)
                accs[h] = d if accs[h] is None else accs[h] + d
        L = [jnp.broadcast_to(jnp.sum(l, axis=0, keepdims=True), (8, 128)) for l in L]
        outs = []
        for h in range(4):
            lh = L[0]
            for b in range(1, 4):
                lh = jnp.where(blk == (h + b) % 4, L[b], lh)
            ot = (accs[h].reshape(4, 8, 128) * (1.0 / lh)[None]).reshape(32, 128)
            if h > 0:
                ot = pltpu.roll(ot, 128 - 32 * h, axis=1)
            outs.append(ot)
        ot = jnp.concatenate(outs, axis=0)
        o_s[pl.ds(q0, 128), g * 128:(g + 1) * 128] = ot.T

    def phase_b():
        def make_body(masked):
            def body(sb, c):
                q0 = pl.multiple_of(sb * 128, 128)
                qn = pl.multiple_of(jnp.minimum(sb + 1, NSB - 1) * 128, 128)
                for g in range(G):
                    if g + 1 < G:
                        qk_stage(g + 1, q0, (g + 1) % 2, masked)
                    else:
                        qk_stage(0, qn, 0, masked)
                    pv_stage(g, q0, g % 2)
                return c
            return body

        qk_stage(0, 0, 0, True)
        lax.fori_loop(0, 2, make_body(True), 0)
        lax.fori_loop(2, NSB, make_body(False), 0)

    def oproj_block(i, at_ref):
        r0 = pl.multiple_of(i * TQ, TQ)
        at_ref[...] = jnp.dot(o_s[pl.ds(r0, TQ), :].astype(bf16), wo_v[...], preferred_element_type=f32)

    def resid_block(layer, i, at_ref):
        r0 = pl.multiple_of(i * TQ, TQ)
        x_in = xio[pl.ds(r0, TQ), :].astype(f32)
        x_rs = xres[pl.ds(r0, TQ), :]
        x1 = jnp.where(layer == 0, x_in, x_rs) + at_ref[...]
        xn = _ln(x1)
        xn1_s[pl.ds(r0, TQ), :] = xn
        r = jnp.sum(xn * wr_v[...].astype(f32).reshape(1, D), axis=-1, keepdims=True)
        r_s[pl.ds(r0, TQ), :] = jnp.broadcast_to(r, (TQ, 128))
        x2 = x1 + xn
        xres[pl.ds(r0, TQ), :] = x2
        return x2

    def phase_c(layer):
        @pl.when(layer == 0)
        def _():
            cp_wo.wait()
            cp_wr.wait()

        oproj_block(0, ata)

        def finish(i, at_ref):
            x2 = resid_block(layer, i, at_ref)

            @pl.when(layer == 1)
            def _():
                r0 = pl.multiple_of(i * TQ, TQ)
                xio[pl.ds(r0, TQ), :] = xres[pl.ds(r0, TQ), :].astype(bf16)
                out_copy(i).start()

        def body(j, c):
            i0 = 2 * j
            oproj_block(i0 + 1, atb)
            finish(i0, ata)
            oproj_block(jnp.minimum(i0 + 2, NB - 1), ata)
            finish(i0 + 1, atb)
            return c

        lax.fori_loop(0, NB // 2, body, 0)

    def phase_d(layer):
        @pl.when(layer == 0)
        def _():
            cp_wg.wait()
            cp_wu.wait()
            cp_wd.wait()

        rb = r_s[...].astype(bf16).astype(f32)
        rmax = jnp.max(rb)
        rows = lax.broadcasted_iota(i32, (S, 128), 0)
        idx = jnp.min(jnp.where(rb == rmax, rows, S))
        idx = jnp.clip(idx, 0, S - 1)
        xs = jnp.broadcast_to(xn1_s[pl.ds(idx, 1), :], (16, D)).astype(bf16)
        gate = jnp.dot(xs, wg_v[...], preferred_element_type=f32)
        up = jnp.dot(xs, wu_v[...], preferred_element_type=f32)
        hmid = (gate * jax.nn.sigmoid(gate) * up).astype(bf16)
        y = jnp.dot(hmid, wd_v[...], preferred_element_type=f32)
        scale = jax.nn.sigmoid(jnp.full((1, D), rmax, f32))
        xres[pl.ds(idx, 1), :] = xres[pl.ds(idx, 1), :] + y[0:1] * scale

        @pl.when(layer == 1)
        def _():
            for i in range(NB):
                out_copy(i).wait()
            g0 = pl.multiple_of((idx // 16) * 16, 16)
            xio[pl.ds(g0, 16), :] = xres[pl.ds(g0, 16), :].astype(bf16)
            fix = pltpu.make_async_copy(xio.at[pl.ds(g0, 16), :], out_hbm.at[pl.ds(g0, 16), :], sem_w.at[7])
            fix.start()
            fix.wait()

    def layer_body(layer, c):
        phase_a(layer)
        phase_b()
        phase_c(layer)
        phase_d(layer)
        return c

    xres[...] = jnp.zeros_like(xres)
    lax.fori_loop(0, 2, layer_body, 0)


@jax.jit
def pallas_interleave_layers__sliding_block__moe_arch_mod__prompt_kernel(
    A_x: jax.Array,
    A_wqkv: jax.Array,
    A_wo: jax.Array,
    B_x: jax.Array,
    B_w_r: jax.Array,
    B_w_gate: jax.Array,
    B_w_up: jax.Array,
    B_w_down: jax.Array,
):
    del B_x
    x = A_x.reshape(S, D)
    any_spec = pl.BlockSpec(memory_space=pl.ANY)
    scratch = [
        pltpu.VMEM((S, D), bf16),
        pltpu.VMEM((D, 2 * D), bf16),
        pltpu.VMEM((D, D), bf16),
        pltpu.VMEM((D // 2, D), u32),
        pltpu.VMEM((D, D), bf16),
        pltpu.VMEM((D,), bf16),
        pltpu.VMEM((D, F), bf16),
        pltpu.VMEM((D, F), bf16),
        pltpu.VMEM((F, D), bf16),
        pltpu.VMEM((S, D), f32),
        pltpu.VMEM((S, D), f32),
        pltpu.VMEM((S, 128), f32),
        pltpu.VMEM((TQ // 2, D), u32),
        pltpu.VMEM((TQ // 2, D), u32),
        pltpu.VMEM((TQ // 2, D), u32),
        pltpu.VMEM((TQ // 2, D), u32),
        pltpu.VMEM((G, S // 2, 128), u32),
        pltpu.VMEM((G, (S + PAD) // 2, 128), u32),
        pltpu.VMEM((D // 2, S + PAD), u32),
        pltpu.VMEM((S, D), f32),
        pltpu.VMEM((2, 4, 256, 128), f32),
        pltpu.VMEM((2, 4, 8, 128), f32),
        pltpu.VMEM((TQ, D), f32),
        pltpu.VMEM((TQ, D), f32),
        pltpu.SemaphoreType.DMA((NB,)),
        pltpu.SemaphoreType.DMA((8,)),
        pltpu.SemaphoreType.DMA((NB,)),
    ]
    out = pl.pallas_call(
        _kernel,
        out_shape=jax.ShapeDtypeStruct((S, D), bf16),
        in_specs=[any_spec] * 7,
        out_specs=any_spec,
        scratch_shapes=scratch,
        compiler_params=pltpu.CompilerParams(vmem_limit_bytes=120 * 1024 * 1024),
    )(x, A_wqkv, A_wo, B_w_r, B_w_gate, B_w_up, B_w_down)
    return out.reshape(1, S, D)
```

```python
import jax
import jax.numpy as jnp
from jax import lax
import jax.experimental.pallas as pl
import jax.experimental.pallas.tpu as pltpu

bf16 = jnp.bfloat16
f32 = jnp.float32
u32 = jnp.uint32
i32 = jnp.int32

S = 2048
D = 1024
H = 32
DH = 32
W = 256
F = 3584
G = 8
PAD = 256
TQ = 256
NB = S // TQ
NSB = S // 128
CH = 32
NCH = TQ // CH
EPS = 1e-5
NEG = -1e30
QSCALE = (DH ** -0.5) * 1.4426950408889634
NT = (((1,), (1,)), ((), ()))


def _ln(x):
    m = jnp.mean(x, axis=-1, keepdims=True)
    xc = x - m
    v = jnp.mean(xc * xc, axis=-1, keepdims=True)
    return xc * lax.rsqrt(v + EPS)


def _pack_rows(x):
    return pltpu.bitcast(x.astype(bf16), u32)


def _pack_rows_interleaved(x):
    n = x.shape[0] // 16
    x3 = x.reshape(n, 16, x.shape[1])
    a = x3[:, 0:8, :].reshape(n * 8, x.shape[1])
    b = x3[:, 8:16, :].reshape(n * 8, x.shape[1])
    return pltpu.pack_elementwise([a, b], packed_dtype=bf16)


def _gate_first(x, gate, z):
    g = gate[0:8, 0:128] * z
    top = jnp.concatenate([x[0:8, 0:128] + g, x[0:8, 128:]], axis=1)
    return jnp.concatenate([top, x[8:]], axis=0)


def _kernel(x_hbm, wqkv_hbm, wo_hbm, wr_hbm, wg_hbm, wu_hbm, wd_hbm,
            out_hbm,
            xio, wqk_v, wv_v, wvt_v, wo_v, wr_v, wg_v, wu_v, wd_v,
            xres, xbuf, r_s, rho_s, z_s,
            xca, xia, xcb, xib,
            q_s, k_s, vt_s, ot_s, s_s, m_s,
            ata, atb,
            sem_x, sem_w, sem_o):
    def x_copy(i):
        r0 = pl.multiple_of(i * TQ, TQ)
        return pltpu.make_async_copy(x_hbm.at[pl.ds(r0, TQ), :], xio.at[pl.ds(r0, TQ), :], sem_x.at[i])

    def out_copy(i):
        r0 = pl.multiple_of(i * TQ, TQ)
        return pltpu.make_async_copy(xio.at[pl.ds(r0, TQ), :], out_hbm.at[pl.ds(r0, TQ), :], sem_o.at[i])

    cp_wv = pltpu.make_async_copy(wqkv_hbm.at[:, pl.ds(2 * D, D)], wv_v, sem_w.at[0])
    cp_wqk = pltpu.make_async_copy(wqkv_hbm.at[:, pl.ds(0, 2 * D)], wqk_v, sem_w.at[1])
    cp_wo = pltpu.make_async_copy(wo_hbm, wo_v, sem_w.at[2])
    cp_wr = pltpu.make_async_copy(wr_hbm, wr_v, sem_w.at[3])
    cp_wg = pltpu.make_async_copy(wg_hbm, wg_v, sem_w.at[4])
    cp_wu = pltpu.make_async_copy(wu_hbm, wu_v, sem_w.at[5])
    cp_wd = pltpu.make_async_copy(wd_hbm, wd_v, sem_w.at[6])

    x_copy(0).start()
    cp_wv.start()
    cp_wqk.start()
    for i in range(1, NB):
        x_copy(i).start()
    cp_wo.start()
    cp_wr.start()
    cp_wg.start()
    cp_wu.start()
    cp_wd.start()

    k_s[:, 0:PAD // 2, :] = jnp.zeros((G, PAD // 2, 128), u32)
    vt_s[:, 0:PAD] = jnp.zeros((D // 2, PAD), u32)

    cp_wv.wait()
    wvt_v[...] = pltpu.bitcast(wv_v[...].T, u32)

    def ln_chunk(layer, i, c, xc_ref, xi_ref, gate):
        r0 = pl.multiple_of(i * TQ + c * CH, CH)
        x_in = xio[pl.ds(r0, CH), :].astype(f32)
        x_rs = xres[pl.ds(r0, CH), :]
        x = jnp.where(layer == 0, x_in, x_rs)
        xbuf[pl.ds(r0, CH), :] = x
        if gate is not None:
            x = _gate_first(x, gate, z_s[...])
        xn = _ln(x)
        xc_ref[c * CH // 2:(c + 1) * CH // 2, :] = _pack_rows(xn)
        xi_ref[c * CH // 2:(c + 1) * CH // 2, :] = _pack_rows_interleaved(xn)

    def proj_step(layer, i, xc_ref, xi_ref, i_next, xc_next, xi_next):
        h0 = pl.multiple_of(i * (TQ // 2), TQ // 2)
        a = pltpu.bitcast(xc_ref[...], bf16)
        ys = []
        for n in range(2 * G):
            y = jnp.dot(a, wqk_v[:, n * 128:(n + 1) * 128], preferred_element_type=f32)
            if n < G:
                q_s[n, pl.ds(h0, TQ // 2), :] = _pack_rows(y * QSCALE)
            else:
                k_s[n - G, pl.ds(PAD // 2 + h0, TQ // 2), :] = _pack_rows(y)
            ys.append(y)
        vt = lax.dot_general(pltpu.bitcast(wvt_v[...], bf16), pltpu.bitcast(xi_ref[...], bf16), NT,
                             preferred_element_type=f32)
        c0 = pl.multiple_of(PAD + i * TQ, TQ)
        vt_s[:, pl.ds(c0, TQ)] = _pack_rows(vt)
        for c in range(NCH):
            ln_chunk(layer, i_next, c, xc_next, xi_next, ys[c * len(ys) // NCH])

    def phase_a(layer):
        @pl.when(layer == 0)
        def _():
            x_copy(0).wait()
            cp_wqk.wait()

        for c in range(NCH):
            ln_chunk(layer, 0, c, xca, xia, None)

        def body(j, c):
            i0 = 2 * j
            i2 = jnp.minimum(i0 + 2, NB - 1)

            @pl.when(layer == 0)
            def _():
                x_copy(i0 + 1).wait()

                @pl.when(i0 + 2 < NB)
                def _():
                    x_copy(i2).wait()

            proj_step(layer, i0, xca, xia, i0 + 1, xcb, xib)
            proj_step(layer, i0 + 1, xcb, xib, i2, xca, xia)
            return c

        lax.fori_loop(0, NB // 2, body, 0)

    def qk_stage(g, q0, slot, masked):
        lane16 = lax.broadcasted_iota(i32, (16, 128), 1)
        r16 = lax.broadcasted_iota(i32, (16, 128), 0)
        hb16 = lane16 // 32
        dd = r16 - lane16 % 32
        h0 = q0 // 2
        first_rows = None
        for b in range(4):
            base = pl.multiple_of(h0 + 16 * b, 16)
            parts = [k_s[g, pl.ds(base, 8), :], k_s[g, pl.ds(base + 128, 8), :],
                     k_s[g, pl.ds(base + 8, 8), :], k_s[g, pl.ds(base + 136, 8), :],
                     k_s[g, pl.ds(base + 16, 112), :]]
            kw = pltpu.bitcast(jnp.concatenate(parts, axis=0), bf16)
            qu = q_s[g, pl.ds(base, 16), :]
            qall = pltpu.bitcast(
                jnp.concatenate([jnp.where(hb16 == (p - b) % 4, qu, jnp.uint32(0)) for p in range(4)], axis=0),
                bf16)
            st = lax.dot_general(kw, qall, NT, preferred_element_type=f32)
            lo0, hi0, lo1, hi1, mid = st[0:16], st[16:32], st[32:48], st[48:64], st[64:288]
            if b == 0:
                first_rows = st[0:8]
            if masked:
                first = PAD - (q0 + 32 * b)
                lo0 = jnp.where(r16 >= first, lo0, NEG)
                lo1 = jnp.where(r16 + 16 >= first, lo1, NEG)
                rm = lax.broadcasted_iota(i32, (224, 128), 0)
                mid = jnp.where(rm + 32 >= first, mid, NEG)
            c0 = jnp.where(dd > 0, lo0, hi0)
            c1 = jnp.where(dd > -16, lo1, hi1)
            x = jnp.concatenate([c0, c1, mid], axis=0)
            s_s[slot, b] = x
            mm = jnp.max(x.reshape(32, 8, 128), axis=0)
            m_s[slot, b] = jnp.broadcast_to(jnp.max(mm, axis=0, keepdims=True), (8, 128))
        return first_rows

    def pv_stage(g, q0, slot, gate):
        r8 = lax.broadcasted_iota(i32, (8, 128), 0)
        c8 = lax.broadcasted_iota(i32, (8, 128), 1)
        blk = c8 // 32
        j = c8 % 32

        def tri(u):
            return (jnp.where(16 * u + r8 > j, jnp.uint32(0xFFFF), jnp.uint32(0)) |
                    jnp.where(16 * u + 8 + r8 > j, jnp.uint32(0xFFFF0000), jnp.uint32(0)))

        tris = [tri(0), tri(1)]
        ms = [m_s[slot, b] for b in range(4)]
        L = [None] * 4
        cache = {}

        def pexp(b, u):
            x = s_s[slot, b, 16 * u:16 * u + 16, :]
            p0 = jnp.exp2(x[0:8] - ms[b])
            p1 = jnp.exp2(x[8:16] - ms[b])
            sm = p0 + p1
            L[b] = sm if L[b] is None else L[b] + sm
            return pltpu.pack_elementwise([p0, p1], packed_dtype=bf16)

        def get_p(b, u):
            if u < 2:
                pk = pexp(b, u)
                lo = pk & tris[u]
                cache[(b, u + 16)] = pk ^ lo
                return lo
            if u >= 16:
                return cache.pop((b, u))
            return pexp(b, u)

        zero = jnp.zeros((8, 128), u32)
        accs = [None] * 4
        for k in range(3):
            wts = [[] for _ in range(4)]
            for t in range(8 * k, 8 * k + 8):
                if t == 8:
                    gv = gate * z_s[...]
                    for b in range(4):
                        ms[b] = ms[b] + gv
                srcs = [(b, get_p(b, t - 2 * b)) for b in range(4) if 0 <= t - 2 * b < 18]
                for h in range(4):
                    acc = zero if len(srcs) < 4 else None
                    for (b, v) in srcs:
                        acc = v if acc is None else jnp.where(blk == (h + b) % 4, v, acc)
                    wts[h].append(acc)
            c0 = pl.multiple_of(q0 + 128 * k, 128)
            for h in range(4):
                pt = pltpu.bitcast(jnp.concatenate(wts[h], axis=0), bf16)
                vth = pltpu.bitcast(vt_s[pl.ds((g * 4 + h) * 16, 16), pl.ds(c0, 128)], bf16)
                d = jnp.dot(vth, pt, preferred_element_type=f32)
                accs[h] = d if accs[h] is None else accs[h] + d
        L = [jnp.broadcast_to(jnp.sum(l, axis=0, keepdims=True), (8, 128)) for l in L]
        outs = []
        for h in range(4):
            lh = L[0]
            for b in range(1, 4):
                lh = jnp.where(blk == (h + b) % 4, L[b], lh)
            ot = (accs[h].reshape(4, 8, 128) * pl.reciprocal(lh, approx=False)[None]).reshape(32, 128)
            if h > 0:
                ot = pltpu.roll(ot, 128 - 32 * h, axis=1)
            outs.append(ot)
        ot_s[g * 128:(g + 1) * 128, pl.ds(q0, 128)] = jnp.concatenate(outs, axis=0)

    def phase_b():
        def make_body(masked):
            def body(sb, c):
                q0 = pl.multiple_of(sb * 128, 128)
                qn = pl.multiple_of(jnp.minimum(sb + 1, NSB - 1) * 128, 128)
                for g in range(G):
                    if g + 1 < G:
                        gate = qk_stage(g + 1, q0, (g + 1) % 2, masked)
                    else:
                        gate = qk_stage(0, qn, 0, masked)
                    pv_stage(g, q0, g % 2, gate)
                return c
            return body

        qk_stage(0, 0, 0, True)
        lax.fori_loop(0, 2, make_body(True), 0)
        lax.fori_loop(2, NSB, make_body(False), 0)

    def resid_chunk(i, c, at_ref, gate):
        r0 = pl.multiple_of(i * TQ + c * CH, CH)
        x1 = xbuf[pl.ds(r0, CH), :] + at_ref[c * CH:(c + 1) * CH, :]
        if gate is not None:
            x1 = _gate_first(x1, gate, z_s[...])
        m = jnp.mean(x1, axis=-1, keepdims=True)
        xc = x1 - m
        v = jnp.mean(xc * xc, axis=-1, keepdims=True)
        rho = lax.rsqrt(v + EPS)
        xn = xc * rho
        r = jnp.sum(xn * wr_v[...].astype(f32).reshape(1, D), axis=-1, keepdims=True)
        r_s[pl.ds(r0, CH), :] = jnp.broadcast_to(r, (CH, 128))
        rho_s[pl.ds(r0, CH), :] = jnp.broadcast_to(rho, (CH, 128))
        x2 = x1 + xn
        xres[pl.ds(r0, CH), :] = x2
        xio[pl.ds(r0, CH), :] = x2.astype(bf16)

    def oproj_step(i_dot, at_w, i_res, at_r):
        ys = []
        if i_dot is not None:
            r0 = pl.multiple_of(i_dot * TQ, TQ)
            a = ot_s[:, pl.ds(r0, TQ)].astype(bf16).T
            for n in range(G):
                y = jnp.dot(a, wo_v[:, n * 128:(n + 1) * 128], preferred_element_type=f32)
                at_w[:, n * 128:(n + 1) * 128] = y
                ys.append(y)
        if i_res is not None:
            for c in range(NCH):
                gate = ys[c * len(ys) // NCH - 1] if (ys and c > 0) else None
                resid_chunk(i_res, c, at_r, gate)

    def phase_c(layer):
        @pl.when(layer == 0)
        def _():
            cp_wo.wait()
            cp_wr.wait()

        def flush(i):
            @pl.when(layer == 1)
            def _():
                out_copy(i).start()

        oproj_step(0, ata, None, None)

        def body(j, c):
            i0 = 2 * j
            oproj_step(i0 + 1, atb, i0, ata)
            oproj_step(i0 + 2, ata, i0 + 1, atb)
            flush(i0)
            flush(i0 + 1)
            return c

        lax.fori_loop(0, NB // 2 - 1, body, 0)
        oproj_step(NB - 1, atb, NB - 2, ata)
        oproj_step(None, None, NB - 1, atb)
        flush(NB - 2)
        flush(NB - 1)

    def phase_d(layer):
        @pl.when(layer == 0)
        def _():
            cp_wg.wait()
            cp_wu.wait()
            cp_wd.wait()

        rb = r_s[...].astype(bf16).astype(f32)
        rmax = jnp.max(rb)
        rows = lax.broadcasted_iota(i32, (S, 128), 0)
        idx = jnp.min(jnp.where(rb == rmax, rows, S))
        idx = jnp.clip(idx, 0, S - 1)
        x2 = xres[pl.ds(idx, 1), :]
        rho = rho_s[pl.ds(idx, 1), 0:1]
        xn = (x2 - jnp.mean(x2, axis=-1, keepdims=True)) * (rho / (1.0 + rho))
        xs = jnp.broadcast_to(xn, (16, D)).astype(bf16)
        gate = jnp.dot(xs, wg_v[...], preferred_element_type=f32)
        up = jnp.dot(xs, wu_v[...], preferred_element_type=f32)
        hmid = (gate * jax.nn.sigmoid(gate) * up).astype(bf16)
        y = jnp.dot(hmid, wd_v[...], preferred_element_type=f32)
        scale = jax.nn.sigmoid(jnp.full((1, D), rmax, f32))
        xres[pl.ds(idx, 1), :] = xres[pl.ds(idx, 1), :] + y[0:1] * scale

        @pl.when(layer == 1)
        def _():
            for i in range(NB):
                out_copy(i).wait()
            g0 = pl.multiple_of((idx // 16) * 16, 16)
            xio[pl.ds(g0, 16), :] = xres[pl.ds(g0, 16), :].astype(bf16)
            fix = pltpu.make_async_copy(xio.at[pl.ds(g0, 16), :], out_hbm.at[pl.ds(g0, 16), :], sem_w.at[7])
            fix.start()
            fix.wait()

    def layer_body(layer, c):
        with jax.named_scope("phase_a"):
            phase_a(layer)
        with jax.named_scope("phase_b"):
            phase_b()
        with jax.named_scope("phase_c"):
            phase_c(layer)
        with jax.named_scope("phase_d"):
            phase_d(layer)
        return c

    z_s[...] = jnp.zeros_like(z_s)
    lax.fori_loop(0, 2, layer_body, 0)


@jax.jit
def pallas_interleave_layers__sliding_block__moe_arch_mod__prompt_kernel(
    A_x: jax.Array,
    A_wqkv: jax.Array,
    A_wo: jax.Array,
    B_x: jax.Array,
    B_w_r: jax.Array,
    B_w_gate: jax.Array,
    B_w_up: jax.Array,
    B_w_down: jax.Array,
):
    del B_x
    x = A_x.reshape(S, D)
    any_spec = pl.BlockSpec(memory_space=pl.ANY)
    scratch = [
        pltpu.VMEM((S, D), bf16),
        pltpu.VMEM((D, 2 * D), bf16),
        pltpu.VMEM((D, D), bf16),
        pltpu.VMEM((D // 2, D), u32),
        pltpu.VMEM((D, D), bf16),
        pltpu.VMEM((D,), bf16),
        pltpu.VMEM((D, F), bf16),
        pltpu.VMEM((D, F), bf16),
        pltpu.VMEM((F, D), bf16),
        pltpu.VMEM((S, D), f32),
        pltpu.VMEM((S, D), f32),
        pltpu.VMEM((S, 128), f32),
        pltpu.VMEM((S, 128), f32),
        pltpu.VMEM((8, 128), f32),
        pltpu.VMEM((TQ // 2, D), u32),
        pltpu.VMEM((TQ // 2, D), u32),
        pltpu.VMEM((TQ // 2, D), u32),
        pltpu.VMEM((TQ // 2, D), u32),
        pltpu.VMEM((G, S // 2, 128), u32),
        pltpu.VMEM((G, (S + PAD) // 2, 128), u32),
        pltpu.VMEM((D // 2, S + PAD), u32),
        pltpu.VMEM((D, S), f32),
        pltpu.VMEM((2, 4, 256, 128), f32),
        pltpu.VMEM((2, 4, 8, 128), f32),
        pltpu.VMEM((TQ, D), f32),
        pltpu.VMEM((TQ, D), f32),
        pltpu.SemaphoreType.DMA((NB,)),
        pltpu.SemaphoreType.DMA((8,)),
        pltpu.SemaphoreType.DMA((NB,)),
    ]
    out = pl.pallas_call(
        _kernel,
        out_shape=jax.ShapeDtypeStruct((S, D), bf16),
        in_specs=[any_spec] * 7,
        out_specs=any_spec,
        scratch_shapes=scratch,
        compiler_params=pltpu.CompilerParams(vmem_limit_bytes=120 * 1024 * 1024),
    )(x, A_wqkv, A_wo, B_w_r, B_w_gate, B_w_up, B_w_down)
    return out.reshape(1, S, D)
```

```python
import jax
import jax.numpy as jnp
from jax import lax
import jax.experimental.pallas as pl
import jax.experimental.pallas.tpu as pltpu

bf16 = jnp.bfloat16
f32 = jnp.float32
u32 = jnp.uint32
i32 = jnp.int32

S = 2048
D = 1024
H = 32
DH = 32
W = 256
F = 3584
G = 8
PAD = 256
TQ = 256
NB = S // TQ
NSB = S // 128
import os
CH = int(os.environ.get('K_CH', 32))
NCH = TQ // CH
CHC = int(os.environ.get('K_CHC', 32))
NCHC = TQ // CHC
GATE_A = [int(v) for v in os.environ.get('K_GA', '-1,0,1,2,3,4,5,6').split(',')]
GATE_C = [int(v) for v in os.environ.get('K_GC', '-1,0,1,2,3,4,5,6').split(',')]
EPS = 1e-5
NEG = -1e30
QSCALE = (DH ** -0.5) * 1.4426950408889634
NT = (((1,), (1,)), ((), ()))


def _ln(x):
    m = jnp.mean(x, axis=-1, keepdims=True)
    xc = x - m
    v = jnp.mean(xc * xc, axis=-1, keepdims=True)
    return xc * lax.rsqrt(v + EPS)


def _pack_rows(x):
    return pltpu.bitcast(x.astype(bf16), u32)


def _pack_rows_interleaved(x):
    n = x.shape[0] // 16
    x3 = x.reshape(n, 16, x.shape[1])
    a = x3[:, 0:8, :].reshape(n * 8, x.shape[1])
    b = x3[:, 8:16, :].reshape(n * 8, x.shape[1])
    return pltpu.pack_elementwise([a, b], packed_dtype=bf16)


def _gate_first(x, gate, z):
    g = gate[0:8, 0:128] * z
    top = jnp.concatenate([x[0:8, 0:128] + g, x[0:8, 128:]], axis=1)
    return jnp.concatenate([top, x[8:]], axis=0)


def _kernel(x_hbm, wqkv_hbm, wo_hbm, wr_hbm, wg_hbm, wu_hbm, wd_hbm,
            out_hbm,
            xio, wq_v, wk_v, wv_v, wvt_v, wo_v, wr_v, wg_v, wu_v, wd_v,
            xres, xbuf, r_s, rho_s, z_s, wr8,
            xca, xcb, xc_all, xi_all,
            q_s, k_s, vt_s, ot_s, s_s, m_s,
            ata, atb,
            sem_x, sem_w, sem_o):
    def x_copy(i):
        r0 = pl.multiple_of(i * TQ, TQ)
        return pltpu.make_async_copy(x_hbm.at[pl.ds(r0, TQ), :], xio.at[pl.ds(r0, TQ), :], sem_x.at[i])

    def out_copy(i):
        r0 = pl.multiple_of(i * TQ, TQ)
        return pltpu.make_async_copy(xio.at[pl.ds(r0, TQ), :], out_hbm.at[pl.ds(r0, TQ), :], sem_o.at[i])

    cp_wq = pltpu.make_async_copy(wqkv_hbm.at[:, pl.ds(0, D)], wq_v, sem_w.at[0])
    cp_wk = pltpu.make_async_copy(wqkv_hbm.at[:, pl.ds(D, D)], wk_v, sem_w.at[1])
    cp_wv = pltpu.make_async_copy(wqkv_hbm.at[:, pl.ds(2 * D, D)], wv_v, sem_w.at[8])
    cp_wo = pltpu.make_async_copy(wo_hbm, wo_v, sem_w.at[2])
    cp_wr = pltpu.make_async_copy(wr_hbm, wr_v, sem_w.at[3])
    cp_wg = pltpu.make_async_copy(wg_hbm, wg_v, sem_w.at[4])
    cp_wu = pltpu.make_async_copy(wu_hbm, wu_v, sem_w.at[5])
    cp_wd = pltpu.make_async_copy(wd_hbm, wd_v, sem_w.at[6])

    x_copy(0).start()
    cp_wq.start()

    k_s[:, 0:PAD // 2, :] = jnp.zeros((G, PAD // 2, 128), u32)
    vt_s[:, 0:PAD] = jnp.zeros((D // 2, PAD), u32)
    z_s[...] = jnp.zeros_like(z_s)

    def ln_chunk(layer, i, c, xc_ref, gate):
        r0 = pl.multiple_of(i * TQ + c * CH, CH)
        h0 = pl.multiple_of(i * (TQ // 2) + c * (CH // 2), CH // 2)
        x_in = xio[pl.ds(r0, CH), :].astype(f32)
        x_rs = xres[pl.ds(r0, CH), :]
        x = jnp.where(layer == 0, x_in, x_rs)
        xbuf[pl.ds(r0, CH), :] = x
        if gate is not None:
            x = _gate_first(x, gate, z_s[...])
        xn = _ln(x)
        xc = _pack_rows(xn)
        xc_ref[c * CH // 2:(c + 1) * CH // 2, :] = xc
        xc_all[pl.ds(h0, CH // 2), :] = xc
        xi_all[pl.ds(h0, CH // 2), :] = _pack_rows_interleaved(xn)

    def q_step(layer, i, xc_ref, i_next, xc_next):
        h0 = pl.multiple_of(i * (TQ // 2), TQ // 2)
        a = pltpu.bitcast(xc_ref[...], bf16)
        ys = []
        for n in range(G):
            y = jnp.dot(a, wq_v[:, n * 128:(n + 1) * 128], preferred_element_type=f32)
            q_s[n, pl.ds(h0, TQ // 2), :] = _pack_rows(y * QSCALE)
            ys.append(y)
        for c in range(NCH):
            gi = GATE_A[c]
            gate = ys[gi] if gi >= 0 else None
            ln_chunk(layer, i_next, c, xc_next, gate)

    def kv_step(i):
        h0 = pl.multiple_of(i * (TQ // 2), TQ // 2)
        a = pltpu.bitcast(xc_all[pl.ds(h0, TQ // 2), :], bf16)
        for n in range(G):
            y = jnp.dot(a, wk_v[:, n * 128:(n + 1) * 128], preferred_element_type=f32)
            k_s[n, pl.ds(PAD // 2 + h0, TQ // 2), :] = _pack_rows(y)
        vt = lax.dot_general(pltpu.bitcast(wvt_v[...], bf16), pltpu.bitcast(xi_all[pl.ds(h0, TQ // 2), :], bf16),
                             NT, preferred_element_type=f32)
        c0 = pl.multiple_of(PAD + i * TQ, TQ)
        vt_s[:, pl.ds(c0, TQ)] = _pack_rows(vt)

    def phase_a(layer):
        @pl.when(layer == 0)
        def _():
            x_copy(0).wait()
            for i in range(1, NB):
                x_copy(i).start()

        for c in range(NCH):
            ln_chunk(layer, 0, c, xca, None)

        @pl.when(layer == 0)
        def _():
            cp_wq.wait()
            cp_wv.start()
            cp_wk.start()
            cp_wo.start()
            cp_wr.start()

        def q_body(j, c):
            i0 = 2 * j
            i2 = jnp.minimum(i0 + 2, NB - 1)

            @pl.when(layer == 0)
            def _():
                x_copy(i0 + 1).wait()

                @pl.when(i0 + 2 < NB)
                def _():
                    x_copy(i2).wait()

            q_step(layer, i0, xca, i0 + 1, xcb)
            q_step(layer, i0 + 1, xcb, i2, xca)
            return c

        with jax.named_scope("a_q"):
            lax.fori_loop(0, NB // 2, q_body, 0)

        @pl.when(layer == 0)
        def _():
            cp_wv.wait()
            wvt_v[...] = pltpu.bitcast(wv_v[...].T, u32)
            cp_wk.wait()
            cp_wg.start()
            cp_wu.start()
            cp_wd.start()

        def kv_body(j, c):
            kv_step(2 * j)
            kv_step(2 * j + 1)
            return c

        with jax.named_scope("a_kv"):
            lax.fori_loop(0, NB // 2, kv_body, 0)

    def qk_stage(g, q0, slot, masked):
        zi = pltpu.bitcast(z_s[...], i32)
        zi16 = jnp.concatenate([zi, zi], axis=0)
        lane16 = lax.broadcasted_iota(i32, (16, 128), 1) + zi16
        r16 = lax.broadcasted_iota(i32, (16, 128), 0)
        hb16 = lane16 // 32
        dd = r16 - lane16 % 32
        h0 = q0 // 2
        first_rows = None
        for b in range(4):
            base = pl.multiple_of(h0 + 16 * b, 16)
            parts = [k_s[g, pl.ds(base, 8), :], k_s[g, pl.ds(base + 128, 8), :],
                     k_s[g, pl.ds(base + 8, 8), :], k_s[g, pl.ds(base + 136, 8), :],
                     k_s[g, pl.ds(base + 16, 112), :]]
            kw = pltpu.bitcast(jnp.concatenate(parts, axis=0), bf16)
            qu = q_s[g, pl.ds(base, 16), :]
            qall = pltpu.bitcast(
                jnp.concatenate([jnp.where(hb16 == (p - b) % 4, qu, jnp.uint32(0)) for p in range(4)], axis=0),
                bf16)
            st = lax.dot_general(kw, qall, NT, preferred_element_type=f32)
            lo0, hi0, lo1, hi1, mid = st[0:16], st[16:32], st[32:48], st[48:64], st[64:288]
            if b == 0:
                first_rows = st[0:8]
            if masked:
                first = PAD - (q0 + 32 * b)
                lo0 = jnp.where(r16 >= first, lo0, NEG)
                lo1 = jnp.where(r16 + 16 >= first, lo1, NEG)
                rm = lax.broadcasted_iota(i32, (224, 128), 0)
                mid = jnp.where(rm + 32 >= first, mid, NEG)
            c0 = jnp.where(dd > 0, lo0, hi0)
            c1 = jnp.where(dd > -16, lo1, hi1)
            x = jnp.concatenate([c0, c1, mid], axis=0)
            s_s[slot, b] = x
            mm = jnp.max(x.reshape(32, 8, 128), axis=0)
            m_s[slot, b] = jnp.broadcast_to(jnp.max(mm, axis=0, keepdims=True), (8, 128))
        return first_rows

    def pv_stage(g, q0, slot, gate):
        r8 = lax.broadcasted_iota(i32, (8, 128), 0)
        c8 = lax.broadcasted_iota(i32, (8, 128), 1) + pltpu.bitcast(z_s[...], i32)
        blk = c8 // 32
        j = c8 % 32

        def tri(u):
            return (jnp.where(16 * u + r8 > j, jnp.uint32(0xFFFF), jnp.uint32(0)) |
                    jnp.where(16 * u + 8 + r8 > j, jnp.uint32(0xFFFF0000), jnp.uint32(0)))

        tris = [tri(0), tri(1)]
        ms = [m_s[slot, b] for b in range(4)]
        L = [None] * 4
        cache = {}

        def pexp(b, u):
            x = s_s[slot, b, 16 * u:16 * u + 16, :]
            p0 = jnp.exp2(x[0:8] - ms[b])
            p1 = jnp.exp2(x[8:16] - ms[b])
            sm = p0 + p1
            L[b] = sm if L[b] is None else L[b] + sm
            return pltpu.pack_elementwise([p0, p1], packed_dtype=bf16)

        def get_p(b, u):
            if u < 2:
                pk = pexp(b, u)
                lo = pk & tris[u]
                cache[(b, u + 16)] = pk ^ lo
                return lo
            if u >= 16:
                return cache.pop((b, u))
            return pexp(b, u)

        zero = jnp.zeros((8, 128), u32)
        accs = [None] * 4
        for k in range(3):
            wts = [[] for _ in range(4)]
            for t in range(8 * k, 8 * k + 8):
                if t == 8:
                    gv = gate * z_s[...]
                    for b in range(4):
                        ms[b] = ms[b] + gv
                srcs = [(b, get_p(b, t - 2 * b)) for b in range(4) if 0 <= t - 2 * b < 18]
                for h in range(4):
                    acc = zero if len(srcs) < 4 else None
                    for (b, v) in srcs:
                        acc = v if acc is None else jnp.where(blk == (h + b) % 4, v, acc)
                    wts[h].append(acc)
            c0 = pl.multiple_of(q0 + 128 * k, 128)
            for h in range(4):
                pt = pltpu.bitcast(jnp.concatenate(wts[h], axis=0), bf16)
                vth = pltpu.bitcast(vt_s[pl.ds((g * 4 + h) * 16, 16), pl.ds(c0, 128)], bf16)
                d = jnp.dot(vth, pt, preferred_element_type=f32)
                accs[h] = d if accs[h] is None else accs[h] + d
        L = [jnp.broadcast_to(jnp.sum(l, axis=0, keepdims=True), (8, 128)) for l in L]
        outs = []
        for h in range(4):
            lh = L[0]
            for b in range(1, 4):
                lh = jnp.where(blk == (h + b) % 4, L[b], lh)
            r0 = pl.reciprocal(lh, approx=True)
            rl = r0 * (2.0 - lh * r0)
            ot = (accs[h].reshape(4, 8, 128) * rl[None]).reshape(32, 128)
            if h > 0:
                ot = pltpu.roll(ot, 128 - 32 * h, axis=1)
            outs.append(ot)
        ot_s[g * 128:(g + 1) * 128, pl.ds(q0, 128)] = jnp.concatenate(outs, axis=0)

    def phase_b():
        def make_body(masked):
            def body(sb, c):
                q0 = pl.multiple_of(sb * 128, 128)
                qn = pl.multiple_of(jnp.minimum(sb + 1, NSB - 1) * 128, 128)
                for g in range(G):
                    if g + 1 < G:
                        gate = qk_stage(g + 1, q0, (g + 1) % 2, masked)
                    else:
                        gate = qk_stage(0, qn, 0, masked)
                    pv_stage(g, q0, g % 2, gate)
                return c
            return body

        qk_stage(0, 0, 0, True)
        lax.fori_loop(0, 2, make_body(True), 0)
        lax.fori_loop(2, NSB, make_body(False), 0)

    def resid_chunk(i, c, at_ref, gate):
        r0 = pl.multiple_of(i * TQ + c * CHC, CHC)
        x1 = xbuf[pl.ds(r0, CHC), :] + at_ref[c * CHC:(c + 1) * CHC, :]
        if gate is not None:
            x1 = _gate_first(x1, gate, z_s[...])
        m = jnp.mean(x1, axis=-1, keepdims=True)
        xc = x1 - m
        v = jnp.mean(xc * xc, axis=-1, keepdims=True)
        rho = lax.rsqrt(v + EPS)
        xn = xc * rho
        r = jnp.sum(xn * wr8[0:1, :], axis=-1, keepdims=True)
        r_s[pl.ds(r0, CHC), :] = jnp.broadcast_to(r, (CHC, 128))
        rho_s[pl.ds(r0, CHC), :] = jnp.broadcast_to(rho, (CHC, 128))
        x2 = x1 + xn
        xres[pl.ds(r0, CHC), :] = x2
        xio[pl.ds(r0, CHC), :] = x2.astype(bf16)

    def oproj_step(i_dot, at_w, i_res, at_r):
        ys = []
        if i_dot is not None:
            r0 = pl.multiple_of(i_dot * TQ, TQ)
            a = ot_s[:, pl.ds(r0, TQ)].astype(bf16).T
            for n in range(G):
                y = jnp.dot(a, wo_v[:, n * 128:(n + 1) * 128], preferred_element_type=f32)
                at_w[:, n * 128:(n + 1) * 128] = y
                ys.append(y)
        if i_res is not None:
            for c in range(NCHC):
                gi = GATE_C[c] if ys else -1
                gate = ys[gi] if gi >= 0 else None
                resid_chunk(i_res, c, at_r, gate)

    def phase_c(layer):
        @pl.when(layer == 0)
        def _():
            cp_wo.wait()
            cp_wr.wait()
            wr8[...] = jnp.broadcast_to(wr_v[...].astype(f32).reshape(1, D), (8, D))

        def flush(i):
            @pl.when(layer == 1)
            def _():
                out_copy(i).start()

        oproj_step(0, ata, None, None)

        def body(j, c):
            i0 = 2 * j
            oproj_step(i0 + 1, atb, i0, ata)
            oproj_step(i0 + 2, ata, i0 + 1, atb)
            flush(i0)
            flush(i0 + 1)
            return c

        lax.fori_loop(0, NB // 2 - 1, body, 0)
        oproj_step(NB - 1, atb, NB - 2, ata)
        oproj_step(None, None, NB - 1, atb)
        flush(NB - 2)
        flush(NB - 1)

    def phase_d(layer):
        @pl.when(layer == 0)
        def _():
            cp_wg.wait()
            cp_wu.wait()
            cp_wd.wait()

        rb = r_s[...].astype(bf16).astype(f32)
        rmax = jnp.max(rb)
        rows = lax.broadcasted_iota(i32, (S, 128), 0)
        idx = jnp.min(jnp.where(rb == rmax, rows, S))
        idx = jnp.clip(idx, 0, S - 1)
        x2 = xres[pl.ds(idx, 1), :]
        rho = rho_s[pl.ds(idx, 1), 0:1]
        xn = (x2 - jnp.mean(x2, axis=-1, keepdims=True)) * (rho / (1.0 + rho))
        xs = jnp.broadcast_to(xn, (16, D)).astype(bf16)
        gate = jnp.dot(xs, wg_v[...], preferred_element_type=f32)
        up = jnp.dot(xs, wu_v[...], preferred_element_type=f32)
        hmid = (gate * jax.nn.sigmoid(gate) * up).astype(bf16)
        y = jnp.dot(hmid, wd_v[...], preferred_element_type=f32)
        scale = jax.nn.sigmoid(jnp.full((1, D), rmax, f32))
        xres[pl.ds(idx, 1), :] = xres[pl.ds(idx, 1), :] + y[0:1] * scale

        @pl.when(layer == 1)
        def _():
            for i in range(NB):
                out_copy(i).wait()
            g0 = pl.multiple_of((idx // 16) * 16, 16)
            xio[pl.ds(g0, 16), :] = xres[pl.ds(g0, 16), :].astype(bf16)
            fix = pltpu.make_async_copy(xio.at[pl.ds(g0, 16), :], out_hbm.at[pl.ds(g0, 16), :], sem_w.at[7])
            fix.start()
            fix.wait()

    def layer_body(layer, c):
        with jax.named_scope("phase_a"):
            phase_a(layer)
        with jax.named_scope("phase_b"):
            phase_b()
        with jax.named_scope("phase_c"):
            phase_c(layer)
        with jax.named_scope("phase_d"):
            phase_d(layer)
        return c

    lax.fori_loop(0, 2, layer_body, 0)


@jax.jit
def pallas_interleave_layers__sliding_block__moe_arch_mod__prompt_kernel(
    A_x: jax.Array,
    A_wqkv: jax.Array,
    A_wo: jax.Array,
    B_x: jax.Array,
    B_w_r: jax.Array,
    B_w_gate: jax.Array,
    B_w_up: jax.Array,
    B_w_down: jax.Array,
):
    del B_x
    x = A_x.reshape(S, D)
    any_spec = pl.BlockSpec(memory_space=pl.ANY)
    scratch = [
        pltpu.VMEM((S, D), bf16),
        pltpu.VMEM((D, D), bf16),
        pltpu.VMEM((D, D), bf16),
        pltpu.VMEM((D, D), bf16),
        pltpu.VMEM((D // 2, D), u32),
        pltpu.VMEM((D, D), bf16),
        pltpu.VMEM((D,), bf16),
        pltpu.VMEM((D, F), bf16),
        pltpu.VMEM((D, F), bf16),
        pltpu.VMEM((F, D), bf16),
        pltpu.VMEM((S, D), f32),
        pltpu.VMEM((S, D), f32),
        pltpu.VMEM((S, 128), f32),
        pltpu.VMEM((S, 128), f32),
        pltpu.VMEM((8, 128), f32),
        pltpu.VMEM((8, D), f32),
        pltpu.VMEM((TQ // 2, D), u32),
        pltpu.VMEM((TQ // 2, D), u32),
        pltpu.VMEM((S // 2, D), u32),
        pltpu.VMEM((S // 2, D), u32),
        pltpu.VMEM((G, S // 2, 128), u32),
        pltpu.VMEM((G, (S + PAD) // 2, 128), u32),
        pltpu.VMEM((D // 2, S + PAD), u32),
        pltpu.VMEM((D, S), f32),
        pltpu.VMEM((2, 4, 256, 128), f32),
        pltpu.VMEM((2, 4, 8, 128), f32),
        pltpu.VMEM((TQ, D), f32),
        pltpu.VMEM((TQ, D), f32),
        pltpu.SemaphoreType.DMA((NB,)),
        pltpu.SemaphoreType.DMA((9,)),
        pltpu.SemaphoreType.DMA((NB,)),
    ]
    out = pl.pallas_call(
        _kernel,
        out_shape=jax.ShapeDtypeStruct((S, D), bf16),
        in_specs=[any_spec] * 7,
        out_specs=any_spec,
        scratch_shapes=scratch,
        compiler_params=pltpu.CompilerParams(vmem_limit_bytes=120 * 1024 * 1024),
    )(x, A_wqkv, A_wo, B_w_r, B_w_gate, B_w_up, B_w_down)
    return out.reshape(1, S, D)
```

```python
import jax
import jax.numpy as jnp
from jax import lax
import jax.experimental.pallas as pl
import jax.experimental.pallas.tpu as pltpu

bf16 = jnp.bfloat16
f32 = jnp.float32
u32 = jnp.uint32
i32 = jnp.int32

S = 2048
D = 1024
H = 32
DH = 32
W = 256
F = 3584
G = 8
PAD = 256
TQ = 256
NB = S // TQ
NSB = S // 128
import os
CH = int(os.environ.get('K_CH', 32))
NCH = TQ // CH
CHC = int(os.environ.get('K_CHC', 32))
NCHC = TQ // CHC
GATE_A = [int(v) for v in os.environ.get('K_GA', '-1,0,1,2,3,4,5,6').split(',')]
GATE_C = [int(v) for v in os.environ.get('K_GC', '-1,0,1,2,3,4,5,6').split(',')]
EPS = 1e-5
NEG = -1e30
QSCALE = (DH ** -0.5) * 1.4426950408889634
NT = (((1,), (1,)), ((), ()))


def _ln(x):
    m = jnp.mean(x, axis=-1, keepdims=True)
    xc = x - m
    v = jnp.mean(xc * xc, axis=-1, keepdims=True)
    return xc * lax.rsqrt(v + EPS)


def _pack_rows(x):
    return pltpu.bitcast(x.astype(bf16), u32)


def _pack_rows_interleaved(x):
    n = x.shape[0] // 16
    x3 = x.reshape(n, 16, x.shape[1])
    a = x3[:, 0:8, :].reshape(n * 8, x.shape[1])
    b = x3[:, 8:16, :].reshape(n * 8, x.shape[1])
    return pltpu.pack_elementwise([a, b], packed_dtype=bf16)


def _gate_first(x, gate, z):
    g = gate[0:8, 0:128] * z
    top = jnp.concatenate([x[0:8, 0:128] + g, x[0:8, 128:]], axis=1)
    return jnp.concatenate([top, x[8:]], axis=0)


def _kernel(x_hbm, wqkv_hbm, wo_hbm, wr_hbm, wg_hbm, wu_hbm, wd_hbm,
            out_hbm,
            xio, wq_v, wk_v, wv_v, wvt_v, wo_v, wr_v, wg_v, wu_v, wd_v,
            xres, xbuf, r_s, rho_s, z_s, wr8,
            xca, xcb, xc_all, xi_all,
            q_s, k_s, vt_s, ot_s, s_s, m_s,
            ata, atb,
            sem_x, sem_w, sem_o):
    def x_copy(i):
        r0 = pl.multiple_of(i * TQ, TQ)
        return pltpu.make_async_copy(x_hbm.at[pl.ds(r0, TQ), :], xio.at[pl.ds(r0, TQ), :], sem_x.at[i])

    def out_copy(i):
        r0 = pl.multiple_of(i * TQ, TQ)
        return pltpu.make_async_copy(xio.at[pl.ds(r0, TQ), :], out_hbm.at[pl.ds(r0, TQ), :], sem_o.at[i])

    cp_wqa = pltpu.make_async_copy(wqkv_hbm.at[:, pl.ds(0, D // 2)], wq_v.at[:, pl.ds(0, D // 2)], sem_w.at[0])
    cp_wqb = pltpu.make_async_copy(wqkv_hbm.at[:, pl.ds(D // 2, D // 2)], wq_v.at[:, pl.ds(D // 2, D // 2)],
                                   sem_w.at[9])
    cp_wk = pltpu.make_async_copy(wqkv_hbm.at[:, pl.ds(D, D)], wk_v, sem_w.at[1])
    cp_wv = pltpu.make_async_copy(wqkv_hbm.at[:, pl.ds(2 * D, D)], wv_v, sem_w.at[8])
    cp_wo = pltpu.make_async_copy(wo_hbm, wo_v, sem_w.at[2])
    cp_wr = pltpu.make_async_copy(wr_hbm, wr_v, sem_w.at[3])
    cp_wg = pltpu.make_async_copy(wg_hbm, wg_v, sem_w.at[4])
    cp_wu = pltpu.make_async_copy(wu_hbm, wu_v, sem_w.at[5])
    cp_wd = pltpu.make_async_copy(wd_hbm, wd_v, sem_w.at[6])

    x_copy(0).start()
    cp_wqa.start()

    z_s[...] = jnp.zeros_like(z_s)

    def ln_chunk(layer, i, c, xc_ref, gate):
        r0 = i * TQ + c * CH
        h0 = i * (TQ // 2) + c * (CH // 2)
        if not isinstance(r0, int):
            r0 = pl.multiple_of(r0, CH)
            h0 = pl.multiple_of(h0, CH // 2)
        x_in = xio[pl.ds(r0, CH), :].astype(f32)
        x_rs = xres[pl.ds(r0, CH), :]
        x = jnp.where(layer == 0, x_in, x_rs)
        xbuf[pl.ds(r0, CH), :] = x
        if gate is not None:
            x = _gate_first(x, gate, z_s[...])
        xn = _ln(x)
        xc = _pack_rows(xn)
        xc_ref[c * CH // 2:(c + 1) * CH // 2, :] = xc
        xc_all[pl.ds(h0, CH // 2), :] = xc
        xi_all[pl.ds(h0, CH // 2), :] = _pack_rows_interleaved(xn)

    def q_step(layer, i, xc_ref, i_next, xc_next, part=(0, G)):
        h0 = i * (TQ // 2)
        if not isinstance(h0, int):
            h0 = pl.multiple_of(h0, TQ // 2)
        a = pltpu.bitcast(xc_ref[...], bf16)
        ys = {}
        for n in range(*part):
            y = jnp.dot(a, wq_v[:, n * 128:(n + 1) * 128], preferred_element_type=f32)
            q_s[n, pl.ds(h0, TQ // 2), :] = _pack_rows(y * QSCALE)
            ys[n] = y
        if i_next is not None:
            for c in range(part[0] * NCH // G, part[1] * NCH // G):
                ln_chunk(layer, i_next, c, xc_next, ys.get(GATE_A[c]))

    def kv_step(i):
        h0 = pl.multiple_of(i * (TQ // 2), TQ // 2)
        a = pltpu.bitcast(xc_all[pl.ds(h0, TQ // 2), :], bf16)
        for n in range(G):
            y = jnp.dot(a, wk_v[:, n * 128:(n + 1) * 128], preferred_element_type=f32)
            k_s[n, pl.ds(PAD // 2 + h0, TQ // 2), :] = _pack_rows(y)
        vt = lax.dot_general(pltpu.bitcast(wvt_v[...], bf16), pltpu.bitcast(xi_all[pl.ds(h0, TQ // 2), :], bf16),
                             NT, preferred_element_type=f32)
        c0 = pl.multiple_of(PAD + i * TQ, TQ)
        vt_s[:, pl.ds(c0, TQ)] = _pack_rows(vt)

    def phase_a(layer):
        @pl.when(layer == 0)
        def _():
            x_copy(0).wait()
            x_copy(1).start()
            cp_wqb.start()

        for c in range(NCH):
            ln_chunk(layer, 0, c, xca, None)

        @pl.when(layer == 0)
        def _():
            cp_wqa.wait()
            x_copy(1).wait()
            for i in range(2, NB):
                x_copy(i).start()

        q_step(layer, 0, xca, 1, xcb, part=(0, G // 2))

        @pl.when(layer == 0)
        def _():
            cp_wqb.wait()
            cp_wv.start()
            cp_wk.start()
            cp_wo.start()
            cp_wr.start()

        q_step(layer, 0, xca, 1, xcb, part=(G // 2, G))

        def q_body(j, c):
            i1 = 2 * j + 1

            @pl.when(layer == 0)
            def _():
                x_copy(i1 + 1).wait()
                x_copy(i1 + 2).wait()

            q_step(layer, i1, xcb, i1 + 1, xca)
            q_step(layer, i1 + 1, xca, i1 + 2, xcb)
            return c

        with jax.named_scope("a_q"):
            lax.fori_loop(0, NB // 2 - 1, q_body, 0)

        @pl.when(layer == 0)
        def _():
            cp_wv.wait()

        q_step(layer, NB - 1, xcb, None, None)
        wvt_v[...] = pltpu.bitcast(wv_v[...].T, u32)

        @pl.when(layer == 0)
        def _():
            cp_wk.wait()
            cp_wg.start()
            cp_wu.start()
            cp_wd.start()

        def kv_body(j, c):
            kv_step(2 * j)
            kv_step(2 * j + 1)
            return c

        with jax.named_scope("a_kv"):
            lax.fori_loop(0, NB // 2, kv_body, 0)

    def qk_stage(g, q0, slot, kstart):
        zi = pltpu.bitcast(z_s[...], i32)
        zi16 = jnp.concatenate([zi, zi], axis=0)
        lane16 = lax.broadcasted_iota(i32, (16, 128), 1) + zi16
        r16 = lax.broadcasted_iota(i32, (16, 128), 0)
        hb16 = lane16 // 32
        dd = r16 - lane16 % 32
        h0 = q0 // 2
        first_rows = None
        for b in range(4):
            first = max(0, kstart - 32 * b)
            base = h0 + 16 * b
            if not isinstance(base, int):
                base = pl.multiple_of(base, 16)
            mid0 = max(first, 32)
            if first == 0:
                parts = [k_s[g, pl.ds(base, 8), :], k_s[g, pl.ds(base + 128, 8), :],
                         k_s[g, pl.ds(base + 8, 8), :], k_s[g, pl.ds(base + 136, 8), :]]
            else:
                parts = [k_s[g, pl.ds(base + 128, 16), :]]
            if mid0 < 256:
                parts.append(k_s[g, pl.ds(base + mid0 // 2, (256 - mid0) // 2), :])
            kw = pltpu.bitcast(jnp.concatenate(parts, axis=0), bf16)
            qu = q_s[g, pl.ds(base, 16), :]
            qall = pltpu.bitcast(
                jnp.concatenate([jnp.where(hb16 == (p - b) % 4, qu, jnp.uint32(0)) for p in range(4)], axis=0),
                bf16)
            st = lax.dot_general(kw, qall, NT, preferred_element_type=f32)
            if b == 0:
                first_rows = st[0:8]
            if first == 0:
                c0 = jnp.where(dd > 0, st[0:16], st[16:32])
                c1 = jnp.where(dd > -16, st[32:48], st[48:64])
                mid = st[64:]
            else:
                c0 = jnp.where(dd > 0, NEG, st[0:16])
                c1 = jnp.where(dd > -16, NEG, st[16:32])
                mid = st[32:]
            s_s[slot, b, 0:16, :] = c0
            s_s[slot, b, 16:32, :] = c1
            x = jnp.concatenate([c0, c1], axis=0)
            if mid0 < 256:
                s_s[slot, b, mid0:256, :] = mid
                x = jnp.concatenate([x, mid], axis=0)
            mm = jnp.max(x.reshape(x.shape[0] // 8, 8, 128), axis=0)
            m_s[slot, b] = jnp.broadcast_to(jnp.max(mm, axis=0, keepdims=True), (8, 128))
        return first_rows

    def pv_stage(g, q0, slot, gate, kstart):
        r8 = lax.broadcasted_iota(i32, (8, 128), 0)
        c8 = lax.broadcasted_iota(i32, (8, 128), 1) + pltpu.bitcast(z_s[...], i32)
        blk = c8 // 32
        j = c8 % 32

        def tri(u):
            return (jnp.where(16 * u + r8 > j, jnp.uint32(0xFFFF), jnp.uint32(0)) |
                    jnp.where(16 * u + 8 + r8 > j, jnp.uint32(0xFFFF0000), jnp.uint32(0)))

        tris = [tri(0), tri(1)] if kstart < 128 else None
        ms = [m_s[slot, b] for b in range(4)]
        L = [None] * 4
        cache = {}

        def pexp(b, u):
            x = s_s[slot, b, 16 * u:16 * u + 16, :]
            p0 = jnp.exp2(x[0:8] - ms[b])
            p1 = jnp.exp2(x[8:16] - ms[b])
            sm = p0 + p1
            L[b] = sm if L[b] is None else L[b] + sm
            return pltpu.pack_elementwise([p0, p1], packed_dtype=bf16)

        def get_p(b, u):
            first = max(0, kstart - 32 * b)
            if u < 0 or u >= 18 or 16 * u < first:
                return None
            if first > 0:
                return pexp(b, u - 16) if u >= 16 else pexp(b, u)
            if u < 2:
                pk = pexp(b, u)
                lo = pk & tris[u]
                cache[(b, u + 16)] = pk ^ lo
                return lo
            if u >= 16:
                return cache.pop((b, u))
            return pexp(b, u)

        zero = jnp.zeros((8, 128), u32)
        accs = [None] * 4
        for k in range(kstart // 128, 3):
            wts = [[] for _ in range(4)]
            for t in range(8 * k, 8 * k + 8):
                if t == 8 and kstart == 0:
                    gv = gate * z_s[...]
                    for b in range(4):
                        ms[b] = ms[b] + gv
                srcs = [(b, get_p(b, t - 2 * b)) for b in range(4)]
                srcs = [(b, v) for (b, v) in srcs if v is not None]
                for h in range(4):
                    acc = zero if len(srcs) < 4 else None
                    for (b, v) in srcs:
                        acc = v if acc is None else jnp.where(blk == (h + b) % 4, v, acc)
                    wts[h].append(acc)
            c0 = q0 + 128 * k
            if not isinstance(c0, int):
                c0 = pl.multiple_of(c0, 128)
            for h in range(4):
                pt = pltpu.bitcast(jnp.concatenate(wts[h], axis=0), bf16)
                vth = pltpu.bitcast(vt_s[pl.ds((g * 4 + h) * 16, 16), pl.ds(c0, 128)], bf16)
                d = jnp.dot(vth, pt, preferred_element_type=f32)
                accs[h] = d if accs[h] is None else accs[h] + d
        L = [jnp.broadcast_to(jnp.sum(l, axis=0, keepdims=True), (8, 128)) for l in L]
        outs = []
        for h in range(4):
            lh = L[0]
            for b in range(1, 4):
                lh = jnp.where(blk == (h + b) % 4, L[b], lh)
            r0 = pl.reciprocal(lh, approx=True)
            rl = r0 * (2.0 - lh * r0)
            ot = (accs[h].reshape(4, 8, 128) * rl[None]).reshape(32, 128)
            if h > 0:
                ot = pltpu.roll(ot, 128 - 32 * h, axis=1)
            outs.append(ot)
        ot_s[g * 128:(g + 1) * 128, pl.ds(q0, 128)] = jnp.concatenate(outs, axis=0)

    def sub_block(q0, qn, kstart, kstart_next):
        for g in range(G):
            if g + 1 < G:
                gate = qk_stage(g + 1, q0, (g + 1) % 2, kstart)
            else:
                gate = qk_stage(0, qn, 0, kstart_next)
            pv_stage(g, q0, g % 2, gate, kstart)

    def phase_b():
        qk_stage(0, 0, 0, PAD)
        sub_block(0, 128, PAD, PAD - 128)
        sub_block(128, 256, PAD - 128, 0)

        def body(sb, c):
            q0 = pl.multiple_of(sb * 128, 128)
            qn = pl.multiple_of(jnp.minimum(sb + 1, NSB - 1) * 128, 128)
            sub_block(q0, qn, 0, 0)
            return c

        lax.fori_loop(2, NSB, body, 0)

    def resid_chunk(i, c, at_ref, gate):
        r0 = pl.multiple_of(i * TQ + c * CHC, CHC)
        x1 = xbuf[pl.ds(r0, CHC), :] + at_ref[c * CHC:(c + 1) * CHC, :]
        if gate is not None:
            x1 = _gate_first(x1, gate, z_s[...])
        m = jnp.mean(x1, axis=-1, keepdims=True)
        xc = x1 - m
        v = jnp.mean(xc * xc, axis=-1, keepdims=True)
        rho = lax.rsqrt(v + EPS)
        xn = xc * rho
        r = jnp.sum(xn * wr8[0:1, :], axis=-1, keepdims=True)
        r_s[pl.ds(r0, CHC), :] = jnp.broadcast_to(r, (CHC, 128))
        rho_s[pl.ds(r0, CHC), :] = jnp.broadcast_to(rho, (CHC, 128))
        x2 = x1 + xn
        xres[pl.ds(r0, CHC), :] = x2
        xio[pl.ds(r0, CHC), :] = x2.astype(bf16)

    def oproj_step(i_dot, at_w, i_res, at_r):
        ys = []
        if i_dot is not None:
            r0 = pl.multiple_of(i_dot * TQ, TQ)
            a = ot_s[:, pl.ds(r0, TQ)].astype(bf16).T
            for n in range(G):
                y = jnp.dot(a, wo_v[:, n * 128:(n + 1) * 128], preferred_element_type=f32)
                at_w[:, n * 128:(n + 1) * 128] = y
                ys.append(y)
        if i_res is not None:
            for c in range(NCHC):
                gi = GATE_C[c] if ys else -1
                gate = ys[gi] if gi >= 0 else None
                resid_chunk(i_res, c, at_r, gate)

    def phase_c(layer):
        @pl.when(layer == 0)
        def _():
            cp_wo.wait()
            cp_wr.wait()
            wr8[...] = jnp.broadcast_to(wr_v[...].astype(f32).reshape(1, D), (8, D))

        def flush(i):
            @pl.when(layer == 1)
            def _():
                out_copy(i).start()

        oproj_step(0, ata, None, None)

        def body(j, c):
            i0 = 2 * j
            oproj_step(i0 + 1, atb, i0, ata)
            oproj_step(i0 + 2, ata, i0 + 1, atb)
            flush(i0)
            flush(i0 + 1)
            return c

        lax.fori_loop(0, NB // 2 - 1, body, 0)
        oproj_step(NB - 1, atb, NB - 2, ata)
        oproj_step(None, None, NB - 1, atb)
        flush(NB - 2)
        flush(NB - 1)

    def phase_d(layer):
        @pl.when(layer == 0)
        def _():
            cp_wg.wait()
            cp_wu.wait()
            cp_wd.wait()

        rb = r_s[...].astype(bf16).astype(f32)
        rmax = jnp.max(rb)
        rows = lax.broadcasted_iota(i32, (S, 128), 0)
        idx = jnp.min(jnp.where(rb == rmax, rows, S))
        idx = jnp.clip(idx, 0, S - 1)
        x2 = xres[pl.ds(idx, 1), :]
        rho = rho_s[pl.ds(idx, 1), 0:1]
        xn = (x2 - jnp.mean(x2, axis=-1, keepdims=True)) * (rho / (1.0 + rho))
        xs = jnp.broadcast_to(xn, (16, D)).astype(bf16)
        gate = jnp.dot(xs, wg_v[...], preferred_element_type=f32)
        up = jnp.dot(xs, wu_v[...], preferred_element_type=f32)
        hmid = (gate * jax.nn.sigmoid(gate) * up).astype(bf16)
        y = jnp.dot(hmid, wd_v[...], preferred_element_type=f32)
        scale = jax.nn.sigmoid(jnp.full((1, D), rmax, f32))
        xres[pl.ds(idx, 1), :] = xres[pl.ds(idx, 1), :] + y[0:1] * scale

        @pl.when(layer == 1)
        def _():
            for i in range(NB):
                out_copy(i).wait()
            g0 = pl.multiple_of((idx // 16) * 16, 16)
            xio[pl.ds(g0, 16), :] = xres[pl.ds(g0, 16), :].astype(bf16)
            fix = pltpu.make_async_copy(xio.at[pl.ds(g0, 16), :], out_hbm.at[pl.ds(g0, 16), :], sem_w.at[7])
            fix.start()
            fix.wait()

    def layer_body(layer, c):
        with jax.named_scope("phase_a"):
            phase_a(layer)
        with jax.named_scope("phase_b"):
            phase_b()
        with jax.named_scope("phase_c"):
            phase_c(layer)
        with jax.named_scope("phase_d"):
            phase_d(layer)
        return c

    lax.fori_loop(0, 2, layer_body, 0)


@jax.jit
def pallas_interleave_layers__sliding_block__moe_arch_mod__prompt_kernel(
    A_x: jax.Array,
    A_wqkv: jax.Array,
    A_wo: jax.Array,
    B_x: jax.Array,
    B_w_r: jax.Array,
    B_w_gate: jax.Array,
    B_w_up: jax.Array,
    B_w_down: jax.Array,
):
    del B_x
    x = A_x.reshape(S, D)
    any_spec = pl.BlockSpec(memory_space=pl.ANY)
    scratch = [
        pltpu.VMEM((S, D), bf16),
        pltpu.VMEM((D, D), bf16),
        pltpu.VMEM((D, D), bf16),
        pltpu.VMEM((D, D), bf16),
        pltpu.VMEM((D // 2, D), u32),
        pltpu.VMEM((D, D), bf16),
        pltpu.VMEM((D,), bf16),
        pltpu.VMEM((D, F), bf16),
        pltpu.VMEM((D, F), bf16),
        pltpu.VMEM((F, D), bf16),
        pltpu.VMEM((S, D), f32),
        pltpu.VMEM((S, D), f32),
        pltpu.VMEM((S, 128), f32),
        pltpu.VMEM((S, 128), f32),
        pltpu.VMEM((8, 128), f32),
        pltpu.VMEM((8, D), f32),
        pltpu.VMEM((TQ // 2, D), u32),
        pltpu.VMEM((TQ // 2, D), u32),
        pltpu.VMEM((S // 2, D), u32),
        pltpu.VMEM((S // 2, D), u32),
        pltpu.VMEM((G, S // 2, 128), u32),
        pltpu.VMEM((G, (S + PAD) // 2, 128), u32),
        pltpu.VMEM((D // 2, S + PAD), u32),
        pltpu.VMEM((D, S), f32),
        pltpu.VMEM((2, 4, 256, 128), f32),
        pltpu.VMEM((2, 4, 8, 128), f32),
        pltpu.VMEM((TQ, D), f32),
        pltpu.VMEM((TQ, D), f32),
        pltpu.SemaphoreType.DMA((NB,)),
        pltpu.SemaphoreType.DMA((10,)),
        pltpu.SemaphoreType.DMA((NB,)),
    ]
    out = pl.pallas_call(
        _kernel,
        out_shape=jax.ShapeDtypeStruct((S, D), bf16),
        in_specs=[any_spec] * 7,
        out_specs=any_spec,
        scratch_shapes=scratch,
        compiler_params=pltpu.CompilerParams(vmem_limit_bytes=120 * 1024 * 1024),
    )(x, A_wqkv, A_wo, B_w_r, B_w_gate, B_w_up, B_w_down)
    return out.reshape(1, S, D)
```

```python
import jax
import jax.numpy as jnp
from jax import lax
import jax.experimental.pallas as pl
import jax.experimental.pallas.tpu as pltpu

bf16 = jnp.bfloat16
f32 = jnp.float32
u32 = jnp.uint32
i32 = jnp.int32

S = 2048
D = 1024
H = 32
DH = 32
W = 256
F = 3584
G = 8
PAD = 256
TQ = 256
NB = S // TQ
TKV = 512
NSB = S // 128
import os
CH = int(os.environ.get('K_CH', 32))
NCH = TQ // CH
CHC = int(os.environ.get('K_CHC', 32))
NCHC = TQ // CHC
GATE_A = [int(v) for v in os.environ.get('K_GA', '-1,0,1,2,3,4,5,6').split(',')]
GATE_C = [int(v) for v in os.environ.get('K_GC', '-1,0,1,2,3,4,5,6').split(',')]
EPS = 1e-5
NEG = -1e30
QSCALE = (DH ** -0.5) * 1.4426950408889634
NT = (((1,), (1,)), ((), ()))


def _ln(x):
    m = jnp.mean(x, axis=-1, keepdims=True)
    xc = x - m
    v = jnp.mean(xc * xc, axis=-1, keepdims=True)
    return xc * lax.rsqrt(v + EPS)


def _pack_rows(x):
    return pltpu.bitcast(x.astype(bf16), u32)


def _pack_rows_interleaved(x):
    n = x.shape[0] // 16
    x3 = x.reshape(n, 16, x.shape[1])
    a = x3[:, 0:8, :].reshape(n * 8, x.shape[1])
    b = x3[:, 8:16, :].reshape(n * 8, x.shape[1])
    return pltpu.pack_elementwise([a, b], packed_dtype=bf16)


def _gate_first(x, gate, z):
    g = gate[0:8, 0:128] * z
    top = jnp.concatenate([x[0:8, 0:128] + g, x[0:8, 128:]], axis=1)
    return jnp.concatenate([top, x[8:]], axis=0)


def _kernel(x_hbm, wqkv_hbm, wo_hbm, wr_hbm, wg_hbm, wu_hbm, wd_hbm,
            out_hbm,
            xio, wq_v, wk_v, wv_v, wvt_v, wo_v, wr_v, wg_v, wu_v, wd_v,
            xres, xbuf, best_v, best_i, rho_s, z_s, wr8,
            xca, xcb, xc_all, xi_all,
            q_s, k_s, vt_s, ot_s, s_s, m_s,
            ata, atb,
            sem_x, sem_w, sem_o):
    def x_copy(i):
        r0 = pl.multiple_of(i * TQ, TQ)
        return pltpu.make_async_copy(x_hbm.at[pl.ds(r0, TQ), :], xio.at[pl.ds(r0, TQ), :], sem_x.at[i])

    def out_copy(i):
        r0 = pl.multiple_of(i * TQ, TQ)
        return pltpu.make_async_copy(xio.at[pl.ds(r0, TQ), :], out_hbm.at[pl.ds(r0, TQ), :], sem_o.at[i])

    cp_wqa = pltpu.make_async_copy(wqkv_hbm.at[:, pl.ds(0, D // 2)], wq_v.at[:, pl.ds(0, D // 2)], sem_w.at[0])
    cp_wqb = pltpu.make_async_copy(wqkv_hbm.at[:, pl.ds(D // 2, D // 2)], wq_v.at[:, pl.ds(D // 2, D // 2)],
                                   sem_w.at[9])
    cp_wk = pltpu.make_async_copy(wqkv_hbm.at[:, pl.ds(D, D)], wk_v, sem_w.at[1])
    cp_wv = pltpu.make_async_copy(wqkv_hbm.at[:, pl.ds(2 * D, D)], wv_v, sem_w.at[8])
    cp_wo = pltpu.make_async_copy(wo_hbm, wo_v, sem_w.at[2])
    cp_wr = pltpu.make_async_copy(wr_hbm, wr_v, sem_w.at[3])
    cp_wg = pltpu.make_async_copy(wg_hbm, wg_v, sem_w.at[4])
    cp_wu = pltpu.make_async_copy(wu_hbm, wu_v, sem_w.at[5])
    cp_wd = pltpu.make_async_copy(wd_hbm, wd_v, sem_w.at[6])

    x_copy(0).start()
    cp_wqa.start()

    z_s[...] = jnp.zeros_like(z_s)
    xres[0:CH, :] = jnp.zeros((CH, D), f32)

    def ln_chunk(layer, i, c, xc_ref, gate):
        r0 = i * TQ + c * CH
        h0 = i * (TQ // 2) + c * (CH // 2)
        if not isinstance(r0, int):
            r0 = pl.multiple_of(r0, CH)
            h0 = pl.multiple_of(h0, CH // 2)
        x_in = xio[pl.ds(r0, CH), :].astype(f32)
        x_rs = xres[pl.ds(pl.multiple_of(r0 * layer, CH), CH), :]
        x = jnp.where(layer == 0, x_in, x_rs)
        xbuf[pl.ds(r0, CH), :] = x
        if gate is not None:
            x = _gate_first(x, gate, z_s[...])
        xn = _ln(x)
        xc = _pack_rows(xn)
        xc_ref[c * CH // 2:(c + 1) * CH // 2, :] = xc
        xc_all[pl.ds(h0, CH // 2), :] = xc
        xi_all[pl.ds(h0, CH // 2), :] = _pack_rows_interleaved(xn)

    def q_step(layer, i, xc_ref, i_next, xc_next, part=(0, G)):
        h0 = i * (TQ // 2)
        if not isinstance(h0, int):
            h0 = pl.multiple_of(h0, TQ // 2)
        a = pltpu.bitcast(xc_ref[...], bf16)
        ys = {}
        for n in range(*part):
            y = jnp.dot(a, wq_v[:, n * 128:(n + 1) * 128], preferred_element_type=f32)
            q_s[n, pl.ds(h0, TQ // 2), :] = _pack_rows(y * QSCALE)
            ys[n] = y
        if i_next is not None:
            for c in range(part[0] * NCH // G, part[1] * NCH // G):
                ln_chunk(layer, i_next, c, xc_next, ys.get(GATE_A[c]))

    def kv_step(i):
        h0 = pl.multiple_of(i * (TKV // 2), TKV // 2)
        a = pltpu.bitcast(xc_all[pl.ds(h0, TKV // 2), :], bf16)
        for n in range(G):
            y = jnp.dot(a, wk_v[:, n * 128:(n + 1) * 128], preferred_element_type=f32)
            k_s[n, pl.ds(PAD // 2 + h0, TKV // 2), :] = _pack_rows(y)
        vt = lax.dot_general(pltpu.bitcast(wvt_v[...], bf16), pltpu.bitcast(xi_all[pl.ds(h0, TKV // 2), :], bf16),
                             NT, preferred_element_type=f32)
        c0 = pl.multiple_of(PAD + i * TKV, 256)
        vt_s[:, pl.ds(c0, TKV)] = _pack_rows(vt)

    def phase_a(layer):
        @pl.when(layer == 0)
        def _():
            x_copy(0).wait()
            x_copy(1).start()
            cp_wqb.start()

        for c in range(NCH):
            ln_chunk(layer, 0, c, xca, None)

        @pl.when(layer == 0)
        def _():
            cp_wqa.wait()
            x_copy(1).wait()
            for i in range(2, NB):
                x_copy(i).start()

        q_step(layer, 0, xca, 1, xcb, part=(0, G // 2))

        @pl.when(layer == 0)
        def _():
            cp_wqb.wait()
            cp_wv.start()
            cp_wk.start()
            cp_wo.start()
            cp_wr.start()

        q_step(layer, 0, xca, 1, xcb, part=(G // 2, G))

        def q_body(j, c):
            i1 = 2 * j + 1

            @pl.when(layer == 0)
            def _():
                x_copy(i1 + 1).wait()
                x_copy(i1 + 2).wait()

            q_step(layer, i1, xcb, i1 + 1, xca)
            q_step(layer, i1 + 1, xca, i1 + 2, xcb)
            return c

        with jax.named_scope("a_q"):
            lax.fori_loop(0, NB // 2 - 1, q_body, 0)

        @pl.when(layer == 0)
        def _():
            cp_wv.wait()

        q_step(layer, NB - 1, xcb, None, None)
        wvt_v[...] = pltpu.bitcast(wv_v[...].T, u32)

        @pl.when(layer == 0)
        def _():
            cp_wk.wait()
            cp_wg.start()
            cp_wu.start()
            cp_wd.start()

        def kv_body(j, c):
            kv_step(j)
            return c

        with jax.named_scope("a_kv"):
            lax.fori_loop(0, S // TKV, kv_body, 0)

    def qk_stage(g, q0, slot, kstart):
        zi = pltpu.bitcast(z_s[...], i32)
        zi16 = jnp.concatenate([zi, zi], axis=0)
        lane16 = lax.broadcasted_iota(i32, (16, 128), 1) + zi16
        r16 = lax.broadcasted_iota(i32, (16, 128), 0)
        hb16 = lane16 // 32
        dd = r16 - lane16 % 32
        h0 = q0 // 2
        first_rows = None
        for b in range(4):
            first = max(0, kstart - 32 * b)
            base = h0 + 16 * b
            if not isinstance(base, int):
                base = pl.multiple_of(base, 16)
            mid0 = max(first, 32)
            if first == 0:
                parts = [k_s[g, pl.ds(base, 8), :], k_s[g, pl.ds(base + 128, 8), :],
                         k_s[g, pl.ds(base + 8, 8), :], k_s[g, pl.ds(base + 136, 8), :]]
            else:
                parts = [k_s[g, pl.ds(base + 128, 16), :]]
            if mid0 < 256:
                parts.append(k_s[g, pl.ds(base + mid0 // 2, (256 - mid0) // 2), :])
            kw = pltpu.bitcast(jnp.concatenate(parts, axis=0), bf16)
            qu = q_s[g, pl.ds(base, 16), :]
            qall = pltpu.bitcast(
                jnp.concatenate([jnp.where(hb16 == (p - b) % 4, qu, jnp.uint32(0)) for p in range(4)], axis=0),
                bf16)
            st = lax.dot_general(kw, qall, NT, preferred_element_type=f32)
            if b == 0:
                first_rows = st[0:8]
            if first == 0:
                c0 = jnp.where(dd > 0, st[0:16], st[16:32])
                c1 = jnp.where(dd > -16, st[32:48], st[48:64])
                mid = st[64:]
            else:
                c0 = jnp.where(dd > 0, NEG, st[0:16])
                c1 = jnp.where(dd > -16, NEG, st[16:32])
                mid = st[32:]
            s_s[slot, b, 0:16, :] = c0
            s_s[slot, b, 16:32, :] = c1
            x = jnp.concatenate([c0, c1], axis=0)
            if mid0 < 256:
                s_s[slot, b, mid0:256, :] = mid
                x = jnp.concatenate([x, mid], axis=0)
            mm = jnp.max(x.reshape(x.shape[0] // 8, 8, 128), axis=0)
            m_s[slot, b] = jnp.broadcast_to(jnp.max(mm, axis=0, keepdims=True), (8, 128))
        return first_rows

    def pv_stage(g, q0, slot, gate, kstart):
        r8 = lax.broadcasted_iota(i32, (8, 128), 0)
        c8 = lax.broadcasted_iota(i32, (8, 128), 1) + pltpu.bitcast(z_s[...], i32)
        blk = c8 // 32
        j = c8 % 32

        def tri(u):
            return (jnp.where(16 * u + r8 > j, jnp.uint32(0xFFFF), jnp.uint32(0)) |
                    jnp.where(16 * u + 8 + r8 > j, jnp.uint32(0xFFFF0000), jnp.uint32(0)))

        tris = [tri(0), tri(1)] if kstart < 128 else None
        ms = [m_s[slot, b] for b in range(4)]
        L = [None] * 4
        cache = {}

        def pexp(b, u):
            x = s_s[slot, b, 16 * u:16 * u + 16, :]
            p0 = jnp.exp2(x[0:8] - ms[b])
            p1 = jnp.exp2(x[8:16] - ms[b])
            sm = p0 + p1
            L[b] = sm if L[b] is None else L[b] + sm
            return pltpu.pack_elementwise([p0, p1], packed_dtype=bf16)

        def get_p(b, u):
            first = max(0, kstart - 32 * b)
            if u < 0 or u >= 18 or 16 * u < first:
                return None
            if first > 0:
                return pexp(b, u - 16) if u >= 16 else pexp(b, u)
            if u < 2:
                pk = pexp(b, u)
                lo = pk & tris[u]
                cache[(b, u + 16)] = pk ^ lo
                return lo
            if u >= 16:
                return cache.pop((b, u))
            return pexp(b, u)

        zero = jnp.zeros((8, 128), u32)
        accs = [None] * 4
        for k in range(kstart // 128, 3):
            wts = [[] for _ in range(4)]
            for t in range(8 * k, 8 * k + 8):
                if t == 8 and kstart == 0:
                    gv = gate * z_s[...]
                    for b in range(4):
                        ms[b] = ms[b] + gv
                srcs = [(b, get_p(b, t - 2 * b)) for b in range(4)]
                srcs = [(b, v) for (b, v) in srcs if v is not None]
                for h in range(4):
                    acc = zero if len(srcs) < 4 else None
                    for (b, v) in srcs:
                        acc = v if acc is None else jnp.where(blk == (h + b) % 4, v, acc)
                    wts[h].append(acc)
            c0 = q0 + 128 * k
            if not isinstance(c0, int):
                c0 = pl.multiple_of(c0, 128)
            for h in range(4):
                pt = pltpu.bitcast(jnp.concatenate(wts[h], axis=0), bf16)
                vth = pltpu.bitcast(vt_s[pl.ds((g * 4 + h) * 16, 16), pl.ds(c0, 128)], bf16)
                d = jnp.dot(vth, pt, preferred_element_type=f32)
                accs[h] = d if accs[h] is None else accs[h] + d
        L = [jnp.broadcast_to(jnp.sum(l, axis=0, keepdims=True), (8, 128)) for l in L]
        outs = []
        for h in range(4):
            lh = L[0]
            for b in range(1, 4):
                lh = jnp.where(blk == (h + b) % 4, L[b], lh)
            r0 = pl.reciprocal(lh, approx=True)
            rl = r0 * (2.0 - lh * r0)
            ot = (accs[h].reshape(4, 8, 128) * rl[None]).reshape(32, 128)
            if h > 0:
                ot = pltpu.roll(ot, 128 - 32 * h, axis=1)
            outs.append(ot)
        ot_s[g * 128:(g + 1) * 128, pl.ds(q0, 128)] = jnp.concatenate(outs, axis=0)

    def sub_block(q0, qn, kstart, kstart_next):
        for g in range(G):
            if g + 1 < G:
                gate = qk_stage(g + 1, q0, (g + 1) % 2, kstart)
            else:
                gate = qk_stage(0, qn, 0, kstart_next)
            pv_stage(g, q0, g % 2, gate, kstart)

    def phase_b():
        qk_stage(0, 0, 0, PAD)
        sub_block(0, 128, PAD, PAD - 128)
        sub_block(128, 256, PAD - 128, 0)

        def body(sb, c):
            q0 = pl.multiple_of(sb * 128, 128)
            qn = pl.multiple_of(jnp.minimum(sb + 1, NSB - 1) * 128, 128)
            sub_block(q0, qn, 0, 0)
            return c

        lax.fori_loop(2, NSB, body, 0)

    def resid_chunk(i, c, at_ref, gate):
        r0 = pl.multiple_of(i * TQ + c * CHC, CHC)
        x1 = xbuf[pl.ds(r0, CHC), :] + at_ref[c * CHC:(c + 1) * CHC, :]
        if gate is not None:
            x1 = _gate_first(x1, gate, z_s[...])
        m = jnp.mean(x1, axis=-1, keepdims=True)
        xc = x1 - m
        v = jnp.mean(xc * xc, axis=-1, keepdims=True)
        rho = lax.rsqrt(v + EPS)
        xn = xc * rho
        r = jnp.sum(xn * wr8[0:1, :], axis=-1, keepdims=True)
        rb = jnp.broadcast_to(r, (CHC, 128)).astype(bf16).astype(f32)
        rows = lax.broadcasted_iota(i32, (8, 128), 0) + r0
        bv, bi = best_v[...], best_i[...]
        for q in range(CHC // 8):
            cand = rb[8 * q:8 * q + 8]
            better = cand > bv
            bv = jnp.where(better, cand, bv)
            bi = jnp.where(better, rows + 8 * q, bi)
        best_v[...] = bv
        best_i[...] = bi
        rho_s[pl.ds(r0, CHC), :] = jnp.broadcast_to(rho, (CHC, 128))
        x2 = x1 + xn
        xres[pl.ds(r0, CHC), :] = x2
        xio[pl.ds(r0, CHC), :] = x2.astype(bf16)

    def oproj_step(i_dot, at_w, i_res, at_r):
        ys = []
        if i_dot is not None:
            r0 = pl.multiple_of(i_dot * TQ, TQ)
            a = ot_s[:, pl.ds(r0, TQ)].astype(bf16).T
            for n in range(G):
                y = jnp.dot(a, wo_v[:, n * 128:(n + 1) * 128], preferred_element_type=f32)
                at_w[:, n * 128:(n + 1) * 128] = y
                ys.append(y)
        if i_res is not None:
            for c in range(NCHC):
                gi = GATE_C[c] if ys else -1
                gate = ys[gi] if gi >= 0 else None
                resid_chunk(i_res, c, at_r, gate)

    def phase_c(layer):
        @pl.when(layer == 0)
        def _():
            cp_wo.wait()
            cp_wr.wait()
            wr8[...] = jnp.broadcast_to(wr_v[...].astype(f32).reshape(1, D), (8, D))

        def flush(i):
            @pl.when(layer == 1)
            def _():
                out_copy(i).start()

        best_v[...] = jnp.full((8, 128), -jnp.inf, f32)
        best_i[...] = jnp.zeros((8, 128), i32)
        oproj_step(0, ata, None, None)

        def body(j, c):
            i0 = 2 * j
            oproj_step(i0 + 1, atb, i0, ata)
            oproj_step(i0 + 2, ata, i0 + 1, atb)
            flush(i0)
            flush(i0 + 1)
            return c

        lax.fori_loop(0, NB // 2 - 1, body, 0)
        oproj_step(NB - 1, atb, NB - 2, ata)
        oproj_step(None, None, NB - 1, atb)
        flush(NB - 2)
        flush(NB - 1)

    def phase_d(layer):
        @pl.when(layer == 0)
        def _():
            cp_wg.wait()
            cp_wu.wait()
            cp_wd.wait()

        bv = best_v[...]
        rmax = jnp.max(bv)
        idx = jnp.min(jnp.where(bv == rmax, best_i[...], S))
        idx = jnp.clip(idx, 0, S - 1)
        x2 = xres[pl.ds(idx, 1), :]
        rho = rho_s[pl.ds(idx, 1), 0:1]
        xn = (x2 - jnp.mean(x2, axis=-1, keepdims=True)) * (rho / (1.0 + rho))
        xs = jnp.broadcast_to(xn, (16, D)).astype(bf16)
        gate = jnp.dot(xs, wg_v[...], preferred_element_type=f32)
        up = jnp.dot(xs, wu_v[...], preferred_element_type=f32)
        hmid = (gate * jax.nn.sigmoid(gate) * up).astype(bf16)
        y = jnp.dot(hmid, wd_v[...], preferred_element_type=f32)
        scale = jax.nn.sigmoid(jnp.full((1, D), rmax, f32))
        xres[pl.ds(idx, 1), :] = xres[pl.ds(idx, 1), :] + y[0:1] * scale

        @pl.when(layer == 1)
        def _():
            for i in range(NB):
                out_copy(i).wait()
            g0 = pl.multiple_of((idx // 16) * 16, 16)
            xio[pl.ds(g0, 16), :] = xres[pl.ds(g0, 16), :].astype(bf16)
            fix = pltpu.make_async_copy(xio.at[pl.ds(g0, 16), :], out_hbm.at[pl.ds(g0, 16), :], sem_w.at[7])
            fix.start()
            fix.wait()

    def layer_body(layer, c):
        with jax.named_scope("phase_a"):
            phase_a(layer)
        with jax.named_scope("phase_b"):
            phase_b()
        with jax.named_scope("phase_c"):
            phase_c(layer)
        with jax.named_scope("phase_d"):
            phase_d(layer)
        return c

    lax.fori_loop(0, 2, layer_body, 0)


@jax.jit
def pallas_interleave_layers__sliding_block__moe_arch_mod__prompt_kernel(
    A_x: jax.Array,
    A_wqkv: jax.Array,
    A_wo: jax.Array,
    B_x: jax.Array,
    B_w_r: jax.Array,
    B_w_gate: jax.Array,
    B_w_up: jax.Array,
    B_w_down: jax.Array,
):
    del B_x
    x = A_x.reshape(S, D)
    any_spec = pl.BlockSpec(memory_space=pl.ANY)
    scratch = [
        pltpu.VMEM((S, D), bf16),
        pltpu.VMEM((D, D), bf16),
        pltpu.VMEM((D, D), bf16),
        pltpu.VMEM((D, D), bf16),
        pltpu.VMEM((D // 2, D), u32),
        pltpu.VMEM((D, D), bf16),
        pltpu.VMEM((D,), bf16),
        pltpu.VMEM((D, F), bf16),
        pltpu.VMEM((D, F), bf16),
        pltpu.VMEM((F, D), bf16),
        pltpu.VMEM((S, D), f32),
        pltpu.VMEM((S, D), f32),
        pltpu.VMEM((8, 128), f32),
        pltpu.VMEM((8, 128), i32),
        pltpu.VMEM((S, 128), f32),
        pltpu.VMEM((8, 128), f32),
        pltpu.VMEM((8, D), f32),
        pltpu.VMEM((TQ // 2, D), u32),
        pltpu.VMEM((TQ // 2, D), u32),
        pltpu.VMEM((S // 2, D), u32),
        pltpu.VMEM((S // 2, D), u32),
        pltpu.VMEM((G, S // 2, 128), u32),
        pltpu.VMEM((G, (S + PAD) // 2, 128), u32),
        pltpu.VMEM((D // 2, S + PAD), u32),
        pltpu.VMEM((D, S), f32),
        pltpu.VMEM((2, 4, 256, 128), f32),
        pltpu.VMEM((2, 4, 8, 128), f32),
        pltpu.VMEM((TQ, D), f32),
        pltpu.VMEM((TQ, D), f32),
        pltpu.SemaphoreType.DMA((NB,)),
        pltpu.SemaphoreType.DMA((10,)),
        pltpu.SemaphoreType.DMA((NB,)),
    ]
    out = pl.pallas_call(
        _kernel,
        out_shape=jax.ShapeDtypeStruct((S, D), bf16),
        in_specs=[any_spec] * 7,
        out_specs=any_spec,
        scratch_shapes=scratch,
        compiler_params=pltpu.CompilerParams(vmem_limit_bytes=120 * 1024 * 1024),
    )(x, A_wqkv, A_wo, B_w_r, B_w_gate, B_w_up, B_w_down)
    return out.reshape(1, S, D)
```

```python
import jax
import jax.numpy as jnp
from jax import lax
import jax.experimental.pallas as pl
import jax.experimental.pallas.tpu as pltpu

bf16 = jnp.bfloat16
f32 = jnp.float32
u32 = jnp.uint32
i32 = jnp.int32

S = 2048
D = 1024
H = 32
DH = 32
W = 256
F = 3584
G = 8
PAD = 256
TQ = 256
NB = S // TQ
TKV = 512
NSB = S // 128
import os
CH = int(os.environ.get('K_CH', 32))
NCH = TQ // CH
CHC = int(os.environ.get('K_CHC', 8))
NCHC = TQ // CHC
GATE_A = [c * 8 // NCH - 1 for c in range(NCH)]
NWC = int(os.environ.get('K_NWC', 128))
_GCN, _GCO = [int(v) for v in os.environ.get('K_GC', '8,-1').split(',')]
GATE_C = [min(c * _GCN // NCHC + _GCO, 7) for c in range(NCHC)]
EPS = 1e-5
NEG = -1e30
QSCALE = (DH ** -0.5) * 1.4426950408889634
NT = (((1,), (1,)), ((), ()))


def _ln(x):
    m = jnp.mean(x, axis=-1, keepdims=True)
    xc = x - m
    v = jnp.mean(xc * xc, axis=-1, keepdims=True)
    return xc * lax.rsqrt(v + EPS)


def _pack_rows(x):
    return pltpu.bitcast(x.astype(bf16), u32)


def _pack_rows_interleaved(x):
    n = x.shape[0] // 16
    x3 = x.reshape(n, 16, x.shape[1])
    a = x3[:, 0:8, :].reshape(n * 8, x.shape[1])
    b = x3[:, 8:16, :].reshape(n * 8, x.shape[1])
    return pltpu.pack_elementwise([a, b], packed_dtype=bf16)


def _gate_first(x, gate, z):
    g = gate[0:8, 0:128] * z
    top = jnp.concatenate([x[0:8, 0:128] + g, x[0:8, 128:]], axis=1)
    return top if x.shape[0] == 8 else jnp.concatenate([top, x[8:]], axis=0)


def _kernel(x_hbm, wqkv_hbm, wo_hbm, wr_hbm, wg_hbm, wu_hbm, wd_hbm,
            out_hbm,
            xio, wq_v, wk_v, wv_v, wvt_v, wo_v, wop_v, wr_v, wg_v, wu_v, wd_v,
            xres, xbuf, best_v, best_i, rho_s, z_s, wr8,
            xca, xcb, xc_all, xi_all,
            q_s, k_s, vt_s, ot_s, s_s, m_s,
            ata, atb,
            sem_x, sem_w, sem_o):
    def x_copy(i):
        r0 = pl.multiple_of(i * TQ, TQ)
        return pltpu.make_async_copy(x_hbm.at[pl.ds(r0, TQ), :], xio.at[pl.ds(r0, TQ), :], sem_x.at[i])

    def out_copy(i):
        r0 = pl.multiple_of(i * TQ, TQ)
        return pltpu.make_async_copy(xio.at[pl.ds(r0, TQ), :], out_hbm.at[pl.ds(r0, TQ), :], sem_o.at[i])

    cp_wqa = pltpu.make_async_copy(wqkv_hbm.at[:, pl.ds(0, D // 2)], wq_v.at[:, pl.ds(0, D // 2)], sem_w.at[0])
    cp_wqb = pltpu.make_async_copy(wqkv_hbm.at[:, pl.ds(D // 2, D // 2)], wq_v.at[:, pl.ds(D // 2, D // 2)],
                                   sem_w.at[9])
    cp_wk = pltpu.make_async_copy(wqkv_hbm.at[:, pl.ds(D, D)], wk_v, sem_w.at[1])
    cp_wv = pltpu.make_async_copy(wqkv_hbm.at[:, pl.ds(2 * D, D)], wv_v, sem_w.at[8])
    cp_wo = pltpu.make_async_copy(wo_hbm, wo_v, sem_w.at[2])
    cp_wr = pltpu.make_async_copy(wr_hbm, wr_v, sem_w.at[3])
    cp_wg = pltpu.make_async_copy(wg_hbm, wg_v, sem_w.at[4])
    cp_wu = pltpu.make_async_copy(wu_hbm, wu_v, sem_w.at[5])
    cp_wd = pltpu.make_async_copy(wd_hbm, wd_v, sem_w.at[6])

    x_copy(0).start()
    cp_wqa.start()

    z_s[...] = jnp.zeros_like(z_s)
    xres[0:CH, :] = jnp.zeros((CH, D), f32)

    def ln_chunk(layer, i, c, xc_ref, gate):
        r0 = i * TQ + c * CH
        h0 = i * (TQ // 2) + c * (CH // 2)
        if not isinstance(r0, int):
            r0 = pl.multiple_of(r0, CH)
            h0 = pl.multiple_of(h0, CH // 2)
        x_in = xio[pl.ds(r0, CH), :].astype(f32)
        x_rs = xres[pl.ds(pl.multiple_of(r0 * layer, CH), CH), :]
        x = jnp.where(layer == 0, x_in, x_rs)
        xbuf[pl.ds(r0, CH), :] = x
        if gate is not None:
            x = _gate_first(x, gate, z_s[...])
        xn = _ln(x)
        xc = _pack_rows(xn)
        xc_ref[c * CH // 2:(c + 1) * CH // 2, :] = xc
        xc_all[pl.ds(h0, CH // 2), :] = xc
        xi_all[pl.ds(h0, CH // 2), :] = _pack_rows_interleaved(xn)

    def q_step(layer, i, xc_ref, i_next, xc_next, part=(0, G)):
        h0 = i * (TQ // 2)
        if not isinstance(h0, int):
            h0 = pl.multiple_of(h0, TQ // 2)
        a = pltpu.bitcast(xc_ref[...], bf16)
        ys = {}
        for n in range(*part):
            y = jnp.dot(a, wq_v[:, n * 128:(n + 1) * 128], preferred_element_type=f32)
            q_s[n, pl.ds(h0, TQ // 2), :] = _pack_rows(y * QSCALE)
            ys[n] = y
        if i_next is not None:
            for c in range(part[0] * NCH // G, part[1] * NCH // G):
                ln_chunk(layer, i_next, c, xc_next, ys.get(GATE_A[c]))

    def kv_step(i):
        h0 = pl.multiple_of(i * (TKV // 2), TKV // 2)
        a = pltpu.bitcast(xc_all[pl.ds(h0, TKV // 2), :], bf16)
        for n in range(G):
            y = jnp.dot(a, wk_v[:, n * 128:(n + 1) * 128], preferred_element_type=f32)
            k_s[n, pl.ds(PAD // 2 + h0, TKV // 2), :] = _pack_rows(y)
        vt = lax.dot_general(pltpu.bitcast(wvt_v[...], bf16), pltpu.bitcast(xi_all[pl.ds(h0, TKV // 2), :], bf16),
                             NT, preferred_element_type=f32)
        c0 = pl.multiple_of(PAD + i * TKV, 256)
        vt_s[:, pl.ds(c0, TKV)] = _pack_rows(vt)

    def phase_a(layer):
        @pl.when(layer == 0)
        def _():
            x_copy(0).wait()
            x_copy(1).start()
            cp_wqb.start()

        for c in range(NCH):
            ln_chunk(layer, 0, c, xca, None)

        @pl.when(layer == 0)
        def _():
            cp_wqa.wait()
            x_copy(1).wait()
            for i in range(2, NB):
                x_copy(i).start()

        q_step(layer, 0, xca, 1, xcb, part=(0, G // 2))

        @pl.when(layer == 0)
        def _():
            cp_wqb.wait()
            cp_wv.start()
            cp_wo.start()
            cp_wk.start()
            cp_wr.start()

        q_step(layer, 0, xca, 1, xcb, part=(G // 2, G))

        def q_body(j, c):
            i1 = 2 * j + 1

            @pl.when(layer == 0)
            def _():
                x_copy(i1 + 1).wait()
                x_copy(i1 + 2).wait()

            q_step(layer, i1, xcb, i1 + 1, xca)
            q_step(layer, i1 + 1, xca, i1 + 2, xcb)
            return c

        with jax.named_scope("a_q"):
            lax.fori_loop(0, NB // 2 - 1, q_body, 0)

        @pl.when(layer == 0)
        def _():
            cp_wv.wait()
            cp_wo.wait()

        q_step(layer, NB - 1, xcb, None, None)
        wvt_v[...] = pltpu.bitcast(wv_v[...].T, u32)
        for c in range(D // 64):
            wop_v[c * 32:(c + 1) * 32, :] = _pack_rows_interleaved(wo_v[c * 64:(c + 1) * 64, :].astype(f32))

        @pl.when(layer == 0)
        def _():
            cp_wk.wait()
            cp_wg.start()
            cp_wu.start()
            cp_wd.start()

        def kv_body(j, c):
            kv_step(j)
            return c

        with jax.named_scope("a_kv"):
            lax.fori_loop(0, S // TKV, kv_body, 0)

    def qk_stage(g, q0, slot, kstart):
        zi = pltpu.bitcast(z_s[...], i32)
        zi16 = jnp.concatenate([zi, zi], axis=0)
        lane16 = lax.broadcasted_iota(i32, (16, 128), 1) + zi16
        r16 = lax.broadcasted_iota(i32, (16, 128), 0)
        hb16 = lane16 // 32
        dd = r16 - lane16 % 32
        h0 = q0 // 2
        first_rows = None
        for b in range(4):
            first = max(0, kstart - 32 * b)
            base = h0 + 16 * b
            if not isinstance(base, int):
                base = pl.multiple_of(base, 16)
            mid0 = max(first, 32)
            if first == 0:
                parts = [k_s[g, pl.ds(base, 8), :], k_s[g, pl.ds(base + 128, 8), :],
                         k_s[g, pl.ds(base + 8, 8), :], k_s[g, pl.ds(base + 136, 8), :]]
            else:
                parts = [k_s[g, pl.ds(base + 128, 16), :]]
            if mid0 < 256:
                parts.append(k_s[g, pl.ds(base + mid0 // 2, (256 - mid0) // 2), :])
            kw = pltpu.bitcast(jnp.concatenate(parts, axis=0), bf16)
            qu = q_s[g, pl.ds(base, 16), :]
            qall = pltpu.bitcast(
                jnp.concatenate([jnp.where(hb16 == (p - b) % 4, qu, jnp.uint32(0)) for p in range(4)], axis=0),
                bf16)
            st = lax.dot_general(kw, qall, NT, preferred_element_type=f32)
            if b == 0:
                first_rows = st[0:8]
            if first == 0:
                c0 = jnp.where(dd > 0, st[0:16], st[16:32])
                c1 = jnp.where(dd > -16, st[32:48], st[48:64])
                mid = st[64:]
            else:
                c0 = jnp.where(dd > 0, NEG, st[0:16])
                c1 = jnp.where(dd > -16, NEG, st[16:32])
                mid = st[32:]
            s_s[slot, b, 0:16, :] = c0
            s_s[slot, b, 16:32, :] = c1
            x = jnp.concatenate([c0, c1], axis=0)
            if mid0 < 256:
                s_s[slot, b, mid0:256, :] = mid
                x = jnp.concatenate([x, mid], axis=0)
            mm = jnp.max(x.reshape(x.shape[0] // 8, 8, 128), axis=0)
            m_s[slot, b] = jnp.broadcast_to(jnp.max(mm, axis=0, keepdims=True), (8, 128))
        return first_rows

    def pv_stage(g, q0, slot, gate, kstart):
        r8 = lax.broadcasted_iota(i32, (8, 128), 0)
        c8 = lax.broadcasted_iota(i32, (8, 128), 1) + pltpu.bitcast(z_s[...], i32)
        blk = c8 // 32
        j = c8 % 32

        def tri(u):
            return (jnp.where(16 * u + r8 > j, jnp.uint32(0xFFFF), jnp.uint32(0)) |
                    jnp.where(16 * u + 8 + r8 > j, jnp.uint32(0xFFFF0000), jnp.uint32(0)))

        tris = [tri(0), tri(1)] if kstart < 128 else None
        ms = [m_s[slot, b] for b in range(4)]
        L = [None] * 4
        cache = {}

        def pexp(b, u):
            x = s_s[slot, b, 16 * u:16 * u + 16, :]
            p0 = jnp.exp2(x[0:8] - ms[b])
            p1 = jnp.exp2(x[8:16] - ms[b])
            sm = p0 + p1
            L[b] = sm if L[b] is None else L[b] + sm
            return pltpu.pack_elementwise([p0, p1], packed_dtype=bf16)

        def get_p(b, u):
            first = max(0, kstart - 32 * b)
            if u < 0 or u >= 18 or 16 * u < first:
                return None
            if first > 0:
                return pexp(b, u - 16) if u >= 16 else pexp(b, u)
            if u < 2:
                pk = pexp(b, u)
                lo = pk & tris[u]
                cache[(b, u + 16)] = pk ^ lo
                return lo
            if u >= 16:
                return cache.pop((b, u))
            return pexp(b, u)

        zero = jnp.zeros((8, 128), u32)
        accs = [None] * 4
        for k in range(kstart // 128, 3):
            wts = [[] for _ in range(4)]
            for t in range(8 * k, 8 * k + 8):
                if t == 8 and kstart == 0:
                    gv = gate * z_s[...]
                    for b in range(4):
                        ms[b] = ms[b] + gv
                srcs = [(b, get_p(b, t - 2 * b)) for b in range(4)]
                srcs = [(b, v) for (b, v) in srcs if v is not None]
                for h in range(4):
                    acc = zero if len(srcs) < 4 else None
                    for (b, v) in srcs:
                        acc = v if acc is None else jnp.where(blk == (h + b) % 4, v, acc)
                    wts[h].append(acc)
            c0 = q0 + 128 * k
            if not isinstance(c0, int):
                c0 = pl.multiple_of(c0, 128)
            for h in range(4):
                pt = pltpu.bitcast(jnp.concatenate(wts[h], axis=0), bf16)
                vth = pltpu.bitcast(vt_s[pl.ds((g * 4 + h) * 16, 16), pl.ds(c0, 128)], bf16)
                d = jnp.dot(vth, pt, preferred_element_type=f32)
                accs[h] = d if accs[h] is None else accs[h] + d
        L = [jnp.broadcast_to(jnp.sum(l, axis=0, keepdims=True), (8, 128)) for l in L]
        outs = []
        for h in range(4):
            lh = L[0]
            for b in range(1, 4):
                lh = jnp.where(blk == (h + b) % 4, L[b], lh)
            r0 = pl.reciprocal(lh, approx=True)
            rl = r0 * (2.0 - lh * r0)
            ot = (accs[h].reshape(4, 8, 128) * rl[None]).reshape(32, 128)
            if h > 0:
                ot = pltpu.roll(ot, 128 - 32 * h, axis=1)
            outs.append(ot)
        ot_s[g * 64:(g + 1) * 64, pl.ds(q0, 128)] = _pack_rows_interleaved(jnp.concatenate(outs, axis=0))

    def sub_block(q0, qn, kstart, kstart_next):
        for g in range(G):
            if g + 1 < G:
                gate = qk_stage(g + 1, q0, (g + 1) % 2, kstart)
            else:
                gate = qk_stage(0, qn, 0, kstart_next)
            pv_stage(g, q0, g % 2, gate, kstart)

    def phase_b():
        qk_stage(0, 0, 0, PAD)
        sub_block(0, 128, PAD, PAD - 128)
        sub_block(128, 256, PAD - 128, 0)

        def body(sb, c):
            q0 = pl.multiple_of(sb * 128, 128)
            qn = pl.multiple_of(jnp.minimum(sb + 1, NSB - 1) * 128, 128)
            sub_block(q0, qn, 0, 0)
            return c

        lax.fori_loop(2, NSB, body, 0)

    def resid_chunk(i, c, at_ref, gate):
        r0 = pl.multiple_of(i * TQ + c * CHC, CHC)
        x1 = xbuf[pl.ds(r0, CHC), :] + at_ref[c * CHC:(c + 1) * CHC, :]
        if gate is not None:
            x1 = _gate_first(x1, gate, z_s[...])
        m = jnp.mean(x1, axis=-1, keepdims=True)
        xc = x1 - m
        v = jnp.mean(xc * xc, axis=-1, keepdims=True)
        rho = lax.rsqrt(v + EPS)
        xn = xc * rho
        r = jnp.sum(xn * wr8[0:1, :], axis=-1, keepdims=True)
        rb = jnp.broadcast_to(r, (CHC, 128)).astype(bf16).astype(f32)
        rows = lax.broadcasted_iota(i32, (8, 128), 0) + r0
        bv, bi = best_v[...], best_i[...]
        for q in range(CHC // 8):
            cand = rb[8 * q:8 * q + 8]
            better = cand > bv
            bv = jnp.where(better, cand, bv)
            bi = jnp.where(better, rows + 8 * q, bi)
        best_v[...] = bv
        best_i[...] = bi
        rho_s[pl.ds(r0, CHC), :] = jnp.broadcast_to(rho, (CHC, 128))
        x2 = x1 + xn
        xres[pl.ds(r0, CHC), :] = x2
        xio[pl.ds(r0, CHC), :] = x2.astype(bf16)

    def oproj_step(i_dot, at_w, i_res, at_r):
        ys = []
        if i_dot is not None:
            r0 = pl.multiple_of(i_dot * TQ, TQ)
            a = pltpu.bitcast(ot_s[:, pl.ds(r0, TQ)], bf16).T
            for n in range(D // NWC):
                y = jnp.dot(a, pltpu.bitcast(wop_v[:, n * NWC:(n + 1) * NWC], bf16), preferred_element_type=f32)
                at_w[:, n * NWC:(n + 1) * NWC] = y
                ys.append(y)
        if i_res is not None:
            for c in range(NCHC):
                gi = GATE_C[c] if ys else -1
                gate = ys[gi] if gi >= 0 else None
                resid_chunk(i_res, c, at_r, gate)

    def phase_c(layer):
        @pl.when(layer == 0)
        def _():
            cp_wr.wait()
            wr8[...] = jnp.broadcast_to(wr_v[...].astype(f32).reshape(1, D), (8, D))

        def flush(i):
            @pl.when(layer == 1)
            def _():
                out_copy(i).start()

        best_v[...] = jnp.full((8, 128), -jnp.inf, f32)
        best_i[...] = jnp.zeros((8, 128), i32)
        oproj_step(0, ata, None, None)

        def body(j, c):
            i0 = 2 * j
            oproj_step(i0 + 1, atb, i0, ata)
            oproj_step(i0 + 2, ata, i0 + 1, atb)
            flush(i0)
            flush(i0 + 1)
            return c

        lax.fori_loop(0, NB // 2 - 1, body, 0)
        oproj_step(NB - 1, atb, NB - 2, ata)
        oproj_step(None, None, NB - 1, atb)
        flush(NB - 2)
        flush(NB - 1)

    def phase_d(layer):
        @pl.when(layer == 0)
        def _():
            cp_wg.wait()
            cp_wu.wait()
            cp_wd.wait()

        bv = best_v[...]
        rmax = jnp.max(bv)
        idx = jnp.min(jnp.where(bv == rmax, best_i[...], S))
        idx = jnp.clip(idx, 0, S - 1)
        x2 = xres[pl.ds(idx, 1), :]
        rho = rho_s[pl.ds(idx, 1), 0:1]
        xn = (x2 - jnp.mean(x2, axis=-1, keepdims=True)) * (rho / (1.0 + rho))
        xs = jnp.broadcast_to(xn, (16, D)).astype(bf16)
        gate = jnp.dot(xs, wg_v[...], preferred_element_type=f32)
        up = jnp.dot(xs, wu_v[...], preferred_element_type=f32)
        hmid = (gate * jax.nn.sigmoid(gate) * up).astype(bf16)
        y = jnp.dot(hmid, wd_v[...], preferred_element_type=f32)
        scale = jax.nn.sigmoid(jnp.full((1, D), rmax, f32))
        xres[pl.ds(idx, 1), :] = xres[pl.ds(idx, 1), :] + y[0:1] * scale

        @pl.when(layer == 1)
        def _():
            for i in range(NB):
                out_copy(i).wait()
            g0 = pl.multiple_of((idx // 16) * 16, 16)
            xio[pl.ds(g0, 16), :] = xres[pl.ds(g0, 16), :].astype(bf16)
            fix = pltpu.make_async_copy(xio.at[pl.ds(g0, 16), :], out_hbm.at[pl.ds(g0, 16), :], sem_w.at[7])
            fix.start()
            fix.wait()

    def layer_body(layer, c):
        with jax.named_scope("phase_a"):
            phase_a(layer)
        with jax.named_scope("phase_b"):
            phase_b()
        with jax.named_scope("phase_c"):
            phase_c(layer)
        with jax.named_scope("phase_d"):
            phase_d(layer)
        return c

    lax.fori_loop(0, 2, layer_body, 0)


@jax.jit
def pallas_interleave_layers__sliding_block__moe_arch_mod__prompt_kernel(
    A_x: jax.Array,
    A_wqkv: jax.Array,
    A_wo: jax.Array,
    B_x: jax.Array,
    B_w_r: jax.Array,
    B_w_gate: jax.Array,
    B_w_up: jax.Array,
    B_w_down: jax.Array,
):
    del B_x
    x = A_x.reshape(S, D)
    any_spec = pl.BlockSpec(memory_space=pl.ANY)
    scratch = [
        pltpu.VMEM((S, D), bf16),
        pltpu.VMEM((D, D), bf16),
        pltpu.VMEM((D, D), bf16),
        pltpu.VMEM((D, D), bf16),
        pltpu.VMEM((D // 2, D), u32),
        pltpu.VMEM((D, D), bf16),
        pltpu.VMEM((D // 2, D), u32),
        pltpu.VMEM((D,), bf16),
        pltpu.VMEM((D, F), bf16),
        pltpu.VMEM((D, F), bf16),
        pltpu.VMEM((F, D), bf16),
        pltpu.VMEM((S, D), f32),
        pltpu.VMEM((S, D), f32),
        pltpu.VMEM((8, 128), f32),
        pltpu.VMEM((8, 128), i32),
        pltpu.VMEM((S, 128), f32),
        pltpu.VMEM((8, 128), f32),
        pltpu.VMEM((8, D), f32),
        pltpu.VMEM((TQ // 2, D), u32),
        pltpu.VMEM((TQ // 2, D), u32),
        pltpu.VMEM((S // 2, D), u32),
        pltpu.VMEM((S // 2, D), u32),
        pltpu.VMEM((G, S // 2, 128), u32),
        pltpu.VMEM((G, (S + PAD) // 2, 128), u32),
        pltpu.VMEM((D // 2, S + PAD), u32),
        pltpu.VMEM((D // 2, S), u32),
        pltpu.VMEM((2, 4, 256, 128), f32),
        pltpu.VMEM((2, 4, 8, 128), f32),
        pltpu.VMEM((TQ, D), f32),
        pltpu.VMEM((TQ, D), f32),
        pltpu.SemaphoreType.DMA((NB,)),
        pltpu.SemaphoreType.DMA((10,)),
        pltpu.SemaphoreType.DMA((NB,)),
    ]
    out = pl.pallas_call(
        _kernel,
        out_shape=jax.ShapeDtypeStruct((S, D), bf16),
        in_specs=[any_spec] * 7,
        out_specs=any_spec,
        scratch_shapes=scratch,
        compiler_params=pltpu.CompilerParams(vmem_limit_bytes=120 * 1024 * 1024),
    )(x, A_wqkv, A_wo, B_w_r, B_w_gate, B_w_up, B_w_down)
    return out.reshape(1, S, D)
```

```python
import jax
import jax.numpy as jnp
from jax import lax
import jax.experimental.pallas as pl
import jax.experimental.pallas.tpu as pltpu

bf16 = jnp.bfloat16
f32 = jnp.float32
u32 = jnp.uint32
i32 = jnp.int32

S = 2048
D = 1024
H = 32
DH = 32
W = 256
F = 3584
G = 8
PAD = 256
TQ = 256
NB = S // TQ
TKV = 512
NSB = S // 128
import os
CH = int(os.environ.get('K_CH', 32))
NCH = TQ // CH
CHC = int(os.environ.get('K_CHC', 8))
NCHC = TQ // CHC
GATE_A = [c * 8 // NCH - 1 for c in range(NCH)]
NWC = int(os.environ.get('K_NWC', 128))
_GCN, _GCO = [int(v) for v in os.environ.get('K_GC', '8,-1').split(',')]
GATE_C = [min(c * _GCN // NCHC + _GCO, 7) for c in range(NCHC)]
EPS = 1e-5
NEG = -1e30
QSCALE = (DH ** -0.5) * 1.4426950408889634
NT = (((1,), (1,)), ((), ()))


def _ln(x):
    m = jnp.mean(x, axis=-1, keepdims=True)
    xc = x - m
    v = jnp.mean(xc * xc, axis=-1, keepdims=True)
    return xc * lax.rsqrt(v + EPS)


def _pack_rows(x):
    return pltpu.bitcast(x.astype(bf16), u32)


def _pack_rows_interleaved(x):
    n = x.shape[0] // 16
    x3 = x.reshape(n, 16, x.shape[1])
    a = x3[:, 0:8, :].reshape(n * 8, x.shape[1])
    b = x3[:, 8:16, :].reshape(n * 8, x.shape[1])
    return pltpu.pack_elementwise([a, b], packed_dtype=bf16)


def _gate_first(x, gate, z):
    g = gate[0:8, 0:128] * z
    top = jnp.concatenate([x[0:8, 0:128] + g, x[0:8, 128:]], axis=1)
    return top if x.shape[0] == 8 else jnp.concatenate([top, x[8:]], axis=0)


def _kernel(x_hbm, wqkv_hbm, wo_hbm, wr_hbm, wg_hbm, wu_hbm, wd_hbm,
            out_hbm,
            xio, wq_v, wk_v, wv_v, wvt_v, wo_v, wop_v, wr_v, wg_v, wu_v, wd_v,
            xres, xbuf, best_v, best_i, rho_s, z_s, wr8,
            xca, xcb, xc_all, xi_all,
            q_s, k_s, vt_s, ot_s, s_s, m_s,
            ata, atb, oa, ob,
            sem_x, sem_w, sem_o):
    def x_copy(i):
        r0 = pl.multiple_of(i * TQ, TQ)
        return pltpu.make_async_copy(x_hbm.at[pl.ds(r0, TQ), :], xio.at[pl.ds(r0, TQ), :], sem_x.at[i])

    def out_copy(i):
        r0 = pl.multiple_of(i * TQ, TQ)
        return pltpu.make_async_copy(xio.at[pl.ds(r0, TQ), :], out_hbm.at[pl.ds(r0, TQ), :], sem_o.at[i])

    cp_wqa = pltpu.make_async_copy(wqkv_hbm.at[:, pl.ds(0, D // 2)], wq_v.at[:, pl.ds(0, D // 2)], sem_w.at[0])
    cp_wqb = pltpu.make_async_copy(wqkv_hbm.at[:, pl.ds(D // 2, D // 2)], wq_v.at[:, pl.ds(D // 2, D // 2)],
                                   sem_w.at[9])
    cp_wk = pltpu.make_async_copy(wqkv_hbm.at[:, pl.ds(D, D)], wk_v, sem_w.at[1])
    cp_wv = pltpu.make_async_copy(wqkv_hbm.at[:, pl.ds(2 * D, D)], wv_v, sem_w.at[8])
    cp_wo = pltpu.make_async_copy(wo_hbm, wo_v, sem_w.at[2])
    cp_wr = pltpu.make_async_copy(wr_hbm, wr_v, sem_w.at[3])
    cp_wg = pltpu.make_async_copy(wg_hbm, wg_v, sem_w.at[4])
    cp_wu = pltpu.make_async_copy(wu_hbm, wu_v, sem_w.at[5])
    cp_wd = pltpu.make_async_copy(wd_hbm, wd_v, sem_w.at[6])

    x_copy(0).start()
    cp_wqa.start()

    z_s[...] = jnp.zeros_like(z_s)
    xres[0:CH, :] = jnp.zeros((CH, D), f32)

    def ln_chunk(layer, i, c, xc_ref, gate):
        r0 = i * TQ + c * CH
        h0 = i * (TQ // 2) + c * (CH // 2)
        if not isinstance(r0, int):
            r0 = pl.multiple_of(r0, CH)
            h0 = pl.multiple_of(h0, CH // 2)
        x_in = xio[pl.ds(r0, CH), :].astype(f32)
        x_rs = xres[pl.ds(pl.multiple_of(r0 * layer, CH), CH), :]
        x = jnp.where(layer == 0, x_in, x_rs)
        xbuf[pl.ds(r0, CH), :] = x
        if gate is not None:
            x = _gate_first(x, gate, z_s[...])
        xn = _ln(x)
        xc = _pack_rows(xn)
        xc_ref[c * CH // 2:(c + 1) * CH // 2, :] = xc
        xc_all[pl.ds(h0, CH // 2), :] = xc
        xi_all[pl.ds(h0, CH // 2), :] = _pack_rows_interleaved(xn)

    def q_step(layer, i, xc_ref, i_next, xc_next, part=(0, G)):
        h0 = i * (TQ // 2)
        if not isinstance(h0, int):
            h0 = pl.multiple_of(h0, TQ // 2)
        a = pltpu.bitcast(xc_ref[...], bf16)
        ys = {}
        for n in range(*part):
            y = jnp.dot(a, wq_v[:, n * 128:(n + 1) * 128], preferred_element_type=f32)
            q_s[n, pl.ds(h0, TQ // 2), :] = _pack_rows(y * QSCALE)
            ys[n] = y
        if i_next is not None:
            for c in range(part[0] * NCH // G, part[1] * NCH // G):
                ln_chunk(layer, i_next, c, xc_next, ys.get(GATE_A[c]))

    def kv_step(i):
        h0 = pl.multiple_of(i * (TKV // 2), TKV // 2)
        a = pltpu.bitcast(xc_all[pl.ds(h0, TKV // 2), :], bf16)
        for n in range(G):
            y = jnp.dot(a, wk_v[:, n * 128:(n + 1) * 128], preferred_element_type=f32)
            k_s[n, pl.ds(PAD // 2 + h0, TKV // 2), :] = _pack_rows(y)
        vt = lax.dot_general(pltpu.bitcast(wvt_v[...], bf16), pltpu.bitcast(xi_all[pl.ds(h0, TKV // 2), :], bf16),
                             NT, preferred_element_type=f32)
        c0 = pl.multiple_of(PAD + i * TKV, 256)
        vt_s[:, pl.ds(c0, TKV)] = _pack_rows(vt)

    def phase_a(layer):
        @pl.when(layer == 0)
        def _():
            x_copy(0).wait()
            x_copy(1).start()
            cp_wqb.start()

        for c in range(NCH):
            ln_chunk(layer, 0, c, xca, None)

        @pl.when(layer == 0)
        def _():
            cp_wqa.wait()
            x_copy(1).wait()
            for i in range(2, NB):
                x_copy(i).start()

        q_step(layer, 0, xca, 1, xcb, part=(0, G // 2))

        @pl.when(layer == 0)
        def _():
            cp_wqb.wait()
            cp_wv.start()
            cp_wo.start()
            cp_wk.start()
            cp_wr.start()

        q_step(layer, 0, xca, 1, xcb, part=(G // 2, G))

        def q_body(j, c):
            i1 = 2 * j + 1

            @pl.when(layer == 0)
            def _():
                x_copy(i1 + 1).wait()
                x_copy(i1 + 2).wait()

            q_step(layer, i1, xcb, i1 + 1, xca)
            q_step(layer, i1 + 1, xca, i1 + 2, xcb)
            return c

        with jax.named_scope("a_q"):
            lax.fori_loop(0, NB // 2 - 1, q_body, 0)

        @pl.when(layer == 0)
        def _():
            cp_wv.wait()
            cp_wo.wait()

        q_step(layer, NB - 1, xcb, None, None)
        wvt_v[...] = pltpu.bitcast(wv_v[...].T, u32)
        for c in range(D // 64):
            wop_v[c * 32:(c + 1) * 32, :] = _pack_rows_interleaved(wo_v[c * 64:(c + 1) * 64, :].astype(f32))

        @pl.when(layer == 0)
        def _():
            cp_wk.wait()
            cp_wg.start()
            cp_wu.start()
            cp_wd.start()

        def kv_body(j, c):
            kv_step(j)
            return c

        with jax.named_scope("a_kv"):
            lax.fori_loop(0, S // TKV, kv_body, 0)

    def qk_stage(g, q0, slot, kstart):
        zi = pltpu.bitcast(z_s[...], i32)
        zi16 = jnp.concatenate([zi, zi], axis=0)
        lane16 = lax.broadcasted_iota(i32, (16, 128), 1) + zi16
        r16 = lax.broadcasted_iota(i32, (16, 128), 0)
        hb16 = lane16 // 32
        dd = r16 - lane16 % 32
        h0 = q0 // 2
        first_rows = None
        for b in range(4):
            first = max(0, kstart - 32 * b)
            base = h0 + 16 * b
            if not isinstance(base, int):
                base = pl.multiple_of(base, 16)
            mid0 = max(first, 32)
            if first == 0:
                parts = [k_s[g, pl.ds(base, 8), :], k_s[g, pl.ds(base + 128, 8), :],
                         k_s[g, pl.ds(base + 8, 8), :], k_s[g, pl.ds(base + 136, 8), :]]
            else:
                parts = [k_s[g, pl.ds(base + 128, 16), :]]
            if mid0 < 256:
                parts.append(k_s[g, pl.ds(base + mid0 // 2, (256 - mid0) // 2), :])
            kw = pltpu.bitcast(jnp.concatenate(parts, axis=0), bf16)
            qu = q_s[g, pl.ds(base, 16), :]
            qall = pltpu.bitcast(
                jnp.concatenate([jnp.where(hb16 == (p - b) % 4, qu, jnp.uint32(0)) for p in range(4)], axis=0),
                bf16)
            st = lax.dot_general(kw, qall, NT, preferred_element_type=f32)
            if b == 0:
                first_rows = st[0:8]
            if first == 0:
                c0 = jnp.where(dd > 0, st[0:16], st[16:32])
                c1 = jnp.where(dd > -16, st[32:48], st[48:64])
                mid = st[64:]
            else:
                c0 = jnp.where(dd > 0, NEG, st[0:16])
                c1 = jnp.where(dd > -16, NEG, st[16:32])
                mid = st[32:]
            s_s[slot, b, 0:16, :] = c0
            s_s[slot, b, 16:32, :] = c1
            x = jnp.concatenate([c0, c1], axis=0)
            if mid0 < 256:
                s_s[slot, b, mid0:256, :] = mid
                x = jnp.concatenate([x, mid], axis=0)
            mm = jnp.max(x.reshape(x.shape[0] // 8, 8, 128), axis=0)
            m_s[slot, b] = jnp.broadcast_to(jnp.max(mm, axis=0, keepdims=True), (8, 128))
        return first_rows

    def pv_stage(g, q0, slot, gate, kstart):
        r8 = lax.broadcasted_iota(i32, (8, 128), 0)
        c8 = lax.broadcasted_iota(i32, (8, 128), 1) + pltpu.bitcast(z_s[...], i32)
        blk = c8 // 32
        j = c8 % 32

        def tri(u):
            return (jnp.where(16 * u + r8 > j, jnp.uint32(0xFFFF), jnp.uint32(0)) |
                    jnp.where(16 * u + 8 + r8 > j, jnp.uint32(0xFFFF0000), jnp.uint32(0)))

        tris = [tri(0), tri(1)] if kstart < 128 else None
        ms = [m_s[slot, b] for b in range(4)]
        L = [None] * 4
        cache = {}

        def pexp(b, u):
            x = s_s[slot, b, 16 * u:16 * u + 16, :]
            p0 = jnp.exp2(x[0:8] - ms[b])
            p1 = jnp.exp2(x[8:16] - ms[b])
            sm = p0 + p1
            L[b] = sm if L[b] is None else L[b] + sm
            return pltpu.pack_elementwise([p0, p1], packed_dtype=bf16)

        def get_p(b, u):
            first = max(0, kstart - 32 * b)
            if u < 0 or u >= 18 or 16 * u < first:
                return None
            if first > 0:
                return pexp(b, u - 16) if u >= 16 else pexp(b, u)
            if u < 2:
                pk = pexp(b, u)
                lo = pk & tris[u]
                cache[(b, u + 16)] = pk ^ lo
                return lo
            if u >= 16:
                return cache.pop((b, u))
            return pexp(b, u)

        zero = jnp.zeros((8, 128), u32)
        accs = [None] * 4
        for k in range(kstart // 128, 3):
            wts = [[] for _ in range(4)]
            for t in range(8 * k, 8 * k + 8):
                if t == 8 and kstart == 0:
                    gv = gate * z_s[...]
                    for b in range(4):
                        ms[b] = ms[b] + gv
                srcs = [(b, get_p(b, t - 2 * b)) for b in range(4)]
                srcs = [(b, v) for (b, v) in srcs if v is not None]
                for h in range(4):
                    acc = zero if len(srcs) < 4 else None
                    for (b, v) in srcs:
                        acc = v if acc is None else jnp.where(blk == (h + b) % 4, v, acc)
                    wts[h].append(acc)
            c0 = q0 + 128 * k
            if not isinstance(c0, int):
                c0 = pl.multiple_of(c0, 128)
            for h in range(4):
                pt = pltpu.bitcast(jnp.concatenate(wts[h], axis=0), bf16)
                vth = pltpu.bitcast(vt_s[pl.ds((g * 4 + h) * 16, 16), pl.ds(c0, 128)], bf16)
                d = jnp.dot(vth, pt, preferred_element_type=f32)
                accs[h] = d if accs[h] is None else accs[h] + d
        L = [jnp.broadcast_to(jnp.sum(l, axis=0, keepdims=True), (8, 128)) for l in L]
        outs = []
        for h in range(4):
            lh = L[0]
            for b in range(1, 4):
                lh = jnp.where(blk == (h + b) % 4, L[b], lh)
            r0 = pl.reciprocal(lh, approx=True)
            rl = r0 * (2.0 - lh * r0)
            ot = (accs[h].reshape(4, 8, 128) * rl[None]).reshape(32, 128)
            if h > 0:
                ot = pltpu.roll(ot, 128 - 32 * h, axis=1)
            outs.append(ot)
        ot_s[g * 64:(g + 1) * 64, pl.ds(q0, 128)] = _pack_rows_interleaved(jnp.concatenate(outs, axis=0))

    def sub_block(q0, qn, kstart, kstart_next):
        for g in range(G):
            if g + 1 < G:
                gate = qk_stage(g + 1, q0, (g + 1) % 2, kstart)
            else:
                gate = qk_stage(0, qn, 0, kstart_next)
            pv_stage(g, q0, g % 2, gate, kstart)

    def phase_b():
        qk_stage(0, 0, 0, PAD)
        sub_block(0, 128, PAD, PAD - 128)
        sub_block(128, 256, PAD - 128, 0)

        def body(sb, c):
            q0 = pl.multiple_of(sb * 128, 128)
            qn = pl.multiple_of(jnp.minimum(sb + 1, NSB - 1) * 128, 128)
            sub_block(q0, qn, 0, 0)
            return c

        lax.fori_loop(2, NSB, body, 0)

    def resid_chunk(i, c, at_ref, gate):
        r0 = i * TQ + c * CHC
        if not isinstance(r0, int):
            r0 = pl.multiple_of(r0, CHC)
        x1 = xbuf[pl.ds(r0, CHC), :] + at_ref[c * CHC:(c + 1) * CHC, :]
        if gate is not None:
            x1 = _gate_first(x1, gate, z_s[...])
        m = jnp.mean(x1, axis=-1, keepdims=True)
        xc = x1 - m
        v = jnp.mean(xc * xc, axis=-1, keepdims=True)
        rho = lax.rsqrt(v + EPS)
        xn = xc * rho
        r = jnp.sum(xn * wr8[0:1, :], axis=-1, keepdims=True)
        rb = jnp.broadcast_to(r, (CHC, 128)).astype(bf16).astype(f32)
        rows = lax.broadcasted_iota(i32, (8, 128), 0) + r0
        bv, bi = best_v[...], best_i[...]
        for q in range(CHC // 8):
            cand = rb[8 * q:8 * q + 8]
            better = cand > bv
            bv = jnp.where(better, cand, bv)
            bi = jnp.where(better, rows + 8 * q, bi)
        best_v[...] = bv
        best_i[...] = bi
        rho_s[pl.ds(r0, CHC), :] = jnp.broadcast_to(rho, (CHC, 128))
        x2 = x1 + xn
        xres[pl.ds(r0, CHC), :] = x2
        xio[pl.ds(r0, CHC), :] = x2.astype(bf16)

    def transpose_o(i, o_dst):
        r0 = i * TQ
        if not isinstance(r0, int):
            r0 = pl.multiple_of(r0, TQ)
        o_dst[...] = pltpu.bitcast(pltpu.bitcast(ot_s[:, pl.ds(r0, TQ)], bf16).T, u32)

    def oproj_step(o_src, at_w, i_res, at_r, i_t, o_dst):
        ys = []
        if o_src is not None:
            a = pltpu.bitcast(o_src[...], bf16)
            for n in range(D // NWC):
                y = jnp.dot(a, pltpu.bitcast(wop_v[:, n * NWC:(n + 1) * NWC], bf16), preferred_element_type=f32)
                at_w[:, n * NWC:(n + 1) * NWC] = y
                ys.append(y)
        if i_t is not None:
            transpose_o(i_t, o_dst)
        if i_res is not None:
            for c in range(NCHC):
                gi = GATE_C[c] if ys else -1
                gate = ys[gi] if gi >= 0 else None
                resid_chunk(i_res, c, at_r, gate)

    def phase_c(layer):
        @pl.when(layer == 0)
        def _():
            cp_wr.wait()
            wr8[...] = jnp.broadcast_to(wr_v[...].astype(f32).reshape(1, D), (8, D))

        def flush(i):
            @pl.when(layer == 1)
            def _():
                out_copy(i).start()

        best_v[...] = jnp.full((8, 128), -jnp.inf, f32)
        best_i[...] = jnp.zeros((8, 128), i32)
        transpose_o(0, oa)
        oproj_step(oa, ata, None, None, 1, ob)

        def body(j, c):
            i0 = 2 * j
            oproj_step(ob, atb, i0, ata, i0 + 2, oa)
            oproj_step(oa, ata, i0 + 1, atb, i0 + 3, ob)
            flush(i0)
            flush(i0 + 1)
            return c

        lax.fori_loop(0, NB // 2 - 1, body, 0)
        oproj_step(ob, atb, NB - 2, ata, None, None)
        oproj_step(None, None, NB - 1, atb, None, None)
        flush(NB - 2)
        flush(NB - 1)

    def phase_d(layer):
        @pl.when(layer == 0)
        def _():
            cp_wg.wait()
            cp_wu.wait()
            cp_wd.wait()

        bv = best_v[...]
        rmax = jnp.max(bv)
        idx = jnp.min(jnp.where(bv == rmax, best_i[...], S))
        idx = jnp.clip(idx, 0, S - 1)
        x2 = xres[pl.ds(idx, 1), :]
        rho = rho_s[pl.ds(idx, 1), 0:1]
        xn = (x2 - jnp.mean(x2, axis=-1, keepdims=True)) * (rho / (1.0 + rho))
        xs = jnp.broadcast_to(xn, (16, D)).astype(bf16)
        gate = jnp.dot(xs, wg_v[...], preferred_element_type=f32)
        up = jnp.dot(xs, wu_v[...], preferred_element_type=f32)
        hmid = (gate * jax.nn.sigmoid(gate) * up).astype(bf16)
        y = jnp.dot(hmid, wd_v[...], preferred_element_type=f32)
        scale = jax.nn.sigmoid(jnp.full((1, D), rmax, f32))
        xres[pl.ds(idx, 1), :] = xres[pl.ds(idx, 1), :] + y[0:1] * scale

        @pl.when(layer == 1)
        def _():
            for i in range(NB):
                out_copy(i).wait()
            g0 = pl.multiple_of((idx // 16) * 16, 16)
            xio[pl.ds(g0, 16), :] = xres[pl.ds(g0, 16), :].astype(bf16)
            fix = pltpu.make_async_copy(xio.at[pl.ds(g0, 16), :], out_hbm.at[pl.ds(g0, 16), :], sem_w.at[7])
            fix.start()
            fix.wait()

    def layer_body(layer, c):
        with jax.named_scope("phase_a"):
            phase_a(layer)
        with jax.named_scope("phase_b"):
            phase_b()
        with jax.named_scope("phase_c"):
            phase_c(layer)
        with jax.named_scope("phase_d"):
            phase_d(layer)
        return c

    lax.fori_loop(0, 2, layer_body, 0)


@jax.jit
def pallas_interleave_layers__sliding_block__moe_arch_mod__prompt_kernel(
    A_x: jax.Array,
    A_wqkv: jax.Array,
    A_wo: jax.Array,
    B_x: jax.Array,
    B_w_r: jax.Array,
    B_w_gate: jax.Array,
    B_w_up: jax.Array,
    B_w_down: jax.Array,
):
    del B_x
    x = A_x.reshape(S, D)
    any_spec = pl.BlockSpec(memory_space=pl.ANY)
    scratch = [
        pltpu.VMEM((S, D), bf16),
        pltpu.VMEM((D, D), bf16),
        pltpu.VMEM((D, D), bf16),
        pltpu.VMEM((D, D), bf16),
        pltpu.VMEM((D // 2, D), u32),
        pltpu.VMEM((D, D), bf16),
        pltpu.VMEM((D // 2, D), u32),
        pltpu.VMEM((D,), bf16),
        pltpu.VMEM((D, F), bf16),
        pltpu.VMEM((D, F), bf16),
        pltpu.VMEM((F, D), bf16),
        pltpu.VMEM((S, D), f32),
        pltpu.VMEM((S, D), f32),
        pltpu.VMEM((8, 128), f32),
        pltpu.VMEM((8, 128), i32),
        pltpu.VMEM((S, 128), f32),
        pltpu.VMEM((8, 128), f32),
        pltpu.VMEM((8, D), f32),
        pltpu.VMEM((TQ // 2, D), u32),
        pltpu.VMEM((TQ // 2, D), u32),
        pltpu.VMEM((S // 2, D), u32),
        pltpu.VMEM((S // 2, D), u32),
        pltpu.VMEM((G, S // 2, 128), u32),
        pltpu.VMEM((G, (S + PAD) // 2, 128), u32),
        pltpu.VMEM((D // 2, S + PAD), u32),
        pltpu.VMEM((D // 2, S), u32),
        pltpu.VMEM((2, 4, 256, 128), f32),
        pltpu.VMEM((2, 4, 8, 128), f32),
        pltpu.VMEM((TQ, D), f32),
        pltpu.VMEM((TQ, D), f32),
        pltpu.VMEM((TQ // 2, D), u32),
        pltpu.VMEM((TQ // 2, D), u32),
        pltpu.SemaphoreType.DMA((NB,)),
        pltpu.SemaphoreType.DMA((10,)),
        pltpu.SemaphoreType.DMA((NB,)),
    ]
    out = pl.pallas_call(
        _kernel,
        out_shape=jax.ShapeDtypeStruct((S, D), bf16),
        in_specs=[any_spec] * 7,
        out_specs=any_spec,
        scratch_shapes=scratch,
        compiler_params=pltpu.CompilerParams(vmem_limit_bytes=120 * 1024 * 1024),
    )(x, A_wqkv, A_wo, B_w_r, B_w_gate, B_w_up, B_w_down)
    return out.reshape(1, S, D)
```

```python
import jax
import jax.numpy as jnp
from jax import lax
import jax.experimental.pallas as pl
import jax.experimental.pallas.tpu as pltpu

bf16 = jnp.bfloat16
f32 = jnp.float32
u32 = jnp.uint32
i32 = jnp.int32

S = 2048
D = 1024
H = 32
DH = 32
W = 256
F = 3584
G = 8
PAD = 256
TQ = 256
NB = S // TQ
TKV = 512
NSB = S // 128
import os
CH = int(os.environ.get('K_CH', 32))
NCH = TQ // CH
CHC = int(os.environ.get('K_CHC', 8))
NCHC = TQ // CHC
GATE_A = [c * 8 // NCH - 1 for c in range(NCH)]
NWC = int(os.environ.get('K_NWC', 128))
_GCN, _GCO = [int(v) for v in os.environ.get('K_GC', '8,-1').split(',')]
GATE_C = [min(c * _GCN // NCHC + _GCO, 7) for c in range(NCHC)]
LNR = int(os.environ.get('K_LNR', 8))
GATE_EACH = int(os.environ.get('K_GE', 1))
EPS = 1e-5
NEG = -1e30
QSCALE = (DH ** -0.5) * 1.4426950408889634
NT = (((1,), (1,)), ((), ()))


def _ln(x):
    m = jnp.mean(x, axis=-1, keepdims=True)
    xc = x - m
    v = jnp.mean(xc * xc, axis=-1, keepdims=True)
    return xc * lax.rsqrt(v + EPS)


def _pack_rows(x):
    return pltpu.bitcast(x.astype(bf16), u32)


def _pack_rows_interleaved(x):
    n = x.shape[0] // 16
    x3 = x.reshape(n, 16, x.shape[1])
    a = x3[:, 0:8, :].reshape(n * 8, x.shape[1])
    b = x3[:, 8:16, :].reshape(n * 8, x.shape[1])
    return pltpu.pack_elementwise([a, b], packed_dtype=bf16)


def _gate_first(x, gate, z):
    g = gate[0:8, 0:128] * z
    top = jnp.concatenate([x[0:8, 0:128] + g, x[0:8, 128:]], axis=1)
    return top if x.shape[0] == 8 else jnp.concatenate([top, x[8:]], axis=0)


def _kernel(x_hbm, wqkv_hbm, wo_hbm, wr_hbm, wg_hbm, wu_hbm, wd_hbm,
            out_hbm,
            xio, wq_v, wk_v, wv_v, wvt_v, wo_v, wop_v, wr_v, wg_v, wu_v, wd_v,
            xres, xbuf, best_v, best_i, rho_s, z_s, wr8,
            xca, xcb, xc_all, xi_all,
            q_s, k_s, vt_s, ot_s, s_s, m_s,
            ata, atb, oa, ob,
            sem_x, sem_w, sem_o):
    def x_copy(i):
        r0 = pl.multiple_of(i * TQ, TQ)
        return pltpu.make_async_copy(x_hbm.at[pl.ds(r0, TQ), :], xio.at[pl.ds(r0, TQ), :], sem_x.at[i])

    def out_copy(i):
        r0 = pl.multiple_of(i * TQ, TQ)
        return pltpu.make_async_copy(xio.at[pl.ds(r0, TQ), :], out_hbm.at[pl.ds(r0, TQ), :], sem_o.at[i])

    cp_wqa = pltpu.make_async_copy(wqkv_hbm.at[:, pl.ds(0, D // 2)], wq_v.at[:, pl.ds(0, D // 2)], sem_w.at[0])
    cp_wqb = pltpu.make_async_copy(wqkv_hbm.at[:, pl.ds(D // 2, D // 2)], wq_v.at[:, pl.ds(D // 2, D // 2)],
                                   sem_w.at[9])
    cp_wk = pltpu.make_async_copy(wqkv_hbm.at[:, pl.ds(D, D)], wk_v, sem_w.at[1])
    cp_wv = pltpu.make_async_copy(wqkv_hbm.at[:, pl.ds(2 * D, D)], wv_v, sem_w.at[8])
    cp_wo = pltpu.make_async_copy(wo_hbm, wo_v, sem_w.at[2])
    cp_wr = pltpu.make_async_copy(wr_hbm, wr_v, sem_w.at[3])
    cp_wg = pltpu.make_async_copy(wg_hbm, wg_v, sem_w.at[4])
    cp_wu = pltpu.make_async_copy(wu_hbm, wu_v, sem_w.at[5])
    cp_wd = pltpu.make_async_copy(wd_hbm, wd_v, sem_w.at[6])

    x_copy(0).start()
    cp_wqa.start()

    z_s[...] = jnp.zeros_like(z_s)
    xres[0:CH, :] = jnp.zeros((CH, D), f32)

    def ln_chunk(layer, i, c, xc_ref, gate):
        r0 = i * TQ + c * CH
        h0 = i * (TQ // 2) + c * (CH // 2)
        if not isinstance(r0, int):
            r0 = pl.multiple_of(r0, CH)
            h0 = pl.multiple_of(h0, CH // 2)
        parts = []
        for q in range(CH // LNR):
            rq = r0 + q * LNR
            x_in = xio[pl.ds(rq, LNR), :].astype(f32)
            x_rs = xres[pl.ds(pl.multiple_of(rq * layer, LNR), LNR), :]
            xq = jnp.where(layer == 0, x_in, x_rs)
            xbuf[pl.ds(rq, LNR), :] = xq
            if gate is not None:
                xq = _gate_first(xq, gate, z_s[...])
            parts.append(_ln(xq))
        xn = jnp.concatenate(parts, axis=0)
        xc = _pack_rows(xn)
        xc_ref[c * CH // 2:(c + 1) * CH // 2, :] = xc
        xc_all[pl.ds(h0, CH // 2), :] = xc
        xi_all[pl.ds(h0, CH // 2), :] = _pack_rows_interleaved(xn)

    def q_step(layer, i, xc_ref, i_next, xc_next, part=(0, G)):
        h0 = i * (TQ // 2)
        if not isinstance(h0, int):
            h0 = pl.multiple_of(h0, TQ // 2)
        a = pltpu.bitcast(xc_ref[...], bf16)
        ys = {}
        for n in range(*part):
            y = jnp.dot(a, wq_v[:, n * 128:(n + 1) * 128], preferred_element_type=f32)
            q_s[n, pl.ds(h0, TQ // 2), :] = _pack_rows(y * QSCALE)
            ys[n] = y
        if i_next is not None:
            for c in range(part[0] * NCH // G, part[1] * NCH // G):
                ln_chunk(layer, i_next, c, xc_next, ys.get(GATE_A[c]))

    def kv_step(i):
        h0 = pl.multiple_of(i * (TKV // 2), TKV // 2)
        a = pltpu.bitcast(xc_all[pl.ds(h0, TKV // 2), :], bf16)
        for n in range(G):
            y = jnp.dot(a, wk_v[:, n * 128:(n + 1) * 128], preferred_element_type=f32)
            k_s[n, pl.ds(PAD // 2 + h0, TKV // 2), :] = _pack_rows(y)
        vt = lax.dot_general(pltpu.bitcast(wvt_v[...], bf16), pltpu.bitcast(xi_all[pl.ds(h0, TKV // 2), :], bf16),
                             NT, preferred_element_type=f32)
        c0 = pl.multiple_of(PAD + i * TKV, 256)
        vt_s[:, pl.ds(c0, TKV)] = _pack_rows(vt)

    def phase_a(layer):
        @pl.when(layer == 0)
        def _():
            x_copy(0).wait()
            x_copy(1).start()
            cp_wqb.start()

        for c in range(NCH):
            ln_chunk(layer, 0, c, xca, None)

        @pl.when(layer == 0)
        def _():
            cp_wqa.wait()
            x_copy(1).wait()
            for i in range(2, NB):
                x_copy(i).start()

        q_step(layer, 0, xca, 1, xcb, part=(0, G // 2))

        @pl.when(layer == 0)
        def _():
            cp_wqb.wait()
            cp_wv.start()
            cp_wo.start()
            cp_wk.start()
            cp_wr.start()

        q_step(layer, 0, xca, 1, xcb, part=(G // 2, G))

        def q_body(j, c):
            i1 = 2 * j + 1

            @pl.when(layer == 0)
            def _():
                x_copy(i1 + 1).wait()
                x_copy(i1 + 2).wait()

            q_step(layer, i1, xcb, i1 + 1, xca)
            q_step(layer, i1 + 1, xca, i1 + 2, xcb)
            return c

        with jax.named_scope("a_q"):
            lax.fori_loop(0, NB // 2 - 1, q_body, 0)

        @pl.when(layer == 0)
        def _():
            cp_wv.wait()
            cp_wo.wait()

        q_step(layer, NB - 1, xcb, None, None)
        wvt_v[...] = pltpu.bitcast(wv_v[...].T, u32)
        for c in range(D // 64):
            wop_v[c * 32:(c + 1) * 32, :] = _pack_rows_interleaved(wo_v[c * 64:(c + 1) * 64, :].astype(f32))

        @pl.when(layer == 0)
        def _():
            cp_wk.wait()
            cp_wg.start()
            cp_wu.start()
            cp_wd.start()

        def kv_body(j, c):
            kv_step(j)
            return c

        with jax.named_scope("a_kv"):
            lax.fori_loop(0, S // TKV, kv_body, 0)

    def qk_stage(g, q0, slot, kstart):
        zi = pltpu.bitcast(z_s[...], i32)
        zi16 = jnp.concatenate([zi, zi], axis=0)
        lane16 = lax.broadcasted_iota(i32, (16, 128), 1) + zi16
        r16 = lax.broadcasted_iota(i32, (16, 128), 0)
        hb16 = lane16 // 32
        dd = r16 - lane16 % 32
        h0 = q0 // 2
        first_rows = None
        for b in range(4):
            first = max(0, kstart - 32 * b)
            base = h0 + 16 * b
            if not isinstance(base, int):
                base = pl.multiple_of(base, 16)
            mid0 = max(first, 32)
            if first == 0:
                parts = [k_s[g, pl.ds(base, 8), :], k_s[g, pl.ds(base + 128, 8), :],
                         k_s[g, pl.ds(base + 8, 8), :], k_s[g, pl.ds(base + 136, 8), :]]
            else:
                parts = [k_s[g, pl.ds(base + 128, 16), :]]
            if mid0 < 256:
                parts.append(k_s[g, pl.ds(base + mid0 // 2, (256 - mid0) // 2), :])
            kw = pltpu.bitcast(jnp.concatenate(parts, axis=0), bf16)
            qu = q_s[g, pl.ds(base, 16), :]
            qall = pltpu.bitcast(
                jnp.concatenate([jnp.where(hb16 == (p - b) % 4, qu, jnp.uint32(0)) for p in range(4)], axis=0),
                bf16)
            st = lax.dot_general(kw, qall, NT, preferred_element_type=f32)
            if b == 0:
                first_rows = st[0:8]
            if first == 0:
                c0 = jnp.where(dd > 0, st[0:16], st[16:32])
                c1 = jnp.where(dd > -16, st[32:48], st[48:64])
                mid = st[64:]
            else:
                c0 = jnp.where(dd > 0, NEG, st[0:16])
                c1 = jnp.where(dd > -16, NEG, st[16:32])
                mid = st[32:]
            s_s[slot, b, 0:16, :] = c0
            s_s[slot, b, 16:32, :] = c1
            x = jnp.concatenate([c0, c1], axis=0)
            if mid0 < 256:
                s_s[slot, b, mid0:256, :] = mid
                x = jnp.concatenate([x, mid], axis=0)
            mm = jnp.max(x.reshape(x.shape[0] // 8, 8, 128), axis=0)
            m_s[slot, b] = jnp.broadcast_to(jnp.max(mm, axis=0, keepdims=True), (8, 128))
        return first_rows

    def pv_stage(g, q0, slot, gate, kstart):
        r8 = lax.broadcasted_iota(i32, (8, 128), 0)
        c8 = lax.broadcasted_iota(i32, (8, 128), 1) + pltpu.bitcast(z_s[...], i32)
        blk = c8 // 32
        j = c8 % 32

        def tri(u):
            return (jnp.where(16 * u + r8 > j, jnp.uint32(0xFFFF), jnp.uint32(0)) |
                    jnp.where(16 * u + 8 + r8 > j, jnp.uint32(0xFFFF0000), jnp.uint32(0)))

        tris = [tri(0), tri(1)] if kstart < 128 else None
        ms = [m_s[slot, b] for b in range(4)]
        L = [None] * 4
        cache = {}

        def pexp(b, u):
            x = s_s[slot, b, 16 * u:16 * u + 16, :]
            p0 = jnp.exp2(x[0:8] - ms[b])
            p1 = jnp.exp2(x[8:16] - ms[b])
            sm = p0 + p1
            L[b] = sm if L[b] is None else L[b] + sm
            return pltpu.pack_elementwise([p0, p1], packed_dtype=bf16)

        def get_p(b, u):
            first = max(0, kstart - 32 * b)
            if u < 0 or u >= 18 or 16 * u < first:
                return None
            if first > 0:
                return pexp(b, u - 16) if u >= 16 else pexp(b, u)
            if u < 2:
                pk = pexp(b, u)
                lo = pk & tris[u]
                cache[(b, u + 16)] = pk ^ lo
                return lo
            if u >= 16:
                return cache.pop((b, u))
            return pexp(b, u)

        zero = jnp.zeros((8, 128), u32)
        accs = [None] * 4
        for k in range(kstart // 128, 3):
            wts = [[] for _ in range(4)]
            for t in range(8 * k, 8 * k + 8):
                if t == 8 and kstart == 0:
                    gv = gate * z_s[...]
                    for b in range(4):
                        ms[b] = ms[b] + gv
                srcs = [(b, get_p(b, t - 2 * b)) for b in range(4)]
                srcs = [(b, v) for (b, v) in srcs if v is not None]
                for h in range(4):
                    acc = zero if len(srcs) < 4 else None
                    for (b, v) in srcs:
                        acc = v if acc is None else jnp.where(blk == (h + b) % 4, v, acc)
                    wts[h].append(acc)
            c0 = q0 + 128 * k
            if not isinstance(c0, int):
                c0 = pl.multiple_of(c0, 128)
            for h in range(4):
                pt = pltpu.bitcast(jnp.concatenate(wts[h], axis=0), bf16)
                vth = pltpu.bitcast(vt_s[pl.ds((g * 4 + h) * 16, 16), pl.ds(c0, 128)], bf16)
                d = jnp.dot(vth, pt, preferred_element_type=f32)
                accs[h] = d if accs[h] is None else accs[h] + d
        L = [jnp.broadcast_to(jnp.sum(l, axis=0, keepdims=True), (8, 128)) for l in L]
        outs = []
        for h in range(4):
            lh = L[0]
            for b in range(1, 4):
                lh = jnp.where(blk == (h + b) % 4, L[b], lh)
            r0 = pl.reciprocal(lh, approx=True)
            rl = r0 * (2.0 - lh * r0)
            ot = (accs[h].reshape(4, 8, 128) * rl[None]).reshape(32, 128)
            if h > 0:
                ot = pltpu.roll(ot, 128 - 32 * h, axis=1)
            outs.append(ot)
        ot_s[g * 64:(g + 1) * 64, pl.ds(q0, 128)] = _pack_rows_interleaved(jnp.concatenate(outs, axis=0))

    def sub_block(q0, qn, kstart, kstart_next):
        for g in range(G):
            if g + 1 < G:
                gate = qk_stage(g + 1, q0, (g + 1) % 2, kstart)
            else:
                gate = qk_stage(0, qn, 0, kstart_next)
            pv_stage(g, q0, g % 2, gate, kstart)

    def phase_b():
        qk_stage(0, 0, 0, PAD)
        sub_block(0, 128, PAD, PAD - 128)
        sub_block(128, 256, PAD - 128, 0)

        def body(sb, c):
            q0 = pl.multiple_of(sb * 128, 128)
            qn = pl.multiple_of(jnp.minimum(sb + 1, NSB - 1) * 128, 128)
            sub_block(q0, qn, 0, 0)
            return c

        lax.fori_loop(2, NSB, body, 0, unroll=int(os.environ.get('K_UB', 2)))

    def resid_chunk(i, c, at_ref, gate):
        r0 = i * TQ + c * CHC
        if not isinstance(r0, int):
            r0 = pl.multiple_of(r0, CHC)
        x1 = xbuf[pl.ds(r0, CHC), :] + at_ref[c * CHC:(c + 1) * CHC, :]
        if gate is not None:
            x1 = _gate_first(x1, gate, z_s[...])
        m = jnp.mean(x1, axis=-1, keepdims=True)
        xc = x1 - m
        v = jnp.mean(xc * xc, axis=-1, keepdims=True)
        rho = lax.rsqrt(v + EPS)
        xn = xc * rho
        r = jnp.sum(xn * wr8[0:1, :], axis=-1, keepdims=True)
        rb = jnp.broadcast_to(r, (CHC, 128)).astype(bf16).astype(f32)
        rows = lax.broadcasted_iota(i32, (8, 128), 0) + r0
        bv, bi = best_v[...], best_i[...]
        for q in range(CHC // 8):
            cand = rb[8 * q:8 * q + 8]
            better = cand > bv
            bv = jnp.where(better, cand, bv)
            bi = jnp.where(better, rows + 8 * q, bi)
        best_v[...] = bv
        best_i[...] = bi
        rho_s[pl.ds(r0, CHC), :] = jnp.broadcast_to(rho, (CHC, 128))
        x2 = x1 + xn
        xres[pl.ds(r0, CHC), :] = x2
        xio[pl.ds(r0, CHC), :] = x2.astype(bf16)

    def transpose_o(i, o_dst):
        r0 = i * TQ
        if not isinstance(r0, int):
            r0 = pl.multiple_of(r0, TQ)
        o_dst[...] = pltpu.bitcast(pltpu.bitcast(ot_s[:, pl.ds(r0, TQ)], bf16).T, u32)

    def oproj_step(o_src, at_w, i_res, at_r, i_t, o_dst):
        ys = []
        if o_src is not None:
            a = pltpu.bitcast(o_src[...], bf16)
            for n in range(D // NWC):
                y = jnp.dot(a, pltpu.bitcast(wop_v[:, n * NWC:(n + 1) * NWC], bf16), preferred_element_type=f32)
                at_w[:, n * NWC:(n + 1) * NWC] = y
                ys.append(y)
        if i_t is not None:
            transpose_o(i_t, o_dst)
        if i_res is not None:
            for c in range(NCHC):
                gi = GATE_C[c] if ys else -1
                gate = ys[gi] if gi >= 0 else None
                resid_chunk(i_res, c, at_r, gate)

    def phase_c(layer):
        @pl.when(layer == 0)
        def _():
            cp_wr.wait()
            wr8[...] = jnp.broadcast_to(wr_v[...].astype(f32).reshape(1, D), (8, D))

        def flush(i):
            @pl.when(layer == 1)
            def _():
                out_copy(i).start()

        best_v[...] = jnp.full((8, 128), -jnp.inf, f32)
        best_i[...] = jnp.zeros((8, 128), i32)
        transpose_o(0, oa)
        oproj_step(oa, ata, None, None, 1, ob)

        def body(j, c):
            i0 = 2 * j
            oproj_step(ob, atb, i0, ata, i0 + 2, oa)
            oproj_step(oa, ata, i0 + 1, atb, i0 + 3, ob)
            flush(i0)
            flush(i0 + 1)
            return c

        lax.fori_loop(0, NB // 2 - 1, body, 0)
        oproj_step(ob, atb, NB - 2, ata, None, None)
        oproj_step(None, None, NB - 1, atb, None, None)
        flush(NB - 2)
        flush(NB - 1)

    def phase_d(layer):
        @pl.when(layer == 0)
        def _():
            cp_wg.wait()
            cp_wu.wait()
            cp_wd.wait()

        bv = best_v[...]
        rmax = jnp.max(bv)
        idx = jnp.min(jnp.where(bv == rmax, best_i[...], S))
        idx = jnp.clip(idx, 0, S - 1)
        x2 = xres[pl.ds(idx, 1), :]
        rho = rho_s[pl.ds(idx, 1), 0:1]
        xn = (x2 - jnp.mean(x2, axis=-1, keepdims=True)) * (rho / (1.0 + rho))
        xs = jnp.broadcast_to(xn, (16, D)).astype(bf16)
        gate = jnp.dot(xs, wg_v[...], preferred_element_type=f32)
        up = jnp.dot(xs, wu_v[...], preferred_element_type=f32)
        hmid = (gate * jax.nn.sigmoid(gate) * up).astype(bf16)
        y = jnp.dot(hmid, wd_v[...], preferred_element_type=f32)
        scale = jax.nn.sigmoid(jnp.full((1, D), rmax, f32))
        xres[pl.ds(idx, 1), :] = xres[pl.ds(idx, 1), :] + y[0:1] * scale

        @pl.when(layer == 1)
        def _():
            for i in range(NB):
                out_copy(i).wait()
            g0 = pl.multiple_of((idx // 16) * 16, 16)
            xio[pl.ds(g0, 16), :] = xres[pl.ds(g0, 16), :].astype(bf16)
            fix = pltpu.make_async_copy(xio.at[pl.ds(g0, 16), :], out_hbm.at[pl.ds(g0, 16), :], sem_w.at[7])
            fix.start()
            fix.wait()

    def layer_body(layer, c):
        with jax.named_scope("phase_a"):
            phase_a(layer)
        with jax.named_scope("phase_b"):
            phase_b()
        with jax.named_scope("phase_c"):
            phase_c(layer)
        with jax.named_scope("phase_d"):
            phase_d(layer)
        return c

    lax.fori_loop(0, 2, layer_body, 0)


@jax.jit
def pallas_interleave_layers__sliding_block__moe_arch_mod__prompt_kernel(
    A_x: jax.Array,
    A_wqkv: jax.Array,
    A_wo: jax.Array,
    B_x: jax.Array,
    B_w_r: jax.Array,
    B_w_gate: jax.Array,
    B_w_up: jax.Array,
    B_w_down: jax.Array,
):
    del B_x
    x = A_x.reshape(S, D)
    any_spec = pl.BlockSpec(memory_space=pl.ANY)
    scratch = [
        pltpu.VMEM((S, D), bf16),
        pltpu.VMEM((D, D), bf16),
        pltpu.VMEM((D, D), bf16),
        pltpu.VMEM((D, D), bf16),
        pltpu.VMEM((D // 2, D), u32),
        pltpu.VMEM((D, D), bf16),
        pltpu.VMEM((D // 2, D), u32),
        pltpu.VMEM((D,), bf16),
        pltpu.VMEM((D, F), bf16),
        pltpu.VMEM((D, F), bf16),
        pltpu.VMEM((F, D), bf16),
        pltpu.VMEM((S, D), f32),
        pltpu.VMEM((S, D), f32),
        pltpu.VMEM((8, 128), f32),
        pltpu.VMEM((8, 128), i32),
        pltpu.VMEM((S, 128), f32),
        pltpu.VMEM((8, 128), f32),
        pltpu.VMEM((8, D), f32),
        pltpu.VMEM((TQ // 2, D), u32),
        pltpu.VMEM((TQ // 2, D), u32),
        pltpu.VMEM((S // 2, D), u32),
        pltpu.VMEM((S // 2, D), u32),
        pltpu.VMEM((G, S // 2, 128), u32),
        pltpu.VMEM((G, (S + PAD) // 2, 128), u32),
        pltpu.VMEM((D // 2, S + PAD), u32),
        pltpu.VMEM((D // 2, S), u32),
        pltpu.VMEM((2, 4, 256, 128), f32),
        pltpu.VMEM((2, 4, 8, 128), f32),
        pltpu.VMEM((TQ, D), f32),
        pltpu.VMEM((TQ, D), f32),
        pltpu.VMEM((TQ // 2, D), u32),
        pltpu.VMEM((TQ // 2, D), u32),
        pltpu.SemaphoreType.DMA((NB,)),
        pltpu.SemaphoreType.DMA((10,)),
        pltpu.SemaphoreType.DMA((NB,)),
    ]
    out = pl.pallas_call(
        _kernel,
        out_shape=jax.ShapeDtypeStruct((S, D), bf16),
        in_specs=[any_spec] * 7,
        out_specs=any_spec,
        scratch_shapes=scratch,
        compiler_params=pltpu.CompilerParams(vmem_limit_bytes=120 * 1024 * 1024),
    )(x, A_wqkv, A_wo, B_w_r, B_w_gate, B_w_up, B_w_down)
    return out.reshape(1, S, D)
```

```python
import jax
import jax.numpy as jnp
from jax import lax
import jax.experimental.pallas as pl
import jax.experimental.pallas.tpu as pltpu

bf16 = jnp.bfloat16
f32 = jnp.float32
u32 = jnp.uint32
i32 = jnp.int32

S = 2048
D = 1024
H = 32
DH = 32
W = 256
F = 3584
G = 8
PAD = 256
TQ = 256
NB = S // TQ
TKV = 512
NSB = S // 128
import os
CH = int(os.environ.get('K_CH', 32))
NCH = TQ // CH
CHC = int(os.environ.get('K_CHC', 8))
NCHC = TQ // CHC
GATE_A = [c * 8 // NCH - 1 for c in range(NCH)]
NWC = int(os.environ.get('K_NWC', 128))
_GCN, _GCO = [int(v) for v in os.environ.get('K_GC', '8,-1').split(',')]
GATE_C = [min(c * _GCN // NCHC + _GCO, 7) for c in range(NCHC)]
LNR = int(os.environ.get('K_LNR', 8))
GATE_EACH = int(os.environ.get('K_GE', 1))
FC = int(os.environ.get('K_FC', 256))
EPS = 1e-5
NEG = -1e30
QSCALE = (DH ** -0.5) * 1.4426950408889634
NT = (((1,), (1,)), ((), ()))


def _ln(x):
    m = jnp.mean(x, axis=-1, keepdims=True)
    xc = x - m
    v = jnp.mean(xc * xc, axis=-1, keepdims=True)
    return xc * lax.rsqrt(v + EPS)


def _pack_rows(x):
    return pltpu.bitcast(x.astype(bf16), u32)


def _pack_rows_interleaved(x):
    n = x.shape[0] // 16
    x3 = x.reshape(n, 16, x.shape[1])
    a = x3[:, 0:8, :].reshape(n * 8, x.shape[1])
    b = x3[:, 8:16, :].reshape(n * 8, x.shape[1])
    return pltpu.pack_elementwise([a, b], packed_dtype=bf16)


def _gate_first(x, gate, z):
    g = gate[0:8, 0:128] * z
    top = jnp.concatenate([x[0:8, 0:128] + g, x[0:8, 128:]], axis=1)
    return top if x.shape[0] == 8 else jnp.concatenate([top, x[8:]], axis=0)


def _kernel(x_hbm, wqkv_hbm, wo_hbm, wr_hbm, wg_hbm, wu_hbm, wd_hbm,
            out_hbm,
            xio, wq_v, wk_v, wv_v, wvt_v, wo_v, wop_v, wr_v, wg_v, wu_v, wd_v,
            xres, xbuf, best_v, best_i, rho_s, z_s, wr8,
            xca, xcb, xc_all, xi_all,
            q_s, k_s, vt_s, ot_s, s_s, m_s,
            ata, atb, oa, ob,
            sem_x, sem_w, sem_o):
    def x_copy(i):
        r0 = pl.multiple_of(i * TQ, TQ)
        return pltpu.make_async_copy(x_hbm.at[pl.ds(r0, TQ), :], xio.at[pl.ds(r0, TQ), :], sem_x.at[i])

    def out_copy(i):
        r0 = pl.multiple_of(i * TQ, TQ)
        return pltpu.make_async_copy(xio.at[pl.ds(r0, TQ), :], out_hbm.at[pl.ds(r0, TQ), :], sem_o.at[i])

    cp_wqa = pltpu.make_async_copy(wqkv_hbm.at[:, pl.ds(0, D // 2)], wq_v.at[:, pl.ds(0, D // 2)], sem_w.at[0])
    cp_wqb = pltpu.make_async_copy(wqkv_hbm.at[:, pl.ds(D // 2, D // 2)], wq_v.at[:, pl.ds(D // 2, D // 2)],
                                   sem_w.at[9])
    cp_wk = pltpu.make_async_copy(wqkv_hbm.at[:, pl.ds(D, D)], wk_v, sem_w.at[1])
    cp_wv = pltpu.make_async_copy(wqkv_hbm.at[:, pl.ds(2 * D, D)], wv_v, sem_w.at[8])
    cp_wo = pltpu.make_async_copy(wo_hbm, wo_v, sem_w.at[2])
    cp_wr = pltpu.make_async_copy(wr_hbm, wr_v, sem_w.at[3])
    cp_wg = pltpu.make_async_copy(wg_hbm, wg_v, sem_w.at[4])
    cp_wu = pltpu.make_async_copy(wu_hbm, wu_v, sem_w.at[5])
    cp_wd = pltpu.make_async_copy(wd_hbm, wd_v, sem_w.at[6])

    x_copy(0).start()
    cp_wqa.start()

    z_s[...] = jnp.zeros_like(z_s)
    xres[0:CH, :] = jnp.zeros((CH, D), f32)

    def ln_chunk(layer, i, c, xc_ref, gate):
        r0 = i * TQ + c * CH
        h0 = i * (TQ // 2) + c * (CH // 2)
        if not isinstance(r0, int):
            r0 = pl.multiple_of(r0, CH)
            h0 = pl.multiple_of(h0, CH // 2)
        parts = []
        for q in range(CH // LNR):
            rq = r0 + q * LNR
            x_in = xio[pl.ds(rq, LNR), :].astype(f32)
            x_rs = xres[pl.ds(pl.multiple_of(rq * layer, LNR), LNR), :]
            xq = jnp.where(layer == 0, x_in, x_rs)
            xbuf[pl.ds(rq, LNR), :] = xq
            if gate is not None:
                xq = _gate_first(xq, gate, z_s[...])
            parts.append(_ln(xq))
        xn = jnp.concatenate(parts, axis=0)
        xc = _pack_rows(xn)
        xc_ref[c * CH // 2:(c + 1) * CH // 2, :] = xc
        xc_all[pl.ds(h0, CH // 2), :] = xc
        xi_all[pl.ds(h0, CH // 2), :] = _pack_rows_interleaved(xn)

    def q_step(layer, i, xc_ref, i_next, xc_next, part=(0, G)):
        h0 = i * (TQ // 2)
        if not isinstance(h0, int):
            h0 = pl.multiple_of(h0, TQ // 2)
        a = pltpu.bitcast(xc_ref[...], bf16)
        ys = {}
        for n in range(*part):
            y = jnp.dot(a, wq_v[:, n * 128:(n + 1) * 128], preferred_element_type=f32)
            q_s[n, pl.ds(h0, TQ // 2), :] = _pack_rows(y * QSCALE)
            ys[n] = y
        if i_next is not None:
            for c in range(part[0] * NCH // G, part[1] * NCH // G):
                ln_chunk(layer, i_next, c, xc_next, ys.get(GATE_A[c]))

    def kv_step(i):
        h0 = pl.multiple_of(i * (TKV // 2), TKV // 2)
        a = pltpu.bitcast(xc_all[pl.ds(h0, TKV // 2), :], bf16)
        for n in range(G):
            y = jnp.dot(a, wk_v[:, n * 128:(n + 1) * 128], preferred_element_type=f32)
            k_s[n, pl.ds(PAD // 2 + h0, TKV // 2), :] = _pack_rows(y)
        vt = lax.dot_general(pltpu.bitcast(wvt_v[...], bf16), pltpu.bitcast(xi_all[pl.ds(h0, TKV // 2), :], bf16),
                             NT, preferred_element_type=f32)
        c0 = pl.multiple_of(PAD + i * TKV, 256)
        vt_s[:, pl.ds(c0, TKV)] = _pack_rows(vt)

    def phase_a(layer):
        @pl.when(layer == 0)
        def _():
            x_copy(0).wait()
            x_copy(1).start()
            cp_wqb.start()

        for c in range(NCH):
            ln_chunk(layer, 0, c, xca, None)

        @pl.when(layer == 0)
        def _():
            cp_wqa.wait()
            x_copy(1).wait()
            for i in range(2, NB):
                x_copy(i).start()

        q_step(layer, 0, xca, 1, xcb, part=(0, G // 2))

        @pl.when(layer == 0)
        def _():
            cp_wqb.wait()
            cp_wv.start()
            cp_wo.start()
            cp_wk.start()
            cp_wr.start()

        q_step(layer, 0, xca, 1, xcb, part=(G // 2, G))

        def q_body(j, c):
            i1 = 2 * j + 1

            @pl.when(layer == 0)
            def _():
                x_copy(i1 + 1).wait()
                x_copy(i1 + 2).wait()

            q_step(layer, i1, xcb, i1 + 1, xca)
            q_step(layer, i1 + 1, xca, i1 + 2, xcb)
            return c

        with jax.named_scope("a_q"):
            lax.fori_loop(0, NB // 2 - 1, q_body, 0)

        @pl.when(layer == 0)
        def _():
            cp_wv.wait()
            cp_wo.wait()

        q_step(layer, NB - 1, xcb, None, None)
        wvt_v[...] = pltpu.bitcast(wv_v[...].T, u32)
        for c in range(D // 64):
            wop_v[c * 32:(c + 1) * 32, :] = _pack_rows_interleaved(wo_v[c * 64:(c + 1) * 64, :].astype(f32))

        @pl.when(layer == 0)
        def _():
            cp_wk.wait()
            cp_wg.start()
            cp_wu.start()
            cp_wd.start()

        def kv_body(j, c):
            kv_step(j)
            return c

        with jax.named_scope("a_kv"):
            lax.fori_loop(0, S // TKV, kv_body, 0)

    def qk_stage(g, q0, slot, kstart):
        zi = pltpu.bitcast(z_s[...], i32)
        zi16 = jnp.concatenate([zi, zi], axis=0)
        lane16 = lax.broadcasted_iota(i32, (16, 128), 1) + zi16
        r16 = lax.broadcasted_iota(i32, (16, 128), 0)
        hb16 = lane16 // 32
        dd = r16 - lane16 % 32
        h0 = q0 // 2
        first_rows = None
        for b in range(4):
            first = max(0, kstart - 32 * b)
            base = h0 + 16 * b
            if not isinstance(base, int):
                base = pl.multiple_of(base, 16)
            mid0 = max(first, 32)
            if first == 0:
                parts = [k_s[g, pl.ds(base, 8), :], k_s[g, pl.ds(base + 128, 8), :],
                         k_s[g, pl.ds(base + 8, 8), :], k_s[g, pl.ds(base + 136, 8), :]]
            else:
                parts = [k_s[g, pl.ds(base + 128, 16), :]]
            if mid0 < 256:
                parts.append(k_s[g, pl.ds(base + mid0 // 2, (256 - mid0) // 2), :])
            kw = pltpu.bitcast(jnp.concatenate(parts, axis=0), bf16)
            qu = q_s[g, pl.ds(base, 16), :]
            qall = pltpu.bitcast(
                jnp.concatenate([jnp.where(hb16 == (p - b) % 4, qu, jnp.uint32(0)) for p in range(4)], axis=0),
                bf16)
            st = lax.dot_general(kw, qall, NT, preferred_element_type=f32)
            if b == 0:
                first_rows = st[0:8]
            if first == 0:
                c0 = jnp.where(dd > 0, st[0:16], st[16:32])
                c1 = jnp.where(dd > -16, st[32:48], st[48:64])
                mid = st[64:]
            else:
                c0 = jnp.where(dd > 0, NEG, st[0:16])
                c1 = jnp.where(dd > -16, NEG, st[16:32])
                mid = st[32:]
            s_s[slot, b, 0:16, :] = c0
            s_s[slot, b, 16:32, :] = c1
            x = jnp.concatenate([c0, c1], axis=0)
            if mid0 < 256:
                s_s[slot, b, mid0:256, :] = mid
                x = jnp.concatenate([x, mid], axis=0)
            mm = jnp.max(x.reshape(x.shape[0] // 8, 8, 128), axis=0)
            m_s[slot, b] = jnp.broadcast_to(jnp.max(mm, axis=0, keepdims=True), (8, 128))
        return first_rows

    def pv_stage(g, q0, slot, gate, kstart):
        r8 = lax.broadcasted_iota(i32, (8, 128), 0)
        c8 = lax.broadcasted_iota(i32, (8, 128), 1) + pltpu.bitcast(z_s[...], i32)
        blk = c8 // 32
        j = c8 % 32

        def tri(u):
            return (jnp.where(16 * u + r8 > j, jnp.uint32(0xFFFF), jnp.uint32(0)) |
                    jnp.where(16 * u + 8 + r8 > j, jnp.uint32(0xFFFF0000), jnp.uint32(0)))

        tris = [tri(0), tri(1)] if kstart < 128 else None
        ms = [m_s[slot, b] for b in range(4)]
        L = [None] * 4
        cache = {}

        def pexp(b, u):
            x = s_s[slot, b, 16 * u:16 * u + 16, :]
            p0 = jnp.exp2(x[0:8] - ms[b])
            p1 = jnp.exp2(x[8:16] - ms[b])
            sm = p0 + p1
            L[b] = sm if L[b] is None else L[b] + sm
            return pltpu.pack_elementwise([p0, p1], packed_dtype=bf16)

        def get_p(b, u):
            first = max(0, kstart - 32 * b)
            if u < 0 or u >= 18 or 16 * u < first:
                return None
            if first > 0:
                return pexp(b, u - 16) if u >= 16 else pexp(b, u)
            if u < 2:
                pk = pexp(b, u)
                lo = pk & tris[u]
                cache[(b, u + 16)] = pk ^ lo
                return lo
            if u >= 16:
                return cache.pop((b, u))
            return pexp(b, u)

        zero = jnp.zeros((8, 128), u32)
        accs = [None] * 4
        for k in range(kstart // 128, 3):
            wts = [[] for _ in range(4)]
            for t in range(8 * k, 8 * k + 8):
                if t == 8 and kstart == 0:
                    gv = gate * z_s[...]
                    for b in range(4):
                        ms[b] = ms[b] + gv
                srcs = [(b, get_p(b, t - 2 * b)) for b in range(4)]
                srcs = [(b, v) for (b, v) in srcs if v is not None]
                for h in range(4):
                    acc = zero if len(srcs) < 4 else None
                    for (b, v) in srcs:
                        acc = v if acc is None else jnp.where(blk == (h + b) % 4, v, acc)
                    wts[h].append(acc)
            c0 = q0 + 128 * k
            if not isinstance(c0, int):
                c0 = pl.multiple_of(c0, 128)
            for h in range(4):
                pt = pltpu.bitcast(jnp.concatenate(wts[h], axis=0), bf16)
                vth = pltpu.bitcast(vt_s[pl.ds((g * 4 + h) * 16, 16), pl.ds(c0, 128)], bf16)
                d = jnp.dot(vth, pt, preferred_element_type=f32)
                accs[h] = d if accs[h] is None else accs[h] + d
        L = [jnp.broadcast_to(jnp.sum(l, axis=0, keepdims=True), (8, 128)) for l in L]
        outs = []
        for h in range(4):
            lh = L[0]
            for b in range(1, 4):
                lh = jnp.where(blk == (h + b) % 4, L[b], lh)
            r0 = pl.reciprocal(lh, approx=True)
            rl = r0 * (2.0 - lh * r0)
            ot = (accs[h].reshape(4, 8, 128) * rl[None]).reshape(32, 128)
            if h > 0:
                ot = pltpu.roll(ot, 128 - 32 * h, axis=1)
            outs.append(ot)
        ot_s[g * 64:(g + 1) * 64, pl.ds(q0, 128)] = _pack_rows_interleaved(jnp.concatenate(outs, axis=0))

    def sub_block(q0, qn, kstart, kstart_next):
        for g in range(G):
            if g + 1 < G:
                gate = qk_stage(g + 1, q0, (g + 1) % 2, kstart)
            else:
                gate = qk_stage(0, qn, 0, kstart_next)
            pv_stage(g, q0, g % 2, gate, kstart)

    def phase_b():
        qk_stage(0, 0, 0, PAD)
        sub_block(0, 128, PAD, PAD - 128)
        sub_block(128, 256, PAD - 128, 0)

        def body(sb, c):
            q0 = pl.multiple_of(sb * 128, 128)
            qn = pl.multiple_of(jnp.minimum(sb + 1, NSB - 1) * 128, 128)
            sub_block(q0, qn, 0, 0)
            return c

        lax.fori_loop(2, NSB, body, 0, unroll=int(os.environ.get('K_UB', 2)))

    def resid_chunk(i, c, at_ref, gate):
        r0 = i * TQ + c * CHC
        if not isinstance(r0, int):
            r0 = pl.multiple_of(r0, CHC)
        x1 = xbuf[pl.ds(r0, CHC), :] + at_ref[c * CHC:(c + 1) * CHC, :]
        if gate is not None:
            x1 = _gate_first(x1, gate, z_s[...])
        m = jnp.mean(x1, axis=-1, keepdims=True)
        xc = x1 - m
        v = jnp.mean(xc * xc, axis=-1, keepdims=True)
        rho = lax.rsqrt(v + EPS)
        xn = xc * rho
        r = jnp.sum(xn * wr8[0:1, :], axis=-1, keepdims=True)
        rb = jnp.broadcast_to(r, (CHC, 128)).astype(bf16).astype(f32)
        rows = lax.broadcasted_iota(i32, (8, 128), 0) + r0
        bv, bi = best_v[...], best_i[...]
        for q in range(CHC // 8):
            cand = rb[8 * q:8 * q + 8]
            better = cand > bv
            bv = jnp.where(better, cand, bv)
            bi = jnp.where(better, rows + 8 * q, bi)
        best_v[...] = bv
        best_i[...] = bi
        rho_s[pl.ds(r0, CHC), :] = jnp.broadcast_to(rho, (CHC, 128))
        x2 = x1 + xn
        xres[pl.ds(r0, CHC), :] = x2
        xio[pl.ds(r0, CHC), :] = x2.astype(bf16)

    def transpose_o(i, o_dst):
        r0 = i * TQ
        if not isinstance(r0, int):
            r0 = pl.multiple_of(r0, TQ)
        o_dst[...] = pltpu.bitcast(pltpu.bitcast(ot_s[:, pl.ds(r0, TQ)], bf16).T, u32)

    def oproj_step(o_src, at_w, i_res, at_r, i_t, o_dst):
        ys = []
        if o_src is not None:
            a = pltpu.bitcast(o_src[...], bf16)
            for n in range(D // NWC):
                y = jnp.dot(a, pltpu.bitcast(wop_v[:, n * NWC:(n + 1) * NWC], bf16), preferred_element_type=f32)
                at_w[:, n * NWC:(n + 1) * NWC] = y
                ys.append(y)
        if i_t is not None:
            transpose_o(i_t, o_dst)
        if i_res is not None:
            for c in range(NCHC):
                gi = GATE_C[c] if ys else -1
                gate = ys[gi] if gi >= 0 else None
                resid_chunk(i_res, c, at_r, gate)

    def phase_c(layer):
        @pl.when(layer == 0)
        def _():
            cp_wr.wait()
            wr8[...] = jnp.broadcast_to(wr_v[...].astype(f32).reshape(1, D), (8, D))

        def flush(i):
            @pl.when(layer == 1)
            def _():
                out_copy(i).start()

        best_v[...] = jnp.full((8, 128), -jnp.inf, f32)
        best_i[...] = jnp.zeros((8, 128), i32)
        transpose_o(0, oa)
        oproj_step(oa, ata, None, None, 1, ob)

        def body(j, c):
            i0 = 2 * j
            oproj_step(ob, atb, i0, ata, i0 + 2, oa)
            oproj_step(oa, ata, i0 + 1, atb, i0 + 3, ob)
            flush(i0)
            flush(i0 + 1)
            return c

        lax.fori_loop(0, NB // 2 - 1, body, 0)
        oproj_step(ob, atb, NB - 2, ata, None, None)
        oproj_step(None, None, NB - 1, atb, None, None)
        flush(NB - 2)
        flush(NB - 1)

    def phase_d(layer):
        @pl.when(layer == 0)
        def _():
            cp_wg.wait()
            cp_wu.wait()
            cp_wd.wait()

        bv = best_v[...]
        rmax = jnp.max(bv)
        idx = jnp.min(jnp.where(bv == rmax, best_i[...], S))
        idx = jnp.clip(idx, 0, S - 1)
        x2 = xres[pl.ds(idx, 1), :]
        rho = rho_s[pl.ds(idx, 1), 0:1]
        xn = (x2 - jnp.mean(x2, axis=-1, keepdims=True)) * (rho / (1.0 + rho))
        xs = jnp.broadcast_to(xn, (16, D)).astype(bf16)
        nf = F // FC
        hs = []
        y = None
        for c in range(nf + 1):
            if c < nf:
                gate = jnp.dot(xs, wg_v[:, c * FC:(c + 1) * FC], preferred_element_type=f32)
                up = jnp.dot(xs, wu_v[:, c * FC:(c + 1) * FC], preferred_element_type=f32)
                hs.append((gate * jax.nn.sigmoid(gate) * up).astype(bf16))
            if c > 0:
                d = jnp.dot(hs[c - 1], wd_v[(c - 1) * FC:c * FC, :], preferred_element_type=f32)
                y = d if y is None else y + d
        scale = jax.nn.sigmoid(jnp.full((1, D), rmax, f32))
        xres[pl.ds(idx, 1), :] = xres[pl.ds(idx, 1), :] + y[0:1] * scale

        @pl.when(layer == 1)
        def _():
            for i in range(NB):
                out_copy(i).wait()
            g0 = pl.multiple_of((idx // 16) * 16, 16)
            xio[pl.ds(g0, 16), :] = xres[pl.ds(g0, 16), :].astype(bf16)
            fix = pltpu.make_async_copy(xio.at[pl.ds(g0, 16), :], out_hbm.at[pl.ds(g0, 16), :], sem_w.at[7])
            fix.start()
            fix.wait()

    def layer_body(layer, c):
        with jax.named_scope("phase_a"):
            phase_a(layer)
        with jax.named_scope("phase_b"):
            phase_b()
        with jax.named_scope("phase_c"):
            phase_c(layer)
        with jax.named_scope("phase_d"):
            phase_d(layer)
        return c

    lax.fori_loop(0, 2, layer_body, 0)


@jax.jit
def pallas_interleave_layers__sliding_block__moe_arch_mod__prompt_kernel(
    A_x: jax.Array,
    A_wqkv: jax.Array,
    A_wo: jax.Array,
    B_x: jax.Array,
    B_w_r: jax.Array,
    B_w_gate: jax.Array,
    B_w_up: jax.Array,
    B_w_down: jax.Array,
):
    del B_x
    x = A_x.reshape(S, D)
    any_spec = pl.BlockSpec(memory_space=pl.ANY)
    scratch = [
        pltpu.VMEM((S, D), bf16),
        pltpu.VMEM((D, D), bf16),
        pltpu.VMEM((D, D), bf16),
        pltpu.VMEM((D, D), bf16),
        pltpu.VMEM((D // 2, D), u32),
        pltpu.VMEM((D, D), bf16),
        pltpu.VMEM((D // 2, D), u32),
        pltpu.VMEM((D,), bf16),
        pltpu.VMEM((D, F), bf16),
        pltpu.VMEM((D, F), bf16),
        pltpu.VMEM((F, D), bf16),
        pltpu.VMEM((S, D), f32),
        pltpu.VMEM((S, D), f32),
        pltpu.VMEM((8, 128), f32),
        pltpu.VMEM((8, 128), i32),
        pltpu.VMEM((S, 128), f32),
        pltpu.VMEM((8, 128), f32),
        pltpu.VMEM((8, D), f32),
        pltpu.VMEM((TQ // 2, D), u32),
        pltpu.VMEM((TQ // 2, D), u32),
        pltpu.VMEM((S // 2, D), u32),
        pltpu.VMEM((S // 2, D), u32),
        pltpu.VMEM((G, S // 2, 128), u32),
        pltpu.VMEM((G, (S + PAD) // 2, 128), u32),
        pltpu.VMEM((D // 2, S + PAD), u32),
        pltpu.VMEM((D // 2, S), u32),
        pltpu.VMEM((2, 4, 256, 128), f32),
        pltpu.VMEM((2, 4, 8, 128), f32),
        pltpu.VMEM((TQ, D), f32),
        pltpu.VMEM((TQ, D), f32),
        pltpu.VMEM((TQ // 2, D), u32),
        pltpu.VMEM((TQ // 2, D), u32),
        pltpu.SemaphoreType.DMA((NB,)),
        pltpu.SemaphoreType.DMA((10,)),
        pltpu.SemaphoreType.DMA((NB,)),
    ]
    out = pl.pallas_call(
        _kernel,
        out_shape=jax.ShapeDtypeStruct((S, D), bf16),
        in_specs=[any_spec] * 7,
        out_specs=any_spec,
        scratch_shapes=scratch,
        compiler_params=pltpu.CompilerParams(vmem_limit_bytes=120 * 1024 * 1024),
    )(x, A_wqkv, A_wo, B_w_r, B_w_gate, B_w_up, B_w_down)
    return out.reshape(1, S, D)
```

```python
import jax
import jax.numpy as jnp
from jax import lax
import jax.experimental.pallas as pl
import jax.experimental.pallas.tpu as pltpu

bf16 = jnp.bfloat16
f32 = jnp.float32
u32 = jnp.uint32
i32 = jnp.int32

S = 2048
D = 1024
H = 32
DH = 32
W = 256
F = 3584
G = 8
PAD = 256
TQ = 256
NB = S // TQ
TKV = 512
NSB = S // 128
import os
CH = int(os.environ.get('K_CH', 32))
NCH = TQ // CH
CHC = int(os.environ.get('K_CHC', 8))
NCHC = TQ // CHC
GATE_A = [c * 8 // NCH - 1 for c in range(NCH)]
NWC = int(os.environ.get('K_NWC', 128))
_GCN, _GCO = [int(v) for v in os.environ.get('K_GC', '8,-1').split(',')]
GATE_C = [min(c * _GCN // NCHC + _GCO, 7) for c in range(NCHC)]
LNR = int(os.environ.get('K_LNR', 8))
GATE_EACH = int(os.environ.get('K_GE', 1))
FC = int(os.environ.get('K_FC', 256))
CHAIN_A = int(os.environ.get('K_CHA', 3))
CHAIN_C = int(os.environ.get('K_CHAINC', 0))
B_GATE = dict(tuple(int(v) for v in kv.split(':')) for kv in os.environ.get('K_BG', '8:0').split(','))
B_CHAIN = [int(v) for v in os.environ.get('K_BC', '').split(',') if v]
EPS = 1e-5
NEG = -1e30
QSCALE = (DH ** -0.5) * 1.4426950408889634
NT = (((1,), (1,)), ((), ()))


def _ln(x):
    m = jnp.mean(x, axis=-1, keepdims=True)
    xc = x - m
    v = jnp.mean(xc * xc, axis=-1, keepdims=True)
    return xc * lax.rsqrt(v + EPS)


def _pack_rows(x):
    return pltpu.bitcast(x.astype(bf16), u32)


def _pack_rows_interleaved(x):
    n = x.shape[0] // 16
    x3 = x.reshape(n, 16, x.shape[1])
    a = x3[:, 0:8, :].reshape(n * 8, x.shape[1])
    b = x3[:, 8:16, :].reshape(n * 8, x.shape[1])
    return pltpu.pack_elementwise([a, b], packed_dtype=bf16)


def _gate_first(x, gate, z):
    g = gate[0:8, 0:128] * z
    top = jnp.concatenate([x[0:8, 0:128] + g, x[0:8, 128:]], axis=1)
    return top if x.shape[0] == 8 else jnp.concatenate([top, x[8:]], axis=0)


def _kernel(x_hbm, wqkv_hbm, wo_hbm, wr_hbm, wg_hbm, wu_hbm, wd_hbm,
            out_hbm,
            xio, wq_v, wk_v, wv_v, wvt_v, wo_v, wop_v, wr_v, wg_v, wu_v, wd_v,
            xres, xbuf, best_v, best_i, rho_s, z_s, wr8,
            xca, xcb, xc_all, xi_all,
            q_s, k_s, vt_s, ot_s, s_s, m_s,
            ata, atb, oa, ob,
            sem_x, sem_w, sem_o):
    def x_copy(i):
        r0 = pl.multiple_of(i * TQ, TQ)
        return pltpu.make_async_copy(x_hbm.at[pl.ds(r0, TQ), :], xio.at[pl.ds(r0, TQ), :], sem_x.at[i])

    def out_copy(i):
        r0 = pl.multiple_of(i * TQ, TQ)
        return pltpu.make_async_copy(xio.at[pl.ds(r0, TQ), :], out_hbm.at[pl.ds(r0, TQ), :], sem_o.at[i])

    cp_wqa = pltpu.make_async_copy(wqkv_hbm.at[:, pl.ds(0, D // 2)], wq_v.at[:, pl.ds(0, D // 2)], sem_w.at[0])
    cp_wqb = pltpu.make_async_copy(wqkv_hbm.at[:, pl.ds(D // 2, D // 2)], wq_v.at[:, pl.ds(D // 2, D // 2)],
                                   sem_w.at[9])
    cp_wk = pltpu.make_async_copy(wqkv_hbm.at[:, pl.ds(D, D)], wk_v, sem_w.at[1])
    cp_wv = pltpu.make_async_copy(wqkv_hbm.at[:, pl.ds(2 * D, D)], wv_v, sem_w.at[8])
    cp_wo = pltpu.make_async_copy(wo_hbm, wo_v, sem_w.at[2])
    cp_wr = pltpu.make_async_copy(wr_hbm, wr_v, sem_w.at[3])
    cp_wg = pltpu.make_async_copy(wg_hbm, wg_v, sem_w.at[4])
    cp_wu = pltpu.make_async_copy(wu_hbm, wu_v, sem_w.at[5])
    cp_wd = pltpu.make_async_copy(wd_hbm, wd_v, sem_w.at[6])

    x_copy(0).start()
    cp_wqa.start()

    z_s[...] = jnp.zeros_like(z_s)
    xres[0:CH, :] = jnp.zeros((CH, D), f32)

    def ln_chunk(layer, i, c, xc_ref, gate, chain=None):
        r0 = i * TQ + c * CH
        h0 = i * (TQ // 2) + c * (CH // 2)
        if not isinstance(r0, int):
            r0 = pl.multiple_of(r0, CH)
            h0 = pl.multiple_of(h0, CH // 2)
        parts = []
        for q in range(CH // LNR):
            rq = r0 + q * LNR
            x_in = xio[pl.ds(rq, LNR), :].astype(f32)
            x_rs = xres[pl.ds(pl.multiple_of(rq * layer, LNR), LNR), :]
            xq = jnp.where(layer == 0, x_in, x_rs)
            xbuf[pl.ds(rq, LNR), :] = xq
            if chain is not None and len(chain) >= CHAIN_A:
                xq = _gate_first(xq, chain[-CHAIN_A], z_s[...])
            elif gate is not None:
                xq = _gate_first(xq, gate, z_s[...])
            parts.append(_ln(xq))
            if chain is not None:
                chain.append(parts[-1])
        xn = jnp.concatenate(parts, axis=0)
        xc = _pack_rows(xn)
        xc_ref[c * CH // 2:(c + 1) * CH // 2, :] = xc
        xc_all[pl.ds(h0, CH // 2), :] = xc
        xi_all[pl.ds(h0, CH // 2), :] = _pack_rows_interleaved(xn)

    def q_step(layer, i, xc_ref, i_next, xc_next, part=(0, G)):
        h0 = i * (TQ // 2)
        if not isinstance(h0, int):
            h0 = pl.multiple_of(h0, TQ // 2)
        a = pltpu.bitcast(xc_ref[...], bf16)
        ys = {}
        for n in range(*part):
            y = jnp.dot(a, wq_v[:, n * 128:(n + 1) * 128], preferred_element_type=f32)
            q_s[n, pl.ds(h0, TQ // 2), :] = _pack_rows(y * QSCALE)
            ys[n] = y
        if i_next is not None:
            chain = [] if CHAIN_A > 0 else None
            for c in range(part[0] * NCH // G, part[1] * NCH // G):
                ln_chunk(layer, i_next, c, xc_next, ys.get(GATE_A[c]), chain)

    def kv_step(i):
        h0 = pl.multiple_of(i * (TKV // 2), TKV // 2)
        a = pltpu.bitcast(xc_all[pl.ds(h0, TKV // 2), :], bf16)
        for n in range(G):
            y = jnp.dot(a, wk_v[:, n * 128:(n + 1) * 128], preferred_element_type=f32)
            k_s[n, pl.ds(PAD // 2 + h0, TKV // 2), :] = _pack_rows(y)
        vt = lax.dot_general(pltpu.bitcast(wvt_v[...], bf16), pltpu.bitcast(xi_all[pl.ds(h0, TKV // 2), :], bf16),
                             NT, preferred_element_type=f32)
        c0 = pl.multiple_of(PAD + i * TKV, 256)
        vt_s[:, pl.ds(c0, TKV)] = _pack_rows(vt)

    def phase_a(layer):
        @pl.when(layer == 0)
        def _():
            x_copy(0).wait()
            x_copy(1).start()
            cp_wqb.start()

        for c in range(NCH):
            ln_chunk(layer, 0, c, xca, None)

        @pl.when(layer == 0)
        def _():
            cp_wqa.wait()
            x_copy(1).wait()
            for i in range(2, NB):
                x_copy(i).start()

        q_step(layer, 0, xca, 1, xcb, part=(0, G // 2))

        @pl.when(layer == 0)
        def _():
            cp_wqb.wait()
            cp_wv.start()
            cp_wo.start()
            cp_wk.start()
            cp_wr.start()

        q_step(layer, 0, xca, 1, xcb, part=(G // 2, G))

        def q_body(j, c):
            i1 = 2 * j + 1

            @pl.when(layer == 0)
            def _():
                x_copy(i1 + 1).wait()
                x_copy(i1 + 2).wait()

            q_step(layer, i1, xcb, i1 + 1, xca)
            q_step(layer, i1 + 1, xca, i1 + 2, xcb)
            return c

        with jax.named_scope("a_q"):
            lax.fori_loop(0, NB // 2 - 1, q_body, 0)

        @pl.when(layer == 0)
        def _():
            cp_wv.wait()
            cp_wo.wait()

        q_step(layer, NB - 1, xcb, None, None)
        wvt_v[...] = pltpu.bitcast(wv_v[...].T, u32)
        for c in range(D // 64):
            wop_v[c * 32:(c + 1) * 32, :] = _pack_rows_interleaved(wo_v[c * 64:(c + 1) * 64, :].astype(f32))

        @pl.when(layer == 0)
        def _():
            cp_wk.wait()
            cp_wg.start()
            cp_wu.start()
            cp_wd.start()

        def kv_body(j, c):
            kv_step(j)
            return c

        with jax.named_scope("a_kv"):
            lax.fori_loop(0, S // TKV, kv_body, 0)

    def qk_stage(g, q0, slot, kstart):
        zi = pltpu.bitcast(z_s[...], i32)
        zi16 = jnp.concatenate([zi, zi], axis=0)
        lane16 = lax.broadcasted_iota(i32, (16, 128), 1) + zi16
        r16 = lax.broadcasted_iota(i32, (16, 128), 0)
        hb16 = lane16 // 32
        dd = r16 - lane16 % 32
        h0 = q0 // 2
        first_rows = None
        for b in range(4):
            first = max(0, kstart - 32 * b)
            base = h0 + 16 * b
            if not isinstance(base, int):
                base = pl.multiple_of(base, 16)
            mid0 = max(first, 32)
            if first == 0:
                parts = [k_s[g, pl.ds(base, 8), :], k_s[g, pl.ds(base + 128, 8), :],
                         k_s[g, pl.ds(base + 8, 8), :], k_s[g, pl.ds(base + 136, 8), :]]
            else:
                parts = [k_s[g, pl.ds(base + 128, 16), :]]
            if mid0 < 256:
                parts.append(k_s[g, pl.ds(base + mid0 // 2, (256 - mid0) // 2), :])
            kw = pltpu.bitcast(jnp.concatenate(parts, axis=0), bf16)
            qu = q_s[g, pl.ds(base, 16), :]
            qall = pltpu.bitcast(
                jnp.concatenate([jnp.where(hb16 == (p - b) % 4, qu, jnp.uint32(0)) for p in range(4)], axis=0),
                bf16)
            st = lax.dot_general(kw, qall, NT, preferred_element_type=f32)
            if b == 0:
                first_rows = [st[16 * r:16 * r + 8] for r in range(st.shape[0] // 16)]
            if first == 0:
                c0 = jnp.where(dd > 0, st[0:16], st[16:32])
                c1 = jnp.where(dd > -16, st[32:48], st[48:64])
                mid = st[64:]
            else:
                c0 = jnp.where(dd > 0, NEG, st[0:16])
                c1 = jnp.where(dd > -16, NEG, st[16:32])
                mid = st[32:]
            s_s[slot, b, 0:16, :] = c0
            s_s[slot, b, 16:32, :] = c1
            x = jnp.concatenate([c0, c1], axis=0)
            if mid0 < 256:
                s_s[slot, b, mid0:256, :] = mid
                x = jnp.concatenate([x, mid], axis=0)
            mm = jnp.max(x.reshape(x.shape[0] // 8, 8, 128), axis=0)
            m_s[slot, b] = jnp.broadcast_to(jnp.max(mm, axis=0, keepdims=True), (8, 128))
        return first_rows

    def pv_stage(g, q0, slot, gate, kstart):
        r8 = lax.broadcasted_iota(i32, (8, 128), 0)
        c8 = lax.broadcasted_iota(i32, (8, 128), 1) + pltpu.bitcast(z_s[...], i32)
        blk = c8 // 32
        j = c8 % 32

        def tri(u):
            return (jnp.where(16 * u + r8 > j, jnp.uint32(0xFFFF), jnp.uint32(0)) |
                    jnp.where(16 * u + 8 + r8 > j, jnp.uint32(0xFFFF0000), jnp.uint32(0)))

        tris = [tri(0), tri(1)] if kstart < 128 else None
        ms = [m_s[slot, b] for b in range(4)]
        L = [None] * 4
        cache = {}

        def pexp(b, u):
            x = s_s[slot, b, 16 * u:16 * u + 16, :]
            p0 = jnp.exp2(x[0:8] - ms[b])
            p1 = jnp.exp2(x[8:16] - ms[b])
            sm = p0 + p1
            L[b] = sm if L[b] is None else L[b] + sm
            return pltpu.pack_elementwise([p0, p1], packed_dtype=bf16)

        def get_p(b, u):
            first = max(0, kstart - 32 * b)
            if u < 0 or u >= 18 or 16 * u < first:
                return None
            if first > 0:
                return pexp(b, u - 16) if u >= 16 else pexp(b, u)
            if u < 2:
                pk = pexp(b, u)
                lo = pk & tris[u]
                cache[(b, u + 16)] = pk ^ lo
                return lo
            if u >= 16:
                return cache.pop((b, u))
            return pexp(b, u)

        zero = jnp.zeros((8, 128), u32)
        accs = [None] * 4
        for k in range(kstart // 128, 3):
            wts = [[] for _ in range(4)]
            for t in range(8 * k, 8 * k + 8):
                if t in B_GATE and kstart == 0:
                    gv = gate[B_GATE[t]] * z_s[...]
                    for b in range(4):
                        ms[b] = ms[b] + gv
                if t in B_CHAIN and kstart == 0:
                    for b in range(4):
                        ms[b] = ms[b] + L[b] * z_s[...]
                srcs = [(b, get_p(b, t - 2 * b)) for b in range(4)]
                srcs = [(b, v) for (b, v) in srcs if v is not None]
                for h in range(4):
                    acc = zero if len(srcs) < 4 else None
                    for (b, v) in srcs:
                        acc = v if acc is None else jnp.where(blk == (h + b) % 4, v, acc)
                    wts[h].append(acc)
            c0 = q0 + 128 * k
            if not isinstance(c0, int):
                c0 = pl.multiple_of(c0, 128)
            for h in range(4):
                pt = pltpu.bitcast(jnp.concatenate(wts[h], axis=0), bf16)
                vth = pltpu.bitcast(vt_s[pl.ds((g * 4 + h) * 16, 16), pl.ds(c0, 128)], bf16)
                d = jnp.dot(vth, pt, preferred_element_type=f32)
                accs[h] = d if accs[h] is None else accs[h] + d
        L = [jnp.broadcast_to(jnp.sum(l, axis=0, keepdims=True), (8, 128)) for l in L]
        outs = []
        for h in range(4):
            lh = L[0]
            for b in range(1, 4):
                lh = jnp.where(blk == (h + b) % 4, L[b], lh)
            r0 = pl.reciprocal(lh, approx=True)
            rl = r0 * (2.0 - lh * r0)
            ot = (accs[h].reshape(4, 8, 128) * rl[None]).reshape(32, 128)
            if h > 0:
                ot = pltpu.roll(ot, 128 - 32 * h, axis=1)
            outs.append(ot)
        ot_s[g * 64:(g + 1) * 64, pl.ds(q0, 128)] = _pack_rows_interleaved(jnp.concatenate(outs, axis=0))

    def sub_block(q0, qn, kstart, kstart_next):
        for g in range(G):
            if g + 1 < G:
                gate = qk_stage(g + 1, q0, (g + 1) % 2, kstart)
            else:
                gate = qk_stage(0, qn, 0, kstart_next)
            pv_stage(g, q0, g % 2, gate, kstart)

    def phase_b():
        qk_stage(0, 0, 0, PAD)
        sub_block(0, 128, PAD, PAD - 128)
        sub_block(128, 256, PAD - 128, 0)

        def body(sb, c):
            q0 = pl.multiple_of(sb * 128, 128)
            qn = pl.multiple_of(jnp.minimum(sb + 1, NSB - 1) * 128, 128)
            sub_block(q0, qn, 0, 0)
            return c

        lax.fori_loop(2, NSB, body, 0, unroll=int(os.environ.get('K_UB', 2)))

    def resid_chunk(i, c, at_ref, gate, chain=None):
        r0 = i * TQ + c * CHC
        if not isinstance(r0, int):
            r0 = pl.multiple_of(r0, CHC)
        x1 = xbuf[pl.ds(r0, CHC), :] + at_ref[c * CHC:(c + 1) * CHC, :]
        if chain is not None and len(chain) >= CHAIN_C:
            x1 = _gate_first(x1, chain[-CHAIN_C], z_s[...])
        elif gate is not None:
            x1 = _gate_first(x1, gate, z_s[...])
        m = jnp.mean(x1, axis=-1, keepdims=True)
        xc = x1 - m
        v = jnp.mean(xc * xc, axis=-1, keepdims=True)
        rho = lax.rsqrt(v + EPS)
        xn = xc * rho
        r = jnp.sum(xn * wr8[0:1, :], axis=-1, keepdims=True)
        rb = jnp.broadcast_to(r, (CHC, 128)).astype(bf16).astype(f32)
        rows = lax.broadcasted_iota(i32, (8, 128), 0) + r0
        bv, bi = best_v[...], best_i[...]
        for q in range(CHC // 8):
            cand = rb[8 * q:8 * q + 8]
            better = cand > bv
            bv = jnp.where(better, cand, bv)
            bi = jnp.where(better, rows + 8 * q, bi)
        best_v[...] = bv
        best_i[...] = bi
        rho_s[pl.ds(r0, CHC), :] = jnp.broadcast_to(rho, (CHC, 128))
        x2 = x1 + xn
        if chain is not None:
            chain.append(x2)
        xres[pl.ds(r0, CHC), :] = x2
        xio[pl.ds(r0, CHC), :] = x2.astype(bf16)

    def transpose_o(i, o_dst):
        r0 = i * TQ
        if not isinstance(r0, int):
            r0 = pl.multiple_of(r0, TQ)
        o_dst[...] = pltpu.bitcast(pltpu.bitcast(ot_s[:, pl.ds(r0, TQ)], bf16).T, u32)

    def oproj_step(o_src, at_w, i_res, at_r, i_t, o_dst):
        ys = []
        if o_src is not None:
            a = pltpu.bitcast(o_src[...], bf16)
            for n in range(D // NWC):
                y = jnp.dot(a, pltpu.bitcast(wop_v[:, n * NWC:(n + 1) * NWC], bf16), preferred_element_type=f32)
                at_w[:, n * NWC:(n + 1) * NWC] = y
                ys.append(y)
        if i_t is not None:
            transpose_o(i_t, o_dst)
        if i_res is not None:
            chain = [] if (CHAIN_C > 0 and ys) else None
            for c in range(NCHC):
                gi = GATE_C[c] if ys else -1
                gate = ys[gi] if gi >= 0 else None
                resid_chunk(i_res, c, at_r, gate, chain)

    def phase_c(layer):
        @pl.when(layer == 0)
        def _():
            cp_wr.wait()
            wr8[...] = jnp.broadcast_to(wr_v[...].astype(f32).reshape(1, D), (8, D))

        def flush(i):
            @pl.when(layer == 1)
            def _():
                out_copy(i).start()

        best_v[...] = jnp.full((8, 128), -jnp.inf, f32)
        best_i[...] = jnp.zeros((8, 128), i32)
        transpose_o(0, oa)
        oproj_step(oa, ata, None, None, 1, ob)

        def body(j, c):
            i0 = 2 * j
            oproj_step(ob, atb, i0, ata, i0 + 2, oa)
            oproj_step(oa, ata, i0 + 1, atb, i0 + 3, ob)
            flush(i0)
            flush(i0 + 1)
            return c

        lax.fori_loop(0, NB // 2 - 1, body, 0)
        oproj_step(ob, atb, NB - 2, ata, None, None)
        oproj_step(None, None, NB - 1, atb, None, None)
        flush(NB - 2)
        flush(NB - 1)

    def phase_d(layer):
        @pl.when(layer == 0)
        def _():
            cp_wg.wait()
            cp_wu.wait()
            cp_wd.wait()

        bv = best_v[...]
        rmax = jnp.max(bv)
        idx = jnp.min(jnp.where(bv == rmax, best_i[...], S))
        idx = jnp.clip(idx, 0, S - 1)
        x2 = xres[pl.ds(idx, 1), :]
        rho = rho_s[pl.ds(idx, 1), 0:1]
        xn = (x2 - jnp.mean(x2, axis=-1, keepdims=True)) * (rho / (1.0 + rho))
        xs = jnp.broadcast_to(xn, (16, D)).astype(bf16)
        nf = F // FC
        hs = []
        y = None
        for c in range(nf + 1):
            if c < nf:
                gate = jnp.dot(xs, wg_v[:, c * FC:(c + 1) * FC], preferred_element_type=f32)
                up = jnp.dot(xs, wu_v[:, c * FC:(c + 1) * FC], preferred_element_type=f32)
                hs.append((gate * jax.nn.sigmoid(gate) * up).astype(bf16))
            if c > 0:
                d = jnp.dot(hs[c - 1], wd_v[(c - 1) * FC:c * FC, :], preferred_element_type=f32)
                y = d if y is None else y + d
        scale = jax.nn.sigmoid(jnp.full((1, D), rmax, f32))
        xres[pl.ds(idx, 1), :] = xres[pl.ds(idx, 1), :] + y[0:1] * scale

        @pl.when(layer == 1)
        def _():
            for i in range(NB):
                out_copy(i).wait()
            g0 = pl.multiple_of((idx // 16) * 16, 16)
            xio[pl.ds(g0, 16), :] = xres[pl.ds(g0, 16), :].astype(bf16)
            fix = pltpu.make_async_copy(xio.at[pl.ds(g0, 16), :], out_hbm.at[pl.ds(g0, 16), :], sem_w.at[7])
            fix.start()
            fix.wait()

    def layer_body(layer, c):
        with jax.named_scope("phase_a"):
            phase_a(layer)
        with jax.named_scope("phase_b"):
            phase_b()
        with jax.named_scope("phase_c"):
            phase_c(layer)
        with jax.named_scope("phase_d"):
            phase_d(layer)
        return c

    lax.fori_loop(0, 2, layer_body, 0)


@jax.jit
def pallas_interleave_layers__sliding_block__moe_arch_mod__prompt_kernel(
    A_x: jax.Array,
    A_wqkv: jax.Array,
    A_wo: jax.Array,
    B_x: jax.Array,
    B_w_r: jax.Array,
    B_w_gate: jax.Array,
    B_w_up: jax.Array,
    B_w_down: jax.Array,
):
    del B_x
    x = A_x.reshape(S, D)
    any_spec = pl.BlockSpec(memory_space=pl.ANY)
    scratch = [
        pltpu.VMEM((S, D), bf16),
        pltpu.VMEM((D, D), bf16),
        pltpu.VMEM((D, D), bf16),
        pltpu.VMEM((D, D), bf16),
        pltpu.VMEM((D // 2, D), u32),
        pltpu.VMEM((D, D), bf16),
        pltpu.VMEM((D // 2, D), u32),
        pltpu.VMEM((D,), bf16),
        pltpu.VMEM((D, F), bf16),
        pltpu.VMEM((D, F), bf16),
        pltpu.VMEM((F, D), bf16),
        pltpu.VMEM((S, D), f32),
        pltpu.VMEM((S, D), f32),
        pltpu.VMEM((8, 128), f32),
        pltpu.VMEM((8, 128), i32),
        pltpu.VMEM((S, 128), f32),
        pltpu.VMEM((8, 128), f32),
        pltpu.VMEM((8, D), f32),
        pltpu.VMEM((TQ // 2, D), u32),
        pltpu.VMEM((TQ // 2, D), u32),
        pltpu.VMEM((S // 2, D), u32),
        pltpu.VMEM((S // 2, D), u32),
        pltpu.VMEM((G, S // 2, 128), u32),
        pltpu.VMEM((G, (S + PAD) // 2, 128), u32),
        pltpu.VMEM((D // 2, S + PAD), u32),
        pltpu.VMEM((D // 2, S), u32),
        pltpu.VMEM((2, 4, 256, 128), f32),
        pltpu.VMEM((2, 4, 8, 128), f32),
        pltpu.VMEM((TQ, D), f32),
        pltpu.VMEM((TQ, D), f32),
        pltpu.VMEM((TQ // 2, D), u32),
        pltpu.VMEM((TQ // 2, D), u32),
        pltpu.SemaphoreType.DMA((NB,)),
        pltpu.SemaphoreType.DMA((10,)),
        pltpu.SemaphoreType.DMA((NB,)),
    ]
    out = pl.pallas_call(
        _kernel,
        out_shape=jax.ShapeDtypeStruct((S, D), bf16),
        in_specs=[any_spec] * 7,
        out_specs=any_spec,
        scratch_shapes=scratch,
        compiler_params=pltpu.CompilerParams(vmem_limit_bytes=120 * 1024 * 1024),
    )(x, A_wqkv, A_wo, B_w_r, B_w_gate, B_w_up, B_w_down)
    return out.reshape(1, S, D)
```

```python
import jax
import jax.numpy as jnp
from jax import lax
import jax.experimental.pallas as pl
import jax.experimental.pallas.tpu as pltpu

bf16 = jnp.bfloat16
f32 = jnp.float32
u32 = jnp.uint32
i32 = jnp.int32

S = 2048
D = 1024
H = 32
DH = 32
W = 256
F = 3584
G = 8
PAD = 256
TQ = 256
NB = S // TQ
TKV = 512
NSB = S // 128
import os
CH = int(os.environ.get('K_CH', 32))
NCH = TQ // CH
CHC = int(os.environ.get('K_CHC', 8))
NCHC = TQ // CHC
GATE_A = [c * 8 // NCH - 1 for c in range(NCH)]
NWC = int(os.environ.get('K_NWC', 128))
_GCN, _GCO = [int(v) for v in os.environ.get('K_GC', '8,-1').split(',')]
GATE_C = [min(c * _GCN // NCHC + _GCO, 7) for c in range(NCHC)]
LNR = int(os.environ.get('K_LNR', 8))
GATE_EACH = int(os.environ.get('K_GE', 1))
FC = int(os.environ.get('K_FC', 256))
CHAIN_A = int(os.environ.get('K_CHA', 3))
CHAIN_C = int(os.environ.get('K_CHAINC', 0))
B_GATE = dict(tuple(int(v) for v in kv.split(':')) for kv in os.environ.get('K_BG', '8:0').split(','))
B_CHAIN = [int(v) for v in os.environ.get('K_BC', '').split(',') if v]
EPS = 1e-5
NEG = -1e30
QSCALE = (DH ** -0.5) * 1.4426950408889634
NT = (((1,), (1,)), ((), ()))


def _ln(x):
    m = jnp.mean(x, axis=-1, keepdims=True)
    xc = x - m
    v = jnp.mean(xc * xc, axis=-1, keepdims=True)
    return xc * lax.rsqrt(v + EPS)


def _pack_rows(x):
    return pltpu.bitcast(x.astype(bf16), u32)


def _pack_rows_interleaved(x):
    n = x.shape[0] // 16
    x3 = x.reshape(n, 16, x.shape[1])
    a = x3[:, 0:8, :].reshape(n * 8, x.shape[1])
    b = x3[:, 8:16, :].reshape(n * 8, x.shape[1])
    return pltpu.pack_elementwise([a, b], packed_dtype=bf16)


def _gate_first(x, gate, z):
    g = gate[0:8, 0:128] * z
    top = jnp.concatenate([x[0:8, 0:128] + g, x[0:8, 128:]], axis=1)
    return top if x.shape[0] == 8 else jnp.concatenate([top, x[8:]], axis=0)


def _kernel(x_hbm, wqkv_hbm, wo_hbm, wr_hbm, wg_hbm, wu_hbm, wd_hbm,
            out_hbm,
            xio, wq_v, wk_v, wv_v, wvt_v, wo_v, wop_v, wr_v, wg_v, wu_v, wd_v,
            xres, xbuf, best_v, best_i, rho_s, z_s, wr8,
            xca, xcb, xc_all, xi_all,
            q_s, k_s, vt_s, ot_s, s_s, m_s,
            ata, atb, oa, ob,
            sem_x, sem_w, sem_o):
    def x_copy(i):
        r0 = pl.multiple_of(i * TQ, TQ)
        return pltpu.make_async_copy(x_hbm.at[pl.ds(r0, TQ), :], xio.at[pl.ds(r0, TQ), :], sem_x.at[i])

    def out_copy(i):
        r0 = pl.multiple_of(i * TQ, TQ)
        return pltpu.make_async_copy(xio.at[pl.ds(r0, TQ), :], out_hbm.at[pl.ds(r0, TQ), :], sem_o.at[i])

    cp_wqa = pltpu.make_async_copy(wqkv_hbm.at[:, pl.ds(0, D // 2)], wq_v.at[:, pl.ds(0, D // 2)], sem_w.at[0])
    cp_wqb = pltpu.make_async_copy(wqkv_hbm.at[:, pl.ds(D // 2, D // 2)], wq_v.at[:, pl.ds(D // 2, D // 2)],
                                   sem_w.at[9])
    cp_wk = pltpu.make_async_copy(wqkv_hbm.at[:, pl.ds(D, D)], wk_v, sem_w.at[1])
    cp_wv = pltpu.make_async_copy(wqkv_hbm.at[:, pl.ds(2 * D, D)], wv_v, sem_w.at[8])
    cp_wo = pltpu.make_async_copy(wo_hbm, wo_v, sem_w.at[2])
    cp_wr = pltpu.make_async_copy(wr_hbm, wr_v, sem_w.at[3])
    cp_wg = pltpu.make_async_copy(wg_hbm, wg_v, sem_w.at[4])
    cp_wu = pltpu.make_async_copy(wu_hbm, wu_v, sem_w.at[5])
    cp_wd = pltpu.make_async_copy(wd_hbm, wd_v, sem_w.at[6])

    x_copy(0).start()
    cp_wqa.start()

    z_s[...] = jnp.zeros_like(z_s)
    xres[0:CH, :] = jnp.zeros((CH, D), f32)

    def ln_chunk(layer, i, c, xc_ref, gate, chain=None):
        r0 = i * TQ + c * CH
        h0 = i * (TQ // 2) + c * (CH // 2)
        if not isinstance(r0, int):
            r0 = pl.multiple_of(r0, CH)
            h0 = pl.multiple_of(h0, CH // 2)
        parts = []
        for q in range(CH // LNR):
            rq = r0 + q * LNR
            x_in = xio[pl.ds(rq, LNR), :].astype(f32)
            x_rs = xres[pl.ds(pl.multiple_of(rq * layer, LNR), LNR), :]
            xq = jnp.where(layer == 0, x_in, x_rs)
            xbuf[pl.ds(rq, LNR), :] = xq
            if chain is not None and len(chain) >= CHAIN_A:
                xq = _gate_first(xq, chain[-CHAIN_A], z_s[...])
            elif gate is not None:
                xq = _gate_first(xq, gate, z_s[...])
            parts.append(_ln(xq))
            if chain is not None:
                chain.append(parts[-1])
        xn = jnp.concatenate(parts, axis=0)
        xc = _pack_rows(xn)
        xc_ref[c * CH // 2:(c + 1) * CH // 2, :] = xc
        xc_all[pl.ds(h0, CH // 2), :] = xc
        xi_all[pl.ds(h0, CH // 2), :] = _pack_rows_interleaved(xn)

    def q_step(layer, i, xc_ref, i_next, xc_next, part=(0, G)):
        h0 = i * (TQ // 2)
        if not isinstance(h0, int):
            h0 = pl.multiple_of(h0, TQ // 2)
        a = pltpu.bitcast(xc_ref[...], bf16)
        ys = {}
        for n in range(*part):
            y = jnp.dot(a, wq_v[:, n * 128:(n + 1) * 128], preferred_element_type=f32)
            q_s[n, pl.ds(h0, TQ // 2), :] = _pack_rows(y * QSCALE)
            ys[n] = y
        if i_next is not None:
            chain = [] if CHAIN_A > 0 else None
            for c in range(part[0] * NCH // G, part[1] * NCH // G):
                ln_chunk(layer, i_next, c, xc_next, ys.get(GATE_A[c]), chain)

    def kv_step(i):
        h0 = pl.multiple_of(i * (TKV // 2), TKV // 2)
        a = pltpu.bitcast(xc_all[pl.ds(h0, TKV // 2), :], bf16)
        for n in range(G):
            y = jnp.dot(a, wk_v[:, n * 128:(n + 1) * 128], preferred_element_type=f32)
            k_s[n, pl.ds(PAD // 2 + h0, TKV // 2), :] = _pack_rows(y)
        vt = lax.dot_general(pltpu.bitcast(wvt_v[...], bf16), pltpu.bitcast(xi_all[pl.ds(h0, TKV // 2), :], bf16),
                             NT, preferred_element_type=f32)
        c0 = pl.multiple_of(PAD + i * TKV, 256)
        vt_s[:, pl.ds(c0, TKV)] = _pack_rows(vt)

    def phase_a(layer):
        @pl.when(layer == 0)
        def _():
            x_copy(0).wait()
            x_copy(1).start()
            cp_wqb.start()

        for c in range(NCH):
            ln_chunk(layer, 0, c, xca, None)

        @pl.when(layer == 0)
        def _():
            cp_wqa.wait()
            x_copy(1).wait()
            for i in range(2, NB):
                x_copy(i).start()

        q_step(layer, 0, xca, 1, xcb, part=(0, G // 2))

        @pl.when(layer == 0)
        def _():
            cp_wqb.wait()
            cp_wv.start()
            cp_wo.start()
            cp_wk.start()
            cp_wr.start()

        q_step(layer, 0, xca, 1, xcb, part=(G // 2, G))

        def q_body(j, c):
            i1 = 2 * j + 1

            @pl.when(layer == 0)
            def _():
                x_copy(i1 + 1).wait()
                x_copy(i1 + 2).wait()

            q_step(layer, i1, xcb, i1 + 1, xca)
            q_step(layer, i1 + 1, xca, i1 + 2, xcb)
            return c

        with jax.named_scope("a_q"):
            lax.fori_loop(0, NB // 2 - 1, q_body, 0)

        @pl.when(layer == 0)
        def _():
            cp_wv.wait()
            cp_wo.wait()

        q_step(layer, NB - 1, xcb, None, None)
        wvt_v[...] = pltpu.bitcast(wv_v[...].T, u32)
        for c in range(D // 64):
            wop_v[c * 32:(c + 1) * 32, :] = _pack_rows_interleaved(wo_v[c * 64:(c + 1) * 64, :].astype(f32))

        @pl.when(layer == 0)
        def _():
            cp_wk.wait()
            cp_wg.start()
            cp_wu.start()
            cp_wd.start()

        def kv_body(j, c):
            kv_step(j)
            return c

        with jax.named_scope("a_kv"):
            lax.fori_loop(0, S // TKV, kv_body, 0)

    def qk_stage(g, q0, slot, kstart):
        zi = pltpu.bitcast(z_s[...], i32)
        zi16 = jnp.concatenate([zi, zi], axis=0)
        lane16 = lax.broadcasted_iota(i32, (16, 128), 1) + zi16
        r16 = lax.broadcasted_iota(i32, (16, 128), 0)
        hb16 = lane16 // 32
        dd = r16 - lane16 % 32
        h0 = q0 // 2
        first_rows = None
        for b in range(4):
            first = max(0, kstart - 32 * b)
            base = h0 + 16 * b
            if not isinstance(base, int):
                base = pl.multiple_of(base, 16)
            mid0 = max(first, 32)
            if first == 0:
                parts = [k_s[g, pl.ds(base, 8), :], k_s[g, pl.ds(base + 128, 8), :],
                         k_s[g, pl.ds(base + 8, 8), :], k_s[g, pl.ds(base + 136, 8), :]]
            else:
                parts = [k_s[g, pl.ds(base + 128, 16), :]]
            if mid0 < 256:
                parts.append(k_s[g, pl.ds(base + mid0 // 2, (256 - mid0) // 2), :])
            kw = pltpu.bitcast(jnp.concatenate(parts, axis=0), bf16)
            qu = q_s[g, pl.ds(base, 16), :]
            qall = pltpu.bitcast(
                jnp.concatenate([jnp.where(hb16 == (p - b) % 4, qu, jnp.uint32(0)) for p in range(4)], axis=0),
                bf16)
            st = lax.dot_general(kw, qall, NT, preferred_element_type=f32)
            if b == 0:
                first_rows = [st[16 * r:16 * r + 8] for r in range(st.shape[0] // 16)]
            if first == 0:
                c0 = jnp.where(dd > 0, st[0:16], st[16:32])
                c1 = jnp.where(dd > -16, st[32:48], st[48:64])
                mid = st[64:]
            else:
                c0 = jnp.where(dd > 0, NEG, st[0:16])
                c1 = jnp.where(dd > -16, NEG, st[16:32])
                mid = st[32:]
            s_s[slot, b, 0:16, :] = c0
            s_s[slot, b, 16:32, :] = c1
            x = jnp.concatenate([c0, c1], axis=0)
            if mid0 < 256:
                s_s[slot, b, mid0:256, :] = mid
                x = jnp.concatenate([x, mid], axis=0)
            mm = jnp.max(x.reshape(x.shape[0] // 8, 8, 128), axis=0)
            m_s[slot, b] = jnp.broadcast_to(jnp.max(mm, axis=0, keepdims=True), (8, 128))
        return first_rows

    def pv_stage(g, q0, slot, gate, kstart):
        r8 = lax.broadcasted_iota(i32, (8, 128), 0)
        c8 = lax.broadcasted_iota(i32, (8, 128), 1) + pltpu.bitcast(z_s[...], i32)
        blk = c8 // 32
        j = c8 % 32

        def tri(u):
            return (jnp.where(16 * u + r8 > j, jnp.uint32(0xFFFF), jnp.uint32(0)) |
                    jnp.where(16 * u + 8 + r8 > j, jnp.uint32(0xFFFF0000), jnp.uint32(0)))

        tris = [tri(0), tri(1)] if kstart < 128 else None
        ms = [m_s[slot, b] for b in range(4)]
        L = [None] * 4
        cache = {}

        def pexp(b, u):
            x = s_s[slot, b, 16 * u:16 * u + 16, :]
            p0 = jnp.exp2(x[0:8] - ms[b])
            p1 = jnp.exp2(x[8:16] - ms[b])
            sm = p0 + p1
            L[b] = sm if L[b] is None else L[b] + sm
            return pltpu.pack_elementwise([p0, p1], packed_dtype=bf16)

        def get_p(b, u):
            first = max(0, kstart - 32 * b)
            if u < 0 or u >= 18 or 16 * u < first:
                return None
            if first > 0:
                return pexp(b, u - 16) if u >= 16 else pexp(b, u)
            if u < 2:
                pk = pexp(b, u)
                lo = pk & tris[u]
                cache[(b, u + 16)] = pk ^ lo
                return lo
            if u >= 16:
                return cache.pop((b, u))
            return pexp(b, u)

        zero = jnp.zeros((8, 128), u32)
        accs = [None] * 4
        for k in range(kstart // 128, 3):
            wts = [[] for _ in range(4)]
            for t in range(8 * k, 8 * k + 8):
                if t in B_GATE and kstart == 0:
                    gv = gate[B_GATE.get(t, 0)] * z_s[...]
                    for b in range(4):
                        ms[b] = ms[b] + gv
                if t in B_CHAIN and kstart == 0:
                    for b in range(4):
                        ms[b] = ms[b] + L[b] * z_s[...]
                srcs = [(b, get_p(b, t - 2 * b)) for b in range(4)]
                srcs = [(b, v) for (b, v) in srcs if v is not None]
                for h in range(4):
                    acc = zero if len(srcs) < 4 else None
                    for (b, v) in srcs:
                        acc = v if acc is None else jnp.where(blk == (h + b) % 4, v, acc)
                    wts[h].append(acc)
            c0 = q0 + 128 * k
            if not isinstance(c0, int):
                c0 = pl.multiple_of(c0, 128)
            for h in range(4):
                pt = pltpu.bitcast(jnp.concatenate(wts[h], axis=0), bf16)
                vth = pltpu.bitcast(vt_s[pl.ds((g * 4 + h) * 16, 16), pl.ds(c0, 128)], bf16)
                d = jnp.dot(vth, pt, preferred_element_type=f32)
                accs[h] = d if accs[h] is None else accs[h] + d
        L = [jnp.broadcast_to(jnp.sum(l, axis=0, keepdims=True), (8, 128)) for l in L]
        outs = []
        for h in range(4):
            lh = L[0]
            for b in range(1, 4):
                lh = jnp.where(blk == (h + b) % 4, L[b], lh)
            r0 = pl.reciprocal(lh, approx=True)
            rl = r0 * (2.0 - lh * r0)
            ot = (accs[h].reshape(4, 8, 128) * rl[None]).reshape(32, 128)
            if h > 0:
                ot = pltpu.roll(ot, 128 - 32 * h, axis=1)
            outs.append(ot)
        ot_s[g * 64:(g + 1) * 64, pl.ds(q0, 128)] = _pack_rows_interleaved(jnp.concatenate(outs, axis=0))

    def sub_block(q0, qn, kstart, kstart_next):
        for g in range(G):
            if g + 1 < G:
                gate = qk_stage(g + 1, q0, (g + 1) % 2, kstart)
            else:
                gate = qk_stage(0, qn, 0, kstart_next)
            pv_stage(g, q0, g % 2, gate, kstart)

    def phase_b():
        qk_stage(0, 0, 2, PAD)
        qk_stage(0, 128, 0, PAD - 128)
        for g in range(G):
            if g + 1 < G:
                qk_stage(g + 1, 0, 2 + (g + 1) % 2, PAD)
            pv_stage(g, 0, 2 + g % 2, None, PAD)
            if g + 1 < G:
                qk_stage(g + 1, 128, (g + 1) % 2, PAD - 128)
            else:
                qk_stage(0, 256, 0, 0)
            pv_stage(g, 128, g % 2, None, PAD - 128)

        def body(sb, c):
            q0 = pl.multiple_of(sb * 128, 128)
            qn = pl.multiple_of(jnp.minimum(sb + 1, NSB - 1) * 128, 128)
            sub_block(q0, qn, 0, 0)
            return c

        lax.fori_loop(2, NSB, body, 0, unroll=int(os.environ.get('K_UB', 2)))

    def resid_chunk(i, c, at_ref, gate, chain=None):
        r0 = i * TQ + c * CHC
        if not isinstance(r0, int):
            r0 = pl.multiple_of(r0, CHC)
        x1 = xbuf[pl.ds(r0, CHC), :] + at_ref[c * CHC:(c + 1) * CHC, :]
        if chain is not None and len(chain) >= CHAIN_C:
            x1 = _gate_first(x1, chain[-CHAIN_C], z_s[...])
        elif gate is not None:
            x1 = _gate_first(x1, gate, z_s[...])
        m = jnp.mean(x1, axis=-1, keepdims=True)
        xc = x1 - m
        v = jnp.mean(xc * xc, axis=-1, keepdims=True)
        rho = lax.rsqrt(v + EPS)
        xn = xc * rho
        r = jnp.sum(xn * wr8[0:1, :], axis=-1, keepdims=True)
        rb = jnp.broadcast_to(r, (CHC, 128)).astype(bf16).astype(f32)
        rows = lax.broadcasted_iota(i32, (8, 128), 0) + r0
        bv, bi = best_v[...], best_i[...]
        for q in range(CHC // 8):
            cand = rb[8 * q:8 * q + 8]
            better = cand > bv
            bv = jnp.where(better, cand, bv)
            bi = jnp.where(better, rows + 8 * q, bi)
        best_v[...] = bv
        best_i[...] = bi
        rho_s[pl.ds(r0, CHC), :] = jnp.broadcast_to(rho, (CHC, 128))
        x2 = x1 + xn
        if chain is not None:
            chain.append(x2)
        xres[pl.ds(r0, CHC), :] = x2
        xio[pl.ds(r0, CHC), :] = x2.astype(bf16)

    def transpose_o(i, o_dst):
        r0 = i * TQ
        if not isinstance(r0, int):
            r0 = pl.multiple_of(r0, TQ)
        o_dst[...] = pltpu.bitcast(pltpu.bitcast(ot_s[:, pl.ds(r0, TQ)], bf16).T, u32)

    def oproj_step(o_src, at_w, i_res, at_r, i_t, o_dst):
        ys = []
        if o_src is not None:
            a = pltpu.bitcast(o_src[...], bf16)
            for n in range(D // NWC):
                y = jnp.dot(a, pltpu.bitcast(wop_v[:, n * NWC:(n + 1) * NWC], bf16), preferred_element_type=f32)
                at_w[:, n * NWC:(n + 1) * NWC] = y
                ys.append(y)
        if i_t is not None:
            transpose_o(i_t, o_dst)
        if i_res is not None:
            chain = [] if (CHAIN_C > 0 and ys) else None
            for c in range(NCHC):
                gi = GATE_C[c] if ys else -1
                gate = ys[gi] if gi >= 0 else None
                resid_chunk(i_res, c, at_r, gate, chain)

    def phase_c(layer):
        @pl.when(layer == 0)
        def _():
            cp_wr.wait()
            wr8[...] = jnp.broadcast_to(wr_v[...].astype(f32).reshape(1, D), (8, D))

        def flush(i):
            @pl.when(layer == 1)
            def _():
                out_copy(i).start()

        best_v[...] = jnp.full((8, 128), -jnp.inf, f32)
        best_i[...] = jnp.zeros((8, 128), i32)
        transpose_o(0, oa)
        oproj_step(oa, ata, None, None, 1, ob)

        def body(j, c):
            i0 = 2 * j
            oproj_step(ob, atb, i0, ata, i0 + 2, oa)
            oproj_step(oa, ata, i0 + 1, atb, i0 + 3, ob)
            flush(i0)
            flush(i0 + 1)
            return c

        lax.fori_loop(0, NB // 2 - 1, body, 0)
        oproj_step(ob, atb, NB - 2, ata, None, None)
        oproj_step(None, None, NB - 1, atb, None, None)
        flush(NB - 2)
        flush(NB - 1)

    def phase_d(layer):
        @pl.when(layer == 0)
        def _():
            cp_wg.wait()
            cp_wu.wait()
            cp_wd.wait()

        bv = best_v[...]
        rmax = jnp.max(bv)
        idx = jnp.min(jnp.where(bv == rmax, best_i[...], S))
        idx = jnp.clip(idx, 0, S - 1)
        x2 = xres[pl.ds(idx, 1), :]
        rho = rho_s[pl.ds(idx, 1), 0:1]
        xn = (x2 - jnp.mean(x2, axis=-1, keepdims=True)) * (rho / (1.0 + rho))
        xs = jnp.broadcast_to(xn, (16, D)).astype(bf16)
        nf = F // FC
        hs = []
        y = None
        for c in range(nf + 1):
            if c < nf:
                gate = jnp.dot(xs, wg_v[:, c * FC:(c + 1) * FC], preferred_element_type=f32)
                up = jnp.dot(xs, wu_v[:, c * FC:(c + 1) * FC], preferred_element_type=f32)
                hs.append((gate * jax.nn.sigmoid(gate) * up).astype(bf16))
            if c > 0:
                d = jnp.dot(hs[c - 1], wd_v[(c - 1) * FC:c * FC, :], preferred_element_type=f32)
                y = d if y is None else y + d
        scale = jax.nn.sigmoid(jnp.full((1, D), rmax, f32))
        xres[pl.ds(idx, 1), :] = xres[pl.ds(idx, 1), :] + y[0:1] * scale

        @pl.when(layer == 1)
        def _():
            for i in range(NB):
                out_copy(i).wait()
            g0 = pl.multiple_of((idx // 16) * 16, 16)
            xio[pl.ds(g0, 16), :] = xres[pl.ds(g0, 16), :].astype(bf16)
            fix = pltpu.make_async_copy(xio.at[pl.ds(g0, 16), :], out_hbm.at[pl.ds(g0, 16), :], sem_w.at[7])
            fix.start()
            fix.wait()

    def layer_body(layer, c):
        with jax.named_scope("phase_a"):
            phase_a(layer)
        with jax.named_scope("phase_b"):
            phase_b()
        with jax.named_scope("phase_c"):
            phase_c(layer)
        with jax.named_scope("phase_d"):
            phase_d(layer)
        return c

    lax.fori_loop(0, 2, layer_body, 0)


@jax.jit
def pallas_interleave_layers__sliding_block__moe_arch_mod__prompt_kernel(
    A_x: jax.Array,
    A_wqkv: jax.Array,
    A_wo: jax.Array,
    B_x: jax.Array,
    B_w_r: jax.Array,
    B_w_gate: jax.Array,
    B_w_up: jax.Array,
    B_w_down: jax.Array,
):
    del B_x
    x = A_x.reshape(S, D)
    any_spec = pl.BlockSpec(memory_space=pl.ANY)
    scratch = [
        pltpu.VMEM((S, D), bf16),
        pltpu.VMEM((D, D), bf16),
        pltpu.VMEM((D, D), bf16),
        pltpu.VMEM((D, D), bf16),
        pltpu.VMEM((D // 2, D), u32),
        pltpu.VMEM((D, D), bf16),
        pltpu.VMEM((D // 2, D), u32),
        pltpu.VMEM((D,), bf16),
        pltpu.VMEM((D, F), bf16),
        pltpu.VMEM((D, F), bf16),
        pltpu.VMEM((F, D), bf16),
        pltpu.VMEM((S, D), f32),
        pltpu.VMEM((S, D), f32),
        pltpu.VMEM((8, 128), f32),
        pltpu.VMEM((8, 128), i32),
        pltpu.VMEM((S, 128), f32),
        pltpu.VMEM((8, 128), f32),
        pltpu.VMEM((8, D), f32),
        pltpu.VMEM((TQ // 2, D), u32),
        pltpu.VMEM((TQ // 2, D), u32),
        pltpu.VMEM((S // 2, D), u32),
        pltpu.VMEM((S // 2, D), u32),
        pltpu.VMEM((G, S // 2, 128), u32),
        pltpu.VMEM((G, (S + PAD) // 2, 128), u32),
        pltpu.VMEM((D // 2, S + PAD), u32),
        pltpu.VMEM((D // 2, S), u32),
        pltpu.VMEM((4, 4, 256, 128), f32),
        pltpu.VMEM((4, 4, 8, 128), f32),
        pltpu.VMEM((TQ, D), f32),
        pltpu.VMEM((TQ, D), f32),
        pltpu.VMEM((TQ // 2, D), u32),
        pltpu.VMEM((TQ // 2, D), u32),
        pltpu.SemaphoreType.DMA((NB,)),
        pltpu.SemaphoreType.DMA((10,)),
        pltpu.SemaphoreType.DMA((NB,)),
    ]
    out = pl.pallas_call(
        _kernel,
        out_shape=jax.ShapeDtypeStruct((S, D), bf16),
        in_specs=[any_spec] * 7,
        out_specs=any_spec,
        scratch_shapes=scratch,
        compiler_params=pltpu.CompilerParams(vmem_limit_bytes=120 * 1024 * 1024),
    )(x, A_wqkv, A_wo, B_w_r, B_w_gate, B_w_up, B_w_down)
    return out.reshape(1, S, D)
```

```python
import jax
import jax.numpy as jnp
from jax import lax
import jax.experimental.pallas as pl
import jax.experimental.pallas.tpu as pltpu

bf16 = jnp.bfloat16
f32 = jnp.float32
u32 = jnp.uint32
i32 = jnp.int32

S = 2048
D = 1024
H = 32
DH = 32
W = 256
F = 3584
G = 8
PAD = 256
TQ = 256
NB = S // TQ
TKV = 512
NSB = S // 128
import os
CH = int(os.environ.get('K_CH', 32))
NCH = TQ // CH
CHC = int(os.environ.get('K_CHC', 8))
NCHC = TQ // CHC
GATE_A = [c * 8 // NCH - 1 for c in range(NCH)]
NWC = int(os.environ.get('K_NWC', 128))
_GCN, _GCO = [int(v) for v in os.environ.get('K_GC', '8,-1').split(',')]
GATE_C = [min(c * _GCN // NCHC + _GCO, 7) for c in range(NCHC)]
LNR = int(os.environ.get('K_LNR', 8))
GATE_EACH = int(os.environ.get('K_GE', 1))
FC = int(os.environ.get('K_FC', 256))
CHAIN_A = int(os.environ.get('K_CHA', 3))
CHAIN_C = int(os.environ.get('K_CHAINC', 0))
B_GATE = dict(tuple(int(v) for v in kv.split(':')) for kv in os.environ.get('K_BG', '6:0').split(','))
B_CHAIN = [int(v) for v in os.environ.get('K_BC', '').split(',') if v]
B_ORDER = [int(v) for v in os.environ.get('K_BO', '1,0,2').split(',')]
EPS = 1e-5
NEG = -1e30
QSCALE = (DH ** -0.5) * 1.4426950408889634
NT = (((1,), (1,)), ((), ()))


def _ln(x):
    m = jnp.mean(x, axis=-1, keepdims=True)
    xc = x - m
    v = jnp.mean(xc * xc, axis=-1, keepdims=True)
    return xc * lax.rsqrt(v + EPS)


def _pack_rows(x):
    return pltpu.bitcast(x.astype(bf16), u32)


def _pack_rows_interleaved(x):
    n = x.shape[0] // 16
    x3 = x.reshape(n, 16, x.shape[1])
    a = x3[:, 0:8, :].reshape(n * 8, x.shape[1])
    b = x3[:, 8:16, :].reshape(n * 8, x.shape[1])
    return pltpu.pack_elementwise([a, b], packed_dtype=bf16)


def _gate_first(x, gate, z):
    g = gate[0:8, 0:128] * z
    top = jnp.concatenate([x[0:8, 0:128] + g, x[0:8, 128:]], axis=1)
    return top if x.shape[0] == 8 else jnp.concatenate([top, x[8:]], axis=0)


def _kernel(x_hbm, wqkv_hbm, wo_hbm, wr_hbm, wg_hbm, wu_hbm, wd_hbm,
            out_hbm,
            xio, wq_v, wk_v, wv_v, wvt_v, wo_v, wop_v, wr_v, wg_v, wu_v, wd_v,
            xres, xbuf, best_v, best_i, rho_s, z_s, wr8,
            xca, xcb, xc_all, xi_all,
            q_s, k_s, vt_s, ot_s, s_s, m_s,
            ata, atb, oa, ob,
            sem_x, sem_w, sem_o):
    def x_copy(i):
        r0 = pl.multiple_of(i * TQ, TQ)
        return pltpu.make_async_copy(x_hbm.at[pl.ds(r0, TQ), :], xio.at[pl.ds(r0, TQ), :], sem_x.at[i])

    def out_copy(i):
        r0 = pl.multiple_of(i * TQ, TQ)
        return pltpu.make_async_copy(xio.at[pl.ds(r0, TQ), :], out_hbm.at[pl.ds(r0, TQ), :], sem_o.at[i])

    cp_wqa = pltpu.make_async_copy(wqkv_hbm.at[:, pl.ds(0, D // 2)], wq_v.at[:, pl.ds(0, D // 2)], sem_w.at[0])
    cp_wqb = pltpu.make_async_copy(wqkv_hbm.at[:, pl.ds(D // 2, D // 2)], wq_v.at[:, pl.ds(D // 2, D // 2)],
                                   sem_w.at[9])
    cp_wk = pltpu.make_async_copy(wqkv_hbm.at[:, pl.ds(D, D)], wk_v, sem_w.at[1])
    cp_wv = pltpu.make_async_copy(wqkv_hbm.at[:, pl.ds(2 * D, D)], wv_v, sem_w.at[8])
    cp_wo = pltpu.make_async_copy(wo_hbm, wo_v, sem_w.at[2])
    cp_wr = pltpu.make_async_copy(wr_hbm, wr_v, sem_w.at[3])
    cp_wg = pltpu.make_async_copy(wg_hbm, wg_v, sem_w.at[4])
    cp_wu = pltpu.make_async_copy(wu_hbm, wu_v, sem_w.at[5])
    cp_wd = pltpu.make_async_copy(wd_hbm, wd_v, sem_w.at[6])

    x_copy(0).start()
    cp_wqa.start()

    z_s[...] = jnp.zeros_like(z_s)
    xres[0:CH, :] = jnp.zeros((CH, D), f32)

    def ln_chunk(layer, i, c, xc_ref, gate, chain=None):
        r0 = i * TQ + c * CH
        h0 = i * (TQ // 2) + c * (CH // 2)
        if not isinstance(r0, int):
            r0 = pl.multiple_of(r0, CH)
            h0 = pl.multiple_of(h0, CH // 2)
        parts = []
        for q in range(CH // LNR):
            rq = r0 + q * LNR
            x_in = xio[pl.ds(rq, LNR), :].astype(f32)
            x_rs = xres[pl.ds(pl.multiple_of(rq * layer, LNR), LNR), :]
            xq = jnp.where(layer == 0, x_in, x_rs)
            xbuf[pl.ds(rq, LNR), :] = xq
            if chain is not None and len(chain) >= CHAIN_A:
                xq = _gate_first(xq, chain[-CHAIN_A], z_s[...])
            elif gate is not None:
                xq = _gate_first(xq, gate, z_s[...])
            parts.append(_ln(xq))
            if chain is not None:
                chain.append(parts[-1])
        xn = jnp.concatenate(parts, axis=0)
        xc = _pack_rows(xn)
        xc_ref[c * CH // 2:(c + 1) * CH // 2, :] = xc
        xc_all[pl.ds(h0, CH // 2), :] = xc
        xi_all[pl.ds(h0, CH // 2), :] = _pack_rows_interleaved(xn)

    def q_step(layer, i, xc_ref, i_next, xc_next, part=(0, G)):
        h0 = i * (TQ // 2)
        if not isinstance(h0, int):
            h0 = pl.multiple_of(h0, TQ // 2)
        a = pltpu.bitcast(xc_ref[...], bf16)
        ys = {}
        for n in range(*part):
            y = jnp.dot(a, wq_v[:, n * 128:(n + 1) * 128], preferred_element_type=f32)
            q_s[n, pl.ds(h0, TQ // 2), :] = _pack_rows(y * QSCALE)
            ys[n] = y
        if i_next is not None:
            chain = [] if CHAIN_A > 0 else None
            for c in range(part[0] * NCH // G, part[1] * NCH // G):
                ln_chunk(layer, i_next, c, xc_next, ys.get(GATE_A[c]), chain)

    def kv_step(i):
        h0 = pl.multiple_of(i * (TKV // 2), TKV // 2)
        a = pltpu.bitcast(xc_all[pl.ds(h0, TKV // 2), :], bf16)
        for n in range(G):
            y = jnp.dot(a, wk_v[:, n * 128:(n + 1) * 128], preferred_element_type=f32)
            k_s[n, pl.ds(PAD // 2 + h0, TKV // 2), :] = _pack_rows(y)
        vt = lax.dot_general(pltpu.bitcast(wvt_v[...], bf16), pltpu.bitcast(xi_all[pl.ds(h0, TKV // 2), :], bf16),
                             NT, preferred_element_type=f32)
        c0 = pl.multiple_of(PAD + i * TKV, 256)
        vt_s[:, pl.ds(c0, TKV)] = _pack_rows(vt)

    def phase_a(layer):
        @pl.when(layer == 0)
        def _():
            x_copy(0).wait()
            x_copy(1).start()
            cp_wqb.start()

        for c in range(NCH):
            ln_chunk(layer, 0, c, xca, None)

        @pl.when(layer == 0)
        def _():
            cp_wqa.wait()
            x_copy(1).wait()
            for i in range(2, NB):
                x_copy(i).start()

        q_step(layer, 0, xca, 1, xcb, part=(0, G // 2))

        @pl.when(layer == 0)
        def _():
            cp_wqb.wait()
            cp_wv.start()
            cp_wo.start()
            cp_wk.start()
            cp_wr.start()

        q_step(layer, 0, xca, 1, xcb, part=(G // 2, G))

        def q_body(j, c):
            i1 = 2 * j + 1

            @pl.when(layer == 0)
            def _():
                x_copy(i1 + 1).wait()
                x_copy(i1 + 2).wait()

            q_step(layer, i1, xcb, i1 + 1, xca)
            q_step(layer, i1 + 1, xca, i1 + 2, xcb)
            return c

        with jax.named_scope("a_q"):
            lax.fori_loop(0, NB // 2 - 1, q_body, 0)

        @pl.when(layer == 0)
        def _():
            cp_wv.wait()
            cp_wo.wait()

        q_step(layer, NB - 1, xcb, None, None)
        wvt_v[...] = pltpu.bitcast(wv_v[...].T, u32)
        for c in range(D // 64):
            wop_v[c * 32:(c + 1) * 32, :] = _pack_rows_interleaved(wo_v[c * 64:(c + 1) * 64, :].astype(f32))

        @pl.when(layer == 0)
        def _():
            cp_wk.wait()
            cp_wg.start()
            cp_wu.start()
            cp_wd.start()

        def kv_body(j, c):
            kv_step(j)
            return c

        with jax.named_scope("a_kv"):
            lax.fori_loop(0, S // TKV, kv_body, 0)

    def qk_stage(g, q0, slot, kstart):
        zi = pltpu.bitcast(z_s[...], i32)
        zi16 = jnp.concatenate([zi, zi], axis=0)
        lane16 = lax.broadcasted_iota(i32, (16, 128), 1) + zi16
        r16 = lax.broadcasted_iota(i32, (16, 128), 0)
        hb16 = lane16 // 32
        dd = r16 - lane16 % 32
        h0 = q0 // 2
        first_rows = None
        for b in range(4):
            first = max(0, kstart - 32 * b)
            base = h0 + 16 * b
            if not isinstance(base, int):
                base = pl.multiple_of(base, 16)
            mid0 = max(first, 32)
            if first == 0:
                parts = [k_s[g, pl.ds(base, 8), :], k_s[g, pl.ds(base + 128, 8), :],
                         k_s[g, pl.ds(base + 8, 8), :], k_s[g, pl.ds(base + 136, 8), :]]
            else:
                parts = [k_s[g, pl.ds(base + 128, 16), :]]
            if mid0 < 256:
                parts.append(k_s[g, pl.ds(base + mid0 // 2, (256 - mid0) // 2), :])
            kw = pltpu.bitcast(jnp.concatenate(parts, axis=0), bf16)
            qu = q_s[g, pl.ds(base, 16), :]
            qall = pltpu.bitcast(
                jnp.concatenate([jnp.where(hb16 == (p - b) % 4, qu, jnp.uint32(0)) for p in range(4)], axis=0),
                bf16)
            st = lax.dot_general(kw, qall, NT, preferred_element_type=f32)
            if b == 0:
                first_rows = [st[16 * r:16 * r + 8] for r in range(st.shape[0] // 16)]
            if first == 0:
                c0 = jnp.where(dd > 0, st[0:16], st[16:32])
                c1 = jnp.where(dd > -16, st[32:48], st[48:64])
                mid = st[64:]
            else:
                c0 = jnp.where(dd > 0, NEG, st[0:16])
                c1 = jnp.where(dd > -16, NEG, st[16:32])
                mid = st[32:]
            s_s[slot, b, 0:16, :] = c0
            s_s[slot, b, 16:32, :] = c1
            x = jnp.concatenate([c0, c1], axis=0)
            if mid0 < 256:
                s_s[slot, b, mid0:256, :] = mid
                x = jnp.concatenate([x, mid], axis=0)
            mm = jnp.max(x.reshape(x.shape[0] // 8, 8, 128), axis=0)
            m_s[slot, b] = jnp.broadcast_to(jnp.max(mm, axis=0, keepdims=True), (8, 128))
        return first_rows

    def pv_stage(g, q0, slot, gate, kstart):
        r8 = lax.broadcasted_iota(i32, (8, 128), 0)
        c8 = lax.broadcasted_iota(i32, (8, 128), 1) + pltpu.bitcast(z_s[...], i32)
        blk = c8 // 32
        j = c8 % 32

        def tri(u):
            return (jnp.where(16 * u + r8 > j, jnp.uint32(0xFFFF), jnp.uint32(0)) |
                    jnp.where(16 * u + 8 + r8 > j, jnp.uint32(0xFFFF0000), jnp.uint32(0)))

        tris = [tri(0), tri(1)] if kstart < 128 else None
        ms = [m_s[slot, b] for b in range(4)]
        L = [None] * 4
        cache = {}

        def pexp(b, u):
            x = s_s[slot, b, 16 * u:16 * u + 16, :]
            p0 = jnp.exp2(x[0:8] - ms[b])
            p1 = jnp.exp2(x[8:16] - ms[b])
            sm = p0 + p1
            L[b] = sm if L[b] is None else L[b] + sm
            return pltpu.pack_elementwise([p0, p1], packed_dtype=bf16)

        def get_p(b, u):
            first = max(0, kstart - 32 * b)
            if u < 0 or u >= 18 or 16 * u < first:
                return None
            if first > 0:
                return pexp(b, u - 16) if u >= 16 else pexp(b, u)
            if u < 2 or u >= 16:
                if (b, u) not in cache:
                    pk = pexp(b, u % 16)
                    lo = pk & tris[u % 16]
                    cache[(b, u % 16)] = lo
                    cache[(b, u % 16 + 16)] = pk ^ lo
                return cache.pop((b, u))
            return pexp(b, u)

        zero = jnp.zeros((8, 128), u32)
        accs = [None] * 4
        for k in [k for k in B_ORDER if k >= kstart // 128]:
            wts = [[] for _ in range(4)]
            for t in range(8 * k, 8 * k + 8):
                if t in B_GATE and kstart == 0:
                    gv = gate[B_GATE.get(t, 0)] * z_s[...]
                    for b in range(4):
                        ms[b] = ms[b] + gv
                if t in B_CHAIN and kstart == 0:
                    for b in range(4):
                        ms[b] = ms[b] + L[b] * z_s[...]
                srcs = [(b, get_p(b, t - 2 * b)) for b in range(4)]
                srcs = [(b, v) for (b, v) in srcs if v is not None]
                for h in range(4):
                    acc = zero if len(srcs) < 4 else None
                    for (b, v) in srcs:
                        acc = v if acc is None else jnp.where(blk == (h + b) % 4, v, acc)
                    wts[h].append(acc)
            c0 = q0 + 128 * k
            if not isinstance(c0, int):
                c0 = pl.multiple_of(c0, 128)
            for h in range(4):
                pt = pltpu.bitcast(jnp.concatenate(wts[h], axis=0), bf16)
                vth = pltpu.bitcast(vt_s[pl.ds((g * 4 + h) * 16, 16), pl.ds(c0, 128)], bf16)
                d = jnp.dot(vth, pt, preferred_element_type=f32)
                accs[h] = d if accs[h] is None else accs[h] + d
        L = [jnp.broadcast_to(jnp.sum(l, axis=0, keepdims=True), (8, 128)) for l in L]
        outs = []
        for h in range(4):
            lh = L[0]
            for b in range(1, 4):
                lh = jnp.where(blk == (h + b) % 4, L[b], lh)
            r0 = pl.reciprocal(lh, approx=True)
            rl = r0 * (2.0 - lh * r0)
            ot = (accs[h].reshape(4, 8, 128) * rl[None]).reshape(32, 128)
            if h > 0:
                ot = pltpu.roll(ot, 128 - 32 * h, axis=1)
            outs.append(ot)
        ot_s[g * 64:(g + 1) * 64, pl.ds(q0, 128)] = _pack_rows_interleaved(jnp.concatenate(outs, axis=0))

    def sub_block(q0, qn, kstart, kstart_next):
        for g in range(G):
            if g + 1 < G:
                gate = qk_stage(g + 1, q0, (g + 1) % 2, kstart)
            else:
                gate = qk_stage(0, qn, 0, kstart_next)
            pv_stage(g, q0, g % 2, gate, kstart)

    def phase_b():
        qk_stage(0, 0, 2, PAD)
        qk_stage(0, 128, 0, PAD - 128)
        for g in range(G):
            if g + 1 < G:
                qk_stage(g + 1, 0, 2 + (g + 1) % 2, PAD)
            pv_stage(g, 0, 2 + g % 2, None, PAD)
            if g + 1 < G:
                qk_stage(g + 1, 128, (g + 1) % 2, PAD - 128)
            else:
                qk_stage(0, 256, 0, 0)
            pv_stage(g, 128, g % 2, None, PAD - 128)

        def body(sb, c):
            q0 = pl.multiple_of(sb * 128, 128)
            qn = pl.multiple_of(jnp.minimum(sb + 1, NSB - 1) * 128, 128)
            sub_block(q0, qn, 0, 0)
            return c

        lax.fori_loop(2, NSB, body, 0, unroll=int(os.environ.get('K_UB', 2)))

    def resid_chunk(i, c, at_ref, gate, chain=None):
        r0 = i * TQ + c * CHC
        if not isinstance(r0, int):
            r0 = pl.multiple_of(r0, CHC)
        x1 = xbuf[pl.ds(r0, CHC), :] + at_ref[c * CHC:(c + 1) * CHC, :]
        if chain is not None and len(chain) >= CHAIN_C:
            x1 = _gate_first(x1, chain[-CHAIN_C], z_s[...])
        elif gate is not None:
            x1 = _gate_first(x1, gate, z_s[...])
        m = jnp.mean(x1, axis=-1, keepdims=True)
        xc = x1 - m
        v = jnp.mean(xc * xc, axis=-1, keepdims=True)
        rho = lax.rsqrt(v + EPS)
        xn = xc * rho
        r = jnp.sum(xn * wr8[0:1, :], axis=-1, keepdims=True)
        rb = jnp.broadcast_to(r, (CHC, 128)).astype(bf16).astype(f32)
        rows = lax.broadcasted_iota(i32, (8, 128), 0) + r0
        bv, bi = best_v[...], best_i[...]
        for q in range(CHC // 8):
            cand = rb[8 * q:8 * q + 8]
            better = cand > bv
            bv = jnp.where(better, cand, bv)
            bi = jnp.where(better, rows + 8 * q, bi)
        best_v[...] = bv
        best_i[...] = bi
        rho_s[pl.ds(r0, CHC), :] = jnp.broadcast_to(rho, (CHC, 128))
        x2 = x1 + xn
        if chain is not None:
            chain.append(x2)
        xres[pl.ds(r0, CHC), :] = x2
        xio[pl.ds(r0, CHC), :] = x2.astype(bf16)

    def transpose_o(i, o_dst):
        r0 = i * TQ
        if not isinstance(r0, int):
            r0 = pl.multiple_of(r0, TQ)
        o_dst[...] = pltpu.bitcast(pltpu.bitcast(ot_s[:, pl.ds(r0, TQ)], bf16).T, u32)

    def oproj_step(o_src, at_w, i_res, at_r, i_t, o_dst):
        ys = []
        if o_src is not None:
            a = pltpu.bitcast(o_src[...], bf16)
            for n in range(D // NWC):
                y = jnp.dot(a, pltpu.bitcast(wop_v[:, n * NWC:(n + 1) * NWC], bf16), preferred_element_type=f32)
                at_w[:, n * NWC:(n + 1) * NWC] = y
                ys.append(y)
        if i_t is not None:
            transpose_o(i_t, o_dst)
        if i_res is not None:
            chain = [] if (CHAIN_C > 0 and ys) else None
            for c in range(NCHC):
                gi = GATE_C[c] if ys else -1
                gate = ys[gi] if gi >= 0 else None
                resid_chunk(i_res, c, at_r, gate, chain)

    def phase_c(layer):
        @pl.when(layer == 0)
        def _():
            cp_wr.wait()
            wr8[...] = jnp.broadcast_to(wr_v[...].astype(f32).reshape(1, D), (8, D))

        def flush(i):
            @pl.when(layer == 1)
            def _():
                out_copy(i).start()

        best_v[...] = jnp.full((8, 128), -jnp.inf, f32)
        best_i[...] = jnp.zeros((8, 128), i32)
        transpose_o(0, oa)
        oproj_step(oa, ata, None, None, 1, ob)

        def body(j, c):
            i0 = 2 * j
            oproj_step(ob, atb, i0, ata, i0 + 2, oa)
            oproj_step(oa, ata, i0 + 1, atb, i0 + 3, ob)
            flush(i0)
            flush(i0 + 1)
            return c

        lax.fori_loop(0, NB // 2 - 1, body, 0)
        oproj_step(ob, atb, NB - 2, ata, None, None)
        oproj_step(None, None, NB - 1, atb, None, None)
        flush(NB - 2)
        flush(NB - 1)

    def phase_d(layer):
        @pl.when(layer == 0)
        def _():
            cp_wg.wait()
            cp_wu.wait()
            cp_wd.wait()

        bv = best_v[...]
        rmax = jnp.max(bv)
        idx = jnp.min(jnp.where(bv == rmax, best_i[...], S))
        idx = jnp.clip(idx, 0, S - 1)
        x2 = xres[pl.ds(idx, 1), :]
        rho = rho_s[pl.ds(idx, 1), 0:1]
        xn = (x2 - jnp.mean(x2, axis=-1, keepdims=True)) * (rho / (1.0 + rho))
        xs = jnp.broadcast_to(xn, (16, D)).astype(bf16)
        nf = F // FC
        hs = []
        y = None
        for c in range(nf + 1):
            if c < nf:
                gate = jnp.dot(xs, wg_v[:, c * FC:(c + 1) * FC], preferred_element_type=f32)
                up = jnp.dot(xs, wu_v[:, c * FC:(c + 1) * FC], preferred_element_type=f32)
                hs.append((gate * jax.nn.sigmoid(gate) * up).astype(bf16))
            if c > 0:
                d = jnp.dot(hs[c - 1], wd_v[(c - 1) * FC:c * FC, :], preferred_element_type=f32)
                y = d if y is None else y + d
        scale = jax.nn.sigmoid(jnp.full((1, D), rmax, f32))
        xres[pl.ds(idx, 1), :] = xres[pl.ds(idx, 1), :] + y[0:1] * scale

        @pl.when(layer == 1)
        def _():
            for i in range(NB):
                out_copy(i).wait()
            g0 = pl.multiple_of((idx // 16) * 16, 16)
            xio[pl.ds(g0, 16), :] = xres[pl.ds(g0, 16), :].astype(bf16)
            fix = pltpu.make_async_copy(xio.at[pl.ds(g0, 16), :], out_hbm.at[pl.ds(g0, 16), :], sem_w.at[7])
            fix.start()
            fix.wait()

    def layer_body(layer, c):
        with jax.named_scope("phase_a"):
            phase_a(layer)
        with jax.named_scope("phase_b"):
            phase_b()
        with jax.named_scope("phase_c"):
            phase_c(layer)
        with jax.named_scope("phase_d"):
            phase_d(layer)
        return c

    lax.fori_loop(0, 2, layer_body, 0)


@jax.jit
def pallas_interleave_layers__sliding_block__moe_arch_mod__prompt_kernel(
    A_x: jax.Array,
    A_wqkv: jax.Array,
    A_wo: jax.Array,
    B_x: jax.Array,
    B_w_r: jax.Array,
    B_w_gate: jax.Array,
    B_w_up: jax.Array,
    B_w_down: jax.Array,
):
    del B_x
    x = A_x.reshape(S, D)
    any_spec = pl.BlockSpec(memory_space=pl.ANY)
    scratch = [
        pltpu.VMEM((S, D), bf16),
        pltpu.VMEM((D, D), bf16),
        pltpu.VMEM((D, D), bf16),
        pltpu.VMEM((D, D), bf16),
        pltpu.VMEM((D // 2, D), u32),
        pltpu.VMEM((D, D), bf16),
        pltpu.VMEM((D // 2, D), u32),
        pltpu.VMEM((D,), bf16),
        pltpu.VMEM((D, F), bf16),
        pltpu.VMEM((D, F), bf16),
        pltpu.VMEM((F, D), bf16),
        pltpu.VMEM((S, D), f32),
        pltpu.VMEM((S, D), f32),
        pltpu.VMEM((8, 128), f32),
        pltpu.VMEM((8, 128), i32),
        pltpu.VMEM((S, 128), f32),
        pltpu.VMEM((8, 128), f32),
        pltpu.VMEM((8, D), f32),
        pltpu.VMEM((TQ // 2, D), u32),
        pltpu.VMEM((TQ // 2, D), u32),
        pltpu.VMEM((S // 2, D), u32),
        pltpu.VMEM((S // 2, D), u32),
        pltpu.VMEM((G, S // 2, 128), u32),
        pltpu.VMEM((G, (S + PAD) // 2, 128), u32),
        pltpu.VMEM((D // 2, S + PAD), u32),
        pltpu.VMEM((D // 2, S), u32),
        pltpu.VMEM((4, 4, 256, 128), f32),
        pltpu.VMEM((4, 4, 8, 128), f32),
        pltpu.VMEM((TQ, D), f32),
        pltpu.VMEM((TQ, D), f32),
        pltpu.VMEM((TQ // 2, D), u32),
        pltpu.VMEM((TQ // 2, D), u32),
        pltpu.SemaphoreType.DMA((NB,)),
        pltpu.SemaphoreType.DMA((10,)),
        pltpu.SemaphoreType.DMA((NB,)),
    ]
    out = pl.pallas_call(
        _kernel,
        out_shape=jax.ShapeDtypeStruct((S, D), bf16),
        in_specs=[any_spec] * 7,
        out_specs=any_spec,
        scratch_shapes=scratch,
        compiler_params=pltpu.CompilerParams(vmem_limit_bytes=120 * 1024 * 1024),
    )(x, A_wqkv, A_wo, B_w_r, B_w_gate, B_w_up, B_w_down)
    return out.reshape(1, S, D)
```

```python
import jax
import jax.numpy as jnp
from jax import lax
import jax.experimental.pallas as pl
import jax.experimental.pallas.tpu as pltpu

bf16 = jnp.bfloat16
f32 = jnp.float32
u32 = jnp.uint32
i32 = jnp.int32

S = 2048
D = 1024
H = 32
DH = 32
W = 256
F = 3584
G = 8
PAD = 256
TQ = 256
NB = S // TQ
TKV = 512
NSB = S // 128
CH = 32
LNR = 8
NCH = TQ // CH
CHC = 8
NCHC = TQ // CHC
FC = 256
GATE_A = [c * 8 // NCH - 1 for c in range(NCH)]
CHAIN_A = 3
GATE_C = [c * 8 // NCHC - 1 for c in range(NCHC)]
B_ORDER = [1, 0, 2]
B_GATE_T = 6
EPS = 1e-5
NEG = -1e30
QSCALE = (DH ** -0.5) * 1.4426950408889634
NT = (((1,), (1,)), ((), ()))


def _ln(x):
    m = jnp.mean(x, axis=-1, keepdims=True)
    xc = x - m
    v = jnp.mean(xc * xc, axis=-1, keepdims=True)
    return xc * lax.rsqrt(v + EPS)


def _pack_rows(x):
    return pltpu.bitcast(x.astype(bf16), u32)


def _pack_rows_interleaved(x):
    n = x.shape[0] // 16
    x3 = x.reshape(n, 16, x.shape[1])
    a = x3[:, 0:8, :].reshape(n * 8, x.shape[1])
    b = x3[:, 8:16, :].reshape(n * 8, x.shape[1])
    return pltpu.pack_elementwise([a, b], packed_dtype=bf16)


def _gate_first(x, gate, z):
    g = gate[0:8, 0:128] * z
    top = jnp.concatenate([x[0:8, 0:128] + g, x[0:8, 128:]], axis=1)
    return top if x.shape[0] == 8 else jnp.concatenate([top, x[8:]], axis=0)


def _kernel(x_hbm, wqkv_hbm, wo_hbm, wr_hbm, wg_hbm, wu_hbm, wd_hbm,
            out_hbm,
            xio, wq_v, wk_v, wv_v, wvt_v, wo_v, wop_v, wr_v, wg_v, wu_v, wd_v,
            xres, xbuf, best_v, best_i, rho_s, z_s, wr8,
            xca, xcb, xc_all, xi_all,
            q_s, k_s, vt_s, ot_s, s_s, m_s,
            ata, atb, oa, ob,
            sem_x, sem_w, sem_o):
    def x_copy(i):
        r0 = pl.multiple_of(i * TQ, TQ)
        return pltpu.make_async_copy(x_hbm.at[pl.ds(r0, TQ), :], xio.at[pl.ds(r0, TQ), :], sem_x.at[i])

    def out_copy(i):
        r0 = pl.multiple_of(i * TQ, TQ)
        return pltpu.make_async_copy(xio.at[pl.ds(r0, TQ), :], out_hbm.at[pl.ds(r0, TQ), :], sem_o.at[i])

    cp_wqa = pltpu.make_async_copy(wqkv_hbm.at[:, pl.ds(0, D // 2)], wq_v.at[:, pl.ds(0, D // 2)], sem_w.at[0])
    cp_wqb = pltpu.make_async_copy(wqkv_hbm.at[:, pl.ds(D // 2, D // 2)], wq_v.at[:, pl.ds(D // 2, D // 2)],
                                   sem_w.at[9])
    cp_wk = pltpu.make_async_copy(wqkv_hbm.at[:, pl.ds(D, D)], wk_v, sem_w.at[1])
    cp_wv = pltpu.make_async_copy(wqkv_hbm.at[:, pl.ds(2 * D, D)], wv_v, sem_w.at[8])
    cp_wo = pltpu.make_async_copy(wo_hbm, wo_v, sem_w.at[2])
    cp_wr = pltpu.make_async_copy(wr_hbm, wr_v, sem_w.at[3])
    cp_wg = pltpu.make_async_copy(wg_hbm, wg_v, sem_w.at[4])
    cp_wu = pltpu.make_async_copy(wu_hbm, wu_v, sem_w.at[5])
    cp_wd = pltpu.make_async_copy(wd_hbm, wd_v, sem_w.at[6])

    x_copy(0).start()
    cp_wqa.start()

    z_s[...] = jnp.zeros_like(z_s)
    xres[0:CH, :] = jnp.zeros((CH, D), f32)

    def ln_chunk(layer, i, c, xc_ref, gate, chain=None):
        r0 = i * TQ + c * CH
        h0 = i * (TQ // 2) + c * (CH // 2)
        if not isinstance(r0, int):
            r0 = pl.multiple_of(r0, CH)
            h0 = pl.multiple_of(h0, CH // 2)
        parts = []
        for q in range(CH // LNR):
            rq = r0 + q * LNR
            x_in = xio[pl.ds(rq, LNR), :].astype(f32)
            x_rs = xres[pl.ds(pl.multiple_of(rq * layer, LNR), LNR), :]
            xq = jnp.where(layer == 0, x_in, x_rs)
            xbuf[pl.ds(rq, LNR), :] = xq
            if chain is not None and len(chain) >= CHAIN_A:
                xq = _gate_first(xq, chain[-CHAIN_A], z_s[...])
            elif gate is not None:
                xq = _gate_first(xq, gate, z_s[...])
            parts.append(_ln(xq))
            if chain is not None:
                chain.append(parts[-1])
        xn = jnp.concatenate(parts, axis=0)
        xc = _pack_rows(xn)
        xc_ref[c * CH // 2:(c + 1) * CH // 2, :] = xc
        xc_all[pl.ds(h0, CH // 2), :] = xc
        xi_all[pl.ds(h0, CH // 2), :] = _pack_rows_interleaved(xn)

    def q_step(layer, i, xc_ref, i_next, xc_next, part=(0, G)):
        h0 = i * (TQ // 2)
        if not isinstance(h0, int):
            h0 = pl.multiple_of(h0, TQ // 2)
        a = pltpu.bitcast(xc_ref[...], bf16)
        ys = {}
        for n in range(*part):
            y = jnp.dot(a, wq_v[:, n * 128:(n + 1) * 128], preferred_element_type=f32)
            q_s[n, pl.ds(h0, TQ // 2), :] = _pack_rows(y * QSCALE)
            ys[n] = y
        if i_next is not None:
            chain = []
            for c in range(part[0] * NCH // G, part[1] * NCH // G):
                ln_chunk(layer, i_next, c, xc_next, ys.get(GATE_A[c]), chain)

    def kv_step(i):
        h0 = pl.multiple_of(i * (TKV // 2), TKV // 2)
        a = pltpu.bitcast(xc_all[pl.ds(h0, TKV // 2), :], bf16)
        for n in range(G):
            y = jnp.dot(a, wk_v[:, n * 128:(n + 1) * 128], preferred_element_type=f32)
            k_s[n, pl.ds(PAD // 2 + h0, TKV // 2), :] = _pack_rows(y)
        vt = lax.dot_general(pltpu.bitcast(wvt_v[...], bf16), pltpu.bitcast(xi_all[pl.ds(h0, TKV // 2), :], bf16),
                             NT, preferred_element_type=f32)
        c0 = pl.multiple_of(PAD + i * TKV, 256)
        vt_s[:, pl.ds(c0, TKV)] = _pack_rows(vt)

    def phase_a(layer):
        @pl.when(layer == 0)
        def _():
            x_copy(0).wait()
            x_copy(1).start()
            cp_wqb.start()

        for c in range(NCH):
            ln_chunk(layer, 0, c, xca, None)

        @pl.when(layer == 0)
        def _():
            cp_wqa.wait()
            x_copy(1).wait()
            for i in range(2, NB):
                x_copy(i).start()

        q_step(layer, 0, xca, 1, xcb, part=(0, G // 2))

        @pl.when(layer == 0)
        def _():
            cp_wqb.wait()
            cp_wv.start()
            cp_wo.start()
            cp_wk.start()
            cp_wr.start()

        q_step(layer, 0, xca, 1, xcb, part=(G // 2, G))

        def q_body(j, c):
            i1 = 2 * j + 1

            @pl.when(layer == 0)
            def _():
                x_copy(i1 + 1).wait()
                x_copy(i1 + 2).wait()

            q_step(layer, i1, xcb, i1 + 1, xca)
            q_step(layer, i1 + 1, xca, i1 + 2, xcb)
            return c

        with jax.named_scope("a_q"):
            lax.fori_loop(0, NB // 2 - 1, q_body, 0)

        @pl.when(layer == 0)
        def _():
            cp_wv.wait()
            cp_wo.wait()

        q_step(layer, NB - 1, xcb, None, None)
        wvt_v[...] = pltpu.bitcast(wv_v[...].T, u32)
        for c in range(D // 64):
            wop_v[c * 32:(c + 1) * 32, :] = _pack_rows_interleaved(wo_v[c * 64:(c + 1) * 64, :].astype(f32))

        @pl.when(layer == 0)
        def _():
            cp_wk.wait()
            cp_wg.start()
            cp_wu.start()
            cp_wd.start()

        def kv_body(j, c):
            kv_step(j)
            return c

        with jax.named_scope("a_kv"):
            lax.fori_loop(0, S // TKV, kv_body, 0)

    def qk_stage(g, q0, slot, kstart):
        zi = pltpu.bitcast(z_s[...], i32)
        zi16 = jnp.concatenate([zi, zi], axis=0)
        lane16 = lax.broadcasted_iota(i32, (16, 128), 1) + zi16
        r16 = lax.broadcasted_iota(i32, (16, 128), 0)
        hb16 = lane16 // 32
        dd = r16 - lane16 % 32
        h0 = q0 // 2
        first_rows = None
        for b in range(4):
            first = max(0, kstart - 32 * b)
            base = h0 + 16 * b
            if not isinstance(base, int):
                base = pl.multiple_of(base, 16)
            mid0 = max(first, 32)
            if first == 0:
                parts = [k_s[g, pl.ds(base, 8), :], k_s[g, pl.ds(base + 128, 8), :],
                         k_s[g, pl.ds(base + 8, 8), :], k_s[g, pl.ds(base + 136, 8), :]]
            else:
                parts = [k_s[g, pl.ds(base + 128, 16), :]]
            if mid0 < 256:
                parts.append(k_s[g, pl.ds(base + mid0 // 2, (256 - mid0) // 2), :])
            kw = pltpu.bitcast(jnp.concatenate(parts, axis=0), bf16)
            qu = q_s[g, pl.ds(base, 16), :]
            qall = pltpu.bitcast(
                jnp.concatenate([jnp.where(hb16 == (p - b) % 4, qu, jnp.uint32(0)) for p in range(4)], axis=0),
                bf16)
            st = lax.dot_general(kw, qall, NT, preferred_element_type=f32)
            if b == 0:
                first_rows = st[0:8]
            if first == 0:
                c0 = jnp.where(dd > 0, st[0:16], st[16:32])
                c1 = jnp.where(dd > -16, st[32:48], st[48:64])
                mid = st[64:]
            else:
                c0 = jnp.where(dd > 0, NEG, st[0:16])
                c1 = jnp.where(dd > -16, NEG, st[16:32])
                mid = st[32:]
            s_s[slot, b, 0:16, :] = c0
            s_s[slot, b, 16:32, :] = c1
            x = jnp.concatenate([c0, c1], axis=0)
            if mid0 < 256:
                s_s[slot, b, mid0:256, :] = mid
                x = jnp.concatenate([x, mid], axis=0)
            mm = jnp.max(x.reshape(x.shape[0] // 8, 8, 128), axis=0)
            m_s[slot, b] = jnp.broadcast_to(jnp.max(mm, axis=0, keepdims=True), (8, 128))
        return first_rows

    def pv_stage(g, q0, slot, gate, kstart):
        r8 = lax.broadcasted_iota(i32, (8, 128), 0)
        c8 = lax.broadcasted_iota(i32, (8, 128), 1) + pltpu.bitcast(z_s[...], i32)
        blk = c8 // 32
        j = c8 % 32

        def tri(u):
            return (jnp.where(16 * u + r8 > j, jnp.uint32(0xFFFF), jnp.uint32(0)) |
                    jnp.where(16 * u + 8 + r8 > j, jnp.uint32(0xFFFF0000), jnp.uint32(0)))

        tris = [tri(0), tri(1)] if kstart < 128 else None
        ms = [m_s[slot, b] for b in range(4)]
        L = [None] * 4
        cache = {}

        def pexp(b, u):
            x = s_s[slot, b, 16 * u:16 * u + 16, :]
            p0 = jnp.exp2(x[0:8] - ms[b])
            p1 = jnp.exp2(x[8:16] - ms[b])
            sm = p0 + p1
            L[b] = sm if L[b] is None else L[b] + sm
            return pltpu.pack_elementwise([p0, p1], packed_dtype=bf16)

        def get_p(b, u):
            first = max(0, kstart - 32 * b)
            if u < 0 or u >= 18 or 16 * u < first:
                return None
            if first > 0:
                return pexp(b, u - 16) if u >= 16 else pexp(b, u)
            if u < 2 or u >= 16:
                if (b, u) not in cache:
                    pk = pexp(b, u % 16)
                    lo = pk & tris[u % 16]
                    cache[(b, u % 16)] = lo
                    cache[(b, u % 16 + 16)] = pk ^ lo
                return cache.pop((b, u))
            return pexp(b, u)

        zero = jnp.zeros((8, 128), u32)
        accs = [None] * 4
        for k in [k for k in B_ORDER if k >= kstart // 128]:
            wts = [[] for _ in range(4)]
            for t in range(8 * k, 8 * k + 8):
                if t == B_GATE_T and gate is not None:
                    gv = gate * z_s[...]
                    for b in range(4):
                        ms[b] = ms[b] + gv
                srcs = [(b, get_p(b, t - 2 * b)) for b in range(4)]
                srcs = [(b, v) for (b, v) in srcs if v is not None]
                for h in range(4):
                    acc = zero if len(srcs) < 4 else None
                    for (b, v) in srcs:
                        acc = v if acc is None else jnp.where(blk == (h + b) % 4, v, acc)
                    wts[h].append(acc)
            c0 = q0 + 128 * k
            if not isinstance(c0, int):
                c0 = pl.multiple_of(c0, 128)
            for h in range(4):
                pt = pltpu.bitcast(jnp.concatenate(wts[h], axis=0), bf16)
                vth = pltpu.bitcast(vt_s[pl.ds((g * 4 + h) * 16, 16), pl.ds(c0, 128)], bf16)
                d = jnp.dot(vth, pt, preferred_element_type=f32)
                accs[h] = d if accs[h] is None else accs[h] + d
        L = [jnp.broadcast_to(jnp.sum(l, axis=0, keepdims=True), (8, 128)) for l in L]
        outs = []
        for h in range(4):
            lh = L[0]
            for b in range(1, 4):
                lh = jnp.where(blk == (h + b) % 4, L[b], lh)
            r0 = pl.reciprocal(lh, approx=True)
            rl = r0 * (2.0 - lh * r0)
            ot = (accs[h].reshape(4, 8, 128) * rl[None]).reshape(32, 128)
            if h > 0:
                ot = pltpu.roll(ot, 128 - 32 * h, axis=1)
            outs.append(ot)
        ot_s[g * 64:(g + 1) * 64, pl.ds(q0, 128)] = _pack_rows_interleaved(jnp.concatenate(outs, axis=0))

    def sub_block(q0, qn):
        for g in range(G):
            if g + 1 < G:
                gate = qk_stage(g + 1, q0, (g + 1) % 2, 0)
            else:
                gate = qk_stage(0, qn, 0, 0)
            pv_stage(g, q0, g % 2, gate, 0)

    def transpose_o(i, o_dst):
        r0 = i * TQ
        if not isinstance(r0, int):
            r0 = pl.multiple_of(r0, TQ)
        o_dst[...] = pltpu.bitcast(pltpu.bitcast(ot_s[:, pl.ds(r0, TQ)], bf16).T, u32)

    def phase_b():
        qk_stage(0, 0, 2, PAD)
        qk_stage(0, 128, 0, PAD - 128)
        for g in range(G):
            if g + 1 < G:
                qk_stage(g + 1, 0, 2 + (g + 1) % 2, PAD)
            pv_stage(g, 0, 2 + g % 2, None, PAD)
            if g + 1 < G:
                qk_stage(g + 1, 128, (g + 1) % 2, PAD - 128)
            else:
                qk_stage(0, 256, 0, 0)
            pv_stage(g, 128, g % 2, None, PAD - 128)
        transpose_o(0, oa)

        def body(j, c):
            q0 = pl.multiple_of(j * 256, 256)
            q1 = pl.multiple_of(q0 + 128, 128)
            qn = pl.multiple_of(jnp.minimum(q0 + 256, S - 128), 128)
            sub_block(q0, q1)
            sub_block(q1, qn)
            return c

        lax.fori_loop(1, NSB // 2, body, 0)

    def resid_chunk(i, c, at_ref, gate):
        r0 = i * TQ + c * CHC
        if not isinstance(r0, int):
            r0 = pl.multiple_of(r0, CHC)
        x1 = xbuf[pl.ds(r0, CHC), :] + at_ref[c * CHC:(c + 1) * CHC, :]
        if gate is not None:
            x1 = _gate_first(x1, gate, z_s[...])
        m = jnp.mean(x1, axis=-1, keepdims=True)
        xc = x1 - m
        v = jnp.mean(xc * xc, axis=-1, keepdims=True)
        rho = lax.rsqrt(v + EPS)
        xn = xc * rho
        r = jnp.sum(xn * wr8[0:1, :], axis=-1, keepdims=True)
        rb = jnp.broadcast_to(r, (CHC, 128)).astype(bf16).astype(f32)
        rows = lax.broadcasted_iota(i32, (8, 128), 0) + r0
        bv, bi = best_v[...], best_i[...]
        for q in range(CHC // 8):
            cand = rb[8 * q:8 * q + 8]
            better = cand > bv
            bv = jnp.where(better, cand, bv)
            bi = jnp.where(better, rows + 8 * q, bi)
        best_v[...] = bv
        best_i[...] = bi
        rho_s[pl.ds(r0, CHC), :] = jnp.broadcast_to(rho, (CHC, 128))
        x2 = x1 + xn
        xres[pl.ds(r0, CHC), :] = x2
        xio[pl.ds(r0, CHC), :] = x2.astype(bf16)

    def oproj_step(o_src, at_w, i_res, at_r, i_t, o_dst):
        ys = []
        if o_src is not None:
            a = pltpu.bitcast(o_src[...], bf16)
            for n in range(G):
                y = jnp.dot(a, pltpu.bitcast(wop_v[:, n * 128:(n + 1) * 128], bf16), preferred_element_type=f32)
                at_w[:, n * 128:(n + 1) * 128] = y
                ys.append(y)
        if i_t is not None:
            transpose_o(i_t, o_dst)
        if i_res is not None:
            for c in range(NCHC):
                gi = GATE_C[c] if ys else -1
                resid_chunk(i_res, c, at_r, ys[gi] if gi >= 0 else None)

    def phase_c(layer):
        @pl.when(layer == 0)
        def _():
            cp_wr.wait()
            wr8[...] = jnp.broadcast_to(wr_v[...].astype(f32).reshape(1, D), (8, D))

        def flush(i):
            @pl.when(layer == 1)
            def _():
                out_copy(i).start()

        best_v[...] = jnp.full((8, 128), -jnp.inf, f32)
        best_i[...] = jnp.zeros((8, 128), i32)
        oproj_step(oa, ata, None, None, 1, ob)

        def body(j, c):
            i0 = 2 * j
            oproj_step(ob, atb, i0, ata, i0 + 2, oa)
            oproj_step(oa, ata, i0 + 1, atb, i0 + 3, ob)
            flush(i0)
            flush(i0 + 1)
            return c

        lax.fori_loop(0, NB // 2 - 1, body, 0)
        oproj_step(ob, atb, NB - 2, ata, None, None)
        oproj_step(None, None, NB - 1, atb, None, None)
        flush(NB - 2)
        flush(NB - 1)

    def phase_d(layer):
        @pl.when(layer == 0)
        def _():
            cp_wg.wait()
            cp_wu.wait()
            cp_wd.wait()

        bv = best_v[...]
        rmax = jnp.max(bv)
        idx = jnp.min(jnp.where(bv == rmax, best_i[...], S))
        idx = jnp.clip(idx, 0, S - 1)
        x2 = xres[pl.ds(idx, 1), :]
        rho = rho_s[pl.ds(idx, 1), 0:1]
        xn = (x2 - jnp.mean(x2, axis=-1, keepdims=True)) * (rho / (1.0 + rho))
        xs = jnp.broadcast_to(xn, (16, D)).astype(bf16)
        nf = F // FC
        hs = []
        y = None
        for c in range(nf + 1):
            if c < nf:
                gate = jnp.dot(xs, wg_v[:, c * FC:(c + 1) * FC], preferred_element_type=f32)
                up = jnp.dot(xs, wu_v[:, c * FC:(c + 1) * FC], preferred_element_type=f32)
                hs.append((gate * jax.nn.sigmoid(gate) * up).astype(bf16))
            if c > 0:
                d = jnp.dot(hs[c - 1], wd_v[(c - 1) * FC:c * FC, :], preferred_element_type=f32)
                y = d if y is None else y + d
        scale = jax.nn.sigmoid(jnp.full((1, D), rmax, f32))
        xres[pl.ds(idx, 1), :] = xres[pl.ds(idx, 1), :] + y[0:1] * scale

        @pl.when(layer == 1)
        def _():
            for i in range(NB):
                out_copy(i).wait()
            g0 = pl.multiple_of((idx // 16) * 16, 16)
            xio[pl.ds(g0, 16), :] = xres[pl.ds(g0, 16), :].astype(bf16)
            fix = pltpu.make_async_copy(xio.at[pl.ds(g0, 16), :], out_hbm.at[pl.ds(g0, 16), :], sem_w.at[7])
            fix.start()
            fix.wait()

    def layer_body(layer, c):
        with jax.named_scope("phase_a"):
            phase_a(layer)
        with jax.named_scope("phase_b"):
            phase_b()
        with jax.named_scope("phase_c"):
            phase_c(layer)
        with jax.named_scope("phase_d"):
            phase_d(layer)
        return c

    lax.fori_loop(0, 2, layer_body, 0)


@jax.jit
def pallas_interleave_layers__sliding_block__moe_arch_mod__prompt_kernel(
    A_x: jax.Array,
    A_wqkv: jax.Array,
    A_wo: jax.Array,
    B_x: jax.Array,
    B_w_r: jax.Array,
    B_w_gate: jax.Array,
    B_w_up: jax.Array,
    B_w_down: jax.Array,
):
    del B_x
    x = A_x.reshape(S, D)
    any_spec = pl.BlockSpec(memory_space=pl.ANY)
    scratch = [
        pltpu.VMEM((S, D), bf16),
        pltpu.VMEM((D, D), bf16),
        pltpu.VMEM((D, D), bf16),
        pltpu.VMEM((D, D), bf16),
        pltpu.VMEM((D // 2, D), u32),
        pltpu.VMEM((D, D), bf16),
        pltpu.VMEM((D // 2, D), u32),
        pltpu.VMEM((D,), bf16),
        pltpu.VMEM((D, F), bf16),
        pltpu.VMEM((D, F), bf16),
        pltpu.VMEM((F, D), bf16),
        pltpu.VMEM((S, D), f32),
        pltpu.VMEM((S, D), f32),
        pltpu.VMEM((8, 128), f32),
        pltpu.VMEM((8, 128), i32),
        pltpu.VMEM((S, 128), f32),
        pltpu.VMEM((8, 128), f32),
        pltpu.VMEM((8, D), f32),
        pltpu.VMEM((TQ // 2, D), u32),
        pltpu.VMEM((TQ // 2, D), u32),
        pltpu.VMEM((S // 2, D), u32),
        pltpu.VMEM((S // 2, D), u32),
        pltpu.VMEM((G, S // 2, 128), u32),
        pltpu.VMEM((G, (S + PAD) // 2, 128), u32),
        pltpu.VMEM((D // 2, S + PAD), u32),
        pltpu.VMEM((D // 2, S), u32),
        pltpu.VMEM((4, 4, 256, 128), f32),
        pltpu.VMEM((4, 4, 8, 128), f32),
        pltpu.VMEM((TQ, D), f32),
        pltpu.VMEM((TQ, D), f32),
        pltpu.VMEM((TQ // 2, D), u32),
        pltpu.VMEM((TQ // 2, D), u32),
        pltpu.SemaphoreType.DMA((NB,)),
        pltpu.SemaphoreType.DMA((10,)),
        pltpu.SemaphoreType.DMA((NB,)),
    ]
    out = pl.pallas_call(
        _kernel,
        out_shape=jax.ShapeDtypeStruct((S, D), bf16),
        in_specs=[any_spec] * 7,
        out_specs=any_spec,
        scratch_shapes=scratch,
        compiler_params=pltpu.CompilerParams(vmem_limit_bytes=120 * 1024 * 1024),
    )(x, A_wqkv, A_wo, B_w_r, B_w_gate, B_w_up, B_w_down)
    return out.reshape(1, S, D)
```

```python
import jax
import jax.numpy as jnp
from jax import lax
import jax.experimental.pallas as pl
import jax.experimental.pallas.tpu as pltpu

bf16 = jnp.bfloat16
f32 = jnp.float32
u32 = jnp.uint32
i32 = jnp.int32

S = 2048
D = 1024
H = 32
DH = 32
W = 256
F = 3584
G = 8
PAD = 256
TQ = 256
NB = S // TQ
TKV = 512
NSB = S // 128
CH = 32
LNR = 8
NCH = TQ // CH
CHC = 8
NCHC = TQ // CHC
FC = 256
GATE_A = [c * 8 // NCH - 1 for c in range(NCH)]
CHAIN_A = 3
GATE_C = [c * 8 // NCHC - 1 for c in range(NCHC)]
B_ORDER = [1, 0, 2]
B_GATE_T = 6
EPS = 1e-5
NEG = -1e30
QSCALE = (DH ** -0.5) * 1.4426950408889634
NT = (((1,), (1,)), ((), ()))


def _ln(x):
    m = jnp.mean(x, axis=-1, keepdims=True)
    xc = x - m
    v = jnp.mean(xc * xc, axis=-1, keepdims=True)
    return xc * lax.rsqrt(v + EPS)


def _pack_rows(x):
    return pltpu.bitcast(x.astype(bf16), u32)


def _pack_rows_interleaved(x):
    n = x.shape[0] // 16
    x3 = x.reshape(n, 16, x.shape[1])
    a = x3[:, 0:8, :].reshape(n * 8, x.shape[1])
    b = x3[:, 8:16, :].reshape(n * 8, x.shape[1])
    return pltpu.pack_elementwise([a, b], packed_dtype=bf16)


def _gate_first(x, gate, z):
    g = gate[0:8, 0:128] * z
    top = jnp.concatenate([x[0:8, 0:128] + g, x[0:8, 128:]], axis=1)
    return top if x.shape[0] == 8 else jnp.concatenate([top, x[8:]], axis=0)


def _latin_merge(src, blk):
    present = [v for v in src if v is not None]
    zero = jnp.zeros_like(present[0])

    def sel(mask, x, y):
        if x is None and y is None:
            return None
        return jnp.where(mask, zero if x is None else x, zero if y is None else y)

    if len(present) == 1:
        b = [v is not None for v in src].index(True)
        return [jnp.where(blk == (h + b) % 4, src[b], zero) for h in range(4)]
    odd = (blk & 1) == 1
    low = blk < 2
    pair = [sel(odd, src[(a + 1) % 4], src[a]) for a in range(4)]
    out = [sel(low, pair[(-h) % 4], pair[(2 - h) % 4]) for h in range(4)]
    return [zero if v is None else v for v in out]


def _kernel(x_hbm, wqkv_hbm, wo_hbm, wr_hbm, wg_hbm, wu_hbm, wd_hbm,
            out_hbm,
            xio, wq_v, wk_v, wv_v, wvt_v, wo_v, wop_v, wr_v, wg_v, wu_v, wd_v,
            xres, xbuf, best_v, best_i, rho_s, z_s, wr8,
            xca, xcb, xc_all, xi_all,
            q_s, k_s, vt_s, ot_s, s_s, m_s,
            ata, atb, oa, ob,
            sem_x, sem_w, sem_o):
    def x_copy(i):
        r0 = pl.multiple_of(i * TQ, TQ)
        return pltpu.make_async_copy(x_hbm.at[pl.ds(r0, TQ), :], xio.at[pl.ds(r0, TQ), :], sem_x.at[i])

    def out_copy(i):
        r0 = pl.multiple_of(i * TQ, TQ)
        return pltpu.make_async_copy(xio.at[pl.ds(r0, TQ), :], out_hbm.at[pl.ds(r0, TQ), :], sem_o.at[i])

    cp_wqa = pltpu.make_async_copy(wqkv_hbm.at[:, pl.ds(0, D // 2)], wq_v.at[:, pl.ds(0, D // 2)], sem_w.at[0])
    cp_wqb = pltpu.make_async_copy(wqkv_hbm.at[:, pl.ds(D // 2, D // 2)], wq_v.at[:, pl.ds(D // 2, D // 2)],
                                   sem_w.at[9])
    cp_wk = pltpu.make_async_copy(wqkv_hbm.at[:, pl.ds(D, D)], wk_v, sem_w.at[1])
    cp_wv = pltpu.make_async_copy(wqkv_hbm.at[:, pl.ds(2 * D, D)], wv_v, sem_w.at[8])
    cp_wo = pltpu.make_async_copy(wo_hbm, wo_v, sem_w.at[2])
    cp_wr = pltpu.make_async_copy(wr_hbm, wr_v, sem_w.at[3])
    cp_wg = pltpu.make_async_copy(wg_hbm, wg_v, sem_w.at[4])
    cp_wu = pltpu.make_async_copy(wu_hbm, wu_v, sem_w.at[5])
    cp_wd = pltpu.make_async_copy(wd_hbm, wd_v, sem_w.at[6])

    x_copy(0).start()
    cp_wqa.start()

    z_s[...] = jnp.zeros_like(z_s)
    xres[0:CH, :] = jnp.zeros((CH, D), f32)

    def ln_chunk(layer, i, c, xc_ref, gate, chain=None):
        r0 = i * TQ + c * CH
        h0 = i * (TQ // 2) + c * (CH // 2)
        if not isinstance(r0, int):
            r0 = pl.multiple_of(r0, CH)
            h0 = pl.multiple_of(h0, CH // 2)
        parts = []
        for q in range(CH // LNR):
            rq = r0 + q * LNR
            x_in = xio[pl.ds(rq, LNR), :].astype(f32)
            x_rs = xres[pl.ds(pl.multiple_of(rq * layer, LNR), LNR), :]
            xq = jnp.where(layer == 0, x_in, x_rs)
            xbuf[pl.ds(rq, LNR), :] = xq
            if chain is not None and len(chain) >= CHAIN_A:
                xq = _gate_first(xq, chain[-CHAIN_A], z_s[...])
            elif gate is not None:
                xq = _gate_first(xq, gate, z_s[...])
            parts.append(_ln(xq))
            if chain is not None:
                chain.append(parts[-1])
        xn = jnp.concatenate(parts, axis=0)
        xc = _pack_rows(xn)
        xc_ref[c * CH // 2:(c + 1) * CH // 2, :] = xc
        xc_all[pl.ds(h0, CH // 2), :] = xc
        xi_all[pl.ds(h0, CH // 2), :] = _pack_rows_interleaved(xn)

    def q_step(layer, i, xc_ref, i_next, xc_next, part=(0, G)):
        h0 = i * (TQ // 2)
        if not isinstance(h0, int):
            h0 = pl.multiple_of(h0, TQ // 2)
        a = pltpu.bitcast(xc_ref[...], bf16)
        ys = {}
        for n in range(*part):
            y = jnp.dot(a, wq_v[:, n * 128:(n + 1) * 128], preferred_element_type=f32)
            q_s[n, pl.ds(h0, TQ // 2), :] = _pack_rows(y * QSCALE)
            ys[n] = y
        if i_next is not None:
            chain = []
            for c in range(part[0] * NCH // G, part[1] * NCH // G):
                ln_chunk(layer, i_next, c, xc_next, ys.get(GATE_A[c]), chain)

    def kv_step(i):
        h0 = pl.multiple_of(i * (TKV // 2), TKV // 2)
        a = pltpu.bitcast(xc_all[pl.ds(h0, TKV // 2), :], bf16)
        for n in range(G):
            y = jnp.dot(a, wk_v[:, n * 128:(n + 1) * 128], preferred_element_type=f32)
            k_s[n, pl.ds(PAD // 2 + h0, TKV // 2), :] = _pack_rows(y)
        vt = lax.dot_general(pltpu.bitcast(wvt_v[...], bf16), pltpu.bitcast(xi_all[pl.ds(h0, TKV // 2), :], bf16),
                             NT, preferred_element_type=f32)
        c0 = pl.multiple_of(PAD + i * TKV, 256)
        vt_s[:, pl.ds(c0, TKV)] = _pack_rows(vt)

    def phase_a(layer):
        @pl.when(layer == 0)
        def _():
            x_copy(0).wait()
            x_copy(1).start()
            cp_wqb.start()

        for c in range(NCH):
            ln_chunk(layer, 0, c, xca, None)

        @pl.when(layer == 0)
        def _():
            cp_wqa.wait()
            x_copy(1).wait()
            for i in range(2, NB):
                x_copy(i).start()

        q_step(layer, 0, xca, 1, xcb, part=(0, G // 2))

        @pl.when(layer == 0)
        def _():
            cp_wqb.wait()
            cp_wv.start()
            cp_wo.start()
            cp_wk.start()
            cp_wr.start()

        q_step(layer, 0, xca, 1, xcb, part=(G // 2, G))

        def q_body(j, c):
            i1 = 2 * j + 1

            @pl.when(layer == 0)
            def _():
                x_copy(i1 + 1).wait()
                x_copy(i1 + 2).wait()

            q_step(layer, i1, xcb, i1 + 1, xca)
            q_step(layer, i1 + 1, xca, i1 + 2, xcb)
            return c

        with jax.named_scope("a_q"):
            lax.fori_loop(0, NB // 2 - 1, q_body, 0)

        @pl.when(layer == 0)
        def _():
            cp_wv.wait()
            cp_wo.wait()

        q_step(layer, NB - 1, xcb, None, None)
        wvt_v[...] = pltpu.bitcast(wv_v[...].T, u32)
        for c in range(D // 64):
            wop_v[c * 32:(c + 1) * 32, :] = _pack_rows_interleaved(wo_v[c * 64:(c + 1) * 64, :].astype(f32))

        @pl.when(layer == 0)
        def _():
            cp_wk.wait()
            cp_wg.start()
            cp_wu.start()
            cp_wd.start()

        def kv_body(j, c):
            kv_step(j)
            return c

        with jax.named_scope("a_kv"):
            lax.fori_loop(0, S // TKV, kv_body, 0)

    def qk_stage(g, q0, slot, kstart):
        zi = pltpu.bitcast(z_s[...], i32)
        zi16 = jnp.concatenate([zi, zi], axis=0)
        lane16 = lax.broadcasted_iota(i32, (16, 128), 1) + zi16
        r16 = lax.broadcasted_iota(i32, (16, 128), 0)
        hb16 = lane16 // 32
        dd = r16 - lane16 % 32
        h0 = q0 // 2
        first_rows = None
        for b in range(4):
            first = max(0, kstart - 32 * b)
            base = h0 + 16 * b
            if not isinstance(base, int):
                base = pl.multiple_of(base, 16)
            mid0 = max(first, 32)
            if first == 0:
                parts = [k_s[g, pl.ds(base, 8), :], k_s[g, pl.ds(base + 128, 8), :],
                         k_s[g, pl.ds(base + 8, 8), :], k_s[g, pl.ds(base + 136, 8), :]]
            else:
                parts = [k_s[g, pl.ds(base + 128, 16), :]]
            if mid0 < 256:
                parts.append(k_s[g, pl.ds(base + mid0 // 2, (256 - mid0) // 2), :])
            kw = pltpu.bitcast(jnp.concatenate(parts, axis=0), bf16)
            qu = q_s[g, pl.ds(base, 16), :]
            qall = pltpu.bitcast(
                jnp.concatenate([jnp.where(hb16 == (p - b) % 4, qu, jnp.uint32(0)) for p in range(4)], axis=0),
                bf16)
            st = lax.dot_general(kw, qall, NT, preferred_element_type=f32)
            if b == 0:
                first_rows = st[0:8]
            if first == 0:
                c0 = jnp.where(dd > 0, st[0:16], st[16:32])
                c1 = jnp.where(dd > -16, st[32:48], st[48:64])
                mid = st[64:]
            else:
                c0 = jnp.where(dd > 0, NEG, st[0:16])
                c1 = jnp.where(dd > -16, NEG, st[16:32])
                mid = st[32:]
            s_s[slot, b, 0:16, :] = c0
            s_s[slot, b, 16:32, :] = c1
            x = jnp.concatenate([c0, c1], axis=0)
            if mid0 < 256:
                s_s[slot, b, mid0:256, :] = mid
                x = jnp.concatenate([x, mid], axis=0)
            mm = jnp.max(x.reshape(x.shape[0] // 8, 8, 128), axis=0)
            m_s[slot, b] = jnp.broadcast_to(jnp.max(mm, axis=0, keepdims=True), (8, 128))
        return first_rows

    def pv_stage(g, q0, slot, gate, kstart):
        r8 = lax.broadcasted_iota(i32, (8, 128), 0)
        c8 = lax.broadcasted_iota(i32, (8, 128), 1) + pltpu.bitcast(z_s[...], i32)
        blk = c8 // 32
        j = c8 % 32

        def tri(u):
            return (jnp.where(16 * u + r8 > j, jnp.uint32(0xFFFF), jnp.uint32(0)) |
                    jnp.where(16 * u + 8 + r8 > j, jnp.uint32(0xFFFF0000), jnp.uint32(0)))

        tris = [tri(0), tri(1)] if kstart < 128 else None
        ms = [m_s[slot, b] for b in range(4)]
        L = [None] * 4
        cache = {}

        def pexp(b, u):
            x = s_s[slot, b, 16 * u:16 * u + 16, :]
            p0 = jnp.exp2(x[0:8] - ms[b])
            p1 = jnp.exp2(x[8:16] - ms[b])
            sm = p0 + p1
            L[b] = sm if L[b] is None else L[b] + sm
            return pltpu.pack_elementwise([p0, p1], packed_dtype=bf16)

        def get_p(b, u):
            first = max(0, kstart - 32 * b)
            if u < 0 or u >= 18 or 16 * u < first:
                return None
            if first > 0:
                return pexp(b, u - 16) if u >= 16 else pexp(b, u)
            if u < 2 or u >= 16:
                if (b, u) not in cache:
                    pk = pexp(b, u % 16)
                    lo = pk & tris[u % 16]
                    cache[(b, u % 16)] = lo
                    cache[(b, u % 16 + 16)] = pk ^ lo
                return cache.pop((b, u))
            return pexp(b, u)

        accs = [None] * 4
        for k in [k for k in B_ORDER if k >= kstart // 128]:
            wts = [[] for _ in range(4)]
            for t in range(8 * k, 8 * k + 8):
                if t == B_GATE_T and gate is not None:
                    gv = gate * z_s[...]
                    for b in range(4):
                        ms[b] = ms[b] + gv
                src = [get_p(b, t - 2 * b) for b in range(4)]
                for h, w in enumerate(_latin_merge(src, blk)):
                    wts[h].append(w)
            c0 = q0 + 128 * k
            if not isinstance(c0, int):
                c0 = pl.multiple_of(c0, 128)
            for h in range(4):
                pt = pltpu.bitcast(jnp.concatenate(wts[h], axis=0), bf16)
                vth = pltpu.bitcast(vt_s[pl.ds((g * 4 + h) * 16, 16), pl.ds(c0, 128)], bf16)
                d = jnp.dot(vth, pt, preferred_element_type=f32)
                accs[h] = d if accs[h] is None else accs[h] + d
        L = [jnp.broadcast_to(jnp.sum(l, axis=0, keepdims=True), (8, 128)) for l in L]
        outs = []
        for h, lh in enumerate(_latin_merge(L, blk)):
            r0 = pl.reciprocal(lh, approx=True)
            rl = r0 * (2.0 - lh * r0)
            ot = (accs[h].reshape(4, 8, 128) * rl[None]).reshape(32, 128)
            if h > 0:
                ot = pltpu.roll(ot, 128 - 32 * h, axis=1)
            outs.append(ot)
        ot_s[g * 64:(g + 1) * 64, pl.ds(q0, 128)] = _pack_rows_interleaved(jnp.concatenate(outs, axis=0))

    def sub_block(q0, qn):
        for g in range(G):
            if g + 1 < G:
                gate = qk_stage(g + 1, q0, (g + 1) % 2, 0)
            else:
                gate = qk_stage(0, qn, 0, 0)
            pv_stage(g, q0, g % 2, gate, 0)

    def transpose_o(i, o_dst):
        r0 = i * TQ
        if not isinstance(r0, int):
            r0 = pl.multiple_of(r0, TQ)
        o_dst[...] = pltpu.bitcast(pltpu.bitcast(ot_s[:, pl.ds(r0, TQ)], bf16).T, u32)

    def phase_b():
        qk_stage(0, 0, 2, PAD)
        qk_stage(0, 128, 0, PAD - 128)
        for g in range(G):
            if g + 1 < G:
                qk_stage(g + 1, 0, 2 + (g + 1) % 2, PAD)
            pv_stage(g, 0, 2 + g % 2, None, PAD)
            if g + 1 < G:
                qk_stage(g + 1, 128, (g + 1) % 2, PAD - 128)
            else:
                qk_stage(0, 256, 0, 0)
            pv_stage(g, 128, g % 2, None, PAD - 128)
        transpose_o(0, oa)

        def body(j, c):
            q0 = pl.multiple_of(j * 256, 256)
            q1 = pl.multiple_of(q0 + 128, 128)
            qn = pl.multiple_of(jnp.minimum(q0 + 256, S - 128), 128)
            sub_block(q0, q1)
            sub_block(q1, qn)
            return c

        lax.fori_loop(1, NSB // 2, body, 0)

    def resid_chunk(i, c, at_ref, gate):
        r0 = i * TQ + c * CHC
        if not isinstance(r0, int):
            r0 = pl.multiple_of(r0, CHC)
        x1 = xbuf[pl.ds(r0, CHC), :] + at_ref[c * CHC:(c + 1) * CHC, :]
        if gate is not None:
            x1 = _gate_first(x1, gate, z_s[...])
        m = jnp.mean(x1, axis=-1, keepdims=True)
        xc = x1 - m
        v = jnp.mean(xc * xc, axis=-1, keepdims=True)
        rho = lax.rsqrt(v + EPS)
        xn = xc * rho
        r = jnp.sum(xn * wr8[0:1, :], axis=-1, keepdims=True)
        rb = jnp.broadcast_to(r, (CHC, 128)).astype(bf16).astype(f32)
        rows = lax.broadcasted_iota(i32, (8, 128), 0) + r0
        bv, bi = best_v[...], best_i[...]
        for q in range(CHC // 8):
            cand = rb[8 * q:8 * q + 8]
            better = cand > bv
            bv = jnp.where(better, cand, bv)
            bi = jnp.where(better, rows + 8 * q, bi)
        best_v[...] = bv
        best_i[...] = bi
        rho_s[pl.ds(r0, CHC), :] = jnp.broadcast_to(rho, (CHC, 128))
        x2 = x1 + xn
        xres[pl.ds(r0, CHC), :] = x2
        xio[pl.ds(r0, CHC), :] = x2.astype(bf16)

    def oproj_step(o_src, at_w, i_res, at_r, i_t, o_dst):
        ys = []
        if o_src is not None:
            a = pltpu.bitcast(o_src[...], bf16)
            for n in range(G):
                y = jnp.dot(a, pltpu.bitcast(wop_v[:, n * 128:(n + 1) * 128], bf16), preferred_element_type=f32)
                at_w[:, n * 128:(n + 1) * 128] = y
                ys.append(y)
        if i_t is not None:
            transpose_o(i_t, o_dst)
        if i_res is not None:
            for c in range(NCHC):
                gi = GATE_C[c] if ys else -1
                resid_chunk(i_res, c, at_r, ys[gi] if gi >= 0 else None)

    def phase_c(layer):
        @pl.when(layer == 0)
        def _():
            cp_wr.wait()
            wr8[...] = jnp.broadcast_to(wr_v[...].astype(f32).reshape(1, D), (8, D))

        def flush(i):
            @pl.when(layer == 1)
            def _():
                out_copy(i).start()

        best_v[...] = jnp.full((8, 128), -jnp.inf, f32)
        best_i[...] = jnp.zeros((8, 128), i32)
        oproj_step(oa, ata, None, None, 1, ob)

        def body(j, c):
            i0 = 2 * j
            oproj_step(ob, atb, i0, ata, i0 + 2, oa)
            oproj_step(oa, ata, i0 + 1, atb, i0 + 3, ob)
            flush(i0)
            flush(i0 + 1)
            return c

        lax.fori_loop(0, NB // 2 - 1, body, 0)
        oproj_step(ob, atb, NB - 2, ata, None, None)
        oproj_step(None, None, NB - 1, atb, None, None)
        flush(NB - 2)
        flush(NB - 1)

    def phase_d(layer):
        @pl.when(layer == 0)
        def _():
            cp_wg.wait()
            cp_wu.wait()
            cp_wd.wait()

        bv = best_v[...]
        rmax = jnp.max(bv)
        idx = jnp.min(jnp.where(bv == rmax, best_i[...], S))
        idx = jnp.clip(idx, 0, S - 1)
        x2 = xres[pl.ds(idx, 1), :]
        rho = rho_s[pl.ds(idx, 1), 0:1]
        xn = (x2 - jnp.mean(x2, axis=-1, keepdims=True)) * (rho / (1.0 + rho))
        xs = jnp.broadcast_to(xn, (16, D)).astype(bf16)
        nf = F // FC
        hs = []
        y = None
        for c in range(nf + 1):
            if c < nf:
                gate = jnp.dot(xs, wg_v[:, c * FC:(c + 1) * FC], preferred_element_type=f32)
                up = jnp.dot(xs, wu_v[:, c * FC:(c + 1) * FC], preferred_element_type=f32)
                hs.append((gate * jax.nn.sigmoid(gate) * up).astype(bf16))
            if c > 0:
                d = jnp.dot(hs[c - 1], wd_v[(c - 1) * FC:c * FC, :], preferred_element_type=f32)
                y = d if y is None else y + d
        scale = jax.nn.sigmoid(jnp.full((1, D), rmax, f32))
        xres[pl.ds(idx, 1), :] = xres[pl.ds(idx, 1), :] + y[0:1] * scale

        @pl.when(layer == 1)
        def _():
            for i in range(NB):
                out_copy(i).wait()
            g0 = pl.multiple_of((idx // 16) * 16, 16)
            xio[pl.ds(g0, 16), :] = xres[pl.ds(g0, 16), :].astype(bf16)
            fix = pltpu.make_async_copy(xio.at[pl.ds(g0, 16), :], out_hbm.at[pl.ds(g0, 16), :], sem_w.at[7])
            fix.start()
            fix.wait()

    def layer_body(layer, c):
        with jax.named_scope("phase_a"):
            phase_a(layer)
        with jax.named_scope("phase_b"):
            phase_b()
        with jax.named_scope("phase_c"):
            phase_c(layer)
        with jax.named_scope("phase_d"):
            phase_d(layer)
        return c

    lax.fori_loop(0, 2, layer_body, 0)


@jax.jit
def pallas_interleave_layers__sliding_block__moe_arch_mod__prompt_kernel(
    A_x: jax.Array,
    A_wqkv: jax.Array,
    A_wo: jax.Array,
    B_x: jax.Array,
    B_w_r: jax.Array,
    B_w_gate: jax.Array,
    B_w_up: jax.Array,
    B_w_down: jax.Array,
):
    del B_x
    x = A_x.reshape(S, D)
    any_spec = pl.BlockSpec(memory_space=pl.ANY)
    scratch = [
        pltpu.VMEM((S, D), bf16),
        pltpu.VMEM((D, D), bf16),
        pltpu.VMEM((D, D), bf16),
        pltpu.VMEM((D, D), bf16),
        pltpu.VMEM((D // 2, D), u32),
        pltpu.VMEM((D, D), bf16),
        pltpu.VMEM((D // 2, D), u32),
        pltpu.VMEM((D,), bf16),
        pltpu.VMEM((D, F), bf16),
        pltpu.VMEM((D, F), bf16),
        pltpu.VMEM((F, D), bf16),
        pltpu.VMEM((S, D), f32),
        pltpu.VMEM((S, D), f32),
        pltpu.VMEM((8, 128), f32),
        pltpu.VMEM((8, 128), i32),
        pltpu.VMEM((S, 128), f32),
        pltpu.VMEM((8, 128), f32),
        pltpu.VMEM((8, D), f32),
        pltpu.VMEM((TQ // 2, D), u32),
        pltpu.VMEM((TQ // 2, D), u32),
        pltpu.VMEM((S // 2, D), u32),
        pltpu.VMEM((S // 2, D), u32),
        pltpu.VMEM((G, S // 2, 128), u32),
        pltpu.VMEM((G, (S + PAD) // 2, 128), u32),
        pltpu.VMEM((D // 2, S + PAD), u32),
        pltpu.VMEM((D // 2, S), u32),
        pltpu.VMEM((4, 4, 256, 128), f32),
        pltpu.VMEM((4, 4, 8, 128), f32),
        pltpu.VMEM((TQ, D), f32),
        pltpu.VMEM((TQ, D), f32),
        pltpu.VMEM((TQ // 2, D), u32),
        pltpu.VMEM((TQ // 2, D), u32),
        pltpu.SemaphoreType.DMA((NB,)),
        pltpu.SemaphoreType.DMA((10,)),
        pltpu.SemaphoreType.DMA((NB,)),
    ]
    out = pl.pallas_call(
        _kernel,
        out_shape=jax.ShapeDtypeStruct((S, D), bf16),
        in_specs=[any_spec] * 7,
        out_specs=any_spec,
        scratch_shapes=scratch,
        compiler_params=pltpu.CompilerParams(vmem_limit_bytes=120 * 1024 * 1024),
    )(x, A_wqkv, A_wo, B_w_r, B_w_gate, B_w_up, B_w_down)
    return out.reshape(1, S, D)
```

```python
import jax
import jax.numpy as jnp
from jax import lax
import jax.experimental.pallas as pl
import jax.experimental.pallas.tpu as pltpu

bf16 = jnp.bfloat16
f32 = jnp.float32
u32 = jnp.uint32
i32 = jnp.int32

S = 2048
D = 1024
H = 32
DH = 32
W = 256
F = 3584
G = 8
PAD = 256
TQ = 256
NB = S // TQ
TKV = 512
NSB = S // 128
CH = 32
LNR = 8
NCH = TQ // CH
CHC = 8
NCHC = TQ // CHC
FC = 256
GATE_A = [c * 8 // NCH - 1 for c in range(NCH)]
CHAIN_A = 3
GATE_C = [c * 8 // NCHC - 1 for c in range(NCHC)]
B_ORDER = [1, 0, 2]
B_GATE_T = 6
EPS = 1e-5
NEG = -1e30
QSCALE = (DH ** -0.5) * 1.4426950408889634
NT = (((1,), (1,)), ((), ()))


def _ln(x):
    m = jnp.mean(x, axis=-1, keepdims=True)
    xc = x - m
    v = jnp.mean(xc * xc, axis=-1, keepdims=True)
    return xc * lax.rsqrt(v + EPS)


def _pack_rows(x):
    return pltpu.bitcast(x.astype(bf16), u32)


def _pack_rows_interleaved(x):
    n = x.shape[0] // 16
    x3 = x.reshape(n, 16, x.shape[1])
    a = x3[:, 0:8, :].reshape(n * 8, x.shape[1])
    b = x3[:, 8:16, :].reshape(n * 8, x.shape[1])
    return pltpu.pack_elementwise([a, b], packed_dtype=bf16)


def _gate_first(x, gate, z):
    g = gate[0:8, 0:128] * z
    top = jnp.concatenate([x[0:8, 0:128] + g, x[0:8, 128:]], axis=1)
    return top if x.shape[0] == 8 else jnp.concatenate([top, x[8:]], axis=0)


def _latin_merge(src, blk):
    present = [v for v in src if v is not None]
    zero = jnp.zeros_like(present[0])

    def sel(mask, x, y):
        if x is None and y is None:
            return None
        return jnp.where(mask, zero if x is None else x, zero if y is None else y)

    if len(present) == 1:
        b = [v is not None for v in src].index(True)
        return [jnp.where(blk == (h + b) % 4, src[b], zero) for h in range(4)]
    odd = (blk & 1) == 1
    low = blk < 2
    pair = [sel(odd, src[(a + 1) % 4], src[a]) for a in range(4)]
    out = [sel(low, pair[(-h) % 4], pair[(2 - h) % 4]) for h in range(4)]
    return [zero if v is None else v for v in out]


def _kernel(x_hbm, wqkv_hbm, wo_hbm, wr_hbm, wg_hbm, wu_hbm, wd_hbm,
            out_hbm,
            xio, wq_v, wk_v, wv_v, wvt_v, wo_v, wop_v, wr_v, wg_v, wu_v, wd_v,
            xres, xbuf, best_v, best_i, rho_s, z_s, wr8,
            xca, xcb, xc_all, xi_all,
            q_s, k_s, vt_s, ot_s, s_s, m_s, pend_acc, pend_l,
            ata, atb, oa, ob,
            sem_x, sem_w, sem_o):
    def x_copy(i):
        r0 = pl.multiple_of(i * TQ, TQ)
        return pltpu.make_async_copy(x_hbm.at[pl.ds(r0, TQ), :], xio.at[pl.ds(r0, TQ), :], sem_x.at[i])

    def out_copy(i):
        r0 = pl.multiple_of(i * TQ, TQ)
        return pltpu.make_async_copy(xio.at[pl.ds(r0, TQ), :], out_hbm.at[pl.ds(r0, TQ), :], sem_o.at[i])

    cp_wqa = pltpu.make_async_copy(wqkv_hbm.at[:, pl.ds(0, D // 2)], wq_v.at[:, pl.ds(0, D // 2)], sem_w.at[0])
    cp_wqb = pltpu.make_async_copy(wqkv_hbm.at[:, pl.ds(D // 2, D // 2)], wq_v.at[:, pl.ds(D // 2, D // 2)],
                                   sem_w.at[9])
    cp_wk = pltpu.make_async_copy(wqkv_hbm.at[:, pl.ds(D, D)], wk_v, sem_w.at[1])
    cp_wv = pltpu.make_async_copy(wqkv_hbm.at[:, pl.ds(2 * D, D)], wv_v, sem_w.at[8])
    cp_wo = pltpu.make_async_copy(wo_hbm, wo_v, sem_w.at[2])
    cp_wr = pltpu.make_async_copy(wr_hbm, wr_v, sem_w.at[3])
    cp_wg = pltpu.make_async_copy(wg_hbm, wg_v, sem_w.at[4])
    cp_wu = pltpu.make_async_copy(wu_hbm, wu_v, sem_w.at[5])
    cp_wd = pltpu.make_async_copy(wd_hbm, wd_v, sem_w.at[6])

    x_copy(0).start()
    cp_wqa.start()

    z_s[...] = jnp.zeros_like(z_s)
    xres[0:CH, :] = jnp.zeros((CH, D), f32)

    def ln_chunk(layer, i, c, xc_ref, gate, chain=None):
        r0 = i * TQ + c * CH
        h0 = i * (TQ // 2) + c * (CH // 2)
        if not isinstance(r0, int):
            r0 = pl.multiple_of(r0, CH)
            h0 = pl.multiple_of(h0, CH // 2)
        parts = []
        for q in range(CH // LNR):
            rq = r0 + q * LNR
            x_in = xio[pl.ds(rq, LNR), :].astype(f32)
            x_rs = xres[pl.ds(pl.multiple_of(rq * layer, LNR), LNR), :]
            xq = jnp.where(layer == 0, x_in, x_rs)
            xbuf[pl.ds(rq, LNR), :] = xq
            if chain is not None and len(chain) >= CHAIN_A:
                xq = _gate_first(xq, chain[-CHAIN_A], z_s[...])
            elif gate is not None:
                xq = _gate_first(xq, gate, z_s[...])
            parts.append(_ln(xq))
            if chain is not None:
                chain.append(parts[-1])
        xn = jnp.concatenate(parts, axis=0)
        xc = _pack_rows(xn)
        xc_ref[c * CH // 2:(c + 1) * CH // 2, :] = xc
        xc_all[pl.ds(h0, CH // 2), :] = xc
        xi_all[pl.ds(h0, CH // 2), :] = _pack_rows_interleaved(xn)

    def q_step(layer, i, xc_ref, i_next, xc_next, part=(0, G)):
        h0 = i * (TQ // 2)
        if not isinstance(h0, int):
            h0 = pl.multiple_of(h0, TQ // 2)
        a = pltpu.bitcast(xc_ref[...], bf16)
        ys = {}
        for n in range(*part):
            y = jnp.dot(a, wq_v[:, n * 128:(n + 1) * 128], preferred_element_type=f32)
            q_s[n, pl.ds(h0, TQ // 2), :] = _pack_rows(y * QSCALE)
            ys[n] = y
        if i_next is not None:
            chain = []
            for c in range(part[0] * NCH // G, part[1] * NCH // G):
                ln_chunk(layer, i_next, c, xc_next, ys.get(GATE_A[c]), chain)

    def kv_step(i):
        h0 = pl.multiple_of(i * (TKV // 2), TKV // 2)
        a = pltpu.bitcast(xc_all[pl.ds(h0, TKV // 2), :], bf16)
        for n in range(G):
            y = jnp.dot(a, wk_v[:, n * 128:(n + 1) * 128], preferred_element_type=f32)
            k_s[n, pl.ds(PAD // 2 + h0, TKV // 2), :] = _pack_rows(y)
        vt = lax.dot_general(pltpu.bitcast(wvt_v[...], bf16), pltpu.bitcast(xi_all[pl.ds(h0, TKV // 2), :], bf16),
                             NT, preferred_element_type=f32)
        c0 = pl.multiple_of(PAD + i * TKV, 256)
        vt_s[:, pl.ds(c0, TKV)] = _pack_rows(vt)

    def phase_a(layer):
        @pl.when(layer == 0)
        def _():
            x_copy(0).wait()
            x_copy(1).start()
            cp_wqb.start()

        for c in range(NCH):
            ln_chunk(layer, 0, c, xca, None)

        @pl.when(layer == 0)
        def _():
            cp_wqa.wait()
            x_copy(1).wait()
            for i in range(2, NB):
                x_copy(i).start()

        q_step(layer, 0, xca, 1, xcb, part=(0, G // 2))

        @pl.when(layer == 0)
        def _():
            cp_wqb.wait()
            cp_wv.start()
            cp_wo.start()
            cp_wk.start()
            cp_wr.start()

        q_step(layer, 0, xca, 1, xcb, part=(G // 2, G))

        def q_body(j, c):
            i1 = 2 * j + 1

            @pl.when(layer == 0)
            def _():
                x_copy(i1 + 1).wait()
                x_copy(i1 + 2).wait()

            q_step(layer, i1, xcb, i1 + 1, xca)
            q_step(layer, i1 + 1, xca, i1 + 2, xcb)
            return c

        with jax.named_scope("a_q"):
            lax.fori_loop(0, NB // 2 - 1, q_body, 0)

        @pl.when(layer == 0)
        def _():
            cp_wv.wait()
            cp_wo.wait()

        q_step(layer, NB - 1, xcb, None, None)
        wvt_v[...] = pltpu.bitcast(wv_v[...].T, u32)
        for c in range(D // 64):
            wop_v[c * 32:(c + 1) * 32, :] = _pack_rows_interleaved(wo_v[c * 64:(c + 1) * 64, :].astype(f32))

        @pl.when(layer == 0)
        def _():
            cp_wk.wait()
            cp_wg.start()
            cp_wu.start()
            cp_wd.start()

        def kv_body(j, c):
            kv_step(j)
            return c

        with jax.named_scope("a_kv"):
            lax.fori_loop(0, S // TKV, kv_body, 0)

    def qk_stage(g, q0, slot, kstart):
        zi = pltpu.bitcast(z_s[...], i32)
        zi16 = jnp.concatenate([zi, zi], axis=0)
        lane16 = lax.broadcasted_iota(i32, (16, 128), 1) + zi16
        r16 = lax.broadcasted_iota(i32, (16, 128), 0)
        hb16 = lane16 // 32
        dd = r16 - lane16 % 32
        h0 = q0 // 2
        first_rows = None
        for b in range(4):
            first = max(0, kstart - 32 * b)
            base = h0 + 16 * b
            if not isinstance(base, int):
                base = pl.multiple_of(base, 16)
            mid0 = max(first, 32)
            if first == 0:
                parts = [k_s[g, pl.ds(base, 8), :], k_s[g, pl.ds(base + 128, 8), :],
                         k_s[g, pl.ds(base + 8, 8), :], k_s[g, pl.ds(base + 136, 8), :]]
            else:
                parts = [k_s[g, pl.ds(base + 128, 16), :]]
            if mid0 < 256:
                parts.append(k_s[g, pl.ds(base + mid0 // 2, (256 - mid0) // 2), :])
            kw = pltpu.bitcast(jnp.concatenate(parts, axis=0), bf16)
            qu = q_s[g, pl.ds(base, 16), :]
            qall = pltpu.bitcast(
                jnp.concatenate([jnp.where(hb16 == (p - b) % 4, qu, jnp.uint32(0)) for p in range(4)], axis=0),
                bf16)
            st = lax.dot_general(kw, qall, NT, preferred_element_type=f32)
            if b == 3:
                first_rows = st[0:8]
            if first == 0:
                c0 = jnp.where(dd > 0, st[0:16], st[16:32])
                c1 = jnp.where(dd > -16, st[32:48], st[48:64])
                mid = st[64:]
            else:
                c0 = jnp.where(dd > 0, NEG, st[0:16])
                c1 = jnp.where(dd > -16, NEG, st[16:32])
                mid = st[32:]
            s_s[slot, b, 0:16, :] = c0
            s_s[slot, b, 16:32, :] = c1
            x = jnp.concatenate([c0, c1], axis=0)
            if mid0 < 256:
                s_s[slot, b, mid0:256, :] = mid
                x = jnp.concatenate([x, mid], axis=0)
            mm = jnp.max(x.reshape(x.shape[0] // 8, 8, 128), axis=0)
            m_s[slot, b] = jnp.broadcast_to(jnp.max(mm, axis=0, keepdims=True), (8, 128))
        return first_rows

    def pv_stage(g, q0, slot, gate, kstart, defer=False, finish=True):
        r8 = lax.broadcasted_iota(i32, (8, 128), 0)
        c8 = lax.broadcasted_iota(i32, (8, 128), 1) + pltpu.bitcast(z_s[...], i32)
        blk = c8 // 32
        j = c8 % 32

        def tri(u):
            return (jnp.where(16 * u + r8 > j, jnp.uint32(0xFFFF), jnp.uint32(0)) |
                    jnp.where(16 * u + 8 + r8 > j, jnp.uint32(0xFFFF0000), jnp.uint32(0)))

        tris = [tri(0), tri(1)] if kstart < 128 else None
        ms = [m_s[slot, b] for b in range(4)]
        L = [None] * 4
        cache = {}

        def pexp(b, u):
            x = s_s[slot, b, 16 * u:16 * u + 16, :]
            p0 = jnp.exp2(x[0:8] - ms[b])
            p1 = jnp.exp2(x[8:16] - ms[b])
            sm = p0 + p1
            L[b] = sm if L[b] is None else L[b] + sm
            return pltpu.pack_elementwise([p0, p1], packed_dtype=bf16)

        def get_p(b, u):
            first = max(0, kstart - 32 * b)
            if u < 0 or u >= 18 or 16 * u < first:
                return None
            if first > 0:
                return pexp(b, u - 16) if u >= 16 else pexp(b, u)
            if u < 2 or u >= 16:
                if (b, u) not in cache:
                    pk = pexp(b, u % 16)
                    lo = pk & tris[u % 16]
                    cache[(b, u % 16)] = lo
                    cache[(b, u % 16 + 16)] = pk ^ lo
                return cache.pop((b, u))
            return pexp(b, u)

        accs = [None] * 4
        for k in [k for k in B_ORDER if k >= kstart // 128]:
            wts = [[] for _ in range(4)]
            for t in range(8 * k, 8 * k + 8):
                if t == B_GATE_T and gate is not None:
                    gv = gate * z_s[...]
                    for b in range(4):
                        ms[b] = ms[b] + gv
                src = [get_p(b, t - 2 * b) for b in range(4)]
                for h, w in enumerate(_latin_merge(src, blk)):
                    wts[h].append(w)
            c0 = q0 + 128 * k
            if not isinstance(c0, int):
                c0 = pl.multiple_of(c0, 128)
            for h in range(4):
                pt = pltpu.bitcast(jnp.concatenate(wts[h], axis=0), bf16)
                vth = pltpu.bitcast(vt_s[pl.ds((g * 4 + h) * 16, 16), pl.ds(c0, 128)], bf16)
                d = jnp.dot(vth, pt, preferred_element_type=f32)
                accs[h] = d if accs[h] is None else accs[h] + d
        if defer:
            for h in range(4):
                pend_acc[h * 32:(h + 1) * 32, :] = accs[h]
                pend_l[h] = L[h]
        if finish:
            pv_finish(g, q0, accs, L)

    def pv_finish(g, q0, accs, L):
        blk = (lax.broadcasted_iota(i32, (8, 128), 1) + pltpu.bitcast(z_s[...], i32)) // 32
        L = [jnp.broadcast_to(jnp.sum(l, axis=0, keepdims=True), (8, 128)) for l in L]
        outs = []
        for h, lh in enumerate(_latin_merge(L, blk)):
            r0 = pl.reciprocal(lh, approx=True)
            rl = r0 * (2.0 - lh * r0)
            ot = (accs[h].reshape(4, 8, 128) * rl[None]).reshape(32, 128)
            if h > 0:
                ot = pltpu.roll(ot, 128 - 32 * h, axis=1)
            outs.append(ot)
        ot_s[g * 64:(g + 1) * 64, pl.ds(q0, 128)] = _pack_rows_interleaved(jnp.concatenate(outs, axis=0))

    def finish_pending(q0):
        pv_finish(G - 1, q0, [pend_acc[h * 32:(h + 1) * 32, :] for h in range(4)], [pend_l[h] for h in range(4)])

    def sub_block(q0, qn, defer_last=False):
        for g in range(G):
            if g + 1 < G:
                gate = qk_stage(g + 1, q0, (g + 1) % 2, 0)
            else:
                gate = qk_stage(0, qn, 0, 0)
            last = defer_last and g == G - 1
            pv_stage(g, q0, g % 2, gate, 0, defer=last, finish=not last)

    def transpose_o(i, o_dst):
        r0 = i * TQ
        if not isinstance(r0, int):
            r0 = pl.multiple_of(r0, TQ)
        o_dst[...] = pltpu.bitcast(pltpu.bitcast(ot_s[:, pl.ds(r0, TQ)], bf16).T, u32)

    def phase_b():
        qk_stage(0, 0, 2, PAD)
        qk_stage(0, 128, 0, PAD - 128)
        for g in range(G):
            if g + 1 < G:
                qk_stage(g + 1, 0, 2 + (g + 1) % 2, PAD)
            pv_stage(g, 0, 2 + g % 2, None, PAD)
            if g + 1 < G:
                qk_stage(g + 1, 128, (g + 1) % 2, PAD - 128)
            else:
                qk_stage(0, 256, 0, 0)
            pv_stage(g, 128, g % 2, None, PAD - 128, defer=(g == G - 1))
        transpose_o(0, oa)

        def body(j, c):
            q0 = pl.multiple_of(j * 256, 256)
            q1 = pl.multiple_of(q0 + 128, 128)
            qn = pl.multiple_of(jnp.minimum(q0 + 256, S - 128), 128)
            finish_pending(pl.multiple_of(q0 - 128, 128))
            sub_block(q0, q1)
            sub_block(q1, qn, defer_last=True)
            return c

        lax.fori_loop(1, NSB // 2, body, 0)
        finish_pending(S - 128)

    def resid_chunk(i, c, at_ref, gate):
        r0 = i * TQ + c * CHC
        if not isinstance(r0, int):
            r0 = pl.multiple_of(r0, CHC)
        x1 = xbuf[pl.ds(r0, CHC), :] + at_ref[c * CHC:(c + 1) * CHC, :]
        if gate is not None:
            x1 = _gate_first(x1, gate, z_s[...])
        m = jnp.mean(x1, axis=-1, keepdims=True)
        xc = x1 - m
        v = jnp.mean(xc * xc, axis=-1, keepdims=True)
        rho = lax.rsqrt(v + EPS)
        xn = xc * rho
        r = jnp.sum(xn * wr8[0:1, :], axis=-1, keepdims=True)
        rb = jnp.broadcast_to(r, (CHC, 128)).astype(bf16).astype(f32)
        rows = lax.broadcasted_iota(i32, (8, 128), 0) + r0
        bv, bi = best_v[...], best_i[...]
        for q in range(CHC // 8):
            cand = rb[8 * q:8 * q + 8]
            better = cand > bv
            bv = jnp.where(better, cand, bv)
            bi = jnp.where(better, rows + 8 * q, bi)
        best_v[...] = bv
        best_i[...] = bi
        rho_s[pl.ds(r0, CHC), :] = jnp.broadcast_to(rho, (CHC, 128))
        x2 = x1 + xn
        xres[pl.ds(r0, CHC), :] = x2
        xio[pl.ds(r0, CHC), :] = x2.astype(bf16)

    def oproj_step(o_src, at_w, i_res, at_r, i_t, o_dst):
        ys = []
        if o_src is not None:
            a = pltpu.bitcast(o_src[...], bf16)
            for n in range(G):
                y = jnp.dot(a, pltpu.bitcast(wop_v[:, n * 128:(n + 1) * 128], bf16), preferred_element_type=f32)
                at_w[:, n * 128:(n + 1) * 128] = y
                ys.append(y)
        if i_t is not None:
            transpose_o(i_t, o_dst)
        if i_res is not None:
            for c in range(NCHC):
                gi = GATE_C[c] if ys else -1
                resid_chunk(i_res, c, at_r, ys[gi] if gi >= 0 else None)

    def phase_c(layer):
        @pl.when(layer == 0)
        def _():
            cp_wr.wait()
            wr8[...] = jnp.broadcast_to(wr_v[...].astype(f32).reshape(1, D), (8, D))

        def flush(i):
            @pl.when(layer == 1)
            def _():
                out_copy(i).start()

        best_v[...] = jnp.full((8, 128), -jnp.inf, f32)
        best_i[...] = jnp.zeros((8, 128), i32)
        oproj_step(oa, ata, None, None, 1, ob)

        def body(j, c):
            i0 = 2 * j
            oproj_step(ob, atb, i0, ata, i0 + 2, oa)
            oproj_step(oa, ata, i0 + 1, atb, i0 + 3, ob)
            flush(i0)
            flush(i0 + 1)
            return c

        lax.fori_loop(0, NB // 2 - 1, body, 0)
        oproj_step(ob, atb, NB - 2, ata, None, None)
        oproj_step(None, None, NB - 1, atb, None, None)
        flush(NB - 2)
        flush(NB - 1)

    def phase_d(layer):
        @pl.when(layer == 0)
        def _():
            cp_wg.wait()
            cp_wu.wait()
            cp_wd.wait()

        bv = best_v[...]
        rmax = jnp.max(bv)
        idx = jnp.min(jnp.where(bv == rmax, best_i[...], S))
        idx = jnp.clip(idx, 0, S - 1)
        x2 = xres[pl.ds(idx, 1), :]
        rho = rho_s[pl.ds(idx, 1), 0:1]
        xn = (x2 - jnp.mean(x2, axis=-1, keepdims=True)) * (rho / (1.0 + rho))
        xs = jnp.broadcast_to(xn, (16, D)).astype(bf16)
        nf = F // FC
        hs = []
        y = None
        for c in range(nf + 1):
            if c < nf:
                gate = jnp.dot(xs, wg_v[:, c * FC:(c + 1) * FC], preferred_element_type=f32)
                up = jnp.dot(xs, wu_v[:, c * FC:(c + 1) * FC], preferred_element_type=f32)
                hs.append((gate * jax.nn.sigmoid(gate) * up).astype(bf16))
            if c > 0:
                d = jnp.dot(hs[c - 1], wd_v[(c - 1) * FC:c * FC, :], preferred_element_type=f32)
                y = d if y is None else y + d
        scale = jax.nn.sigmoid(jnp.full((1, D), rmax, f32))
        xres[pl.ds(idx, 1), :] = xres[pl.ds(idx, 1), :] + y[0:1] * scale

        @pl.when(layer == 1)
        def _():
            for i in range(NB):
                out_copy(i).wait()
            g0 = pl.multiple_of((idx // 16) * 16, 16)
            xio[pl.ds(g0, 16), :] = xres[pl.ds(g0, 16), :].astype(bf16)
            fix = pltpu.make_async_copy(xio.at[pl.ds(g0, 16), :], out_hbm.at[pl.ds(g0, 16), :], sem_w.at[7])
            fix.start()
            fix.wait()

    def layer_body(layer, c):
        with jax.named_scope("phase_a"):
            phase_a(layer)
        with jax.named_scope("phase_b"):
            phase_b()
        with jax.named_scope("phase_c"):
            phase_c(layer)
        with jax.named_scope("phase_d"):
            phase_d(layer)
        return c

    lax.fori_loop(0, 2, layer_body, 0)


@jax.jit
def pallas_interleave_layers__sliding_block__moe_arch_mod__prompt_kernel(
    A_x: jax.Array,
    A_wqkv: jax.Array,
    A_wo: jax.Array,
    B_x: jax.Array,
    B_w_r: jax.Array,
    B_w_gate: jax.Array,
    B_w_up: jax.Array,
    B_w_down: jax.Array,
):
    del B_x
    x = A_x.reshape(S, D)
    any_spec = pl.BlockSpec(memory_space=pl.ANY)
    scratch = [
        pltpu.VMEM((S, D), bf16),
        pltpu.VMEM((D, D), bf16),
        pltpu.VMEM((D, D), bf16),
        pltpu.VMEM((D, D), bf16),
        pltpu.VMEM((D // 2, D), u32),
        pltpu.VMEM((D, D), bf16),
        pltpu.VMEM((D // 2, D), u32),
        pltpu.VMEM((D,), bf16),
        pltpu.VMEM((D, F), bf16),
        pltpu.VMEM((D, F), bf16),
        pltpu.VMEM((F, D), bf16),
        pltpu.VMEM((S, D), f32),
        pltpu.VMEM((S, D), f32),
        pltpu.VMEM((8, 128), f32),
        pltpu.VMEM((8, 128), i32),
        pltpu.VMEM((S, 128), f32),
        pltpu.VMEM((8, 128), f32),
        pltpu.VMEM((8, D), f32),
        pltpu.VMEM((TQ // 2, D), u32),
        pltpu.VMEM((TQ // 2, D), u32),
        pltpu.VMEM((S // 2, D), u32),
        pltpu.VMEM((S // 2, D), u32),
        pltpu.VMEM((G, S // 2, 128), u32),
        pltpu.VMEM((G, (S + PAD) // 2, 128), u32),
        pltpu.VMEM((D // 2, S + PAD), u32),
        pltpu.VMEM((D // 2, S), u32),
        pltpu.VMEM((4, 4, 256, 128), f32),
        pltpu.VMEM((4, 4, 8, 128), f32),
        pltpu.VMEM((128, 128), f32),
        pltpu.VMEM((4, 8, 128), f32),
        pltpu.VMEM((TQ, D), f32),
        pltpu.VMEM((TQ, D), f32),
        pltpu.VMEM((TQ // 2, D), u32),
        pltpu.VMEM((TQ // 2, D), u32),
        pltpu.SemaphoreType.DMA((NB,)),
        pltpu.SemaphoreType.DMA((10,)),
        pltpu.SemaphoreType.DMA((NB,)),
    ]
    out = pl.pallas_call(
        _kernel,
        out_shape=jax.ShapeDtypeStruct((S, D), bf16),
        in_specs=[any_spec] * 7,
        out_specs=any_spec,
        scratch_shapes=scratch,
        compiler_params=pltpu.CompilerParams(vmem_limit_bytes=120 * 1024 * 1024),
    )(x, A_wqkv, A_wo, B_w_r, B_w_gate, B_w_up, B_w_down)
    return out.reshape(1, S, D)
```

```python
import jax
import jax.numpy as jnp
from jax import lax
import jax.experimental.pallas as pl
import jax.experimental.pallas.tpu as pltpu

bf16 = jnp.bfloat16
f32 = jnp.float32
u32 = jnp.uint32
i32 = jnp.int32

S = 2048
D = 1024
H = 32
DH = 32
W = 256
F = 3584
G = 8
PAD = 256
TQ = 256
NB = S // TQ
TKV = 512
NSB = S // 128
CH = 32
LNR = 8
NCH = TQ // CH
CHC = 8
NCHC = TQ // CHC
FC = 256
GATE_A = [c * 8 // NCH - 1 for c in range(NCH)]
CHAIN_A = 3
GATE_C = [c * 8 // NCHC - 1 for c in range(NCHC)]
B_ORDER = [1, 0, 2]
B_GATE_T = 6
EPS = 1e-5
NEG = -1e30
QSCALE = (DH ** -0.5) * 1.4426950408889634
NT = (((1,), (1,)), ((), ()))


def _ln(x):
    m = jnp.mean(x, axis=-1, keepdims=True)
    xc = x - m
    v = jnp.mean(xc * xc, axis=-1, keepdims=True)
    return xc * lax.rsqrt(v + EPS)


def _pack_rows(x):
    return pltpu.bitcast(x.astype(bf16), u32)


def _pack_rows_interleaved(x):
    n = x.shape[0] // 16
    x3 = x.reshape(n, 16, x.shape[1])
    a = x3[:, 0:8, :].reshape(n * 8, x.shape[1])
    b = x3[:, 8:16, :].reshape(n * 8, x.shape[1])
    return pltpu.pack_elementwise([a, b], packed_dtype=bf16)


def _gate_first(x, gate, z):
    g = gate[0:8, 0:128] * z
    top = jnp.concatenate([x[0:8, 0:128] + g, x[0:8, 128:]], axis=1)
    return top if x.shape[0] == 8 else jnp.concatenate([top, x[8:]], axis=0)


def _latin_merge(src, blk):
    present = [v for v in src if v is not None]
    zero = jnp.zeros_like(present[0])

    def sel(mask, x, y):
        if x is None and y is None:
            return None
        return jnp.where(mask, zero if x is None else x, zero if y is None else y)

    if len(present) == 1:
        b = [v is not None for v in src].index(True)
        return [jnp.where(blk == (h + b) % 4, src[b], zero) for h in range(4)]
    odd = (blk & 1) == 1
    low = blk < 2
    pair = [sel(odd, src[(a + 1) % 4], src[a]) for a in range(4)]
    out = [sel(low, pair[(-h) % 4], pair[(2 - h) % 4]) for h in range(4)]
    return [zero if v is None else v for v in out]


def _kernel(x_hbm, wqkv_hbm, wo_hbm, wr_hbm, wg_hbm, wu_hbm, wd_hbm,
            out_hbm,
            xio, wq_v, wk_v, wv_v, wvt_v, wo_v, wop_v, wr_v, wg_v, wu_v, wd_v,
            xres, xbuf, best_v, best_i, rho_s, mean_s, z_s, wr8,
            xca, xcb, xc_all, xi_all,
            q_s, k_s, vt_s, ot_s, s_s, m_s, pend_acc, pend_l,
            ata, atb, oa, ob,
            sem_x, sem_w, sem_o):
    def x_copy(i):
        r0 = pl.multiple_of(i * TQ, TQ)
        return pltpu.make_async_copy(x_hbm.at[pl.ds(r0, TQ), :], xio.at[pl.ds(r0, TQ), :], sem_x.at[i])

    def out_copy(i):
        r0 = pl.multiple_of(i * TQ, TQ)
        return pltpu.make_async_copy(xio.at[pl.ds(r0, TQ), :], out_hbm.at[pl.ds(r0, TQ), :], sem_o.at[i])

    cp_wqa = pltpu.make_async_copy(wqkv_hbm.at[:, pl.ds(0, D // 2)], wq_v.at[:, pl.ds(0, D // 2)], sem_w.at[0])
    cp_wqb = pltpu.make_async_copy(wqkv_hbm.at[:, pl.ds(D // 2, D // 2)], wq_v.at[:, pl.ds(D // 2, D // 2)],
                                   sem_w.at[9])
    cp_wk = pltpu.make_async_copy(wqkv_hbm.at[:, pl.ds(D, D)], wk_v, sem_w.at[1])
    cp_wv = pltpu.make_async_copy(wqkv_hbm.at[:, pl.ds(2 * D, D)], wv_v, sem_w.at[8])
    cp_wo = pltpu.make_async_copy(wo_hbm, wo_v, sem_w.at[2])
    cp_wr = pltpu.make_async_copy(wr_hbm, wr_v, sem_w.at[3])
    cp_wg = pltpu.make_async_copy(wg_hbm, wg_v, sem_w.at[4])
    cp_wu = pltpu.make_async_copy(wu_hbm, wu_v, sem_w.at[5])
    cp_wd = pltpu.make_async_copy(wd_hbm, wd_v, sem_w.at[6])

    x_copy(0).start()
    cp_wqa.start()

    z_s[...] = jnp.zeros_like(z_s)
    xres[0:CH, :] = jnp.zeros((CH, D), f32)

    def ln_chunk(layer, i, c, xc_ref, gate, chain=None):
        r0 = i * TQ + c * CH
        h0 = i * (TQ // 2) + c * (CH // 2)
        if not isinstance(r0, int):
            r0 = pl.multiple_of(r0, CH)
            h0 = pl.multiple_of(h0, CH // 2)
        parts = []
        for q in range(CH // LNR):
            rq = r0 + q * LNR
            x_in = xio[pl.ds(rq, LNR), :].astype(f32)
            x_rs = xres[pl.ds(pl.multiple_of(rq * layer, LNR), LNR), :]
            xq = jnp.where(layer == 0, x_in, x_rs)
            xbuf[pl.ds(rq, LNR), :] = xq
            if chain is not None and len(chain) >= CHAIN_A:
                xq = _gate_first(xq, chain[-CHAIN_A], z_s[...])
            elif gate is not None:
                xq = _gate_first(xq, gate, z_s[...])
            parts.append(_ln(xq))
            if chain is not None:
                chain.append(parts[-1])
        xn = jnp.concatenate(parts, axis=0)
        xc = _pack_rows(xn)
        xc_ref[c * CH // 2:(c + 1) * CH // 2, :] = xc
        xc_all[pl.ds(h0, CH // 2), :] = xc
        xi_all[pl.ds(h0, CH // 2), :] = _pack_rows_interleaved(xn)

    def q_step(layer, i, xc_ref, i_next, xc_next, part=(0, G)):
        h0 = i * (TQ // 2)
        if not isinstance(h0, int):
            h0 = pl.multiple_of(h0, TQ // 2)
        a = pltpu.bitcast(xc_ref[...], bf16)
        ys = {}
        for n in range(*part):
            y = jnp.dot(a, wq_v[:, n * 128:(n + 1) * 128], preferred_element_type=f32)
            q_s[n, pl.ds(h0, TQ // 2), :] = _pack_rows(y * QSCALE)
            ys[n] = y
        if i_next is not None:
            chain = []
            for c in range(part[0] * NCH // G, part[1] * NCH // G):
                ln_chunk(layer, i_next, c, xc_next, ys.get(GATE_A[c]), chain)

    def kv_step(i):
        h0 = pl.multiple_of(i * (TKV // 2), TKV // 2)
        a = pltpu.bitcast(xc_all[pl.ds(h0, TKV // 2), :], bf16)
        for n in range(G):
            y = jnp.dot(a, wk_v[:, n * 128:(n + 1) * 128], preferred_element_type=f32)
            k_s[n, pl.ds(PAD // 2 + h0, TKV // 2), :] = _pack_rows(y)
        vt = lax.dot_general(pltpu.bitcast(wvt_v[...], bf16), pltpu.bitcast(xi_all[pl.ds(h0, TKV // 2), :], bf16),
                             NT, preferred_element_type=f32)
        c0 = pl.multiple_of(PAD + i * TKV, 256)
        vt_s[:, pl.ds(c0, TKV)] = _pack_rows(vt)

    def phase_a(layer):
        @pl.when(layer == 0)
        def _():
            x_copy(0).wait()
            x_copy(1).start()
            cp_wqb.start()

        for c in range(NCH):
            ln_chunk(layer, 0, c, xca, None)

        @pl.when(layer == 0)
        def _():
            cp_wqa.wait()
            x_copy(1).wait()
            for i in range(2, NB):
                x_copy(i).start()

        q_step(layer, 0, xca, 1, xcb, part=(0, G // 2))

        @pl.when(layer == 0)
        def _():
            cp_wqb.wait()
            cp_wv.start()
            cp_wo.start()
            cp_wk.start()
            cp_wr.start()

        q_step(layer, 0, xca, 1, xcb, part=(G // 2, G))

        def q_body(j, c):
            i1 = 2 * j + 1

            @pl.when(layer == 0)
            def _():
                x_copy(i1 + 1).wait()
                x_copy(i1 + 2).wait()

            q_step(layer, i1, xcb, i1 + 1, xca)
            q_step(layer, i1 + 1, xca, i1 + 2, xcb)
            return c

        lax.fori_loop(0, NB // 2 - 1, q_body, 0)

        @pl.when(layer == 0)
        def _():
            cp_wv.wait()
            cp_wo.wait()

        q_step(layer, NB - 1, xcb, None, None)
        wvt_v[...] = pltpu.bitcast(wv_v[...].T, u32)
        for c in range(D // 64):
            wop_v[c * 32:(c + 1) * 32, :] = _pack_rows_interleaved(wo_v[c * 64:(c + 1) * 64, :].astype(f32))

        @pl.when(layer == 0)
        def _():
            cp_wk.wait()
            cp_wr.wait()
            wr8[...] = jnp.broadcast_to(wr_v[...].astype(f32).reshape(1, D), (8, D))
            cp_wg.start()
            cp_wu.start()
            cp_wd.start()

        def kv_body(j, c):
            kv_step(j)
            return c

        lax.fori_loop(0, S // TKV, kv_body, 0)

    def qk_stage(g, q0, slot, kstart):
        zi = pltpu.bitcast(z_s[...], i32)
        zi16 = jnp.concatenate([zi, zi], axis=0)
        lane16 = lax.broadcasted_iota(i32, (16, 128), 1) + zi16
        r16 = lax.broadcasted_iota(i32, (16, 128), 0)
        hb16 = lane16 // 32
        dd = r16 - lane16 % 32
        h0 = q0 // 2
        first_rows = None
        for b in range(4):
            first = max(0, kstart - 32 * b)
            base = h0 + 16 * b
            if not isinstance(base, int):
                base = pl.multiple_of(base, 16)
            mid0 = max(first, 32)
            if first == 0:
                parts = [k_s[g, pl.ds(base, 8), :], k_s[g, pl.ds(base + 128, 8), :],
                         k_s[g, pl.ds(base + 8, 8), :], k_s[g, pl.ds(base + 136, 8), :]]
            else:
                parts = [k_s[g, pl.ds(base + 128, 16), :]]
            if mid0 < 256:
                parts.append(k_s[g, pl.ds(base + mid0 // 2, (256 - mid0) // 2), :])
            kw = pltpu.bitcast(jnp.concatenate(parts, axis=0), bf16)
            qu = q_s[g, pl.ds(base, 16), :]
            qall = pltpu.bitcast(
                jnp.concatenate([jnp.where(hb16 == (p - b) % 4, qu, jnp.uint32(0)) for p in range(4)], axis=0),
                bf16)
            st = lax.dot_general(kw, qall, NT, preferred_element_type=f32)
            if b == 3:
                first_rows = st[0:8]
            if first == 0:
                c0 = jnp.where(dd > 0, st[0:16], st[16:32])
                c1 = jnp.where(dd > -16, st[32:48], st[48:64])
                mid = st[64:]
            else:
                c0 = jnp.where(dd > 0, NEG, st[0:16])
                c1 = jnp.where(dd > -16, NEG, st[16:32])
                mid = st[32:]
            s_s[slot, b, 0:16, :] = c0
            s_s[slot, b, 16:32, :] = c1
            x = jnp.concatenate([c0, c1], axis=0)
            if mid0 < 256:
                s_s[slot, b, mid0:256, :] = mid
                x = jnp.concatenate([x, mid], axis=0)
            mm = jnp.max(x.reshape(x.shape[0] // 8, 8, 128), axis=0)
            m_s[slot, b] = jnp.broadcast_to(jnp.max(mm, axis=0, keepdims=True), (8, 128))
        return first_rows

    def pv_stage(g, q0, slot, gate, kstart, defer=False, finish=True):
        r8 = lax.broadcasted_iota(i32, (8, 128), 0)
        c8 = lax.broadcasted_iota(i32, (8, 128), 1) + pltpu.bitcast(z_s[...], i32)
        blk = c8 // 32
        j = c8 % 32

        def tri(u):
            return (jnp.where(16 * u + r8 > j, jnp.uint32(0xFFFF), jnp.uint32(0)) |
                    jnp.where(16 * u + 8 + r8 > j, jnp.uint32(0xFFFF0000), jnp.uint32(0)))

        tris = [tri(0), tri(1)] if kstart < 128 else None
        ms = [m_s[slot, b] for b in range(4)]
        L = [None] * 4
        cache = {}

        def pexp(b, u):
            x = s_s[slot, b, 16 * u:16 * u + 16, :]
            p0 = jnp.exp2(x[0:8] - ms[b])
            p1 = jnp.exp2(x[8:16] - ms[b])
            sm = p0 + p1
            L[b] = sm if L[b] is None else L[b] + sm
            return pltpu.pack_elementwise([p0, p1], packed_dtype=bf16)

        def get_p(b, u):
            first = max(0, kstart - 32 * b)
            if u < 0 or u >= 18 or 16 * u < first:
                return None
            if first > 0:
                return pexp(b, u - 16) if u >= 16 else pexp(b, u)
            if u < 2 or u >= 16:
                if (b, u) not in cache:
                    pk = pexp(b, u % 16)
                    lo = pk & tris[u % 16]
                    cache[(b, u % 16)] = lo
                    cache[(b, u % 16 + 16)] = pk ^ lo
                return cache.pop((b, u))
            return pexp(b, u)

        accs = [None] * 4
        for k in [k for k in B_ORDER if k >= kstart // 128]:
            wts = [[] for _ in range(4)]
            for t in range(8 * k, 8 * k + 8):
                if t == B_GATE_T and gate is not None:
                    gv = gate * z_s[...]
                    for b in range(4):
                        ms[b] = ms[b] + gv
                src = [get_p(b, t - 2 * b) for b in range(4)]
                for h, w in enumerate(_latin_merge(src, blk)):
                    wts[h].append(w)
            c0 = q0 + 128 * k
            if not isinstance(c0, int):
                c0 = pl.multiple_of(c0, 128)
            for h in range(4):
                pt = pltpu.bitcast(jnp.concatenate(wts[h], axis=0), bf16)
                vth = pltpu.bitcast(vt_s[pl.ds((g * 4 + h) * 16, 16), pl.ds(c0, 128)], bf16)
                d = jnp.dot(vth, pt, preferred_element_type=f32)
                accs[h] = d if accs[h] is None else accs[h] + d
        if defer:
            for h in range(4):
                pend_acc[h * 32:(h + 1) * 32, :] = accs[h]
                pend_l[h] = L[h]
        if finish:
            pv_finish(g, q0, accs, L)

    def pv_finish(g, q0, accs, L):
        blk = (lax.broadcasted_iota(i32, (8, 128), 1) + pltpu.bitcast(z_s[...], i32)) // 32
        L = [jnp.broadcast_to(jnp.sum(l, axis=0, keepdims=True), (8, 128)) for l in L]
        outs = []
        for h, lh in enumerate(_latin_merge(L, blk)):
            r0 = pl.reciprocal(lh, approx=True)
            rl = r0 * (2.0 - lh * r0)
            ot = (accs[h].reshape(4, 8, 128) * rl[None]).reshape(32, 128)
            if h > 0:
                ot = pltpu.roll(ot, 128 - 32 * h, axis=1)
            outs.append(ot)
        ot_s[g * 64:(g + 1) * 64, pl.ds(q0, 128)] = _pack_rows_interleaved(jnp.concatenate(outs, axis=0))

    def finish_pending(q0):
        pv_finish(G - 1, q0, [pend_acc[h * 32:(h + 1) * 32, :] for h in range(4)], [pend_l[h] for h in range(4)])

    def sub_block(q0, qn, defer_last=False):
        for g in range(G):
            if g + 1 < G:
                gate = qk_stage(g + 1, q0, (g + 1) % 2, 0)
            else:
                gate = qk_stage(0, qn, 0, 0)
            last = defer_last and g == G - 1
            pv_stage(g, q0, g % 2, gate, 0, defer=last, finish=not last)

    def transpose_o(i, o_dst):
        r0 = i * TQ
        if not isinstance(r0, int):
            r0 = pl.multiple_of(r0, TQ)
        o_dst[...] = pltpu.bitcast(pltpu.bitcast(ot_s[:, pl.ds(r0, TQ)], bf16).T, u32)

    def phase_b():
        qk_stage(0, 0, 2, PAD)
        qk_stage(0, 128, 0, PAD - 128)
        for g in range(G):
            if g + 1 < G:
                qk_stage(g + 1, 0, 2 + (g + 1) % 2, PAD)
            pv_stage(g, 0, 2 + g % 2, None, PAD)
            if g + 1 < G:
                qk_stage(g + 1, 128, (g + 1) % 2, PAD - 128)
            else:
                qk_stage(0, 256, 0, 0)
            pv_stage(g, 128, g % 2, None, PAD - 128, defer=(g == G - 1))
        transpose_o(0, oa)

        def body(j, c):
            q0 = pl.multiple_of(j * 256, 256)
            q1 = pl.multiple_of(q0 + 128, 128)
            qn = pl.multiple_of(jnp.minimum(q0 + 256, S - 128), 128)
            finish_pending(pl.multiple_of(q0 - 128, 128))
            sub_block(q0, q1)
            sub_block(q1, qn, defer_last=True)
            return c

        lax.fori_loop(1, NSB // 2, body, 0)
        finish_pending(S - 128)

    def resid_chunk(i, c, at_ref, gate):
        r0 = i * TQ + c * CHC
        if not isinstance(r0, int):
            r0 = pl.multiple_of(r0, CHC)
        x1 = xbuf[pl.ds(r0, CHC), :] + at_ref[c * CHC:(c + 1) * CHC, :]
        if gate is not None:
            x1 = _gate_first(x1, gate, z_s[...])
        m = jnp.mean(x1, axis=-1, keepdims=True)
        xc = x1 - m
        v = jnp.mean(xc * xc, axis=-1, keepdims=True)
        rho = lax.rsqrt(v + EPS)
        xn = xc * rho
        r = jnp.sum(xn * wr8[0:1, :], axis=-1, keepdims=True)
        rb = jnp.broadcast_to(r, (CHC, 128)).astype(bf16).astype(f32)
        rows = lax.broadcasted_iota(i32, (8, 128), 0) + r0
        bv, bi = best_v[...], best_i[...]
        for q in range(CHC // 8):
            cand = rb[8 * q:8 * q + 8]
            better = cand > bv
            bv = jnp.where(better, cand, bv)
            bi = jnp.where(better, rows + 8 * q, bi)
        best_v[...] = bv
        best_i[...] = bi
        rho_s[pl.ds(r0, CHC), :] = jnp.broadcast_to(rho, (CHC, 128))
        mean_s[pl.ds(r0, CHC), :] = jnp.broadcast_to(m, (CHC, 128))
        x2 = x1 + xn
        xres[pl.ds(r0, CHC), :] = x2
        xio[pl.ds(r0, CHC), :] = x2.astype(bf16)

    def oproj_step(o_src, at_w, i_res, at_r, i_t, o_dst):
        ys = []
        if o_src is not None:
            a = pltpu.bitcast(o_src[...], bf16)
            for n in range(G):
                y = jnp.dot(a, pltpu.bitcast(wop_v[:, n * 128:(n + 1) * 128], bf16), preferred_element_type=f32)
                at_w[:, n * 128:(n + 1) * 128] = y
                ys.append(y)
        if i_t is not None:
            transpose_o(i_t, o_dst)
        if i_res is not None:
            for c in range(NCHC):
                gi = GATE_C[c] if ys else -1
                resid_chunk(i_res, c, at_r, ys[gi] if gi >= 0 else None)

    def phase_c(layer):
        def flush(i):
            @pl.when(layer == 1)
            def _():
                out_copy(i).start()

        best_v[...] = jnp.full((8, 128), -jnp.inf, f32)
        best_i[...] = jnp.zeros((8, 128), i32)
        oproj_step(oa, ata, None, None, 1, ob)

        @pl.when(layer == 0)
        def _():
            cp_wg.wait()
            cp_wu.wait()
            cp_wd.wait()

        def body(j, c):
            i0 = 2 * j
            oproj_step(ob, atb, i0, ata, i0 + 2, oa)
            oproj_step(oa, ata, i0 + 1, atb, i0 + 3, ob)
            flush(i0)
            flush(i0 + 1)
            return c

        lax.fori_loop(0, NB // 2 - 1, body, 0)
        oproj_step(ob, atb, NB - 2, ata, None, None)
        oproj_step(None, None, NB - 1, atb, None, None)
        flush(NB - 2)
        flush(NB - 1)

    def phase_d(layer):
        bv = best_v[...]
        rmax = jnp.max(bv, axis=0, keepdims=True)
        idx = jnp.min(jnp.where(bv == rmax, best_i[...], S), axis=0, keepdims=True)[0, 0]
        idx = jnp.clip(idx, 0, S - 1)
        x2 = xres[pl.ds(idx, 1), :]
        rho = rho_s[pl.ds(idx, 1), 0:1]
        mean = mean_s[pl.ds(idx, 1), 0:1]
        xn = (x2 - mean) * (rho / (1.0 + rho))
        xs = jnp.broadcast_to(xn, (16, D)).astype(bf16)
        nf = F // FC
        hs = []
        y = None
        for c in range(nf + 1):
            if c < nf:
                gate = jnp.dot(xs, wg_v[:, c * FC:(c + 1) * FC], preferred_element_type=f32)
                up = jnp.dot(xs, wu_v[:, c * FC:(c + 1) * FC], preferred_element_type=f32)
                hs.append((gate * jax.nn.sigmoid(gate) * up).astype(bf16))
            if c > 0:
                d = jnp.dot(hs[c - 1], wd_v[(c - 1) * FC:c * FC, :], preferred_element_type=f32)
                y = d if y is None else y + d
        scale = jax.nn.sigmoid(rmax[:, 0:1])
        xres[pl.ds(idx, 1), :] = xres[pl.ds(idx, 1), :] + y[0:1] * scale

        @pl.when(layer == 1)
        def _():
            for i in range(NB):
                out_copy(i).wait()
            g0 = pl.multiple_of((idx // 16) * 16, 16)
            xio[pl.ds(g0, 16), :] = xres[pl.ds(g0, 16), :].astype(bf16)
            fix = pltpu.make_async_copy(xio.at[pl.ds(g0, 16), :], out_hbm.at[pl.ds(g0, 16), :], sem_w.at[7])
            fix.start()
            fix.wait()

    def layer_body(layer, c):
        phase_a(layer)
        phase_b()
        phase_c(layer)
        phase_d(layer)
        return c

    lax.fori_loop(0, 2, layer_body, 0)


@jax.jit
def pallas_interleave_layers__sliding_block__moe_arch_mod__prompt_kernel(
    A_x: jax.Array,
    A_wqkv: jax.Array,
    A_wo: jax.Array,
    B_x: jax.Array,
    B_w_r: jax.Array,
    B_w_gate: jax.Array,
    B_w_up: jax.Array,
    B_w_down: jax.Array,
):
    del B_x
    x = A_x.reshape(S, D)
    any_spec = pl.BlockSpec(memory_space=pl.ANY)
    scratch = [
        pltpu.VMEM((S, D), bf16),
        pltpu.VMEM((D, D), bf16),
        pltpu.VMEM((D, D), bf16),
        pltpu.VMEM((D, D), bf16),
        pltpu.VMEM((D // 2, D), u32),
        pltpu.VMEM((D, D), bf16),
        pltpu.VMEM((D // 2, D), u32),
        pltpu.VMEM((D,), bf16),
        pltpu.VMEM((D, F), bf16),
        pltpu.VMEM((D, F), bf16),
        pltpu.VMEM((F, D), bf16),
        pltpu.VMEM((S, D), f32),
        pltpu.VMEM((S, D), f32),
        pltpu.VMEM((8, 128), f32),
        pltpu.VMEM((8, 128), i32),
        pltpu.VMEM((S, 128), f32),
        pltpu.VMEM((S, 128), f32),
        pltpu.VMEM((8, 128), f32),
        pltpu.VMEM((8, D), f32),
        pltpu.VMEM((TQ // 2, D), u32),
        pltpu.VMEM((TQ // 2, D), u32),
        pltpu.VMEM((S // 2, D), u32),
        pltpu.VMEM((S // 2, D), u32),
        pltpu.VMEM((G, S // 2, 128), u32),
        pltpu.VMEM((G, (S + PAD) // 2, 128), u32),
        pltpu.VMEM((D // 2, S + PAD), u32),
        pltpu.VMEM((D // 2, S), u32),
        pltpu.VMEM((4, 4, 256, 128), f32),
        pltpu.VMEM((4, 4, 8, 128), f32),
        pltpu.VMEM((128, 128), f32),
        pltpu.VMEM((4, 8, 128), f32),
        pltpu.VMEM((TQ, D), f32),
        pltpu.VMEM((TQ, D), f32),
        pltpu.VMEM((TQ // 2, D), u32),
        pltpu.VMEM((TQ // 2, D), u32),
        pltpu.SemaphoreType.DMA((NB,)),
        pltpu.SemaphoreType.DMA((10,)),
        pltpu.SemaphoreType.DMA((NB,)),
    ]
    out = pl.pallas_call(
        _kernel,
        out_shape=jax.ShapeDtypeStruct((S, D), bf16),
        in_specs=[any_spec] * 7,
        out_specs=any_spec,
        scratch_shapes=scratch,
        compiler_params=pltpu.CompilerParams(vmem_limit_bytes=120 * 1024 * 1024),
    )(x, A_wqkv, A_wo, B_w_r, B_w_gate, B_w_up, B_w_down)
    return out.reshape(1, S, D)
```

```python
import jax
import jax.numpy as jnp
from jax import lax
import jax.experimental.pallas as pl
import jax.experimental.pallas.tpu as pltpu

bf16 = jnp.bfloat16
f32 = jnp.float32
u32 = jnp.uint32
i32 = jnp.int32

S = 2048
D = 1024
H = 32
DH = 32
W = 256
F = 3584
G = 8
PAD = 256
TQ = 256
NB = S // TQ
TKV = 512
NSB = S // 128
CH = 32
LNR = 8
NCH = TQ // CH
CHC = 8
NCHC = TQ // CHC
FC = 256
GATE_A = [c * 8 // NCH - 1 for c in range(NCH)]
CHAIN_A = 3
GATE_C = [c * 8 // NCHC - 1 for c in range(NCHC)]
B_ORDER = [1, 0, 2]
B_GATE_T = 6
EPS = 1e-5
NEG = -1e30
QSCALE = (DH ** -0.5) * 1.4426950408889634
NT = (((1,), (1,)), ((), ()))


def _ln(x):
    m = jnp.mean(x, axis=-1, keepdims=True)
    xc = x - m
    v = jnp.mean(xc * xc, axis=-1, keepdims=True)
    return xc * lax.rsqrt(v + EPS)


def _pack_rows(x):
    return pltpu.bitcast(x.astype(bf16), u32)


def _pack_rows_interleaved(x):
    n = x.shape[0] // 16
    x3 = x.reshape(n, 16, x.shape[1])
    a = x3[:, 0:8, :].reshape(n * 8, x.shape[1])
    b = x3[:, 8:16, :].reshape(n * 8, x.shape[1])
    return pltpu.pack_elementwise([a, b], packed_dtype=bf16)


def _gate_first(x, gate, z):
    g = gate[0:8, 0:128] * z
    top = jnp.concatenate([x[0:8, 0:128] + g, x[0:8, 128:]], axis=1)
    return top if x.shape[0] == 8 else jnp.concatenate([top, x[8:]], axis=0)


def _latin_merge(src, blk):
    present = [v for v in src if v is not None]
    zero = jnp.zeros_like(present[0])

    def sel(mask, x, y):
        if x is None and y is None:
            return None
        return jnp.where(mask, zero if x is None else x, zero if y is None else y)

    if len(present) == 1:
        b = [v is not None for v in src].index(True)
        return [jnp.where(blk == (h + b) % 4, src[b], zero) for h in range(4)]
    odd = (blk & 1) == 1
    low = blk < 2
    pair = [sel(odd, src[(a + 1) % 4], src[a]) for a in range(4)]
    out = [sel(low, pair[(-h) % 4], pair[(2 - h) % 4]) for h in range(4)]
    return [zero if v is None else v for v in out]


def _kernel(x_hbm, wqkv_hbm, wo_hbm, wr_hbm, wg_hbm, wu_hbm, wd_hbm,
            out_hbm,
            xio, wq_v, wk_v, wv_v, wvt_v, wo_v, wop_v, wr_v, wg_v, wu_v, wd_v,
            xres, xbuf, best_v, best_i, rho_s, mean_s, z_s, wr8,
            xca, xcb, xc_all, xi_all,
            q_s, k_s, vt_s, ot_s, s_s, m_s, pend_acc, pend_l,
            ata, atb, oa, ob,
            sem_x, sem_w, sem_o):
    def x_copy(i):
        r0 = pl.multiple_of(i * TQ, TQ)
        return pltpu.make_async_copy(x_hbm.at[pl.ds(r0, TQ), :], xio.at[pl.ds(r0, TQ), :], sem_x.at[i])

    def out_copy(i):
        r0 = pl.multiple_of(i * TQ, TQ)
        return pltpu.make_async_copy(xio.at[pl.ds(r0, TQ), :], out_hbm.at[pl.ds(r0, TQ), :], sem_o.at[i])

    cp_wqa = pltpu.make_async_copy(wqkv_hbm.at[:, pl.ds(0, D // 2)], wq_v.at[:, pl.ds(0, D // 2)], sem_w.at[0])
    cp_wqb = pltpu.make_async_copy(wqkv_hbm.at[:, pl.ds(D // 2, D // 2)], wq_v.at[:, pl.ds(D // 2, D // 2)],
                                   sem_w.at[9])
    cp_wk = pltpu.make_async_copy(wqkv_hbm.at[:, pl.ds(D, D)], wk_v, sem_w.at[1])
    cp_wv = pltpu.make_async_copy(wqkv_hbm.at[:, pl.ds(2 * D, D)], wv_v, sem_w.at[8])
    cp_wo = pltpu.make_async_copy(wo_hbm, wo_v, sem_w.at[2])
    cp_wr = pltpu.make_async_copy(wr_hbm, wr_v, sem_w.at[3])
    cp_wg = pltpu.make_async_copy(wg_hbm, wg_v, sem_w.at[4])
    cp_wu = pltpu.make_async_copy(wu_hbm, wu_v, sem_w.at[5])
    cp_wd = pltpu.make_async_copy(wd_hbm, wd_v, sem_w.at[6])

    x_copy(0).start()
    cp_wqa.start()

    z_s[...] = jnp.zeros_like(z_s)
    xres[0:CH, :] = jnp.zeros((CH, D), f32)

    def ln_chunk(layer, i, c, xc_ref, gate, chain=None):
        r0 = i * TQ + c * CH
        h0 = i * (TQ // 2) + c * (CH // 2)
        if not isinstance(r0, int):
            r0 = pl.multiple_of(r0, CH)
            h0 = pl.multiple_of(h0, CH // 2)
        parts = []
        for q in range(CH // LNR):
            rq = r0 + q * LNR
            x_in = xio[pl.ds(rq, LNR), :].astype(f32)
            x_rs = xres[pl.ds(pl.multiple_of(rq * layer, LNR), LNR), :]
            xq = jnp.where(layer == 0, x_in, x_rs)
            xbuf[pl.ds(rq, LNR), :] = xq
            if chain is not None and len(chain) >= CHAIN_A:
                xq = _gate_first(xq, chain[-CHAIN_A], z_s[...])
            elif gate is not None:
                xq = _gate_first(xq, gate, z_s[...])
            parts.append(_ln(xq))
            if chain is not None:
                chain.append(parts[-1])
        xn = jnp.concatenate(parts, axis=0)
        xc = _pack_rows(xn)
        xc_ref[c * CH // 2:(c + 1) * CH // 2, :] = xc
        xc_all[pl.ds(h0, CH // 2), :] = xc
        xi_all[pl.ds(h0, CH // 2), :] = _pack_rows_interleaved(xn)

    def q_step(layer, i, xc_ref, i_next, xc_next, part=(0, G)):
        h0 = i * (TQ // 2)
        if not isinstance(h0, int):
            h0 = pl.multiple_of(h0, TQ // 2)
        a = pltpu.bitcast(xc_ref[...], bf16)
        ys = {}
        for n in range(*part):
            y = jnp.dot(a, wq_v[:, n * 128:(n + 1) * 128], preferred_element_type=f32)
            q_s[n, pl.ds(h0, TQ // 2), :] = _pack_rows(y * QSCALE)
            ys[n] = y
        if i_next is not None:
            chain = []
            for c in range(part[0] * NCH // G, part[1] * NCH // G):
                ln_chunk(layer, i_next, c, xc_next, ys.get(GATE_A[c]), chain)

    def kv_step(i):
        h0 = pl.multiple_of(i * (TKV // 2), TKV // 2)
        a = pltpu.bitcast(xc_all[pl.ds(h0, TKV // 2), :], bf16)
        for n in range(G):
            y = jnp.dot(a, wk_v[:, n * 128:(n + 1) * 128], preferred_element_type=f32)
            k_s[n, pl.ds(PAD // 2 + h0, TKV // 2), :] = _pack_rows(y)
        vt = lax.dot_general(pltpu.bitcast(wvt_v[...], bf16), pltpu.bitcast(xi_all[pl.ds(h0, TKV // 2), :], bf16),
                             NT, preferred_element_type=f32)
        c0 = pl.multiple_of(PAD + i * TKV, 256)
        vt_s[:, pl.ds(c0, TKV)] = _pack_rows(vt)

    def phase_a(layer):
        @pl.when(layer == 0)
        def _():
            x_copy(0).wait()
            x_copy(1).start()
            cp_wqb.start()

        for c in range(NCH):
            ln_chunk(layer, 0, c, xca, None)

        @pl.when(layer == 0)
        def _():
            cp_wqa.wait()
            x_copy(1).wait()
            for i in range(2, NB):
                x_copy(i).start()

        q_step(layer, 0, xca, 1, xcb, part=(0, G // 2))

        @pl.when(layer == 0)
        def _():
            cp_wqb.wait()
            cp_wv.start()
            cp_wo.start()
            cp_wk.start()
            cp_wr.start()

        q_step(layer, 0, xca, 1, xcb, part=(G // 2, G))

        def q_body(j, c):
            i1 = 2 * j + 1

            @pl.when(layer == 0)
            def _():
                x_copy(i1 + 1).wait()
                x_copy(i1 + 2).wait()

            q_step(layer, i1, xcb, i1 + 1, xca)
            q_step(layer, i1 + 1, xca, i1 + 2, xcb)
            return c

        lax.fori_loop(0, NB // 2 - 1, q_body, 0)

        @pl.when(layer == 0)
        def _():
            cp_wv.wait()
            cp_wo.wait()

        q_step(layer, NB - 1, xcb, None, None)
        wvt_v[...] = pltpu.bitcast(wv_v[...].T, u32)
        for c in range(D // 64):
            wop_v[c * 32:(c + 1) * 32, :] = _pack_rows_interleaved(wo_v[c * 64:(c + 1) * 64, :].astype(f32))

        @pl.when(layer == 0)
        def _():
            cp_wk.wait()
            cp_wr.wait()
            wr8[...] = jnp.broadcast_to(wr_v[...].astype(f32).reshape(1, D), (8, D))
            cp_wg.start()
            cp_wu.start()
            cp_wd.start()

        def kv_body(j, c):
            kv_step(j)
            return c

        lax.fori_loop(0, S // TKV, kv_body, 0)

    def qk_stage(g, q0, slot, kstart):
        zi = pltpu.bitcast(z_s[...], i32)
        zi16 = jnp.concatenate([zi, zi], axis=0)
        lane16 = lax.broadcasted_iota(i32, (16, 128), 1) + zi16
        r16 = lax.broadcasted_iota(i32, (16, 128), 0)
        hb16 = lane16 // 32
        dd = r16 - lane16 % 32
        h0 = q0 // 2
        first_rows = None
        for b in range(4):
            first = max(0, kstart - 32 * b)
            base = h0 + 16 * b
            if not isinstance(base, int):
                base = pl.multiple_of(base, 16)
            mid0 = max(first, 32)
            if first == 0:
                parts = [k_s[g, pl.ds(base, 8), :], k_s[g, pl.ds(base + 128, 8), :],
                         k_s[g, pl.ds(base + 8, 8), :], k_s[g, pl.ds(base + 136, 8), :]]
            else:
                parts = [k_s[g, pl.ds(base + 128, 16), :]]
            if mid0 < 256:
                parts.append(k_s[g, pl.ds(base + mid0 // 2, (256 - mid0) // 2), :])
            kw = pltpu.bitcast(jnp.concatenate(parts, axis=0), bf16)
            qu = q_s[g, pl.ds(base, 16), :]
            qall = pltpu.bitcast(
                jnp.concatenate([jnp.where(hb16 == (p - b) % 4, qu, jnp.uint32(0)) for p in range(4)], axis=0),
                bf16)
            st = lax.dot_general(kw, qall, NT, preferred_element_type=f32)
            if b == 3:
                first_rows = st[0:8]
            if first == 0:
                c0 = jnp.where(dd > 0, st[0:16], st[16:32])
                c1 = jnp.where(dd > -16, st[32:48], st[48:64])
                mid = st[64:]
            else:
                c0 = jnp.where(dd > 0, NEG, st[0:16])
                c1 = jnp.where(dd > -16, NEG, st[16:32])
                mid = st[32:]
            s_s[slot, b, 0:16, :] = c0
            s_s[slot, b, 16:32, :] = c1
            x = jnp.concatenate([c0, c1], axis=0)
            if mid0 < 256:
                s_s[slot, b, mid0:256, :] = mid
                x = jnp.concatenate([x, mid], axis=0)
            mm = jnp.max(x.reshape(x.shape[0] // 8, 8, 128), axis=0)
            m_s[slot, b] = jnp.broadcast_to(jnp.max(mm, axis=0, keepdims=True), (8, 128))
        return first_rows

    def pv_stage(g, q0, slot, gate, kstart, defer=False, finish=True):
        r8 = lax.broadcasted_iota(i32, (8, 128), 0)
        c8 = lax.broadcasted_iota(i32, (8, 128), 1) + pltpu.bitcast(z_s[...], i32)
        blk = c8 // 32
        j = c8 % 32

        def tri(u):
            return (jnp.where(16 * u + r8 > j, jnp.uint32(0xFFFF), jnp.uint32(0)) |
                    jnp.where(16 * u + 8 + r8 > j, jnp.uint32(0xFFFF0000), jnp.uint32(0)))

        tris = [tri(0), tri(1)] if kstart < 128 else None
        ms = [m_s[slot, b] for b in range(4)]
        L = [None] * 4
        cache = {}

        def pexp(b, u):
            x = s_s[slot, b, 16 * u:16 * u + 16, :]
            p0 = jnp.exp2(x[0:8] - ms[b])
            p1 = jnp.exp2(x[8:16] - ms[b])
            sm = p0 + p1
            L[b] = sm if L[b] is None else L[b] + sm
            return pltpu.pack_elementwise([p0, p1], packed_dtype=bf16)

        def get_p(b, u):
            first = max(0, kstart - 32 * b)
            if u < 0 or u >= 18 or 16 * u < first:
                return None
            if first > 0:
                return pexp(b, u - 16) if u >= 16 else pexp(b, u)
            if u < 2 or u >= 16:
                if (b, u) not in cache:
                    pk = pexp(b, u % 16)
                    lo = pk & tris[u % 16]
                    cache[(b, u % 16)] = lo
                    cache[(b, u % 16 + 16)] = pk ^ lo
                return cache.pop((b, u))
            return pexp(b, u)

        accs = [None] * 4
        for k in [k for k in B_ORDER if k >= kstart // 128]:
            wts = [[] for _ in range(4)]
            for t in range(8 * k, 8 * k + 8):
                if t == B_GATE_T and gate is not None:
                    gv = gate * z_s[...]
                    for b in range(4):
                        ms[b] = ms[b] + gv
                src = [get_p(b, t - 2 * b) for b in range(4)]
                for h, w in enumerate(_latin_merge(src, blk)):
                    wts[h].append(w)
            c0 = q0 + 128 * k
            if not isinstance(c0, int):
                c0 = pl.multiple_of(c0, 128)
            for h in range(4):
                pt = pltpu.bitcast(jnp.concatenate(wts[h], axis=0), bf16)
                vth = pltpu.bitcast(vt_s[pl.ds((g * 4 + h) * 16, 16), pl.ds(c0, 128)], bf16)
                d = jnp.dot(vth, pt, preferred_element_type=f32)
                accs[h] = d if accs[h] is None else accs[h] + d
        if defer:
            for h in range(4):
                pend_acc[h * 32:(h + 1) * 32, :] = accs[h]
                pend_l[h] = L[h]
        if finish:
            pv_finish(g, q0, accs, L)

    def pv_finish(g, q0, accs, L):
        blk = (lax.broadcasted_iota(i32, (8, 128), 1) + pltpu.bitcast(z_s[...], i32)) // 32
        L = [jnp.broadcast_to(jnp.sum(l, axis=0, keepdims=True), (8, 128)) for l in L]
        outs = []
        for h, lh in enumerate(_latin_merge(L, blk)):
            r0 = pl.reciprocal(lh, approx=True)
            rl = r0 * (2.0 - lh * r0)
            ot = (accs[h].reshape(4, 8, 128) * rl[None]).reshape(32, 128)
            if h > 0:
                ot = pltpu.roll(ot, 128 - 32 * h, axis=1)
            outs.append(ot)
        ot_s[g * 64:(g + 1) * 64, pl.ds(q0, 128)] = _pack_rows_interleaved(jnp.concatenate(outs, axis=0))

    def finish_pending(q0):
        pv_finish(G - 1, q0, [pend_acc[h * 32:(h + 1) * 32, :] for h in range(4)], [pend_l[h] for h in range(4)])

    def sub_block(q0, qn, defer_last=False):
        for g in range(G):
            if g + 1 < G:
                gate = qk_stage(g + 1, q0, (g + 1) % 2, 0)
            else:
                gate = qk_stage(0, qn, 0, 0)
            last = defer_last and g == G - 1
            pv_stage(g, q0, g % 2, gate, 0, defer=last, finish=not last)

    def transpose_o(i, o_dst):
        r0 = i * TQ
        if not isinstance(r0, int):
            r0 = pl.multiple_of(r0, TQ)
        o_dst[...] = pltpu.bitcast(pltpu.bitcast(ot_s[:, pl.ds(r0, TQ)], bf16).T, u32)

    def phase_b():
        qk_stage(0, 0, 2, PAD)
        qk_stage(0, 128, 0, PAD - 128)
        for g in range(G):
            if g + 1 < G:
                qk_stage(g + 1, 0, 2 + (g + 1) % 2, PAD)
            pv_stage(g, 0, 2 + g % 2, None, PAD)
            if g + 1 < G:
                qk_stage(g + 1, 128, (g + 1) % 2, PAD - 128)
            else:
                qk_stage(0, 256, 0, 0)
            pv_stage(g, 128, g % 2, None, PAD - 128, defer=(g == G - 1))
        transpose_o(0, oa)

        def body(j, c):
            q0 = pl.multiple_of(j * 256, 256)
            q1 = pl.multiple_of(q0 + 128, 128)
            qn = pl.multiple_of(jnp.minimum(q0 + 256, S - 128), 128)
            finish_pending(pl.multiple_of(q0 - 128, 128))
            sub_block(q0, q1)
            sub_block(q1, qn, defer_last=True)
            return c

        lax.fori_loop(1, NSB // 2, body, 0)
        finish_pending(S - 128)

    def resid_chunk(i, c, at_ref, gate, best):
        r0 = i * TQ + c * CHC
        if not isinstance(r0, int):
            r0 = pl.multiple_of(r0, CHC)
        x1 = xbuf[pl.ds(r0, CHC), :] + at_ref[c * CHC:(c + 1) * CHC, :]
        if gate is not None:
            x1 = _gate_first(x1, gate, z_s[...])
        m = jnp.mean(x1, axis=-1, keepdims=True)
        xc = x1 - m
        v = jnp.mean(xc * xc, axis=-1, keepdims=True)
        rho = lax.rsqrt(v + EPS)
        xn = xc * rho
        r = jnp.sum(xn * wr8[0:1, :], axis=-1, keepdims=True)
        rb = jnp.broadcast_to(r, (CHC, 128)).astype(bf16).astype(f32)
        rows = lax.broadcasted_iota(i32, (8, 128), 0) + r0
        bv, bi = best
        for q in range(CHC // 8):
            cand = rb[8 * q:8 * q + 8]
            better = cand > bv
            bv = jnp.where(better, cand, bv)
            bi = jnp.where(better, rows + 8 * q, bi)
        rho_s[pl.ds(r0, CHC), :] = jnp.broadcast_to(rho, (CHC, 128))
        mean_s[pl.ds(r0, CHC), :] = jnp.broadcast_to(m, (CHC, 128))
        x2 = x1 + xn
        xres[pl.ds(r0, CHC), :] = x2
        xio[pl.ds(r0, CHC), :] = x2.astype(bf16)
        return bv, bi

    def oproj_step(o_src, at_w, i_res, at_r, i_t, o_dst):
        ys = []
        if o_src is not None:
            a = pltpu.bitcast(o_src[...], bf16)
            for n in range(G):
                y = jnp.dot(a, pltpu.bitcast(wop_v[:, n * 128:(n + 1) * 128], bf16), preferred_element_type=f32)
                at_w[:, n * 128:(n + 1) * 128] = y
                ys.append(y)
        if i_t is not None:
            transpose_o(i_t, o_dst)
        if i_res is not None:
            best = (best_v[...], best_i[...])
            for c in range(NCHC):
                gi = GATE_C[c] if ys else -1
                best = resid_chunk(i_res, c, at_r, ys[gi] if gi >= 0 else None, best)
                if ys or c == NCHC - 1:
                    best_v[...], best_i[...] = best
                    best = (best_v[...], best_i[...])

    def phase_c(layer):
        def flush(i):
            @pl.when(layer == 1)
            def _():
                out_copy(i).start()

        best_v[...] = jnp.full((8, 128), -jnp.inf, f32)
        best_i[...] = jnp.zeros((8, 128), i32)
        oproj_step(oa, ata, None, None, 1, ob)

        @pl.when(layer == 0)
        def _():
            cp_wg.wait()
            cp_wu.wait()
            cp_wd.wait()

        def body(j, c):
            i0 = 2 * j
            oproj_step(ob, atb, i0, ata, i0 + 2, oa)
            oproj_step(oa, ata, i0 + 1, atb, i0 + 3, ob)
            flush(i0)
            flush(i0 + 1)
            return c

        lax.fori_loop(0, NB // 2 - 1, body, 0)
        oproj_step(ob, atb, NB - 2, ata, None, None)
        oproj_step(None, None, NB - 1, atb, None, None)
        flush(NB - 2)
        flush(NB - 1)

    def phase_d(layer):
        bv = best_v[...]
        rmax = jnp.max(bv, axis=0, keepdims=True)
        idx = jnp.min(jnp.where(bv == rmax, best_i[...], S), axis=0, keepdims=True)[0, 0]
        idx = jnp.clip(idx, 0, S - 1)
        x2 = xres[pl.ds(idx, 1), :]
        rho = rho_s[pl.ds(idx, 1), 0:1]
        mean = mean_s[pl.ds(idx, 1), 0:1]
        xn = (x2 - mean) * (rho / (1.0 + rho))
        xs = jnp.broadcast_to(xn, (16, D)).astype(bf16)
        nf = F // FC
        hs = []
        y = None
        for c in range(nf + 1):
            if c < nf:
                gate = jnp.dot(xs, wg_v[:, c * FC:(c + 1) * FC], preferred_element_type=f32)
                up = jnp.dot(xs, wu_v[:, c * FC:(c + 1) * FC], preferred_element_type=f32)
                hs.append((gate * jax.nn.sigmoid(gate) * up).astype(bf16))
            if c > 0:
                d = jnp.dot(hs[c - 1], wd_v[(c - 1) * FC:c * FC, :], preferred_element_type=f32)
                y = d if y is None else y + d
        scale = jax.nn.sigmoid(rmax[:, 0:1])
        xres[pl.ds(idx, 1), :] = xres[pl.ds(idx, 1), :] + y[0:1] * scale

        @pl.when(layer == 1)
        def _():
            for i in range(NB):
                out_copy(i).wait()
            g0 = pl.multiple_of((idx // 16) * 16, 16)
            xio[pl.ds(g0, 16), :] = xres[pl.ds(g0, 16), :].astype(bf16)
            fix = pltpu.make_async_copy(xio.at[pl.ds(g0, 16), :], out_hbm.at[pl.ds(g0, 16), :], sem_w.at[7])
            fix.start()
            fix.wait()

    def layer_body(layer, c):
        phase_a(layer)
        phase_b()
        phase_c(layer)
        phase_d(layer)
        return c

    lax.fori_loop(0, 2, layer_body, 0)


@jax.jit
def pallas_interleave_layers__sliding_block__moe_arch_mod__prompt_kernel(
    A_x: jax.Array,
    A_wqkv: jax.Array,
    A_wo: jax.Array,
    B_x: jax.Array,
    B_w_r: jax.Array,
    B_w_gate: jax.Array,
    B_w_up: jax.Array,
    B_w_down: jax.Array,
):
    del B_x
    x = A_x.reshape(S, D)
    any_spec = pl.BlockSpec(memory_space=pl.ANY)
    scratch = [
        pltpu.VMEM((S, D), bf16),
        pltpu.VMEM((D, D), bf16),
        pltpu.VMEM((D, D), bf16),
        pltpu.VMEM((D, D), bf16),
        pltpu.VMEM((D // 2, D), u32),
        pltpu.VMEM((D, D), bf16),
        pltpu.VMEM((D // 2, D), u32),
        pltpu.VMEM((D,), bf16),
        pltpu.VMEM((D, F), bf16),
        pltpu.VMEM((D, F), bf16),
        pltpu.VMEM((F, D), bf16),
        pltpu.VMEM((S, D), f32),
        pltpu.VMEM((S, D), f32),
        pltpu.VMEM((8, 128), f32),
        pltpu.VMEM((8, 128), i32),
        pltpu.VMEM((S, 128), f32),
        pltpu.VMEM((S, 128), f32),
        pltpu.VMEM((8, 128), f32),
        pltpu.VMEM((8, D), f32),
        pltpu.VMEM((TQ // 2, D), u32),
        pltpu.VMEM((TQ // 2, D), u32),
        pltpu.VMEM((S // 2, D), u32),
        pltpu.VMEM((S // 2, D), u32),
        pltpu.VMEM((G, S // 2, 128), u32),
        pltpu.VMEM((G, (S + PAD) // 2, 128), u32),
        pltpu.VMEM((D // 2, S + PAD), u32),
        pltpu.VMEM((D // 2, S), u32),
        pltpu.VMEM((4, 4, 256, 128), f32),
        pltpu.VMEM((4, 4, 8, 128), f32),
        pltpu.VMEM((128, 128), f32),
        pltpu.VMEM((4, 8, 128), f32),
        pltpu.VMEM((TQ, D), f32),
        pltpu.VMEM((TQ, D), f32),
        pltpu.VMEM((TQ // 2, D), u32),
        pltpu.VMEM((TQ // 2, D), u32),
        pltpu.SemaphoreType.DMA((NB,)),
        pltpu.SemaphoreType.DMA((10,)),
        pltpu.SemaphoreType.DMA((NB,)),
    ]
    out = pl.pallas_call(
        _kernel,
        out_shape=jax.ShapeDtypeStruct((S, D), bf16),
        in_specs=[any_spec] * 7,
        out_specs=any_spec,
        scratch_shapes=scratch,
        compiler_params=pltpu.CompilerParams(vmem_limit_bytes=120 * 1024 * 1024),
    )(x, A_wqkv, A_wo, B_w_r, B_w_gate, B_w_up, B_w_down)
    return out.reshape(1, S, D)
```

```python
import jax
import jax.numpy as jnp
from jax import lax
import jax.experimental.pallas as pl
import jax.experimental.pallas.tpu as pltpu

bf16 = jnp.bfloat16
f32 = jnp.float32
u32 = jnp.uint32
i32 = jnp.int32

S = 2048
D = 1024
H = 32
DH = 32
W = 256
F = 3584
G = 8
PAD = 256
TQ = 256
NB = S // TQ
TKV = 512
NSB = S // 128
CH = 32
LNR = 8
NCH = TQ // CH
CHC = 8
NCHC = TQ // CHC
FC = 256
GATE_A = [c * 8 // NCH - 1 for c in range(NCH)]
CHAIN_A = 3
GATE_C = [c * 8 // NCHC - 1 for c in range(NCHC)]
B_ORDER = [1, 0, 2]
B_GATE_T = 6
EPS = 1e-5
NEG = -1e30
QSCALE = (DH ** -0.5) * 1.4426950408889634
NT = (((1,), (1,)), ((), ()))


def _ln(x):
    m = jnp.mean(x, axis=-1, keepdims=True)
    xc = x - m
    v = jnp.mean(xc * xc, axis=-1, keepdims=True)
    return xc * lax.rsqrt(v + EPS)


def _pack_rows(x):
    return pltpu.bitcast(x.astype(bf16), u32)


def _pack_rows_interleaved(x):
    n = x.shape[0] // 16
    x3 = x.reshape(n, 16, x.shape[1])
    a = x3[:, 0:8, :].reshape(n * 8, x.shape[1])
    b = x3[:, 8:16, :].reshape(n * 8, x.shape[1])
    return pltpu.pack_elementwise([a, b], packed_dtype=bf16)


def _gate_first(x, gate, z):
    g = gate[0:8, 0:128] * z
    top = jnp.concatenate([x[0:8, 0:128] + g, x[0:8, 128:]], axis=1)
    return top if x.shape[0] == 8 else jnp.concatenate([top, x[8:]], axis=0)


def _latin_merge(src, blk):
    present = [v for v in src if v is not None]
    zero = jnp.zeros_like(present[0])

    def sel(mask, x, y):
        if x is None and y is None:
            return None
        return jnp.where(mask, zero if x is None else x, zero if y is None else y)

    if len(present) == 1:
        b = [v is not None for v in src].index(True)
        return [jnp.where(blk == (h + b) % 4, src[b], zero) for h in range(4)]
    odd = (blk & 1) == 1
    low = blk < 2
    pair = [sel(odd, src[(a + 1) % 4], src[a]) for a in range(4)]
    out = [sel(low, pair[(-h) % 4], pair[(2 - h) % 4]) for h in range(4)]
    return [zero if v is None else v for v in out]


def _kernel(x_hbm, wqkv_hbm, wo_hbm, wr_hbm, wg_hbm, wu_hbm, wd_hbm,
            out_hbm,
            xio, wq_v, wk_v, wv_v, wvt_v, wo_v, wop_v, wr_v, wg_v, wu_v, wd_v,
            xres, xbuf, best_v, best_i, rho_s, mean_s, z_s, wr8,
            xca, xcb, xc_all, xi_all,
            q_s, k_s, vt_s, ot_s, s_s, m_s, pend_acc, pend_l,
            ata, atb, oa, ob,
            sem_x, sem_w, sem_o):
    def x_copy(i):
        r0 = pl.multiple_of(i * TQ, TQ)
        return pltpu.make_async_copy(x_hbm.at[pl.ds(r0, TQ), :], xio.at[pl.ds(r0, TQ), :], sem_x.at[i])

    def out_copy(i):
        r0 = pl.multiple_of(i * TQ, TQ)
        return pltpu.make_async_copy(xio.at[pl.ds(r0, TQ), :], out_hbm.at[pl.ds(r0, TQ), :], sem_o.at[i])

    cp_wqa = pltpu.make_async_copy(wqkv_hbm.at[:, pl.ds(0, D // 2)], wq_v.at[:, pl.ds(0, D // 2)], sem_w.at[0])
    cp_wqb = pltpu.make_async_copy(wqkv_hbm.at[:, pl.ds(D // 2, D // 2)], wq_v.at[:, pl.ds(D // 2, D // 2)],
                                   sem_w.at[9])
    cp_wk = pltpu.make_async_copy(wqkv_hbm.at[:, pl.ds(D, D)], wk_v, sem_w.at[1])
    cp_wv = pltpu.make_async_copy(wqkv_hbm.at[:, pl.ds(2 * D, D)], wv_v, sem_w.at[8])
    cp_wo = pltpu.make_async_copy(wo_hbm, wo_v, sem_w.at[2])
    cp_wr = pltpu.make_async_copy(wr_hbm, wr_v, sem_w.at[3])
    cp_wg = pltpu.make_async_copy(wg_hbm, wg_v, sem_w.at[4])
    cp_wu = pltpu.make_async_copy(wu_hbm, wu_v, sem_w.at[5])
    cp_wd = pltpu.make_async_copy(wd_hbm, wd_v, sem_w.at[6])

    x_copy(0).start()
    cp_wqa.start()

    z_s[...] = jnp.zeros_like(z_s)
    xres[0:CH, :] = jnp.zeros((CH, D), f32)

    def ln_chunk(layer, i, c, xc_ref, gate, chain=None):
        r0 = i * TQ + c * CH
        h0 = i * (TQ // 2) + c * (CH // 2)
        if not isinstance(r0, int):
            r0 = pl.multiple_of(r0, CH)
            h0 = pl.multiple_of(h0, CH // 2)
        parts = []
        for q in range(CH // LNR):
            rq = r0 + q * LNR
            x_in = xio[pl.ds(rq, LNR), :].astype(f32)
            x_rs = xres[pl.ds(pl.multiple_of(rq * layer, LNR), LNR), :]
            xq = jnp.where(layer == 0, x_in, x_rs)
            xbuf[pl.ds(rq, LNR), :] = xq
            if chain is not None and len(chain) >= CHAIN_A:
                xq = _gate_first(xq, chain[-CHAIN_A], z_s[...])
            elif gate is not None:
                xq = _gate_first(xq, gate, z_s[...])
            parts.append(_ln(xq))
            if chain is not None:
                chain.append(parts[-1])
        xn = jnp.concatenate(parts, axis=0)
        xc = _pack_rows(xn)
        xc_ref[c * CH // 2:(c + 1) * CH // 2, :] = xc
        xc_all[pl.ds(h0, CH // 2), :] = xc
        xi_all[pl.ds(h0, CH // 2), :] = _pack_rows_interleaved(xn)

    def q_step(layer, i, xc_ref, i_next, xc_next, part=(0, G)):
        h0 = i * (TQ // 2)
        if not isinstance(h0, int):
            h0 = pl.multiple_of(h0, TQ // 2)
        a = pltpu.bitcast(xc_ref[...], bf16)
        ys = {}
        for n in range(*part):
            y = jnp.dot(a, wq_v[:, n * 128:(n + 1) * 128], preferred_element_type=f32)
            q_s[n, pl.ds(h0, TQ // 2), :] = _pack_rows(y * QSCALE)
            ys[n] = y
        if i_next is not None:
            chain = []
            for c in range(part[0] * NCH // G, part[1] * NCH // G):
                ln_chunk(layer, i_next, c, xc_next, ys.get(GATE_A[c]), chain)

    def kv_step(i):
        h0 = pl.multiple_of(i * (TKV // 2), TKV // 2)
        a = pltpu.bitcast(xc_all[pl.ds(h0, TKV // 2), :], bf16)
        for n in range(G):
            y = jnp.dot(a, wk_v[:, n * 128:(n + 1) * 128], preferred_element_type=f32)
            k_s[n, pl.ds(PAD // 2 + h0, TKV // 2), :] = _pack_rows(y)
        vt = lax.dot_general(pltpu.bitcast(wvt_v[...], bf16), pltpu.bitcast(xi_all[pl.ds(h0, TKV // 2), :], bf16),
                             NT, preferred_element_type=f32)
        c0 = pl.multiple_of(PAD + i * TKV, 256)
        vt_s[:, pl.ds(c0, TKV)] = _pack_rows(vt)

    def phase_a(layer):
        @pl.when(layer == 0)
        def _():
            x_copy(0).wait()
            x_copy(1).start()
            cp_wqb.start()

        for c in range(NCH):
            ln_chunk(layer, 0, c, xca, None)

        @pl.when(layer == 0)
        def _():
            cp_wqa.wait()
            x_copy(1).wait()
            for i in range(2, NB):
                x_copy(i).start()

        q_step(layer, 0, xca, 1, xcb, part=(0, G // 2))

        @pl.when(layer == 0)
        def _():
            cp_wqb.wait()
            cp_wv.start()
            cp_wo.start()
            cp_wk.start()
            cp_wr.start()

        q_step(layer, 0, xca, 1, xcb, part=(G // 2, G))

        def q_body(j, c):
            i1 = 2 * j + 1

            @pl.when(layer == 0)
            def _():
                x_copy(i1 + 1).wait()
                x_copy(i1 + 2).wait()

            q_step(layer, i1, xcb, i1 + 1, xca)
            q_step(layer, i1 + 1, xca, i1 + 2, xcb)
            return c

        lax.fori_loop(0, NB // 2 - 1, q_body, 0)

        @pl.when(layer == 0)
        def _():
            cp_wv.wait()
            cp_wo.wait()

        q_step(layer, NB - 1, xcb, None, None)
        wvt_v[...] = pltpu.bitcast(wv_v[...].T, u32)
        for c in range(D // 64):
            wop_v[c * 32:(c + 1) * 32, :] = _pack_rows_interleaved(wo_v[c * 64:(c + 1) * 64, :].astype(f32))

        @pl.when(layer == 0)
        def _():
            cp_wk.wait()
            cp_wr.wait()
            wr8[...] = jnp.broadcast_to(wr_v[...].astype(f32).reshape(1, D), (8, D))
            cp_wg.start()
            cp_wu.start()
            cp_wd.start()

        def kv_body(j, c):
            kv_step(j)
            return c

        lax.fori_loop(0, S // TKV, kv_body, 0)

    def qk_stage(g, q0, slot, kstart):
        zi = pltpu.bitcast(z_s[...], i32)
        zi16 = jnp.concatenate([zi, zi], axis=0)
        lane16 = lax.broadcasted_iota(i32, (16, 128), 1) + zi16
        r16 = lax.broadcasted_iota(i32, (16, 128), 0)
        hb16 = lane16 // 32
        dd = r16 - lane16 % 32
        h0 = q0 // 2
        first_rows = None
        for b in range(4):
            first = max(0, kstart - 32 * b)
            base = h0 + 16 * b
            if not isinstance(base, int):
                base = pl.multiple_of(base, 16)
            mid0 = max(first, 32)
            if first == 0:
                parts = [k_s[g, pl.ds(base, 8), :], k_s[g, pl.ds(base + 128, 8), :],
                         k_s[g, pl.ds(base + 8, 8), :], k_s[g, pl.ds(base + 136, 8), :]]
            else:
                parts = [k_s[g, pl.ds(base + 128, 16), :]]
            if mid0 < 256:
                parts.append(k_s[g, pl.ds(base + mid0 // 2, (256 - mid0) // 2), :])
            kw = pltpu.bitcast(jnp.concatenate(parts, axis=0), bf16)
            qu = q_s[g, pl.ds(base, 16), :]
            qall = pltpu.bitcast(
                jnp.concatenate([jnp.where(hb16 == (p - b) % 4, qu, jnp.uint32(0)) for p in range(4)], axis=0),
                bf16)
            st = lax.dot_general(kw, qall, NT, preferred_element_type=f32)
            if b == 3:
                first_rows = st[0:8]
            if first == 0:
                c0 = jnp.where(dd > 0, st[0:16], st[16:32])
                c1 = jnp.where(dd > -16, st[32:48], st[48:64])
                mid = st[64:]
            else:
                c0 = jnp.where(dd > 0, NEG, st[0:16])
                c1 = jnp.where(dd > -16, NEG, st[16:32])
                mid = st[32:]
            s_s[slot, b, 0:16, :] = c0
            s_s[slot, b, 16:32, :] = c1
            x = jnp.concatenate([c0, c1], axis=0)
            if mid0 < 256:
                s_s[slot, b, mid0:256, :] = mid
                x = jnp.concatenate([x, mid], axis=0)
            mm = jnp.max(x.reshape(x.shape[0] // 8, 8, 128), axis=0)
            m_s[slot, b] = jnp.broadcast_to(jnp.max(mm, axis=0, keepdims=True), (8, 128))
        return first_rows

    def pv_stage(g, q0, slot, gate, kstart, defer=False, finish=True):
        r8 = lax.broadcasted_iota(i32, (8, 128), 0)
        c8 = lax.broadcasted_iota(i32, (8, 128), 1) + pltpu.bitcast(z_s[...], i32)
        blk = c8 // 32
        j = c8 % 32

        def tri(u):
            return (jnp.where(16 * u + r8 > j, jnp.uint32(0xFFFF), jnp.uint32(0)) |
                    jnp.where(16 * u + 8 + r8 > j, jnp.uint32(0xFFFF0000), jnp.uint32(0)))

        tris = [tri(0), tri(1)] if kstart < 128 else None
        ms = [m_s[slot, b] for b in range(4)]
        L = [None] * 4
        cache = {}

        def pexp(b, u):
            x = s_s[slot, b, 16 * u:16 * u + 16, :]
            p0 = jnp.exp2(x[0:8] - ms[b])
            p1 = jnp.exp2(x[8:16] - ms[b])
            sm = p0 + p1
            L[b] = sm if L[b] is None else L[b] + sm
            return pltpu.pack_elementwise([p0, p1], packed_dtype=bf16)

        def get_p(b, u):
            first = max(0, kstart - 32 * b)
            if u < 0 or u >= 18 or 16 * u < first:
                return None
            if first > 0:
                return pexp(b, u - 16) if u >= 16 else pexp(b, u)
            if u < 2 or u >= 16:
                if (b, u) not in cache:
                    pk = pexp(b, u % 16)
                    lo = pk & tris[u % 16]
                    cache[(b, u % 16)] = lo
                    cache[(b, u % 16 + 16)] = pk ^ lo
                return cache.pop((b, u))
            return pexp(b, u)

        accs = [None] * 4
        for k in [k for k in B_ORDER if k >= kstart // 128]:
            wts = [[] for _ in range(4)]
            for t in range(8 * k, 8 * k + 8):
                if t == B_GATE_T and gate is not None:
                    gv = gate * z_s[...]
                    for b in range(4):
                        ms[b] = ms[b] + gv
                src = [get_p(b, t - 2 * b) for b in range(4)]
                for h, w in enumerate(_latin_merge(src, blk)):
                    wts[h].append(w)
            c0 = q0 + 128 * k
            if not isinstance(c0, int):
                c0 = pl.multiple_of(c0, 128)
            for h in range(4):
                pt = pltpu.bitcast(jnp.concatenate(wts[h], axis=0), bf16)
                vth = pltpu.bitcast(vt_s[pl.ds((g * 4 + h) * 16, 16), pl.ds(c0, 128)], bf16)
                d = jnp.dot(vth, pt, preferred_element_type=f32)
                accs[h] = d if accs[h] is None else accs[h] + d
        if defer:
            for h in range(4):
                pend_acc[h * 32:(h + 1) * 32, :] = accs[h]
                pend_l[h] = L[h]
        if finish:
            pv_finish(g, q0, accs, L)

    def pv_finish(g, q0, accs, L):
        blk = (lax.broadcasted_iota(i32, (8, 128), 1) + pltpu.bitcast(z_s[...], i32)) // 32
        L = [jnp.broadcast_to(jnp.sum(l, axis=0, keepdims=True), (8, 128)) for l in L]
        outs = []
        for h, lh in enumerate(_latin_merge(L, blk)):
            r0 = pl.reciprocal(lh, approx=True)
            rl = r0 * (2.0 - lh * r0)
            ot = (accs[h].reshape(4, 8, 128) * rl[None]).reshape(32, 128)
            if h > 0:
                ot = pltpu.roll(ot, 128 - 32 * h, axis=1)
            outs.append(ot)
        ot_s[g * 64:(g + 1) * 64, pl.ds(q0, 128)] = _pack_rows_interleaved(jnp.concatenate(outs, axis=0))

    def finish_pending(q0):
        pv_finish(G - 1, q0, [pend_acc[h * 32:(h + 1) * 32, :] for h in range(4)], [pend_l[h] for h in range(4)])

    def sub_block(q0, qn, defer_last=False):
        for g in range(G):
            if g + 1 < G:
                gate = qk_stage(g + 1, q0, (g + 1) % 2, 0)
            else:
                gate = qk_stage(0, qn, 0, 0)
            last = defer_last and g == G - 1
            pv_stage(g, q0, g % 2, gate, 0, defer=last, finish=not last)

    def transpose_o(i, o_dst):
        r0 = i * TQ
        if not isinstance(r0, int):
            r0 = pl.multiple_of(r0, TQ)
        o_dst[...] = pltpu.bitcast(pltpu.bitcast(ot_s[:, pl.ds(r0, TQ)], bf16).T, u32)

    def phase_b():
        qk_stage(0, 0, 2, PAD)
        qk_stage(0, 128, 0, PAD - 128)
        for g in range(G):
            if g + 1 < G:
                qk_stage(g + 1, 0, 2 + (g + 1) % 2, PAD)
            pv_stage(g, 0, 2 + g % 2, None, PAD)
            if g + 1 < G:
                qk_stage(g + 1, 128, (g + 1) % 2, PAD - 128)
            else:
                qk_stage(0, 256, 0, 0)
            pv_stage(g, 128, g % 2, None, PAD - 128, defer=(g == G - 1))
        transpose_o(0, oa)

        def body(j, c):
            q0 = pl.multiple_of(j * 256, 256)
            q1 = pl.multiple_of(q0 + 128, 128)
            qn = pl.multiple_of(jnp.minimum(q0 + 256, S - 128), 128)
            finish_pending(pl.multiple_of(q0 - 128, 128))
            sub_block(q0, q1)
            sub_block(q1, qn, defer_last=True)
            return c

        lax.fori_loop(1, NSB // 2, body, 0)
        finish_pending(S - 128)

    def resid_chunk(i, c, at_ref, gate, best):
        r0 = i * TQ + c * CHC
        if not isinstance(r0, int):
            r0 = pl.multiple_of(r0, CHC)
        x1 = xbuf[pl.ds(r0, CHC), :] + at_ref[c * CHC:(c + 1) * CHC, :]
        if gate is not None:
            x1 = _gate_first(x1, gate, z_s[...])
        m = jnp.mean(x1, axis=-1, keepdims=True)
        xc = x1 - m
        v = jnp.mean(xc * xc, axis=-1, keepdims=True)
        rho = lax.rsqrt(v + EPS)
        xn = xc * rho
        r = jnp.sum(xn * wr8[0:1, :], axis=-1, keepdims=True)
        rb = jnp.broadcast_to(r, (CHC, 128)).astype(bf16).astype(f32)
        rows = lax.broadcasted_iota(i32, (8, 128), 0) + r0
        bv, bi = best
        for q in range(CHC // 8):
            cand = rb[8 * q:8 * q + 8]
            better = cand > bv
            bv = jnp.where(better, cand, bv)
            bi = jnp.where(better, rows + 8 * q, bi)
        rho_s[pl.ds(r0, CHC), :] = jnp.broadcast_to(rho, (CHC, 128))
        mean_s[pl.ds(r0, CHC), :] = jnp.broadcast_to(m, (CHC, 128))
        x2 = x1 + xn
        xres[pl.ds(r0, CHC), :] = x2
        xio[pl.ds(r0, CHC), :] = x2.astype(bf16)
        return bv, bi

    def oproj_step(o_src, at_w, i_res, at_r, i_t, o_dst, rows=(0, TQ), chunks=(0, NCHC)):
        ys = []
        if o_src is not None:
            a = pltpu.bitcast(o_src[rows[0] // 2:rows[1] // 2, :], bf16)
            for n in range(G):
                y = jnp.dot(a, pltpu.bitcast(wop_v[:, n * 128:(n + 1) * 128], bf16), preferred_element_type=f32)
                at_w[rows[0]:rows[1], n * 128:(n + 1) * 128] = y
                ys.append(y)
        if i_t is not None:
            transpose_o(i_t, o_dst)
        if i_res is not None:
            best = (best_v[...], best_i[...])
            nch = chunks[1] - chunks[0]
            for c in range(*chunks):
                gi = (c - chunks[0]) * G // nch - 1 if ys else -1
                best = resid_chunk(i_res, c, at_r, ys[gi] if gi >= 0 else None, best)
                if ys or c == chunks[1] - 1:
                    best_v[...], best_i[...] = best
                    best = (best_v[...], best_i[...])

    def phase_c(layer):
        def flush(i):
            @pl.when(layer == 1)
            def _():
                out_copy(i).start()

        best_v[...] = jnp.full((8, 128), -jnp.inf, f32)
        best_i[...] = jnp.zeros((8, 128), i32)
        oproj_step(oa, ata, None, None, 1, ob)

        @pl.when(layer == 0)
        def _():
            cp_wg.wait()
            cp_wu.wait()
            cp_wd.wait()

        def body(j, c):
            i0 = 2 * j
            oproj_step(ob, atb, i0, ata, i0 + 2, oa)
            oproj_step(oa, ata, i0 + 1, atb, i0 + 3, ob)
            flush(i0)
            flush(i0 + 1)
            return c

        lax.fori_loop(0, NB // 2 - 1, body, 0)
        oproj_step(ob, atb, NB - 2, ata, None, None, rows=(0, TQ // 2))
        oproj_step(ob, atb, NB - 1, atb, None, None, rows=(TQ // 2, TQ), chunks=(0, NCHC // 2))
        oproj_step(None, None, NB - 1, atb, None, None, chunks=(NCHC // 2, NCHC))
        flush(NB - 2)
        flush(NB - 1)

    def phase_d(layer):
        bv = best_v[...]
        rmax = jnp.max(bv, axis=0, keepdims=True)
        idx = jnp.min(jnp.where(bv == rmax, best_i[...], S), axis=0, keepdims=True)[0, 0]
        idx = jnp.clip(idx, 0, S - 1)
        x2 = xres[pl.ds(idx, 1), :]
        rho = rho_s[pl.ds(idx, 1), 0:1]
        mean = mean_s[pl.ds(idx, 1), 0:1]
        xn = (x2 - mean) * (rho / (1.0 + rho))
        xs = jnp.broadcast_to(xn, (16, D)).astype(bf16)
        nf = F // FC
        hs = []
        y = None
        for c in range(nf + 1):
            if c < nf:
                gate = jnp.dot(xs, wg_v[:, c * FC:(c + 1) * FC], preferred_element_type=f32)
                up = jnp.dot(xs, wu_v[:, c * FC:(c + 1) * FC], preferred_element_type=f32)
                hs.append((gate * jax.nn.sigmoid(gate) * up).astype(bf16))
            if c > 0:
                d = jnp.dot(hs[c - 1], wd_v[(c - 1) * FC:c * FC, :], preferred_element_type=f32)
                y = d if y is None else y + d
        scale = jax.nn.sigmoid(rmax[:, 0:1])
        xres[pl.ds(idx, 1), :] = xres[pl.ds(idx, 1), :] + y[0:1] * scale

        @pl.when(layer == 1)
        def _():
            for i in range(NB):
                out_copy(i).wait()
            g0 = pl.multiple_of((idx // 16) * 16, 16)
            xio[pl.ds(g0, 16), :] = xres[pl.ds(g0, 16), :].astype(bf16)
            fix = pltpu.make_async_copy(xio.at[pl.ds(g0, 16), :], out_hbm.at[pl.ds(g0, 16), :], sem_w.at[7])
            fix.start()
            fix.wait()

    def layer_body(layer, c):
        phase_a(layer)
        phase_b()
        phase_c(layer)
        phase_d(layer)
        return c

    lax.fori_loop(0, 2, layer_body, 0)


@jax.jit
def pallas_interleave_layers__sliding_block__moe_arch_mod__prompt_kernel(
    A_x: jax.Array,
    A_wqkv: jax.Array,
    A_wo: jax.Array,
    B_x: jax.Array,
    B_w_r: jax.Array,
    B_w_gate: jax.Array,
    B_w_up: jax.Array,
    B_w_down: jax.Array,
):
    del B_x
    x = A_x.reshape(S, D)
    any_spec = pl.BlockSpec(memory_space=pl.ANY)
    scratch = [
        pltpu.VMEM((S, D), bf16),
        pltpu.VMEM((D, D), bf16),
        pltpu.VMEM((D, D), bf16),
        pltpu.VMEM((D, D), bf16),
        pltpu.VMEM((D // 2, D), u32),
        pltpu.VMEM((D, D), bf16),
        pltpu.VMEM((D // 2, D), u32),
        pltpu.VMEM((D,), bf16),
        pltpu.VMEM((D, F), bf16),
        pltpu.VMEM((D, F), bf16),
        pltpu.VMEM((F, D), bf16),
        pltpu.VMEM((S, D), f32),
        pltpu.VMEM((S, D), f32),
        pltpu.VMEM((8, 128), f32),
        pltpu.VMEM((8, 128), i32),
        pltpu.VMEM((S, 128), f32),
        pltpu.VMEM((S, 128), f32),
        pltpu.VMEM((8, 128), f32),
        pltpu.VMEM((8, D), f32),
        pltpu.VMEM((TQ // 2, D), u32),
        pltpu.VMEM((TQ // 2, D), u32),
        pltpu.VMEM((S // 2, D), u32),
        pltpu.VMEM((S // 2, D), u32),
        pltpu.VMEM((G, S // 2, 128), u32),
        pltpu.VMEM((G, (S + PAD) // 2, 128), u32),
        pltpu.VMEM((D // 2, S + PAD), u32),
        pltpu.VMEM((D // 2, S), u32),
        pltpu.VMEM((4, 4, 256, 128), f32),
        pltpu.VMEM((4, 4, 8, 128), f32),
        pltpu.VMEM((128, 128), f32),
        pltpu.VMEM((4, 8, 128), f32),
        pltpu.VMEM((TQ, D), f32),
        pltpu.VMEM((TQ, D), f32),
        pltpu.VMEM((TQ // 2, D), u32),
        pltpu.VMEM((TQ // 2, D), u32),
        pltpu.SemaphoreType.DMA((NB,)),
        pltpu.SemaphoreType.DMA((10,)),
        pltpu.SemaphoreType.DMA((NB,)),
    ]
    out = pl.pallas_call(
        _kernel,
        out_shape=jax.ShapeDtypeStruct((S, D), bf16),
        in_specs=[any_spec] * 7,
        out_specs=any_spec,
        scratch_shapes=scratch,
        compiler_params=pltpu.CompilerParams(vmem_limit_bytes=120 * 1024 * 1024),
    )(x, A_wqkv, A_wo, B_w_r, B_w_gate, B_w_up, B_w_down)
    return out.reshape(1, S, D)
```
